```python
import jax
import jax.numpy as jnp

def _softmax(x, axis=-1):
    return jax.nn.softmax(x, axis=axis)

def _gelu(x):
    return jax.nn.gelu(x, approximate=True)

def _silu(x):
    return jax.nn.silu(x)

def _sigmoid(x):
    return jax.nn.sigmoid(x)

def _layernorm(x, axis=-1, eps=1e-05):
    m = jnp.mean(x, axis=axis, keepdims=True)
    v = jnp.var(x, axis=axis, keepdims=True)
    return (x - m) / jnp.sqrt(v + eps)

def _scatter_add(tgt, idx, src, axis=0):
    return tgt.at[idx].add(src)

def _segment_sum(src, seg, n):
    return jax.ops.segment_sum(src, seg, n)

class _Rng:

    def __init__(self, key):
        self._k = key

    def _next(self):
        self._k, sub = jax.random.split(self._k)
        return sub

    def normal(self, shape):
        return jax.random.normal(self._next(), shape, dtype=jnp.bfloat16)

    def randint(self, lo, hi, shape):
        return jax.random.randint(self._next(), shape, lo, hi, dtype=jnp.int32)

    def uniform(self, shape, lo=0.0, hi=1.0):
        return jax.random.uniform(self._next(), shape, jnp.bfloat16, lo, hi)

    def permutation(self, n):
        return jax.random.permutation(self._next(), n)
kernel_name = 'concat_heads__memory_aug_recurrent_mem_tr__spectral_gfnet__prompt'

def setup_inputs():
    _rng = _Rng(jax.random.key(int.from_bytes(__import__("os").urandom(4), "little")))
    _w = lambda a: (lambda t: t.astype(jnp.bfloat16) if jnp.issubdtype(t.dtype, jnp.floating) else t)(jnp.asarray(a))

    def _A_setup():
        B, S, Dm = (1, 2048, 1024)
        H, Dh = (32, 128)
        M, seg = (8, 32)
        seg = min(seg, S)
        S = S // seg * seg
        return {'x': _w((lambda *s: _rng.normal(s) * 0.05)(B, S, Dm)), 'mem0': _w((lambda *s: _rng.normal(s) * 0.05)(B, M, Dm)), 'Wq': _w((lambda *s: _rng.normal(s) * 0.05)(Dm, H, Dh) * Dm ** (-0.5)), 'Wk': _w((lambda *s: _rng.normal(s) * 0.05)(Dm, H, Dh) * Dm ** (-0.5)), 'Wv': _w((lambda *s: _rng.normal(s) * 0.05)(Dm, H, Dh) * Dm ** (-0.5)), 'Wo': _w((lambda *s: _rng.normal(s) * 0.05)(H, Dh, Dm) * (H * Dh) ** (-0.5)), 'seg_len': seg}
    _A_in = _A_setup()

    def _B_setup():
        B, S, D = (1, 2048, 1024)
        Df = D // 2 + 1
        return {'x': _w((lambda *s: _rng.normal(s) * 0.05)(B, S, D)), 'w_r': _w((lambda *s: _rng.normal(s) * 0.05)(S, Df) * 0.02), 'w_i': _w((lambda *s: _rng.normal(s) * 0.05)(S, Df) * 0.02)}
    _B_in = _B_setup()
    return {'A_x': _A_in['x'], 'A_mem0': _A_in['mem0'], 'A_Wq': _A_in['Wq'], 'A_Wk': _A_in['Wk'], 'A_Wv': _A_in['Wv'], 'A_Wo': _A_in['Wo'], 'A_seg_len': _A_in['seg_len'], 'B_x': _B_in['x'], 'B_w_r': _B_in['w_r'], 'B_w_i': _B_in['w_i']}

def reference(A_x, A_mem0, A_Wq, A_Wk, A_Wv, A_Wo, A_seg_len, B_x, B_w_r, B_w_i):

    def _A_ref(x, mem0, Wq, Wk, Wv, Wo, seg_len):
        B, S, Dm = x.shape
        H, Dh = (Wq.shape[1], Wq.shape[2])
        M = mem0.shape[1]
        scale = Dh ** (-0.5)
        n_seg = S // seg_len
        L = M + seg_len
        idx = jnp.arange(L)
        mask = (idx[:, None] < M) | (idx[:, None] >= idx[None, :])
        mem = mem0
        outs = []
        for s in range(n_seg):
            xs = x[:, s * seg_len:(s + 1) * seg_len, :].copy()
            h = jnp.concatenate([mem, xs], axis=1)
            q = jnp.einsum('btd,dhe->bhte', h, Wq)
            k = jnp.einsum('btd,dhe->bhte', h, Wk)
            v = jnp.einsum('btd,dhe->bhte', h, Wv)
            scores = jnp.einsum('bhqe,bhke->bhqk', q, k) * scale
            scores = jnp.where(mask[None, None], scores, -1000000000.0)
            p = _softmax(scores, axis=-1)
            o = jnp.einsum('bhqk,bhke->bhqe', p, v)
            o = jnp.einsum('bhte,hed->btd', o, Wo)
            mem = o[:, :M, :].copy()
            outs.append(o[:, M:, :])
        return jnp.concatenate(outs, axis=1)

    def _B_ref(x, w_r, w_i):
        B, S, D = x.shape
        X = (lambda x, axes=(-2, -1): jnp.fft.rfft2(x.astype(jnp.float32), axes=axes))(x, axes=(-2, -1))
        W = w_r + 1j * w_i
        X = X * W
        y = (lambda x, s, axes=(-2, -1): jnp.fft.irfft2(x, s=s, axes=axes).astype(jnp.bfloat16))(X, (S, D), axes=(-2, -1))
        return y
    a = _A_ref(A_x, A_mem0, A_Wq, A_Wk, A_Wv, A_Wo, A_seg_len)
    b = _B_ref(B_x, B_w_r, B_w_i)
    return jnp.concatenate([a, b], axis=-1)
```

```python
import functools
import math

import jax
import jax.numpy as jnp
import numpy as np
from jax import lax
import jax.experimental.pallas as pl
import jax.experimental.pallas.tpu as pltpu

bf16, f32, u32, i32 = jnp.bfloat16, jnp.float32, jnp.uint32, jnp.int32

S, DM, H, DH, M, SEG = 2048, 1024, 32, 128, 8, 32
NSEG = S // SEG
FR = SEG - M
G = H // 2
NQ = 4
SPQ = NSEG // NQ
NCH = 6
NST = 3

D = 1024
RS, BS = 32, 64
NG = 5
TR = 256
C8 = float(np.sqrt(0.5))


def _grp(k):
    r = k % 8
    return min(r, 8 - r) % 4


@functools.lru_cache(maxsize=None)
def _tables():
    perm = np.zeros((8, 128), np.int32)
    kcol = np.zeros((4, 128), np.int64)
    for g in range(4):
        for c in range(4):
            ks = [l for l in range(128) if _grp(128 * g + l) == c]
            sl = (c + g) % 4
            perm[g, 32 * sl:32 * sl + 32] = ks
            kcol[c, 32 * sl:32 * sl + 32] = [128 * g + l for l in ks]
    c_ = np.sqrt(0.5)
    E = np.eye(8)
    a = [E[i] + E[i + 4] for i in range(4)]
    b = [E[i] - E[i + 4] for i in range(4)]
    U = [(a[0] + a[2], a[1] + a[3]),
         (b[0] + c_ * (b[1] - b[3]), b[2] + c_ * (b[1] + b[3])),
         (a[0] - a[2], a[1] - a[3]),
         (b[0] - c_ * (b[1] - b[3]), b[2] - c_ * (b[1] + b[3]))]
    d = np.arange(D)
    R = np.zeros((8, 256, 256))
    for c in range(4):
        Bc = np.concatenate([np.kron(U[c][0][:, None], np.eye(128)),
                             np.kron(U[c][1][:, None], np.eye(128))], axis=1)
        ang = 2 * np.pi * ((np.outer(d, kcol[c])) % D) / D
        Ft = np.concatenate([np.cos(ang), -np.sin(ang)], axis=1)
        wt = np.full(256, 2.0)
        if c == 0:
            Ft[:, 128] = (-1.0) ** d
            wt[0] = 1.0
            wt[128] = 1.0
        R[c] = (Bc.T @ Ft) / 4.0
        R[4 + c] = (wt[:, None] * R[c].T) / (S * D)
    L = np.zeros((2 * RS, 128, 128))
    bb = np.arange(BS)
    for p1 in range(RS):
        ang = 2 * np.pi * (np.outer(p1 + RS * bb, bb) % S) / S
        mr, mi = np.cos(ang), -np.sin(ang)
        L[p1] = np.block([[mr, -mi], [mi, mr]])
        L[RS + p1] = L[p1].T
    head = np.zeros(80, np.int32)
    pos = np.zeros(80, np.int32)
    for r in range(80):
        if r < 64:
            head[r] = r // 32
            t = r % 32
            pos[r] = (M + t) if t < FR else (t - FR)
        else:
            head[r] = (r - 64) // 8
            pos[r] = M + FR + (r - 64) % 8
    same = head[:, None] == head[None, :]
    vis = (pos[:, None] < M) | (pos[:, None] >= pos[None, :])
    fill = np.where(same, np.where(vis, 0.0, -1e9), -np.inf).astype(np.float32)
    return perm, R.astype(np.float32), L.astype(np.float32), fill


def _cmul_const(re, im, j, n, sgn):
    ang = sgn * 2 * math.pi * j / n
    c, s = math.cos(ang), math.sin(ang)
    if abs(abs(c) - abs(s)) < 1e-12:
        if c * s > 0:
            return (re - im) * c, (re + im) * c
        return (re + im) * c, (im - re) * c
    return re * c - im * s, re * s + im * c


def _diff_tw(a, b, j, n, sgn):
    if j == 0:
        return a[0] - b[0], a[1] - b[1]
    if 4 * j == n:
        if sgn < 0:
            return a[1] - b[1], b[0] - a[0]
        return b[1] - a[1], a[0] - b[0]
    return _cmul_const(a[0] - b[0], a[1] - b[1], j, n, sgn)


def _fft(v, sgn):
    n = len(v)
    if n == 1:
        return v
    h = n // 2
    ev = _fft([(v[j][0] + v[j + h][0], v[j][1] + v[j + h][1]) for j in range(h)], sgn)
    od = _fft([_diff_tw(v[j], v[j + h], j, n, sgn) for j in range(h)], sgn)
    out = [None] * n
    out[0::2] = ev
    out[1::2] = od
    return out


def _dot(a, b):
    return jnp.dot(a, b, preferred_element_type=f32)


def _asbf(v):
    return pltpu.bitcast(v, bf16)


def _spectral(bx, wr, wi, perm_ref, R_ref, L_ref, za, zb, wp, wait_x, wait_w, wait_l, after_p1):
    lane = lax.broadcasted_iota(i32, (TR, 128), 1)

    def p1(i, c):
        rows = pl.ds(pl.multiple_of(i * TR, TR), TR)
        segs = pl.ds(i * (TR // SEG), TR // SEG)
        x = [bx[segs, :, 128 * e:128 * (e + 1)].reshape(TR, 128).astype(f32) for e in range(8)]
        a = [x[j] + x[j + 4] for j in range(4)]
        b = [x[j] - x[j + 4] for j in range(4)]
        t1 = (b[1] - b[3]) * C8
        t2 = (b[1] + b[3]) * C8
        U = [(a[0] + a[2], a[1] + a[3]), (b[0] + t1, b[2] + t2),
             (a[0] - a[2], a[1] - a[3]), (b[0] - t1, b[2] - t2)]
        for cg in range(4):
            u = jnp.concatenate([U[cg][0].astype(bf16), U[cg][1].astype(bf16)], axis=1)
            z = _dot(u, R_ref[cg])
            zr, zi = z[:, :128], z[:, 128:]
            if cg == 0:
                za[4, 0, rows, :] = jnp.where(lane == 0, zi, 0.0)
                za[4, 1, rows, :] = jnp.zeros((TR, 128), f32)
                zi = jnp.where(lane == 0, 0.0, zi)
            za[cg, 0, rows, :] = zr
            za[cg, 1, rows, :] = zi
        return c

    wait_x()
    lax.fori_loop(0, S // TR, p1, 0)
    after_p1()

    def radix(src, dst, sgn):
        def body(it, c):
            cg = it // (BS // 8)
            t = it % (BS // 8)

            def ld(a):
                r = pl.ds(pl.multiple_of(a * BS + t * 8, 8), 8)
                return (src[cg, 0, r, :], src[cg, 1, r, :])
            h = RS // 2
            for par in range(2):
                if par == 0:
                    v = []
                    for j in range(h):
                        p, q = ld(j), ld(j + h)
                        v.append((p[0] + q[0], p[1] + q[1]))
                else:
                    v = [_diff_tw(ld(j), ld(j + h), j, RS, sgn) for j in range(h)]
                o = _fft(v, sgn)
                for m in range(h):
                    r = pl.ds(pl.multiple_of((2 * m + par) * BS + t * 8, 8), 8)
                    dst[cg, 0, r, :] = o[m][0]
                    dst[cg, 1, r, :] = o[m][1]
            return c
        lax.fori_loop(0, NG * (BS // 8), body, 0)

    radix(za, zb, -1)

    def wprep(i, c):
        rows = pl.ds(pl.multiple_of(i * 128, 128), 128)
        rows2 = pl.ds(pl.multiple_of(i * 64, 64), 64)
        ln = lax.broadcasted_iota(i32, (64, 128), 1)
        for t, w in enumerate((wr, wi)):
            gs = []
            for g in range(4):
                v = pltpu.bitcast(w[rows, 128 * g:128 * (g + 1)], u32)
                idx = jnp.broadcast_to(perm_ref[g:g + 1, :], (64, 128))
                gs.append(jnp.take_along_axis(v, idx, axis=1, mode="promise_in_bounds"))
            for cg in range(4):
                r = gs[(3 - cg) % 4]
                for sl in (2, 1, 0):
                    r = jnp.where(ln < 32 * (sl + 1), gs[(sl - cg) % 4], r)
                wp[t, cg, rows2, :] = r
            col = w[rows, 512:513].astype(f32)
            full = jnp.broadcast_to(col, (128, 128)).astype(bf16)
            wp[t, 4, rows2, :] = pltpu.bitcast(full, u32)
        return c

    wait_w()
    lax.fori_loop(0, S // 128, wprep, 0)
    wait_l()

    def fwd(p):
        rows = slice(p * BS, (p + 1) * BS)
        y = jnp.concatenate(
            [jnp.concatenate([zb[cg, 0, rows, :], zb[cg, 1, rows, :]], axis=0).astype(bf16)
             for cg in range(NG)], axis=1)
        return _dot(L_ref[p], y)

    def filt(p, v):
        outs = []
        for cg in range(NG):
            ws = []
            for t in range(2):
                w = wp[t, cg, pl.ds(p // 2, BS, stride=RS // 2), :]
                w = (w << 16) if p % 2 == 0 else (w & jnp.uint32(0xffff0000))
                ws.append(pltpu.bitcast(w, f32))
            vr = v[:BS, 128 * cg:128 * (cg + 1)]
            vi = v[BS:, 128 * cg:128 * (cg + 1)]
            gr = vr * ws[0] - vi * ws[1]
            gi = vr * ws[1] + vi * ws[0]
            outs.append(jnp.concatenate([gr, gi], axis=0).astype(bf16))
        return jnp.concatenate(outs, axis=1)

    def inv(p, g):
        rows = slice(p * BS, (p + 1) * BS)
        t = _dot(L_ref[RS + p], g)
        for cg in range(NG):
            za[cg, 0, rows, :] = t[:BS, 128 * cg:128 * (cg + 1)]
            za[cg, 1, rows, :] = t[BS:, 128 * cg:128 * (cg + 1)]

    gs = {}
    lag = 2
    for p in range(RS + lag):
        if p < RS:
            gs[p] = filt(p, fwd(p))
        if p >= lag:
            inv(p - lag, gs.pop(p - lag))

    radix(za, zb, +1)

    def p3(i, c):
        rows = pl.ds(pl.multiple_of(i * TR, TR), TR)
        V = []
        for cg in range(4):
            tr = zb[cg, 0, rows, :]
            ti = zb[cg, 1, rows, :]
            if cg == 0:
                ti = jnp.where(lane == 0, zb[4, 0, rows, :], ti)
            u = jnp.concatenate([tr.astype(bf16), ti.astype(bf16)], axis=1)
            z = _dot(u, R_ref[4 + cg])
            V.append((z[:, :128], z[:, 128:]))
        a = [V[0][0] + V[2][0], V[0][1] + V[2][1], V[0][0] - V[2][0], V[0][1] - V[2][1]]
        t1 = (V[1][0] - V[3][0]) * C8
        t2 = (V[1][1] - V[3][1]) * C8
        b = [V[1][0] + V[3][0], t1 + t2, V[1][1] + V[3][1], t2 - t1]
        segs = pl.ds(i * (TR // SEG), TR // SEG)
        for j in range(4):
            bx[segs, :, 128 * j:128 * (j + 1)] = (a[j] + b[j]).astype(bf16).reshape(TR // SEG, SEG, 128)
            bx[segs, :, 128 * (j + 4):128 * (j + 5)] = (a[j] - b[j]).astype(bf16).reshape(TR // SEG, SEG, 128)
        return c

    lax.fori_loop(0, S // TR, p3, 0)


def _kernel(ax_hbm, mem_ref, wq_hbm, wk_hbm, wv_hbm, wo_hbm, bx_hbm, wr_hbm, wi_hbm,
            perm_ref, R_hbm, L_hbm, fill_ref, out_hbm,
            ax, wo, stage, w0, w1, w2, w3, w4, w5, bx, memb, xb, sems):
    wpk = (w0, w1, w2, w3, w4, w5)
    srcs = (wq_hbm, wk_hbm, wv_hbm)

    def chunk_copy(t):
        return pltpu.make_async_copy(srcs[t // 2].at[:, pl.ds(16 * (t % 2), 16), :],
                                     stage.at[t % NST], sems.at[8 + t % NST])

    def wo_copy(j):
        return pltpu.make_async_copy(wo_hbm.at[:, pl.ds(128 * j, 128)], wo.at[j], sems.at[11])

    cp_ax = pltpu.make_async_copy(ax_hbm, ax, sems.at[5])
    cp_outb = pltpu.make_async_copy(bx, out_hbm.at[:, :, pl.ds(DM, D)], sems.at[6])

    def spectral(wr, wi, R, L, za, zb, wp):
        cp_x = pltpu.make_async_copy(bx_hbm, bx, sems.at[0])
        cp_r = pltpu.make_async_copy(R_hbm, R, sems.at[1])
        cp_wr = pltpu.make_async_copy(wr_hbm, wr, sems.at[2])
        cp_wi = pltpu.make_async_copy(wi_hbm, wi, sems.at[3])
        cp_l = pltpu.make_async_copy(L_hbm, L, sems.at[4])
        cp_x.start()
        cp_r.start()

        def wait_x():
            cp_x.wait()
            cp_r.wait()
            cp_wr.start()
            cp_wi.start()
            cp_l.start()

        def after_p1():
            cp_ax.start()
            for t in range(NST):
                chunk_copy(t).start()

        def wait_w():
            cp_wr.wait()
            cp_wi.wait()

        _spectral(bx, wr, wi, perm_ref, R, L, za, zb, wp, wait_x, wait_w, cp_l.wait, after_p1)

    pl.run_scoped(
        spectral,
        pltpu.VMEM((S, D // 2 + 1), bf16), pltpu.VMEM((S, D // 2 + 1), bf16),
        pltpu.VMEM((8, 256, 256), bf16), pltpu.VMEM((2 * RS, 128, 128), bf16),
        pltpu.VMEM((NG, 2, S, 128), f32), pltpu.VMEM((NG, 2, S, 128), f32),
        pltpu.VMEM((2, NG, S // 2, 128), u32))
    cp_outb.start()

    def rmt(qkvb, ob, oa):
        cp_ax.wait()
        xb[...] = ax[:, FR:SEG, :].reshape(NSEG * M, DM)
        memb[...] = mem_ref[...]

        def relayout(t, j):
            for i in range(8):
                d0 = pl.multiple_of(j * 128 + i * 16, 16)
                v = pltpu.bitcast(stage[t % NST, pl.ds(d0, 16)], u32).reshape(8, 2, 8, 128)
                a = jnp.swapaxes(v[:, 0], 0, 1)
                b = jnp.swapaxes(v[:, 1], 0, 1)
                lo = (a & jnp.uint32(0xffff)) | (b << 16)
                hi = (a >> 16) | (b & jnp.uint32(0xffff0000))
                r = jnp.stack([lo, hi], axis=1).reshape(16, 8, 128)
                wpk[t][:, pl.ds(pl.multiple_of(j * 64 + i * 8, 8), 8), :] = r

        def bulk(t, j):
            x = xb[...]
            r0 = _dot(x, _asbf(wpk[t][2 * j])).reshape(NSEG, M, DH)
            r1 = _dot(x, _asbf(wpk[t][2 * j + 1])).reshape(NSEG, M, DH)
            qkvb[8 * t + j] = jnp.concatenate([r0, r1], axis=1).astype(bf16)

        for t in range(NCH + 1):
            if t < NCH:
                chunk_copy(t).wait()

            def body(j, c, t=t):
                if t >= 1:
                    bulk(t - 1, j)
                if t < NCH:
                    relayout(t, j)
                return c
            lax.fori_loop(0, 8, body, 0)
            if t + NST < NCH:
                chunk_copy(t + NST).start()
            if t == NCH - NST:
                for j in range(8):
                    wo_copy(j).start()
        for j in range(8):
            wo_copy(j).wait()

        scale = DH ** -0.5

        def wsel(m, h):
            return _asbf(wpk[2 * m + h // 16][h % 16])

        def step(s, sl):
            lhs = jnp.concatenate([ax[s, 0:FR, :], memb[...]], axis=0)
            qs, ks, vs, ps, os_ = {}, {}, {}, {}, {}

            def proj(m, g):
                r0 = _dot(lhs, wsel(m, 2 * g)).astype(bf16)
                r1 = _dot(lhs, wsel(m, 2 * g + 1)).astype(bf16)
                return jnp.concatenate([r0, r1, qkvb[G * m + g, s]], axis=0)

            def qk(g):
                sc = lax.dot_general(qs.pop(g), ks.pop(g), (((1,), (1,)), ((), ())),
                                     preferred_element_type=f32) * scale
                fill = fill_ref[...]
                sc = jnp.where(fill == 0.0, sc, fill)
                mx = jnp.max(sc, axis=-1, keepdims=True)
                e = jnp.exp(sc - mx)
                l = jnp.sum(e, axis=-1, keepdims=True)
                r = pl.reciprocal(l, approx=True)
                r = r * (2.0 - l * r)
                ps[g] = (e * r).astype(bf16)

            def pv(g):
                o = _dot(ps.pop(g), vs.pop(g))
                os_[2 * g] = o[0:32].astype(bf16)
                os_[2 * g + 1] = o[32:64].astype(bf16)
                ob[sl, :, (2 * g) * DH:(2 * g + 1) * DH] = o[64:72]
                ob[sl, :, (2 * g + 1) * DH:(2 * g + 2) * DH] = o[72:80]

            def oproj(lo, hi, j):
                oc = jnp.concatenate([os_[h] for h in range(lo, hi)], axis=1)
                return _dot(oc, wo[j, lo * DH:hi * DH, :])

            sk, dq, dp = 6, 3, 4
            for t in range(G + sk):
                if t < G:
                    qs[t] = proj(0, t)
                if 0 <= t - dq < G:
                    qk(t - dq)
                if t < G:
                    ks[t] = proj(1, t)
                if t - sk - dp >= 0:
                    pv(t - sk - dp)
                if t - sk >= 0:
                    vs[t - sk] = proj(2, t - sk)
            rem = list(range(G - dp, G))
            acc = []
            for j in range(DM // 128):
                acc.append(oproj(0, 16, j))
                if rem and j >= 1:
                    pv(rem.pop(0))
            for j in range(DM // 128):
                r = acc[j] + oproj(16, 32, j)
                oa[s, :, j * 128:(j + 1) * 128] = r.astype(bf16)
                memb[:, j * 128:(j + 1) * 128] = r[FR:SEG].astype(bf16)

        def out_copy(q):
            return pltpu.make_async_copy(
                oa.at[pl.ds(q * SPQ, SPQ)],
                out_hbm.at[pl.ds(q * SPQ, SPQ), :, pl.ds(0, DM)], sems.at[7])

        def quarter(q, c):
            def one(sl, c2):
                step(q * SPQ + sl, sl)
                return c2
            lax.fori_loop(0, SPQ, one, 0)
            obv = ob[...].reshape(SPQ * M, H * DH).astype(bf16)
            for j in range(DM // 128):
                r = _dot(obv, wo[j]).reshape(SPQ, M, 128).astype(bf16)
                oa[pl.ds(q * SPQ, SPQ), FR:SEG, j * 128:(j + 1) * 128] = r
            out_copy(q).start()
            return c
        lax.fori_loop(0, NQ, quarter, 0)
        for q in range(NQ):
            out_copy(q).wait()

    pl.run_scoped(
        rmt,
        pltpu.VMEM((3 * G, NSEG, 16, DH), bf16),
        pltpu.VMEM((SPQ, M, H * DH), f32),
        pltpu.VMEM((NSEG, SEG, DM), bf16))
    cp_outb.wait()


def pallas_concat_heads__memory_aug_recurrent_mem_tr__spectral_gfnet__prompt_kernel(
    A_x, A_mem0, A_Wq, A_Wk, A_Wv, A_Wo, A_seg_len, B_x, B_w_r, B_w_i,
):
    del A_seg_len
    perm, R, L, fill = _tables()
    hbm = pl.BlockSpec(memory_space=pl.ANY)
    vmem = pl.BlockSpec(memory_space=pltpu.VMEM)
    out = pl.pallas_call(
        _kernel,
        out_shape=jax.ShapeDtypeStruct((NSEG, SEG, DM + D), bf16),
        in_specs=[hbm, vmem, hbm, hbm, hbm, hbm, hbm, hbm, hbm, vmem, hbm, hbm, vmem],
        out_specs=hbm,
        scratch_shapes=[
            pltpu.VMEM((NSEG, SEG, DM), bf16),
            pltpu.VMEM((DM // 128, H * DH, 128), bf16),
            pltpu.VMEM((NST, DM, 16, DH), bf16),
        ] + [pltpu.VMEM((16, DM // 2, DH), u32)] * NCH + [
            pltpu.VMEM((NSEG, SEG, D), bf16),
            pltpu.VMEM((M, DM), bf16),
            pltpu.VMEM((NSEG * M, DM), bf16),
            pltpu.SemaphoreType.DMA((12,)),
        ],
        compiler_params=pltpu.CompilerParams(vmem_limit_bytes=120 * 1024 * 1024),
    )(A_x.reshape(NSEG, SEG, DM), A_mem0.reshape(M, DM), A_Wq, A_Wk, A_Wv,
      A_Wo.reshape(H * DH, DM), B_x.reshape(NSEG, SEG, D), B_w_r, B_w_i,
      jnp.asarray(perm), jnp.asarray(R, bf16), jnp.asarray(L, bf16), jnp.asarray(fill))
    return out.reshape(1, S, DM + D)
```

```python
import functools
import math

import jax
import jax.numpy as jnp
import numpy as np
from jax import lax
import jax.experimental.pallas as pl
import jax.experimental.pallas.tpu as pltpu

bf16, f32, u32, i32 = jnp.bfloat16, jnp.float32, jnp.uint32, jnp.int32

S, DM, H, DH, M, SEG = 2048, 1024, 32, 128, 8, 32
NSEG = S // SEG
FR = SEG - M
G = H // 2
U = 4
NCH = 6
NST = 3
PW = 520
QB = NST * DM

D = 1024
RS, BS = 32, 64
HR = RS // 2
WP = 40
TP = 136
C8 = float(np.sqrt(0.5))


def _pack_rows(a):
    u = np.asarray(a, np.float32).astype(jnp.bfloat16).view(np.uint16).astype(np.uint32)
    return u[..., 0::2, :] | (u[..., 1::2, :] << 16)


@functools.lru_cache(maxsize=None)
def _tables():
    kcol = np.zeros((4, 128), np.int64)
    for l in range(128):
        i0, i1 = l, 128 + (l ^ 1)
        ev, o3 = l % 2 == 0, l % 4 in (0, 3)
        kcol[0, l] = 2 * (i0 if ev else i1)
        kcol[2, l] = 2 * (i1 if ev else i0)
        kcol[1, l] = 2 * (i0 if o3 else i1) + 1
        kcol[3, l] = 2 * (i1 if o3 else i0) + 1
    c_ = np.sqrt(0.5)
    E = np.eye(8)
    a = [E[i] + E[i + 4] for i in range(4)]
    b = [E[i] - E[i + 4] for i in range(4)]
    UU = [(a[0] + a[2], a[1] + a[3]),
          (b[0] + c_ * (b[1] - b[3]), b[2] + c_ * (b[1] + b[3])),
          (a[0] - a[2], a[1] - a[3]),
          (b[0] - c_ * (b[1] - b[3]), b[2] - c_ * (b[1] + b[3]))]
    d = np.arange(D)
    R = np.zeros((8, 256, 256))
    for c in range(4):
        Bc = np.concatenate([np.kron(UU[c][0][:, None], np.eye(128)),
                             np.kron(UU[c][1][:, None], np.eye(128))], axis=1)
        ang = 2 * np.pi * (np.outer(d, kcol[c]) % D) / D
        Ft = np.concatenate([np.cos(ang), -np.sin(ang)], axis=1)
        wt = np.full(256, 2.0)
        if c == 0:
            Ft[:, 128] = (-1.0) ** d
            wt[0] = 1.0
            wt[128] = 1.0
        R[c] = (Bc.T @ Ft) / 4.0
        R[4 + c] = (wt[:, None] * R[c].T) / (S * D)
    L = np.zeros((2 * RS, 128, 128))
    bb = np.arange(BS)
    kord = np.array([ri * 64 + 8 * t + r for t in range(8) for ri in range(2) for r in range(8)])
    for p1 in range(RS):
        ang = 2 * np.pi * (np.outer(p1 + RS * bb, bb) % S) / S
        mr, mi = np.cos(ang), -np.sin(ang)
        full = np.block([[mr, -mi], [mi, mr]])
        L[p1] = full[:, kord]
        L[RS + p1] = full.T
    l_, q_ = np.arange(128), np.arange(16)
    ang = 2 * np.pi * (np.outer(l_, l_) % 128) / 128
    N1 = np.concatenate([np.cos(ang), -np.sin(ang)], axis=1)
    N1 = np.concatenate([(N1[:64] + N1[64:]) / 2, (N1[:64] - N1[64:]) / 2], axis=0)
    ang = 2 * np.pi * np.outer(q_, l_) / S
    TW = np.concatenate([np.cos(ang), -np.sin(ang)], axis=0)
    ang = 2 * np.pi * (np.outer(q_, q_) % 16) / 16
    fr, fi = np.cos(ang), -np.sin(ang)
    F16 = np.block([[fr, -fi], [fi, fr]])
    NY = np.zeros((5, 128, 128))
    NY[0], NY[1], NY[2], NY[3] = N1[:, :128], N1[:, 128:], N1[:, :128].T, N1[:, 128:].T
    NY[4, :32, :32] = F16
    NY[4, 32:64, :32] = F16.T
    LN = np.concatenate([L, NY], axis=0)
    head = np.zeros(80, np.int32)
    pos = np.zeros(80, np.int32)
    for r in range(80):
        if r < 64:
            head[r] = r // 32
            t = r % 32
            pos[r] = (M + t) if t < FR else (t - FR)
        else:
            head[r] = (r - 64) // 8
            pos[r] = M + FR + (r - 64) % 8
    same = head[:, None] == head[None, :]
    vis = (pos[:, None] < M) | (pos[:, None] >= pos[None, :])
    fill = np.where(same, np.where(vis, 0.0, -1e9), -np.inf).astype(np.float32)
    return _pack_rows(R), _pack_rows(LN), TW.astype(np.float32), fill


def _cmul_const(re, im, j, n, sgn):
    ang = sgn * 2 * math.pi * j / n
    c, s = math.cos(ang), math.sin(ang)
    if abs(abs(c) - abs(s)) < 1e-12:
        if c * s > 0:
            return (re - im) * c, (re + im) * c
        return (re + im) * c, (im - re) * c
    return re * c - im * s, re * s + im * c


def _diff_tw(a, b, j, n, sgn):
    if j == 0:
        return a[0] - b[0], a[1] - b[1]
    if 4 * j == n:
        if sgn < 0:
            return a[1] - b[1], b[0] - a[0]
        return b[1] - a[1], a[0] - b[0]
    return _cmul_const(a[0] - b[0], a[1] - b[1], j, n, sgn)


def _tw(v, j, sgn):
    if j == 0:
        return v
    if 4 * j == RS:
        return (v[1], -v[0]) if sgn < 0 else (-v[1], v[0])
    return _cmul_const(v[0], v[1], j, RS, sgn)


def _fft(v, sgn):
    n = len(v)
    if n == 1:
        return v
    h = n // 2
    ev = _fft([(v[j][0] + v[j + h][0], v[j][1] + v[j + h][1]) for j in range(h)], sgn)
    od = _fft([_diff_tw(v[j], v[j + h], j, n, sgn) for j in range(h)], sgn)
    out = [None] * n
    out[0::2] = ev
    out[1::2] = od
    return out


def _dot(a, b):
    return jnp.dot(a, b, preferred_element_type=f32)


def _asbf(v):
    return pltpu.bitcast(v, bf16)


def _cm(ar, ai, br, bi):
    return ar * br - ai * bi, ar * bi + ai * br


def _kernel(ax_hbm, mem_ref, wq_hbm, wk_hbm, wv_hbm, wo_hbm, bx_hbm, wr_hbm, wi_hbm,
            R_hbm, L_hbm, TW_ref, fill_ref, out_hbm,
            ax, xb3, xb, wo, pool, w0, w1, w2, w3, w4, w5, memb, ob, oa,
            bx, wr, wi, R, L, Y, Us, T, wp, nv, sems):
    wpk = (w0, w1, w2, w3, w4, w5)
    srcs = (wq_hbm, wk_hbm, wv_hbm)
    lane8 = lax.broadcasted_iota(i32, (8, 128), 1)

    def bx_copy(t):
        return pltpu.make_async_copy(bx_hbm.at[:, t], bx.at[:, t], sems.at[t])

    def chunk_copy(t, part=None):
        lo, n, sem = (0, DM, 8 + t % NST) if part is None else (part * 256, 256, 20 + part)
        return pltpu.make_async_copy(srcs[t // 2].at[pl.ds(lo, n), pl.ds(16 * (t % 2), 16), :],
                                     pool.at[pl.ds((t % NST) * DM + lo, n)], sems.at[sem])

    def wo_copy(j):
        return pltpu.make_async_copy(wo_hbm.at[:, pl.ds(128 * j, 128)], wo.at[j], sems.at[11])

    cp_r0 = pltpu.make_async_copy(R_hbm.at[pl.ds(0, 4)], R.at[pl.ds(0, 4)], sems.at[12])
    cp_r1 = pltpu.make_async_copy(R_hbm.at[pl.ds(4, 4)], R.at[pl.ds(4, 4)], sems.at[13])
    cp_l = pltpu.make_async_copy(L_hbm, L, sems.at[14])
    cp_wr = pltpu.make_async_copy(wr_hbm, wr, sems.at[15])
    cp_wi = pltpu.make_async_copy(wi_hbm, wi, sems.at[16])
    cp_xb = pltpu.make_async_copy(ax_hbm.at[:, 3], xb3, sems.at[17])
    cp_ax = pltpu.make_async_copy(ax_hbm.at[:, pl.ds(0, 3)], ax, sems.at[18])
    cp_outb = pltpu.make_async_copy(bx, out_hbm.at[:, :, :, pl.ds(DM, D)], sems.at[19])

    bx_copy(0).start()
    cp_r0.start()
    for t in range(1, 8):
        bx_copy(t).start()
    for part in range(4):
        chunk_copy(0, part).start()
    cp_xb.start()

    def prep(t):
        for jj in range(HR // 2):
            lo = [bx[2 * jj:2 * jj + 2, t, :, 128 * e:128 * (e + 1)].astype(f32).reshape(16, 128) for e in range(8)]
            hi = [bx[HR + 2 * jj:HR + 2 * jj + 2, t, :, 128 * e:128 * (e + 1)].astype(f32).reshape(16, 128)
                  for e in range(8)]
            for par in range(2):
                x = [lo[e] + hi[e] if par == 0 else lo[e] - hi[e] for e in range(8)]
                a = [x[j] + x[j + 4] for j in range(4)]
                b = [x[j] - x[j + 4] for j in range(4)]
                t1 = (b[1] - b[3]) * C8
                t2 = (b[1] + b[3]) * C8
                uu = [a[0] + a[2], a[1] + a[3], b[0] + t1, b[2] + t2,
                      a[0] - a[2], a[1] - a[3], b[0] - t1, b[2] - t2]
                for q in range(8):
                    Us[t, par, q, jj] = uu[q].astype(bf16)

    def units1(t):
        nrow = pl.ds(pl.multiple_of((t % 2) * 8, 8), 8)
        V = nv[nrow, :]
        for par in range(2):
            for cg in range(4):
                u = jnp.concatenate([Us[t, par, 2 * cg].reshape(128, 128),
                                     Us[t, par, 2 * cg + 1].reshape(128, 128)], axis=1)
                z = _dot(u, _asbf(R[cg]))
                v = [(z[8 * j:8 * j + 8, :128], z[8 * j:8 * j + 8, 128:]) for j in range(HR)]
                if cg == 0:
                    for j in range(HR):
                        vb = jnp.broadcast_to(v[j][1][:, 0:1], (8, 128))
                        V = jnp.where(lane8 == 64 * par + 4 * j + t // 2, vb, V)
                        v[j] = (v[j][0], jnp.where(lane8 == 0, 0.0, v[j][1]))
                if par == 1:
                    v = [_tw(v[j], j, -1) for j in range(HR)]
                o = _fft(v, -1)
                for m in range(HR):
                    Y[2 * m + par, cg, t] = jnp.concatenate(o[m], axis=0).astype(bf16)
        nv[nrow, :] = V

    nv[...] = jnp.zeros((16, 128), f32)
    bx_copy(0).wait()
    prep(0)
    cp_r0.wait()

    def body1(t, c):
        bx_copy(t + 1).wait()
        units1(t)
        prep(t + 1)
        return c
    lax.fori_loop(0, 7, body1, 0)
    units1(7)

    def piece(t, i):
        v = pltpu.bitcast(pool[pl.ds((t % NST) * DM + i * 16, 16)], u32)
        view = wpk[t].at[pl.ds(pl.multiple_of(i * 8, 8), 15 * PW + 8)]
        for k in range(8):
            a, b = v[2 * k], v[2 * k + 1]
            view[pl.ds(k, 8, stride=PW), :] = (a & jnp.uint32(0xffff)) | (b << 16)
            view[pl.ds(8 * PW + k, 8, stride=PW), :] = (a >> 16) | (b & jnp.uint32(0xffff0000))

    def wprep(pb):
        cols = pl.ds(pl.multiple_of(pb * 128, 128), 128)
        sub = lax.broadcasted_iota(i32, (8, 128), 0)
        msk = (jnp.where(sub % 2 == 0, jnp.uint32(0xffff), jnp.uint32(0))
               | jnp.where((sub % 4 == 0) | (sub % 4 == 3), jnp.uint32(0xffff0000), jnp.uint32(0)))
        for t, w in enumerate((wr, wi)):
            t0 = pltpu.bitcast(w[0:256, cols], u32)
            t1 = pltpu.bitcast(w[256:512, cols], u32)
            ps, qs = [], []
            for j in range(16):
                a = t0[8 * j:8 * j + 8]
                b = t1[8 * j:8 * j + 8]
                b = jnp.where(sub % 2 == 0, pltpu.roll(b, 7, 0), pltpu.roll(b, 1, 0))
                x = (a ^ b) & msk
                ps.append(b ^ x)
                qs.append(a ^ x)
            for h, lst in enumerate((ps, qs)):
                tr = pltpu.bitcast(pltpu.bitcast(jnp.concatenate(lst, axis=0), f32).T, u32)
                for q in range(4):
                    wp[t, h, pl.ds(pl.multiple_of((pb * 4 + q) * WP, 8), 32), :] = tr[32 * q:32 * q + 32]

    for part in range(4):
        chunk_copy(0, part).wait()
        if part == 0:
            chunk_copy(1).start()

        def rel0(i, c, part=part):
            for ii in range(4):
                piece(0, part * 16 + i * 4 + ii)
            return c
        lax.fori_loop(0, 4, rel0, 0)
    cp_xb.wait()
    chunk_copy(2).start()
    xb[...] = pltpu.bitcast(xb3[...].reshape(NSEG * M, DM), u32)
    memb[...] = mem_ref[...]

    for t in range(NCH):
        if t + 1 < NCH:
            chunk_copy(t + 1).wait()
        else:
            cp_wr.wait()
            cp_wi.wait()
        if t == 0:
            chunk_copy(3).start()
        if t == 1:
            cp_wr.start()
            cp_wi.start()
        if t == 2:
            cp_l.start()
            cp_r1.start()
            cp_ax.start()
        if t == 3:
            for j in range(8):
                wo_copy(j).start()

        def body(j, c, t=t):
            for hp in range(4):
                g = j * 4 + hp
                for mc in range(4):
                    k = hp * 4 + mc
                    x = _asbf(xb[mc * 64:(mc + 1) * 64, :])
                    rs = [_dot(x, _asbf(wpk[t][pl.ds(pl.multiple_of((hh * 8 + g) * PW, 8), DM // 2), :]))
                          .reshape(16, M, DH) for hh in range(2)]
                    if t + 1 < NCH:
                        piece(t + 1, j * 32 + (k - 1) % 16)
                        piece(t + 1, j * 32 + (k - 1) % 16 + 16)
                    elif k % 2 == 0:
                        wprep(j * 8 + k // 2)
                    pool[pl.ds(QB + (8 * t + g) * NSEG + mc * 16, 16)] = jnp.concatenate(rs, axis=1).astype(bf16)
            return c
        lax.fori_loop(0, 2, body, 0)
        if t + 1 + NST < NCH:
            chunk_copy(t + 1 + NST).start()

    cp_l.wait()
    cp_r1.wait()

    def fwd(p):
        return _dot(_asbf(L[p]), jnp.concatenate([Y[p, cg].reshape(128, 128) for cg in range(4)], axis=1))

    def filt(p, v):
        grs, gis = [None] * 4, [None] * 4
        for h in range(2):
            wr_ = wp[0, h, pl.ds(p, BS, stride=WP), :]
            wi_ = wp[1, h, pl.ds(p, BS, stride=WP), :]
            for hi in range(2):
                cg = 2 * h + hi
                if hi == 0:
                    a, b = wr_ << 16, wi_ << 16
                else:
                    a, b = wr_ & jnp.uint32(0xffff0000), wi_ & jnp.uint32(0xffff0000)
                grs[cg], gis[cg] = _cm(v[:BS, 128 * cg:128 * (cg + 1)], v[BS:, 128 * cg:128 * (cg + 1)],
                                       pltpu.bitcast(a, f32), pltpu.bitcast(b, f32))
        return jnp.concatenate([jnp.concatenate(grs, axis=1), jnp.concatenate(gis, axis=1)], axis=0).astype(bf16)

    def inv(p, g):
        t = _dot(_asbf(L[RS + p]), g)
        for cg in range(4):
            T[cg, p, 0:128, :] = t[:, 128 * cg:128 * (cg + 1)]

    nyq = {}

    def nyq_stage(k):
        n0 = 2 * RS
        if k == 0:
            v = nv[...].astype(bf16)
            r, i = _cm(_dot(v, _asbf(L[n0])), _dot(v, _asbf(L[n0 + 1])), TW_ref[0:16], TW_ref[16:32])
            nyq[0] = jnp.concatenate([r, i], axis=0).astype(bf16)
        elif k == 1:
            t = _dot(_asbf(L[n0 + 4, 0:16])[:, 0:32], nyq[0])
            ws = []
            for w in (wr, wi):
                row = w[512:513, :].astype(f32)
                ws.append(jnp.concatenate([row[:, 128 * r:128 * (r + 1)] for r in range(16)], axis=0))
            r, i = _cm(t[:16], t[16:], ws[0], ws[1])
            nyq[1] = jnp.concatenate([r, i], axis=0).astype(bf16)
        elif k == 2:
            t = _dot(_asbf(L[n0 + 4, 16:32])[:, 0:32], nyq[1])
            r, i = _cm(t[:16], t[16:], TW_ref[0:16], -TW_ref[16:32])
            nyq[2] = (r.astype(bf16), i.astype(bf16))
        elif k == 3:
            nv[...] = _dot(nyq[2][0], _asbf(L[n0 + 2])) + _dot(nyq[2][1], _asbf(L[n0 + 3]))

    gs = {}
    lag = 2
    for p in range(RS + lag):
        if p < RS:
            gs[p] = filt(p, fwd(p))
        if p >= lag:
            inv(p - lag, gs.pop(p - lag))
        if p % 4 == 1 and p // 4 < 4:
            nyq_stage(p // 4)

    def p3(t, tpar):
        rr = pl.ds(pl.multiple_of(t * 8, 8), 8)
        ri = pl.ds(pl.multiple_of(64 + t * 8, 8), 8)
        res = []
        for par in range(2):
            V = []
            for cg in range(4):
                o = _fft([(T[cg, 2 * m + par, rr, :], T[cg, 2 * m + par, ri, :]) for m in range(HR)], +1)
                if par == 1:
                    o = [_tw(o[j], j, +1) for j in range(HR)]
                if cg == 0:
                    un = nv[8 * tpar:8 * tpar + 8, :]
                    o = [(o[j][0], jnp.where(lane8 == 0, pltpu.roll(un, (128 - 64 * par - 4 * j - t // 2) % 128, 1),
                                             o[j][1])) for j in range(HR)]
                u = jnp.concatenate([jnp.concatenate([q[0] for q in o], axis=0),
                                     jnp.concatenate([q[1] for q in o], axis=0)], axis=1).astype(bf16)
                z = _dot(u, _asbf(R[4 + cg]))
                V.append((z[:, :128], z[:, 128:]))
            a = [V[0][0] + V[2][0], V[0][1] + V[2][1], V[0][0] - V[2][0], V[0][1] - V[2][1]]
            t1 = (V[1][0] - V[3][0]) * C8
            t2 = (V[1][1] - V[3][1]) * C8
            b = [V[1][0] + V[3][0], t1 + t2, V[1][1] + V[3][1], t2 - t1]
            res.append([a[j] + b[j] for j in range(4)] + [a[j] - b[j] for j in range(4)])
        for e in range(8):
            bx[0:HR, t, :, 128 * e:128 * (e + 1)] = (res[0][e] + res[1][e]).reshape(HR, 8, 128).astype(bf16)
            bx[HR:RS, t, :, 128 * e:128 * (e + 1)] = (res[0][e] - res[1][e]).reshape(HR, 8, 128).astype(bf16)

    def body3(tt, c):
        for par in range(4):
            p3(4 * tt + par, par % 2)
        return c
    lax.fori_loop(0, 2, body3, 0)
    cp_outb.start()

    cp_ax.wait()
    for j in range(8):
        wo_copy(j).wait()
    scale = DH ** -0.5
    KS = 768

    def wsel(m, h, lo=0, hi=DM):
        hl = h % 16
        base = ((hl % 2) * 8 + hl // 2) * PW
        return _asbf(wpk[2 * m + h // 16][base + lo // 2:base + hi // 2, :])

    def step(it, u):
        s = it * U + u
        lhs = jnp.concatenate([ax[s].reshape(FR, DM), memb[...]], axis=0)
        qs, ks, vs, ps, os_, pre = {}, {}, {}, {}, {}, {}
        if u > 0:
            for m in range(2):
                for h in range(2):
                    pre[(m, h)] = -_dot(lhs[:, :KS], wsel(m, h, 0, KS))

        def dotw(m, h):
            if (m, h) in pre:
                return _dot(lhs[:, KS:], wsel(m, h, KS, DM)) - pre[(m, h)]
            return _dot(lhs, wsel(m, h))

        def proj(m, g):
            return jnp.concatenate([dotw(m, 2 * g).astype(bf16), dotw(m, 2 * g + 1).astype(bf16),
                                    pool[QB + (G * m + g) * NSEG + s]], axis=0)

        def qk(g):
            sc = lax.dot_general(qs.pop(g), ks.pop(g), (((1,), (1,)), ((), ())),
                                 preferred_element_type=f32) * scale
            fill = fill_ref[...]
            sc = jnp.where(fill == 0.0, sc, fill)
            mx = jnp.max(sc, axis=-1, keepdims=True)
            e = jnp.exp(sc - mx)
            l = jnp.sum(e, axis=-1, keepdims=True)
            r = pl.reciprocal(l, approx=True)
            r = r * (2.0 - l * r)
            ps[g] = (e * r).astype(bf16)

        def pv(g):
            o = _dot(ps.pop(g), vs.pop(g))
            os_[2 * g] = o[0:32].astype(bf16)
            os_[2 * g + 1] = o[32:64].astype(bf16)
            ob[8 * u:8 * u + 8, (2 * g) * DH:(2 * g + 1) * DH] = o[64:72]
            ob[8 * u:8 * u + 8, (2 * g + 1) * DH:(2 * g + 2) * DH] = o[72:80]

        def olhs(lo, hi):
            oc = jnp.concatenate([os_[h] for h in range(lo, hi)], axis=1)
            if u == U - 1:
                oc = jnp.concatenate([oc, ob[:, lo * DH:hi * DH].astype(bf16)], axis=0)
            return oc

        sk, dq, dp = 4, 2, 3
        for t in range(G + sk):
            if t < G:
                qs[t] = proj(0, t)
            if 0 <= t - dq < G:
                qk(t - dq)
            if t < G:
                ks[t] = proj(1, t)
            if t - sk - dp >= 0:
                pv(t - sk - dp)
            if t - sk >= 0:
                vs[t - sk] = proj(2, t - sk)
        rem = list(range(G - dp, G))
        acc = []
        oc = olhs(0, 16)
        for j in range(DM // 128):
            acc.append(-_dot(oc, wo[j, 0:16 * DH, :]))
            if rem:
                pv(rem.pop(0))
        oc = olhs(16, 32)
        for j in range(DM // 128):
            cols = slice(j * 128, (j + 1) * 128)
            r = _dot(oc, wo[j, 16 * DH:32 * DH, :]) - acc[j]
            oa[it * 2 + u // 2, pl.ds((u % 2) * 4, 3), :, cols] = r[0:FR].reshape(3, 8, 128).astype(bf16)
            memb[:, cols] = r[FR:SEG].astype(bf16)
            if u == U - 1:
                for uu in range(U):
                    oa[it * 2 + uu // 2, (uu % 2) * 4 + 3, :, cols] = r[SEG + 8 * uu:SEG + 8 * uu + 8].astype(bf16)

    def out_copy(it):
        return pltpu.make_async_copy(oa.at[pl.ds(it * 2, 2)],
                                     out_hbm.at[pl.ds(it * 2, 2), :, :, pl.ds(0, DM)], sems.at[24])

    def group(it, c):
        for u in range(U):
            step(it, u)
        out_copy(it).start()
        return c
    lax.fori_loop(0, NSEG // U, group, 0)
    for it in range(NSEG // U):
        out_copy(it).wait()
    cp_outb.wait()


def pallas_concat_heads__memory_aug_recurrent_mem_tr__spectral_gfnet__prompt_kernel(
    A_x, A_mem0, A_Wq, A_Wk, A_Wv, A_Wo, A_seg_len, B_x, B_w_r, B_w_i,
):
    del A_seg_len
    R, LN, TW, fill = _tables()
    hbm = pl.BlockSpec(memory_space=pl.ANY)
    vmem = pl.BlockSpec(memory_space=pltpu.VMEM)
    out = pl.pallas_call(
        _kernel,
        out_shape=jax.ShapeDtypeStruct((RS, 8, 8, DM + D), bf16),
        in_specs=[hbm, vmem, hbm, hbm, hbm, hbm, hbm, hbm, hbm, hbm, hbm, vmem, vmem],
        out_specs=hbm,
        scratch_shapes=[
            pltpu.VMEM((NSEG, 3, 8, DM), bf16),
            pltpu.VMEM((NSEG, 8, DM), bf16),
            pltpu.VMEM((NSEG * M // 2, DM), u32),
            pltpu.VMEM((DM // 128, H * DH, 128), bf16),
            pltpu.VMEM((QB + 3 * G * NSEG, 16, DH), bf16),
        ] + [pltpu.VMEM((16 * PW, DH), u32)] * NCH + [
            pltpu.VMEM((M, DM), bf16),
            pltpu.VMEM((U * M, H * DH), f32),
            pltpu.VMEM((RS, 8, 8, DM), bf16),
            pltpu.VMEM((RS, 8, 8, D), bf16),
            pltpu.VMEM((D // 2 + 1, S), bf16),
            pltpu.VMEM((D // 2 + 1, S), bf16),
            pltpu.VMEM((8, 128, 256), u32),
            pltpu.VMEM((2 * RS + 5, 64, 128), u32),
            pltpu.VMEM((RS, 4, 8, 16, 128), bf16),
            pltpu.VMEM((8, 2, 8, 8, 16, 128), bf16),
            pltpu.VMEM((4, RS, TP, 128), f32),
            pltpu.VMEM((2, 2, BS * WP, 128), u32),
            pltpu.VMEM((16, 128), f32),
            pltpu.SemaphoreType.DMA((25,)),
        ],
        compiler_params=pltpu.CompilerParams(vmem_limit_bytes=124 * 1024 * 1024),
    )(A_x.reshape(NSEG, 4, 8, DM), A_mem0.reshape(M, DM), A_Wq, A_Wk, A_Wv,
      A_Wo.reshape(H * DH, DM), B_x.reshape(RS, 8, 8, D), B_w_r.T, B_w_i.T,
      jnp.asarray(R), jnp.asarray(LN), jnp.asarray(TW), jnp.asarray(fill))
    return out.reshape(1, S, DM + D)
```

```python
import functools
import math

import jax
import jax.numpy as jnp
import numpy as np
from jax import lax
import jax.experimental.pallas as pl
import jax.experimental.pallas.tpu as pltpu

bf16, f32, u32, i32 = jnp.bfloat16, jnp.float32, jnp.uint32, jnp.int32

S, DM, H, DH, M, SEG = 2048, 1024, 32, 128, 8, 32
NSEG = S // SEG
FR = SEG - M
G = H // 2
U = 4
NCH = 12
NST = 4
PW = 264

D = 1024
RS, BS = 32, 64
HR = RS // 2
WP = 40
TP = 136
C8 = float(np.sqrt(0.5))


def _pack_rows(a):
    u = np.asarray(a, np.float32).astype(jnp.bfloat16).view(np.uint16).astype(np.uint32)
    return u[..., 0::2, :] | (u[..., 1::2, :] << 16)


@functools.lru_cache(maxsize=None)
def _tables():
    kcol = np.zeros((4, 128), np.int64)
    for l in range(128):
        i0, i1 = l, 128 + (l ^ 1)
        ev, o3 = l % 2 == 0, l % 4 in (0, 3)
        kcol[0, l] = 2 * (i0 if ev else i1)
        kcol[2, l] = 2 * (i1 if ev else i0)
        kcol[1, l] = 2 * (i0 if o3 else i1) + 1
        kcol[3, l] = 2 * (i1 if o3 else i0) + 1
    c_ = np.sqrt(0.5)
    E = np.eye(8)
    a = [E[i] + E[i + 4] for i in range(4)]
    b = [E[i] - E[i + 4] for i in range(4)]
    UU = [(a[0] + a[2], a[1] + a[3]),
          (b[0] + c_ * (b[1] - b[3]), b[2] + c_ * (b[1] + b[3])),
          (a[0] - a[2], a[1] - a[3]),
          (b[0] - c_ * (b[1] - b[3]), b[2] - c_ * (b[1] + b[3]))]
    d = np.arange(D)
    R = np.zeros((8, 256, 256))
    for c in range(4):
        Bc = np.concatenate([np.kron(UU[c][0][:, None], np.eye(128)),
                             np.kron(UU[c][1][:, None], np.eye(128))], axis=1)
        ang = 2 * np.pi * (np.outer(d, kcol[c]) % D) / D
        Ft = np.concatenate([np.cos(ang), -np.sin(ang)], axis=1)
        wt = np.full(256, 2.0)
        if c == 0:
            Ft[:, 128] = (-1.0) ** d
            wt[0] = 1.0
            wt[128] = 1.0
        R[c] = (Bc.T @ Ft) / 4.0
        R[4 + c] = (wt[:, None] * R[c].T) / (S * D)
    L = np.zeros((2 * RS, 128, 128))
    bb = np.arange(BS)
    kord = np.array([ri * 64 + 8 * t + r for t in range(8) for ri in range(2) for r in range(8)])
    for p1 in range(RS):
        ang = 2 * np.pi * (np.outer(p1 + RS * bb, bb) % S) / S
        mr, mi = np.cos(ang), -np.sin(ang)
        full = np.block([[mr, -mi], [mi, mr]])
        L[p1] = full[:, kord]
        L[RS + p1] = full.T
    l_, q_ = np.arange(128), np.arange(16)
    ang = 2 * np.pi * (np.outer(l_, l_) % 128) / 128
    N1 = np.concatenate([np.cos(ang), -np.sin(ang)], axis=1)
    N1 = np.concatenate([(N1[:64] + N1[64:]) / 2, (N1[:64] - N1[64:]) / 2], axis=0)
    ang = 2 * np.pi * np.outer(q_, l_) / S
    TW = np.concatenate([np.cos(ang), -np.sin(ang)], axis=0)
    ang = 2 * np.pi * (np.outer(q_, q_) % 16) / 16
    fr, fi = np.cos(ang), -np.sin(ang)
    F16 = np.block([[fr, -fi], [fi, fr]])
    NY = np.zeros((5, 128, 128))
    NY[0], NY[1], NY[2], NY[3] = N1[:, :128], N1[:, 128:], N1[:, :128].T, N1[:, 128:].T
    NY[4, :32, :32] = F16
    NY[4, 32:64, :32] = F16.T
    LN = np.concatenate([L, NY], axis=0)
    head = np.zeros(80, np.int32)
    pos = np.zeros(80, np.int32)
    for r in range(80):
        if r < 64:
            head[r] = r // 32
            t = r % 32
            pos[r] = (M + t) if t < FR else (t - FR)
        else:
            head[r] = (r - 64) // 8
            pos[r] = M + FR + (r - 64) % 8
    same = head[:, None] == head[None, :]
    vis = (pos[:, None] < M) | (pos[:, None] >= pos[None, :])
    fill = np.where(same, np.where(vis, 0.0, -1e9), -np.inf).astype(np.float32)
    return _pack_rows(R), _pack_rows(LN), TW.astype(np.float32), fill


def _cmul_const(re, im, j, n, sgn):
    ang = sgn * 2 * math.pi * j / n
    c, s = math.cos(ang), math.sin(ang)
    if abs(abs(c) - abs(s)) < 1e-12:
        if c * s > 0:
            return (re - im) * c, (re + im) * c
        return (re + im) * c, (im - re) * c
    return re * c - im * s, re * s + im * c


def _diff_tw(a, b, j, n, sgn):
    if j == 0:
        return a[0] - b[0], a[1] - b[1]
    if 4 * j == n:
        if sgn < 0:
            return a[1] - b[1], b[0] - a[0]
        return b[1] - a[1], a[0] - b[0]
    return _cmul_const(a[0] - b[0], a[1] - b[1], j, n, sgn)


def _tw(v, j, sgn):
    if j == 0:
        return v
    if 4 * j == RS:
        return (v[1], -v[0]) if sgn < 0 else (-v[1], v[0])
    return _cmul_const(v[0], v[1], j, RS, sgn)


def _fft(v, sgn):
    n = len(v)
    if n == 1:
        return v
    h = n // 2
    ev = _fft([(v[j][0] + v[j + h][0], v[j][1] + v[j + h][1]) for j in range(h)], sgn)
    od = _fft([_diff_tw(v[j], v[j + h], j, n, sgn) for j in range(h)], sgn)
    out = [None] * n
    out[0::2] = ev
    out[1::2] = od
    return out


def _dot(a, b):
    return jnp.dot(a, b, preferred_element_type=f32)


def _asbf(v):
    return pltpu.bitcast(v, bf16)


def _cm(ar, ai, br, bi):
    return ar * br - ai * bi, ar * bi + ai * br


BU = 2 * NST + NCH


def _kernel(ax_hbm, mem_hbm, wq_hbm, wk_hbm, wv_hbm, wo_hbm, bx_hbm, wr_hbm, wi_hbm,
            R_hbm, L_hbm, sm_hbm, one_hbm, out_hbm,
            ax, xb3, xb, wo, pool, wpk, memb, ob, oa,
            bx, wr, wi, R, L, sm, Y, T, wp, nv, one, sems):
    srcs = (wq_hbm, wk_hbm, wv_hbm)
    lane8 = lax.broadcasted_iota(i32, (8, 128), 1)

    def chunk_copy(t, part=None):
        lo, n, sem = (0, 512, t % NST) if part is None else (part * 128, 128, 4 + part)
        return pltpu.make_async_copy(srcs[t // 4].at[:, pl.ds(lo, n), pl.ds(8 * (t % 4), 8), :],
                                     pool.at[pl.ds(2 * (t % NST), 2), pl.ds(lo, n)], sems.at[sem])

    def chunk_start(t):
        for m in range(3):
            @pl.when(t // 4 == m)
            def _(m=m):
                pltpu.make_async_copy(srcs[m].at[:, :, pl.ds(pl.multiple_of(8 * (t % 4), 8), 8), :],
                                      pool.at[pl.ds(2 * (t % NST), 2)], sems.at[t % NST]).start()

    def chunk_wait(t):
        blk = pool.at[pl.ds(2 * (t % NST), 2)]
        pltpu.make_async_copy(blk, blk, sems.at[t % NST]).wait()

    def xb_copy(q):
        return pltpu.make_async_copy(ax_hbm.at[pl.ds(16 * q, 16), 3], xb3.at[pl.ds(16 * q, 16)], sems.at[8 + q])

    def bx_copy(q):
        return pltpu.make_async_copy(bx_hbm.at[:, pl.ds(2 * q, 2)], bx.at[:, pl.ds(2 * q, 2)], sems.at[12 + q])

    def w_copy(q, i):
        cols = pl.ds(pl.multiple_of(512 * q, 512), 512)
        return pltpu.make_async_copy((wr_hbm, wi_hbm)[i].at[:, cols], (wr, wi)[i].at[:, cols], sems.at[16 + 4 * i + q])

    def wo_copy(j):
        return pltpu.make_async_copy(wo_hbm.at[:, pl.ds(128 * j, 128)], wo.at[j], sems.at[24])

    cp_r0 = pltpu.make_async_copy(R_hbm.at[pl.ds(0, 4)], R.at[pl.ds(0, 4)], sems.at[25])
    cp_r1 = pltpu.make_async_copy(R_hbm.at[pl.ds(4, 4)], R.at[pl.ds(4, 4)], sems.at[26])
    cp_l = pltpu.make_async_copy(L_hbm, L, sems.at[27])
    cp_ax = pltpu.make_async_copy(ax_hbm.at[:, pl.ds(0, 3)], ax, sems.at[28])
    cp_outb = pltpu.make_async_copy(bx, out_hbm.at[:, :, :, pl.ds(DM, D)], sems.at[29])
    cp_sm = pltpu.make_async_copy(sm_hbm, sm, sems.at[30])
    cp_one = pltpu.make_async_copy(one_hbm, one, sems.at[33])
    cp_mem = pltpu.make_async_copy(mem_hbm, memb, sems.at[31])

    cp_one.start()
    for part in range(4):
        chunk_copy(0, part).start()
    for q in range(4):
        xb_copy(q).start()
    chunk_copy(1).start()
    chunk_copy(2).start()
    chunk_copy(3).start()
    cp_r0.start()
    bx_copy(0).start()
    w_copy(0, 0).start()
    w_copy(0, 1).start()
    cp_sm.start()
    cp_mem.start()

    def prep(t, tpar, jj):
        lo = [bx[2 * jj:2 * jj + 2, t, :, 128 * e:128 * (e + 1)].astype(f32).reshape(16, 128) for e in range(8)]
        hi = [bx[HR + 2 * jj:HR + 2 * jj + 2, t, :, 128 * e:128 * (e + 1)].astype(f32).reshape(16, 128)
              for e in range(8)]
        for par in range(2):
            x = [lo[e] + hi[e] if par == 0 else lo[e] - hi[e] for e in range(8)]
            a = [x[j] + x[j + 4] for j in range(4)]
            b = [x[j] - x[j + 4] for j in range(4)]
            t1 = (b[1] - b[3]) * C8
            t2 = (b[1] + b[3]) * C8
            uu = [a[0] + a[2], a[1] + a[3], b[0] + t1, b[2] + t2,
                  a[0] - a[2], a[1] - a[3], b[0] - t1, b[2] - t2]
            for q in range(8):
                o = (((tpar * 2 + par) * 8 + q) * 8 + jj) * 2
                pool[BU, o:o + 2] = uu[q].reshape(2, 8, 128).astype(bf16)

    def unit1(t, tpar, par, cg):
        o = ((tpar * 2 + par) * 8 + 2 * cg) * 16
        u = jnp.concatenate([pool[BU, o:o + 16].reshape(128, 128),
                             pool[BU, o + 16:o + 32].reshape(128, 128)], axis=1)
        z = _dot(u, _asbf(R[cg]))
        v = [(z[8 * j:8 * j + 8, :128], z[8 * j:8 * j + 8, 128:]) for j in range(HR)]
        if cg == 0:
            V = nv[8 * tpar:8 * tpar + 8, :]
            for j in range(HR):
                vb = jnp.broadcast_to(v[j][1][:, 0:1], (8, 128))
                V = jnp.where(lane8 == 64 * par + 4 * j + t // 2, vb, V)
                v[j] = (v[j][0], jnp.where(lane8 == 0, 0.0, v[j][1]))
            nv[8 * tpar:8 * tpar + 8, :] = V
        if par == 1:
            v = [_tw(v[j], j, -1) for j in range(HR)]
        o = _fft(v, -1)
        for m in range(HR):
            Y[2 * m + par, cg, t] = jnp.concatenate(o[m], axis=0).astype(bf16)

    def wprep(pb, i):
        w = (wr, wi)[i]
        cols = pl.ds(pl.multiple_of(pb * 128, 128), 128)
        sub = lax.broadcasted_iota(i32, (8, 128), 0)
        msk = (jnp.where(sub % 2 == 0, jnp.uint32(0xffff), jnp.uint32(0))
               | jnp.where((sub % 4 == 0) | (sub % 4 == 3), jnp.uint32(0xffff0000), jnp.uint32(0)))
        t0 = pltpu.bitcast(w[0:256, cols], u32)
        t1 = pltpu.bitcast(w[256:512, cols], u32)
        ps, qs = [], []
        for j in range(16):
            a = t0[8 * j:8 * j + 8]
            b = t1[8 * j:8 * j + 8]
            b = jnp.where(sub % 2 == 0, pltpu.roll(b, 7, 0), pltpu.roll(b, 1, 0))
            x = (a ^ b) & msk
            ps.append(b ^ x)
            qs.append(a ^ x)
        for h, lst in enumerate((ps, qs)):
            tr = pltpu.bitcast(pltpu.bitcast(jnp.concatenate(lst, axis=0), f32).T, u32)
            for q in range(4):
                wp[i, h, pl.ds(pl.multiple_of((pb * 4 + q) * WP, 8), 32), :] = tr[32 * q:32 * q + 32]

    def fwd(p):
        return _dot(_asbf(L[p]), jnp.concatenate([Y[p, cg].reshape(128, 128) for cg in range(4)], axis=1))

    def filt(pbase, po, v):
        grs, gis = [None] * 4, [None] * 4
        win = pl.ds(pbase, (BS - 1) * WP + 16)
        for h in range(2):
            wr_ = wp.at[0, h, win][pl.ds(po, BS, stride=WP), :]
            wi_ = wp.at[1, h, win][pl.ds(po, BS, stride=WP), :]
            for hi in range(2):
                cg = 2 * h + hi
                if hi == 0:
                    a, b = wr_ << 16, wi_ << 16
                else:
                    a, b = wr_ & jnp.uint32(0xffff0000), wi_ & jnp.uint32(0xffff0000)
                grs[cg], gis[cg] = _cm(v[:BS, 128 * cg:128 * (cg + 1)], v[BS:, 128 * cg:128 * (cg + 1)],
                                       pltpu.bitcast(a, f32), pltpu.bitcast(b, f32))
        return jnp.concatenate([jnp.concatenate(grs, axis=1), jnp.concatenate(gis, axis=1)], axis=0).astype(bf16)

    def inv(p, g):
        t = _dot(_asbf(L[RS + p]), g)
        for cg in range(4):
            T[cg, p, 0:128, :] = t[:, 128 * cg:128 * (cg + 1)]

    nyq = {}

    def nyq_stage(k):
        n0 = 2 * RS
        twr, twi = sm[80:96, :], sm[96:112, :]
        if k == 0:
            v = nv[0:16, :].astype(bf16)
            r, i = _cm(_dot(v, _asbf(L[n0])), _dot(v, _asbf(L[n0 + 1])), twr, twi)
            nyq[0] = jnp.concatenate([r, i], axis=0).astype(bf16)
        elif k == 1:
            t = _dot(_asbf(L[n0 + 4, 0:16])[:, 0:32], nyq[0])
            ws = []
            for w in (wr, wi):
                row = w[512:513, :].astype(f32)
                ws.append(jnp.concatenate([row[:, 128 * r:128 * (r + 1)] for r in range(16)], axis=0))
            r, i = _cm(t[:16], t[16:], ws[0], ws[1])
            nyq[1] = jnp.concatenate([r, i], axis=0).astype(bf16)
        elif k == 2:
            t = _dot(_asbf(L[n0 + 4, 16:32])[:, 0:32], nyq[1])
            r, i = _cm(t[:16], t[16:], twr, -twi)
            nyq[2] = (r.astype(bf16), i.astype(bf16))
        elif k == 3:
            nv[16:32, :] = _dot(nyq[2][0], _asbf(L[n0 + 2])) + _dot(nyq[2][1], _asbf(L[n0 + 3]))

    def p3a(t, tpar, par, cg):
        rr = pl.ds(pl.multiple_of(t * 8, 8), 8)
        ri = pl.ds(pl.multiple_of(64 + t * 8, 8), 8)
        o = _fft([(T[cg, 2 * m + par, rr, :], T[cg, 2 * m + par, ri, :]) for m in range(HR)], +1)
        if par == 1:
            o = [_tw(o[j], j, +1) for j in range(HR)]
        if cg == 0:
            un = nv[16 + 8 * tpar:24 + 8 * tpar, :]
            o = [(o[j][0], jnp.where(lane8 == 0, pltpu.roll(un, (128 - 64 * par - 4 * j - t // 2) % 128, 1),
                                     o[j][1])) for j in range(HR)]
        return jnp.concatenate([jnp.concatenate([q[0] for q in o], axis=0),
                                jnp.concatenate([q[1] for q in o], axis=0)], axis=1).astype(bf16)

    def p3b(u, cg):
        z = _dot(u, _asbf(R[4 + cg]))
        return z[:, :128], z[:, 128:]

    def p3c(V):
        a = [V[0][0] + V[2][0], V[0][1] + V[2][1], V[0][0] - V[2][0], V[0][1] - V[2][1]]
        t1 = (V[1][0] - V[3][0]) * C8
        t2 = (V[1][1] - V[3][1]) * C8
        b = [V[1][0] + V[3][0], t1 + t2, V[1][1] + V[3][1], t2 - t1]
        return [a[j] + b[j] for j in range(4)] + [a[j] - b[j] for j in range(4)]

    def p3d(t, res):
        for e in range(8):
            bx[0:HR, t, :, 128 * e:128 * (e + 1)] = (res[0][e] + res[1][e]).reshape(HR, 8, 128).astype(bf16)
            bx[HR:RS, t, :, 128 * e:128 * (e + 1)] = (res[0][e] - res[1][e]).reshape(HR, 8, 128).astype(bf16)

    def runit(b0, d0, dst, k):
        a = pltpu.bitcast(jnp.concatenate([pool[b0, d0 + 2 * k], pool[b0 + 1, d0 + 2 * k]], axis=0), u32)
        b = pltpu.bitcast(jnp.concatenate([pool[b0, d0 + 2 * k + 1], pool[b0 + 1, d0 + 2 * k + 1]], axis=0), u32)
        dst[pl.ds(k, 8, stride=PW), :] = (a & jnp.uint32(0xffff)) | (b << 16)
        dst[pl.ds(8 * PW + k, 8, stride=PW), :] = (a >> 16) | (b & jnp.uint32(0xffff0000))

    def relayout_loop(t, lo, n):
        def body(i, c):
            dst = wpk.at[t, pl.ds(pl.multiple_of(i * 32, 32), 15 * PW + 32)]
            for k in range(32):
                runit(2 * (t % NST), i * 64, dst, k)
            return c
        lax.fori_loop(lo, lo + n, body, 0)

    def wsel(w, hl, lo=0, hi=DM):
        base = ((hl % 2) * 8 + hl // 2) * PW
        parts = []
        for kh in range(2):
            a, b = max(lo, 512 * kh), min(hi, 512 * (kh + 1))
            if a < b:
                o = base + 4 * PW * kh - 256 * kh
                parts.append(w[o + a // 2:o + b // 2, :])
        return _asbf(jnp.concatenate(parts, axis=0))

    def bulk(t, rel, side, mcs=range(4)):
        w = wpk.at[t]
        if rel:
            b0, dst = 2 * ((t + 1) & (NST - 1)), wpk.at[t + 1]
        bq = 2 * NST + (t & 15)
        for mc in mcs:
            x = _asbf(xb[mc * 64:(mc + 1) * 64, :])
            for h in range(8):
                n = mc * 8 + h
                r = _dot(x, wsel(w, h)).reshape(16, M, DH)
                if rel:
                    nn = (n - 1) % 32
                    for k in range(8 * nn, 8 * nn + 8):
                        runit(b0, 0, dst, k)
                if side is not None:
                    side(n)
                pool[bq, h * NSEG + mc * 16:h * NSEG + (mc + 1) * 16] = r.astype(bf16)

    with jax.named_scope("rel0"):
        for part in range(4):
            chunk_copy(0, part).wait()
            relayout_loop(0, 2 * part, 2)
    chunk_copy(4).start()
    with jax.named_scope("bulk0"):
        for q in range(4):
            xb_copy(q).wait()
            xb[64 * q:64 * (q + 1), :] = pltpu.bitcast(xb3[16 * q:16 * (q + 1)].reshape(128, DM), u32)
            bulk(0, False, None, mcs=[q])
    with jax.named_scope("rel1"):
        chunk_copy(1).wait()
        relayout_loop(1, 0, 8)
    bx_copy(1).start()
    w_copy(1, 0).start()
    w_copy(1, 1).start()
    chunk_copy(5).start()
    with jax.named_scope("w_c2"):
        chunk_copy(2).wait()
        cp_one.wait()
    with jax.named_scope("bulk1"):
        bulk(one[0], True, None)
    bx_copy(2).start()
    w_copy(2, 0).start()
    w_copy(2, 1).start()
    chunk_copy(6).start()
    bx_copy(3).start()
    w_copy(3, 0).start()
    w_copy(3, 1).start()
    cp_l.start()
    cp_r1.start()
    nv[0:16, :] = jnp.zeros((16, 128), f32)
    cp_r0.wait()

    def body1(q, c):
        t = q + 2
        with jax.named_scope("w_1"):
            chunk_wait(t + 1)
            bx_copy(q).wait()
            w_copy(q, 0).wait()
            w_copy(q, 1).wait()

        def side(n):
            if n < 8:
                prep(2 * q, 0, n)
            if 8 <= n < 16:
                prep(2 * q + 1, 1, n - 8)
            if 12 <= n < 28:
                k = n - 12
                unit1(2 * q + k // 8, k // 8, (k // 4) % 2, k % 4)
            if n % 4 == 1:
                wprep(4 * q + n // 8, (n // 4) % 2)
        with jax.named_scope("bulk_p1"):
            bulk(t, True, side)
        chunk_start(t + 1 + NST)
        return c
    lax.fori_loop(0, 4, body1, 0)

    cp_ax.start()
    with jax.named_scope("w_l"):
        cp_l.wait()
        cp_r1.wait()
        cp_sm.wait()

    def body2(q, c):
        t = q + 6
        with jax.named_scope("w_2"):
            chunk_wait(t + 1)
        gs = {}

        def side(n):
            po = n // 2
            if n % 2 == 0:
                gs[po] = filt(pl.multiple_of(16 * q, 16), po, fwd(16 * q + po))
            elif po >= 1:
                inv(16 * q + po - 1, gs.pop(po - 1))
            if n == 31:
                inv(16 * q + 15, gs.pop(15))
            if n % 4 == 2 and n // 4 < 4:
                nyq_stage(n // 4)
        with jax.named_scope("bulk_p2"):
            bulk(t, True, side)

        @pl.when(q == 0)
        def _():
            chunk_copy(11).start()
            for j in range(8):
                wo_copy(j).start()
        return c
    lax.fori_loop(0, 2, body2, 0)

    def body3(q, c):
        t = q + 8

        @pl.when(q < 3)
        def _():
            with jax.named_scope("w_3"):
                chunk_wait(t + 1)
        us, vs, res = {}, {}, {}

        def side(n):
            if n < 16:
                us[n] = p3a(2 * q + n // 8, n // 8, (n // 4) % 2, n % 4)
            k = n - 2
            if 0 <= k < 16:
                vs[k] = p3b(us.pop(k), k % 4)
            k = n - 4
            if 0 <= k < 16 and k % 4 == 3:
                res[k // 4] = p3c([vs.pop(k - 3 + i) for i in range(4)])
                if k % 8 == 7:
                    p3d(2 * q + k // 8, [res.pop(k // 4 - 1), res.pop(k // 4)])
        with jax.named_scope("bulk_p3"):
            bulk(t, True, side)
        return c
    lax.fori_loop(0, 4, body3, 0)
    cp_outb.start()

    with jax.named_scope("w_wo"):
        cp_ax.wait()
        cp_mem.wait()
        for j in range(8):
            wo_copy(j).wait()
    scale = DH ** -0.5
    KS = 768

    def step(it, u):
        s = it * U + u
        lhs = jnp.concatenate([ax[s].reshape(FR, DM), memb[...]], axis=0)
        qs, ks, vs, ps, os_, pre = {}, {}, {}, {}, {}, {}

        def ws(m, h, lo=0, hi=DM):
            return wsel(wpk.at[4 * m + h // 8], h % 8, lo, hi)
        if u > 0:
            for m in range(2):
                for h in range(2):
                    pre[(m, h)] = -_dot(lhs[:, :KS], ws(m, h, 0, KS))

        def dotw(m, h):
            if (m, h) in pre:
                return _dot(lhs[:, KS:], ws(m, h, KS, DM)) - pre[(m, h)]
            return _dot(lhs, ws(m, h))

        def proj(m, g):
            h = 2 * g
            return jnp.concatenate([dotw(m, h).astype(bf16), dotw(m, h + 1).astype(bf16),
                                    pool[2 * NST + 4 * m + h // 8, (h % 8) * NSEG + s],
                                    pool[2 * NST + 4 * m + h // 8, (h % 8 + 1) * NSEG + s]], axis=0)

        def qk(g):
            sc = lax.dot_general(qs.pop(g), ks.pop(g), (((1,), (1,)), ((), ())),
                                 preferred_element_type=f32) * scale
            fill = sm[0:80, 0:80]
            sc = jnp.where(fill == 0.0, sc, fill)
            mx = jnp.max(sc, axis=-1, keepdims=True)
            e = jnp.exp(sc - mx)
            l = jnp.sum(e, axis=-1, keepdims=True)
            r = pl.reciprocal(l, approx=True)
            r = r * (2.0 - l * r)
            ps[g] = (e * r).astype(bf16)

        def pv(g):
            o = _dot(ps.pop(g), vs.pop(g))
            os_[2 * g] = o[0:32].astype(bf16)
            os_[2 * g + 1] = o[32:64].astype(bf16)
            ob[8 * u:8 * u + 8, (2 * g) * DH:(2 * g + 1) * DH] = o[64:72]
            ob[8 * u:8 * u + 8, (2 * g + 1) * DH:(2 * g + 2) * DH] = o[72:80]

        def olhs(lo, hi):
            oc = jnp.concatenate([os_[h] for h in range(lo, hi)], axis=1)
            if u == U - 1:
                oc = jnp.concatenate([oc, ob[:, lo * DH:hi * DH].astype(bf16)], axis=0)
            return oc

        sk, dq, dp = 4, 2, 3
        for t in range(G + sk):
            if t < G:
                qs[t] = proj(0, t)
            if 0 <= t - dq < G:
                qk(t - dq)
            if t < G:
                ks[t] = proj(1, t)
            if t - sk - dp >= 0:
                pv(t - sk - dp)
            if t - sk >= 0:
                vs[t - sk] = proj(2, t - sk)
        rem = list(range(G - dp, G))
        acc = []
        oc = olhs(0, 16)
        for j in range(DM // 128):
            acc.append(-_dot(oc, wo[j, 0:16 * DH, :]))
            if rem:
                pv(rem.pop(0))
        oc = olhs(16, 32)
        for j in range(DM // 128):
            cols = slice(j * 128, (j + 1) * 128)
            r = _dot(oc, wo[j, 16 * DH:32 * DH, :]) - acc[j]
            oa[it * 2 + u // 2, pl.ds((u % 2) * 4, 3), :, cols] = r[0:FR].reshape(3, 8, 128).astype(bf16)
            memb[:, cols] = r[FR:SEG].astype(bf16)
            if u == U - 1:
                for uu in range(U):
                    oa[it * 2 + uu // 2, (uu % 2) * 4 + 3, :, cols] = r[SEG + 8 * uu:SEG + 8 * uu + 8].astype(bf16)

    def out_copy(it):
        return pltpu.make_async_copy(oa.at[pl.ds(it * 2, 2)],
                                     out_hbm.at[pl.ds(it * 2, 2), :, :, pl.ds(0, DM)], sems.at[32])

    def group(it, c):
        with jax.named_scope("grp"):
            for u in range(U):
                step(it, u)
        out_copy(it).start()
        return c
    lax.fori_loop(0, NSEG // U, group, 0)
    with jax.named_scope("w_out"):
        for it in range(NSEG // U):
            out_copy(it).wait()
        cp_outb.wait()


def pallas_concat_heads__memory_aug_recurrent_mem_tr__spectral_gfnet__prompt_kernel(
    A_x, A_mem0, A_Wq, A_Wk, A_Wv, A_Wo, A_seg_len, B_x, B_w_r, B_w_i,
):
    del A_seg_len
    R, LN, TW, fill = _tables()
    small = np.zeros((112, 128), np.float32)
    small[:80, :80] = fill
    small[80:] = TW
    hbm = pl.BlockSpec(memory_space=pl.ANY)
    out = pl.pallas_call(
        _kernel,
        out_shape=jax.ShapeDtypeStruct((RS, 8, 8, DM + D), bf16),
        in_specs=[hbm] * 13,
        out_specs=hbm,
        scratch_shapes=[
            pltpu.VMEM((NSEG, 3, 8, DM), bf16),
            pltpu.VMEM((NSEG, 8, DM), bf16),
            pltpu.VMEM((NSEG * M // 2, DM), u32),
            pltpu.VMEM((DM // 128, H * DH, 128), bf16),
            pltpu.VMEM((2 * NST + NCH + 1, DM // 2, 8, DH), bf16),
            pltpu.VMEM((NCH + 1, 16 * PW, DH), u32),
            pltpu.VMEM((M, DM), bf16),
            pltpu.VMEM((U * M, H * DH), f32),
            pltpu.VMEM((RS, 8, 8, DM), bf16),
            pltpu.VMEM((RS, 8, 8, D), bf16),
            pltpu.VMEM((D // 2 + 1, S), bf16),
            pltpu.VMEM((D // 2 + 1, S), bf16),
            pltpu.VMEM((8, 128, 256), u32),
            pltpu.VMEM((2 * RS + 5, 64, 128), u32),
            pltpu.VMEM((112, 128), f32),
            pltpu.VMEM((RS, 4, 8, 16, 128), bf16),
            pltpu.VMEM((4, RS, TP, 128), f32),
            pltpu.VMEM((2, 2, BS * WP, 128), u32),
            pltpu.VMEM((32, 128), f32),
            pltpu.SMEM((8,), i32),
            pltpu.SemaphoreType.DMA((34,)),
        ],
        compiler_params=pltpu.CompilerParams(vmem_limit_bytes=124 * 1024 * 1024),
    )(A_x.reshape(NSEG, 4, 8, DM), A_mem0.reshape(M, DM),
      A_Wq.reshape(2, DM // 2, H, DH), A_Wk.reshape(2, DM // 2, H, DH), A_Wv.reshape(2, DM // 2, H, DH),
      A_Wo.reshape(H * DH, DM), B_x.reshape(RS, 8, 8, D), B_w_r.T, B_w_i.T,
      jnp.asarray(R), jnp.asarray(LN), jnp.asarray(small), jnp.asarray(np.arange(1, 9, dtype=np.int32)))
    return out.reshape(1, S, DM + D)
```

```python
import functools
import math

import jax
import jax.numpy as jnp
import numpy as np
from jax import lax
import jax.experimental.pallas as pl
import jax.experimental.pallas.tpu as pltpu

bf16, f32, u32, i32 = jnp.bfloat16, jnp.float32, jnp.uint32, jnp.int32

S, DM, H, DH, M, SEG = 2048, 1024, 32, 128, 8, 32
NSEG = S // SEG
FR = SEG - M
G = H // 2
U = 4
NCH = 12
NST = 4
PW = 264

D = 1024
RS, BS = 32, 64
HR = RS // 2
WP = 40
TP = 136
C8 = float(np.sqrt(0.5))


def _pack_rows(a):
    u = np.asarray(a, np.float32).astype(jnp.bfloat16).view(np.uint16).astype(np.uint32)
    return u[..., 0::2, :] | (u[..., 1::2, :] << 16)


_RHO = (2, 4, 4, 4)


def _in_a(lane, c):
    return (lane % 4 < 2) if c == 0 else ((lane + 2) % 8 < 4)


def _dstage(x, kc, roll64):
    a = [x[j] + x[j + 4] for j in range(4)]
    b = [x[j] - x[j + 4] for j in range(4)]
    t1 = (b[1] - b[3]) * C8
    t2 = (b[1] + b[3]) * C8
    s0, s1 = a[0] + a[2], a[1] + a[3]
    out = [s0 + s1, s0 - s1]
    for c, (u, v) in enumerate(((b[0] + t1, b[2] + t2), (a[0] - a[2], a[1] - a[3]), (b[0] - t1, b[2] - t2))):
        g = u * kc[4 * c] + v * kc[4 * c + 1]
        h = roll64(u * kc[4 * c + 2] + v * kc[4 * c + 3])
        out += [g + h, g - h]
    return out


def _dstage_t(p, kc, roll64):
    uv = []
    for c in range(3):
        g = p[2 + 2 * c] + p[3 + 2 * c]
        h = roll64(p[2 + 2 * c] - p[3 + 2 * c])
        uv.append((g * kc[4 * c] + h * kc[4 * c + 2], g * kc[4 * c + 1] + h * kc[4 * c + 3]))
    s0, s1 = p[0] + p[1], p[0] - p[1]
    a = [s0 + uv[1][0], s1 + uv[1][1], s0 - uv[1][0], s1 - uv[1][1]]
    t1 = (uv[0][0] - uv[2][0]) * C8
    t2 = (uv[0][1] - uv[2][1]) * C8
    b = [uv[0][0] + uv[2][0], t1 + t2, uv[0][1] + uv[2][1], t2 - t1]
    return [a[j] + b[j] for j in range(4)] + [a[j] - b[j] for j in range(4)]


@functools.lru_cache(maxsize=None)
def _tables():
    kcol = np.zeros((4, 128), np.int64)
    for l in range(128):
        i0, i1 = l, 128 + (l ^ 1)
        ev, o3 = l % 2 == 0, l % 4 in (0, 3)
        kcol[0, l] = 2 * (i0 if ev else i1)
        kcol[2, l] = 2 * (i1 if ev else i0)
        kcol[1, l] = 2 * (i0 if o3 else i1) + 1
        kcol[3, l] = 2 * (i1 if o3 else i0) + 1
    lanes = np.arange(128)
    lo = lanes < 64
    KC = np.zeros((12, 128))
    for c, sg in ((1, -1.0), (2, -1.0), (3, 1.0)):
        tr, ti = np.cos(2 * np.pi * c / 16), -np.sin(2 * np.pi * c / 16)
        KC[4 * c - 4] = np.where(lo, 1.0, ti)
        KC[4 * c - 3] = sg * np.where(lo, 0.0, tr)
        KC[4 * c - 2] = np.where(lo, 0.0, tr)
        KC[4 * c - 1] = sg * np.where(lo, 1.0, -ti)
    eye = np.eye(D)
    Bt = _dstage([eye[:, 128 * e:128 * (e + 1)] for e in range(8)], KC, lambda v: np.roll(v, 64, axis=1))
    d = np.arange(D)
    R = np.zeros((16, 128, 128))
    for c in range(4):
        rho = _RHO[c]
        inA = _in_a(lanes, c)
        ang = 2 * np.pi * (np.outer(d, kcol[c]) % D) / D
        fr, fi = np.cos(ang), -np.sin(ang)
        wr_, wi_ = np.full(128, 2.0), np.full(128, 2.0)
        if c == 0:
            fi[:, 0] = (-1.0) ** d
            wr_[0] = 1.0
            wi_[0] = 1.0
        fi, wi_ = np.roll(fi, -rho, axis=1), np.roll(wi_, -rho)
        for h in range(2):
            own = inA if h == 0 else ~inA
            ft, wt = np.where(own, fr, fi), np.where(own, wr_, wi_)
            bt = Bt[2 * c + h]
            r = (bt.T @ ft) / (bt * bt).sum(axis=0)[:, None]
            assert np.abs(bt @ r - ft).max() < 1e-9
            R[2 * c + h] = r
            R[8 + 2 * c + h] = (wt[:, None] * r.T) / (S * D)
    L = np.zeros((2 * RS, 128, 128))
    bb = np.arange(BS)
    kord = np.array([ri * 64 + 8 * t + r for t in range(8) for ri in range(2) for r in range(8)])
    for p1 in range(RS):
        ang = 2 * np.pi * (np.outer(p1 + RS * bb, bb) % S) / S
        mr, mi = np.cos(ang), -np.sin(ang)
        full = np.block([[mr, -mi], [mi, mr]])
        L[p1] = full[:, kord]
        L[RS + p1] = full.T
    l_, q_ = np.arange(128), np.arange(16)
    ang = 2 * np.pi * (np.outer(l_, l_) % 128) / 128
    N1 = np.concatenate([np.cos(ang), -np.sin(ang)], axis=1)
    N1 = np.concatenate([(N1[:64] + N1[64:]) / 2, (N1[:64] - N1[64:]) / 2], axis=0)
    ang = 2 * np.pi * np.outer(q_, l_) / S
    TW = np.concatenate([np.cos(ang), -np.sin(ang)], axis=0)
    ang = 2 * np.pi * (np.outer(q_, q_) % 16) / 16
    fr, fi = np.cos(ang), -np.sin(ang)
    F16 = np.block([[fr, -fi], [fi, fr]])
    NY = np.zeros((5, 128, 128))
    NY[0], NY[1], NY[2], NY[3] = N1[:, :128], N1[:, 128:], N1[:, :128].T, N1[:, 128:].T
    NY[4, :32, :32] = F16
    NY[4, 32:64, :32] = F16.T
    LN = np.concatenate([L, NY], axis=0)
    head = np.zeros(80, np.int32)
    pos = np.zeros(80, np.int32)
    for r in range(80):
        if r < 64:
            head[r] = r // 32
            t = r % 32
            pos[r] = (M + t) if t < FR else (t - FR)
        else:
            head[r] = (r - 64) // 8
            pos[r] = M + FR + (r - 64) % 8
    same = head[:, None] == head[None, :]
    vis = (pos[:, None] < M) | (pos[:, None] >= pos[None, :])
    fill = np.where(same, np.where(vis, 0.0, -1e9), -np.inf).astype(np.float32)
    return _pack_rows(R), _pack_rows(LN), TW.astype(np.float32), fill, KC.astype(np.float32)


def _cmul_const(re, im, j, n, sgn):
    ang = sgn * 2 * math.pi * j / n
    c, s = math.cos(ang), math.sin(ang)
    if abs(abs(c) - abs(s)) < 1e-12:
        if c * s > 0:
            return (re - im) * c, (re + im) * c
        return (re + im) * c, (im - re) * c
    return re * c - im * s, re * s + im * c


def _diff_tw(a, b, j, n, sgn):
    if j == 0:
        return a[0] - b[0], a[1] - b[1]
    if 4 * j == n:
        if sgn < 0:
            return a[1] - b[1], b[0] - a[0]
        return b[1] - a[1], a[0] - b[0]
    return _cmul_const(a[0] - b[0], a[1] - b[1], j, n, sgn)


def _tw(v, j, sgn):
    if j == 0:
        return v
    if 4 * j == RS:
        return (v[1], -v[0]) if sgn < 0 else (-v[1], v[0])
    return _cmul_const(v[0], v[1], j, RS, sgn)


def _fft(v, sgn):
    n = len(v)
    if n == 1:
        return v
    h = n // 2
    ev = _fft([(v[j][0] + v[j + h][0], v[j][1] + v[j + h][1]) for j in range(h)], sgn)
    od = _fft([_diff_tw(v[j], v[j + h], j, n, sgn) for j in range(h)], sgn)
    out = [None] * n
    out[0::2] = ev
    out[1::2] = od
    return out


def _dot(a, b):
    return jnp.dot(a, b, preferred_element_type=f32)


def _asbf(v):
    return pltpu.bitcast(v, bf16)


def _cm(ar, ai, br, bi):
    return ar * br - ai * bi, ar * bi + ai * br


BU = 2 * NST + NCH


def _kernel(ax_hbm, mem_hbm, wq_hbm, wk_hbm, wv_hbm, wo_hbm, bx_hbm, wr_hbm, wi_hbm,
            R_hbm, L_hbm, sm_hbm, one_hbm, out_hbm,
            ax, xb3, xb, wo, pool, wpk, memb, ob, oa,
            bx, wr, wi, R, L, sm, Y, T, wp, nv, one, sems):
    srcs = (wq_hbm, wk_hbm, wv_hbm)
    lane8 = lax.broadcasted_iota(i32, (8, 128), 1)

    def chunk_copy(t):
        return pltpu.make_async_copy(srcs[t // 4].at[:, :, pl.ds(8 * (t % 4), 8), :],
                                     pool.at[pl.ds(2 * (t % NST), 2)], sems.at[t % NST])

    def part_sem(t, part):
        return sems.at[34 + jnp.where(t == 0, 0, 2 + 2 * t) + part]

    def part_start(t, part, n):
        pltpu.make_async_copy(srcs[0].at[:, pl.ds(part * n, n), pl.ds(8 * t, 8), :],
                              pool.at[pl.ds(2 * t, 2), pl.ds(part * n, n)], part_sem(t, part)).start()

    def part_wait(t, part, n):
        blk = pool.at[pl.ds(2 * t, 2), pl.ds(part * n, n)]
        pltpu.make_async_copy(blk, blk, part_sem(t, part)).wait()

    def chunk_start(t):
        for m in range(3):
            @pl.when(t // 4 == m)
            def _(m=m):
                pltpu.make_async_copy(srcs[m].at[:, :, pl.ds(pl.multiple_of(8 * (t % 4), 8), 8), :],
                                      pool.at[pl.ds(2 * (t % NST), 2)], sems.at[t % NST]).start()

    def chunk_wait(t):
        blk = pool.at[pl.ds(2 * (t % NST), 2)]
        pltpu.make_async_copy(blk, blk, sems.at[t % NST]).wait()

    def xb_copy(q):
        return pltpu.make_async_copy(ax_hbm.at[pl.ds(16 * q, 16), 3], xb3.at[pl.ds(16 * q, 16)], sems.at[8 + q])

    def bx_copy(q):
        return pltpu.make_async_copy(bx_hbm.at[:, pl.ds(2 * q, 2)], bx.at[:, pl.ds(2 * q, 2)], sems.at[12 + q])

    def w_copy(q, i):
        cols = pl.ds(pl.multiple_of(512 * q, 512), 512)
        return pltpu.make_async_copy((wr_hbm, wi_hbm)[i].at[:, cols], (wr, wi)[i].at[:, cols], sems.at[16 + 4 * i + q])

    def wo_copy(j):
        return pltpu.make_async_copy(wo_hbm.at[:, pl.ds(128 * j, 128)], wo.at[j], sems.at[24])

    cp_r0 = pltpu.make_async_copy(R_hbm.at[pl.ds(0, 8)], R.at[pl.ds(0, 8)], sems.at[25])
    cp_r1 = pltpu.make_async_copy(R_hbm.at[pl.ds(8, 8)], R.at[pl.ds(8, 8)], sems.at[26])
    cp_l = pltpu.make_async_copy(L_hbm, L, sems.at[27])
    cp_ax = pltpu.make_async_copy(ax_hbm.at[:, pl.ds(0, 3)], ax, sems.at[28])
    cp_outb = pltpu.make_async_copy(bx, out_hbm.at[:, :, :, pl.ds(DM, D)], sems.at[29])
    cp_sm = pltpu.make_async_copy(sm_hbm, sm, sems.at[30])
    cp_one = pltpu.make_async_copy(one_hbm, one, sems.at[33])
    cp_mem = pltpu.make_async_copy(mem_hbm, memb, sems.at[31])

    for part in range(4):
        part_start(0, part, 128)
    cp_one.start()
    xb_copy(0).start()
    xb_copy(1).start()
    part_start(1, 0, 256)
    xb_copy(2).start()
    part_start(1, 1, 256)
    xb_copy(3).start()
    part_start(2, 0, 256)
    part_start(2, 1, 256)
    chunk_copy(3).start()
    cp_r0.start()
    bx_copy(0).start()
    w_copy(0, 0).start()
    w_copy(0, 1).start()
    cp_sm.start()
    cp_mem.start()

    def kc():
        return [jnp.concatenate([sm[112 + 8 * i:120 + 8 * i, :]] * 2, axis=0) for i in range(12)]

    def roll64(v):
        return pltpu.roll(v, 64, 1)

    def dot2(u, w):
        if 0 == 0:
            return _dot(u, w)
        return jnp.concatenate([_dot(u[:64], w), _dot(u[64:], w)], axis=0)

    def prep(t, tpar, jj):
        lo = [bx[2 * jj:2 * jj + 2, t, :, 128 * e:128 * (e + 1)].astype(f32).reshape(16, 128) for e in range(8)]
        hi = [bx[HR + 2 * jj:HR + 2 * jj + 2, t, :, 128 * e:128 * (e + 1)].astype(f32).reshape(16, 128)
              for e in range(8)]
        for par in range(2):
            x = [lo[e] + hi[e] if par == 0 else lo[e] - hi[e] for e in range(8)]
            uu = _dstage(x, kc(), roll64)
            for q in range(8):
                o = (((tpar * 2 + par) * 8 + q) * 8 + jj) * 2
                pool[BU, o:o + 2] = uu[q].reshape(2, 8, 128).astype(bf16)

    def unit1(t, tpar, par, cg):
        o = ((tpar * 2 + par) * 8 + 2 * cg) * 16
        za = dot2(pool[BU, o:o + 16].reshape(128, 128), _asbf(R[2 * cg]))
        zb = dot2(pool[BU, o + 16:o + 32].reshape(128, 128), _asbf(R[2 * cg + 1]))
        ina = _in_a(lane8, cg)
        v = []
        for j in range(HR):
            pa, pb = za[8 * j:8 * j + 8], zb[8 * j:8 * j + 8]
            v.append((jnp.where(ina, pa, pb), pltpu.roll(jnp.where(ina, pb, pa), _RHO[cg], 1)))
        if cg == 0:
            V = nv[8 * tpar:8 * tpar + 8, :]
            for j in range(HR):
                vb = jnp.broadcast_to(v[j][1][:, 0:1], (8, 128))
                V = jnp.where(lane8 == 64 * par + 4 * j + t // 2, vb, V)
                v[j] = (v[j][0], jnp.where(lane8 == 0, 0.0, v[j][1]))
            nv[8 * tpar:8 * tpar + 8, :] = V
        if par == 1:
            v = [_tw(v[j], j, -1) for j in range(HR)]
        o = _fft(v, -1)
        for m in range(HR):
            Y[2 * m + par, cg, t] = jnp.concatenate(o[m], axis=0).astype(bf16)

    def wprep(pb, i):
        w = (wr, wi)[i]
        cols = pl.ds(pl.multiple_of(pb * 128, 128), 128)
        sub = lax.broadcasted_iota(i32, (8, 128), 0)
        msk = (jnp.where(sub % 2 == 0, jnp.uint32(0xffff), jnp.uint32(0))
               | jnp.where((sub % 4 == 0) | (sub % 4 == 3), jnp.uint32(0xffff0000), jnp.uint32(0)))
        t0 = pltpu.bitcast(w[0:256, cols], u32)
        t1 = pltpu.bitcast(w[256:512, cols], u32)
        ps, qs = [], []
        for j in range(16):
            a = t0[8 * j:8 * j + 8]
            b = t1[8 * j:8 * j + 8]
            b = jnp.where(sub % 2 == 0, pltpu.roll(b, 7, 0), pltpu.roll(b, 1, 0))
            x = (a ^ b) & msk
            ps.append(b ^ x)
            qs.append(a ^ x)
        for h, lst in enumerate((ps, qs)):
            tr = pltpu.bitcast(pltpu.bitcast(jnp.concatenate(lst, axis=0), f32).T, u32)
            for q in range(4):
                wp[i, h, pl.ds(pl.multiple_of((pb * 4 + q) * WP, 8), 32), :] = tr[32 * q:32 * q + 32]

    def fwd(p):
        return _dot(_asbf(L[p]), jnp.concatenate([Y[p, cg].reshape(128, 128) for cg in range(4)], axis=1))

    def filt(pbase, po, v):
        grs, gis = [None] * 4, [None] * 4
        win = pl.ds(pbase, (BS - 1) * WP + 8)
        for h in range(2):
            wr_ = wp.at[0, h, win][pl.ds(po, BS, stride=WP), :]
            wi_ = wp.at[1, h, win][pl.ds(po, BS, stride=WP), :]
            for hi in range(2):
                cg = 2 * h + hi
                if hi == 0:
                    a, b = wr_ << 16, wi_ << 16
                else:
                    a, b = wr_ & jnp.uint32(0xffff0000), wi_ & jnp.uint32(0xffff0000)
                grs[cg], gis[cg] = _cm(v[:BS, 128 * cg:128 * (cg + 1)], v[BS:, 128 * cg:128 * (cg + 1)],
                                       pltpu.bitcast(a, f32), pltpu.bitcast(b, f32))
        return jnp.concatenate([jnp.concatenate(grs, axis=1), jnp.concatenate(gis, axis=1)], axis=0).astype(bf16)

    def inv(p, g):
        t = _dot(_asbf(L[RS + p]), g)
        for cg in range(4):
            T[cg, p, 0:128, :] = t[:, 128 * cg:128 * (cg + 1)]

    nyq = {}

    def nyq_stage(k):
        n0 = 2 * RS
        twr, twi = sm[80:96, :], sm[96:112, :]
        if k == 0:
            v = nv[0:16, :].astype(bf16)
            r, i = _cm(_dot(v, _asbf(L[n0])), _dot(v, _asbf(L[n0 + 1])), twr, twi)
            nyq[0] = jnp.concatenate([r, i], axis=0).astype(bf16)
        elif k == 1:
            t = _dot(_asbf(L[n0 + 4, 0:16])[:, 0:32], nyq[0])
            ws = []
            for w in (wr, wi):
                row = w[512:513, :].astype(f32)
                ws.append(jnp.concatenate([row[:, 128 * r:128 * (r + 1)] for r in range(16)], axis=0))
            r, i = _cm(t[:16], t[16:], ws[0], ws[1])
            nyq[1] = jnp.concatenate([r, i], axis=0).astype(bf16)
        elif k == 2:
            t = _dot(_asbf(L[n0 + 4, 16:32])[:, 0:32], nyq[1])
            r, i = _cm(t[:16], t[16:], twr, -twi)
            nyq[2] = (r.astype(bf16), i.astype(bf16))
        elif k == 3:
            nv[16:32, :] = _dot(nyq[2][0], _asbf(L[n0 + 2])) + _dot(nyq[2][1], _asbf(L[n0 + 3]))

    def p3a(t, tpar, par, cg):
        rr = pl.ds(pl.multiple_of(t * 8, 8), 8)
        ri = pl.ds(pl.multiple_of(64 + t * 8, 8), 8)
        o = _fft([(T[cg, 2 * m + par, rr, :], T[cg, 2 * m + par, ri, :]) for m in range(HR)], +1)
        if par == 1:
            o = [_tw(o[j], j, +1) for j in range(HR)]
        if cg == 0:
            un = nv[16 + 8 * tpar:24 + 8 * tpar, :]
            o = [(o[j][0], jnp.where(lane8 == 0, pltpu.roll(un, (128 - 64 * par - 4 * j - t // 2) % 128, 1),
                                     o[j][1])) for j in range(HR)]
        ina = _in_a(lane8, cg)
        ua, ub = [], []
        for re, im in o:
            im = pltpu.roll(im, 128 - _RHO[cg], 1)
            ua.append(jnp.where(ina, re, im))
            ub.append(jnp.where(ina, im, re))
        return [[jnp.concatenate(x[8 * i:8 * i + 8], axis=0).astype(bf16) for i in range(2)] for x in (ua, ub)]

    def p3b(u, tpar, par, cg):
        for h in range(2):
            for i in range(2):
                z = _dot(u[h][i], _asbf(R[8 + 2 * cg + h]))
                o = (par * 8 + 2 * cg + h) * 32 + 16 * i
                pool[BU + tpar, o:o + 16] = _asbf(z).reshape(16, 8, 128)

    def p3c(t, tpar, j0, nj):
        res = []
        for par in range(2):
            p = []
            for q in range(8):
                o = (par * 8 + q) * 32 + 2 * j0
                p.append(pltpu.bitcast(pool[BU + tpar, o:o + 2 * nj].reshape(16 * nj, 128), f32))
            res.append(_dstage_t(p, kc(), roll64))
        for e in range(8):
            cols = slice(128 * e, 128 * (e + 1))
            bx[j0:j0 + nj, t, :, cols] = (res[0][e] + res[1][e]).reshape(nj, 8, 128).astype(bf16)
            bx[HR + j0:HR + j0 + nj, t, :, cols] = (res[0][e] - res[1][e]).reshape(nj, 8, 128).astype(bf16)

    def runit(b0, d0, dst, k):
        a = pltpu.bitcast(jnp.concatenate([pool[b0, d0 + 2 * k], pool[b0 + 1, d0 + 2 * k]], axis=0), u32)
        b = pltpu.bitcast(jnp.concatenate([pool[b0, d0 + 2 * k + 1], pool[b0 + 1, d0 + 2 * k + 1]], axis=0), u32)
        dst[pl.ds(k, 8, stride=PW), :] = (a & jnp.uint32(0xffff)) | (b << 16)
        dst[pl.ds(8 * PW + k, 8, stride=PW), :] = (a >> 16) | (b & jnp.uint32(0xffff0000))

    def wsel(w, hl, lo=0, hi=DM):
        base = ((hl % 2) * 8 + hl // 2) * PW
        parts = []
        for kh in range(2):
            a, b = max(lo, 512 * kh), min(hi, 512 * (kh + 1))
            if a < b:
                o = base + 4 * PW * kh - 256 * kh
                parts.append(w[o + a // 2:o + b // 2, :])
        return _asbf(jnp.concatenate(parts, axis=0))

    def bulk(t, mc0, nmc, tsrc, tdst, k0, nk, side=None, tokrow=0):
        w = wpk.at[t]
        b0 = 2 * (tsrc & (NST - 1))
        dst = wpk.at[tdst, pl.ds(k0, 15 * PW + nk)]
        bq = 2 * NST + (t & 15)
        zero = one[1]
        toks = []
        ns = 8 * nmc
        per = nk // ns
        for mi in range(nmc):
            mc = mc0 + mi
            x = _asbf(xb[mc])
            for h in range(8):
                n = mi * 8 + h
                r = _dot(x, wsel(w, h)).reshape(16, M, DH)
                nn = (n - 1) % ns
                for k in range(per * nn, per * (nn + 1)):
                    runit(b0, 2 * k0, dst, k)
                if side is not None:
                    side(n, lambda back, n=n: toks[n - back] if n >= back else 0)
                    toks.append(pltpu.bitcast(r[tokrow], i32)[0, 0] & zero)
                pool[bq, pl.ds(h * NSEG + mc * 16, 16)] = r.astype(bf16)

    def rel0(i, c):
        @pl.when(i % 2 == 0)
        def _():
            part_wait(0, i // 2, 128)
        dst = wpk.at[0, pl.ds(pl.multiple_of(i * 32, 32), 15 * PW + 32)]
        for k in range(32):
            runit(0, i * 64, dst, k)
        return c
    with jax.named_scope("rel0"):
        lax.fori_loop(0, 8, rel0, 0)
    cp_one.wait()

    def body0(i, c):
        t, mc = i // 4, i % 4
        real = mc >= 2

        @pl.when(t == 0)
        def _():
            xb_copy(mc).wait()
            xb[mc] = pltpu.bitcast(xb3[pl.ds(16 * mc, 16)].reshape(128, DM), u32)

        @pl.when(real)
        def _():
            part_wait(t + 1, mc - 2, 256)
        with jax.named_scope("bulk0"):
            bulk(t, mc, 1, jnp.where(real, t + 1, t), jnp.where(real, t + 1, NCH),
                 pl.multiple_of((mc % 2) * 128, 128), 128)

        @pl.when(i == 1)
        def _():
            chunk_copy(4).start()
            bx_copy(1).start()
            w_copy(1, 0).start()
            w_copy(1, 1).start()

        @pl.when(i == 5)
        def _():
            chunk_copy(5).start()
        return c
    lax.fori_loop(0, 8, body0, 0)
    bx_copy(2).start()
    w_copy(2, 0).start()
    w_copy(2, 1).start()
    chunk_copy(6).start()
    bx_copy(3).start()
    w_copy(3, 0).start()
    w_copy(3, 1).start()
    cp_l.start()
    cp_r1.start()
    nv[0:16, :] = jnp.zeros((16, 128), f32)
    cp_r0.wait()
    cp_sm.wait()

    def body1(q, c):
        t = q + 2
        with jax.named_scope("w_1"):
            chunk_wait(t + 1)
            bx_copy(q).wait()
            w_copy(q, 0).wait()
            w_copy(q, 1).wait()

        def side(n, z):
            sq = 1
            ks = list(range(sq + 1)) if n == 0 else [n + sq]
            for k in ks:
                if k < 16:
                    prep(2 * q + k // 8 + z(2), k // 8, k % 8)
            k = n - 15
            if 0 <= k < 16:
                unit1(2 * q + k // 8, k // 8, (k // 4) % 2, k % 4)
            k, r = divmod(n - 1, 2)
            if r == 0 and 0 <= k < 8:
                wprep(4 * q + k // 2 + z(1), k % 2)
        with jax.named_scope("bulk_p1"):
            bulk(t, 0, 4, t + 1, t + 1, 0, 256, side, 15)
        chunk_start(t + 1 + NST)
        return c
    lax.fori_loop(0, 4, body1, 0)

    cp_ax.start()
    with jax.named_scope("w_l"):
        cp_l.wait()
        cp_r1.wait()

    def body2(q, c):
        t, hf = q // 2 + 6, q % 2

        @pl.when(hf == 0)
        def _():
            with jax.named_scope("w_2"):
                chunk_wait(t + 1)
        gs = {}

        def side(n, z):
            po = n // 2
            if n % 2 == 0:
                gs[po] = filt(pl.multiple_of(8 * q, 8), po, fwd(8 * q + po))
            elif po >= 1:
                inv(8 * q + po - 1, gs.pop(po - 1))
            if n == 15:
                inv(8 * q + 7, gs.pop(7))
            if n % 4 == 2:
                nyq_stage(n // 4)
        with jax.named_scope("bulk_p2"):
            bulk(t, 2 * hf, 2, t + 1, t + 1, pl.multiple_of(hf * 128, 128), 128, side)

        @pl.when(q == 1)
        def _():
            chunk_copy(11).start()
            for j in range(8):
                wo_copy(j).start()
        return c
    lax.fori_loop(0, 4, body2, 0)

    def body3(q, c):
        t = q + 8

        @pl.when(q < 3)
        def _():
            with jax.named_scope("w_3"):
                chunk_wait(t + 1)
        us, vs, res = {}, {}, {}

        def side(n, z):
            sq = 0
            ks = list(range(sq + 1)) if n == 0 else [n + sq]
            for k in ks:
                if k < 16:
                    us[k] = p3a(2 * q + k // 8 + z(2), k // 8, (k // 4) % 2, k % 4)
            k = n - 2
            if 0 <= k < 16:
                p3b(us.pop(k), k // 8, (k // 4) % 2, k % 4)
            k = n - 16
            if 0 <= k < 16:
                p3c(2 * q + k // 8, k // 8, 2 * (k % 8), 2)
        with jax.named_scope("bulk_p3"):
            bulk(t, 0, 4, t + 1, t + 1, 0, 256, side, 0)
        return c
    lax.fori_loop(0, 4, body3, 0)
    cp_outb.start()

    with jax.named_scope("w_wo"):
        cp_ax.wait()
        cp_mem.wait()
        for j in range(8):
            wo_copy(j).wait()
    scale = DH ** -0.5
    KS = 768

    def step(it, u):
        s = it * U + u
        lhs = jnp.concatenate([ax[s].reshape(FR, DM), memb[...]], axis=0)
        qs, ks, vs, ps, os_, pre = {}, {}, {}, {}, {}, {}

        def ws(m, h, lo=0, hi=DM):
            return wsel(wpk.at[4 * m + h // 8], h % 8, lo, hi)
        if u > 0:
            for m in range(2):
                for h in range(2):
                    pre[(m, h)] = -_dot(lhs[:, :KS], ws(m, h, 0, KS))

        def dotw(m, h):
            if (m, h) in pre:
                return _dot(lhs[:, KS:], ws(m, h, KS, DM)) - pre[(m, h)]
            return _dot(lhs, ws(m, h))

        def proj(m, g):
            h = 2 * g
            return jnp.concatenate([dotw(m, h).astype(bf16), dotw(m, h + 1).astype(bf16),
                                    pool[2 * NST + 4 * m + h // 8, (h % 8) * NSEG + s],
                                    pool[2 * NST + 4 * m + h // 8, (h % 8 + 1) * NSEG + s]], axis=0)

        def qk(g):
            sc = lax.dot_general(qs.pop(g), ks.pop(g), (((1,), (1,)), ((), ())),
                                 preferred_element_type=f32) * scale
            fill = sm[0:80, 0:80]
            sc = jnp.where(fill == 0.0, sc, fill)
            mx = jnp.max(sc, axis=-1, keepdims=True)
            e = jnp.exp(sc - mx)
            l = jnp.sum(e, axis=-1, keepdims=True)
            r = pl.reciprocal(l, approx=True)
            r = r * (2.0 - l * r)
            ps[g] = (e * r).astype(bf16)

        def pv(g):
            o = _dot(ps.pop(g), vs.pop(g))
            os_[2 * g] = o[0:32].astype(bf16)
            os_[2 * g + 1] = o[32:64].astype(bf16)
            ob[8 * u:8 * u + 8, (2 * g) * DH:(2 * g + 1) * DH] = o[64:72]
            ob[8 * u:8 * u + 8, (2 * g + 1) * DH:(2 * g + 2) * DH] = o[72:80]

        def olhs(lo, hi):
            oc = jnp.concatenate([os_[h] for h in range(lo, hi)], axis=1)
            if u == U - 1:
                oc = jnp.concatenate([oc, ob[:, lo * DH:hi * DH].astype(bf16)], axis=0)
            return oc

        sk, dq, dp = 4, 2, 3
        for t in range(G + sk):
            if t < G:
                qs[t] = proj(0, t)
            if 0 <= t - dq < G:
                qk(t - dq)
            if t < G:
                ks[t] = proj(1, t)
            if t - sk - dp >= 0:
                pv(t - sk - dp)
            if t - sk >= 0:
                vs[t - sk] = proj(2, t - sk)
        rem = list(range(G - dp, G))
        acc = []
        oc = olhs(0, 16)
        for j in range(DM // 128):
            acc.append(-_dot(oc, wo[j, 0:16 * DH, :]))
            if rem:
                pv(rem.pop(0))
        oc = olhs(16, 32)
        for j in range(DM // 128):
            cols = slice(j * 128, (j + 1) * 128)
            r = _dot(oc, wo[j, 16 * DH:32 * DH, :]) - acc[j]
            oa[it * 2 + u // 2, pl.ds((u % 2) * 4, 3), :, cols] = r[0:FR].reshape(3, 8, 128).astype(bf16)
            memb[:, cols] = r[FR:SEG].astype(bf16)
            if u == U - 1:
                for uu in range(U):
                    oa[it * 2 + uu // 2, (uu % 2) * 4 + 3, :, cols] = r[SEG + 8 * uu:SEG + 8 * uu + 8].astype(bf16)

    def out_copy(it):
        return pltpu.make_async_copy(oa.at[pl.ds(it * 2, 2)],
                                     out_hbm.at[pl.ds(it * 2, 2), :, :, pl.ds(0, DM)], sems.at[32])

    def group(it, c):
        with jax.named_scope("grp"):
            for u in range(U):
                step(it, u)
        out_copy(it).start()
        return c
    lax.fori_loop(0, NSEG // U, group, 0)
    with jax.named_scope("w_out"):
        for it in range(NSEG // U):
            out_copy(it).wait()
        cp_outb.wait()


def pallas_concat_heads__memory_aug_recurrent_mem_tr__spectral_gfnet__prompt_kernel(
    A_x, A_mem0, A_Wq, A_Wk, A_Wv, A_Wo, A_seg_len, B_x, B_w_r, B_w_i,
):
    del A_seg_len
    R, LN, TW, fill, KC = _tables()
    small = np.zeros((208, 128), np.float32)
    small[:80, :80] = fill
    small[80:112] = TW
    small[112:] = np.repeat(KC, 8, axis=0)
    hbm = pl.BlockSpec(memory_space=pl.ANY)
    out = pl.pallas_call(
        _kernel,
        out_shape=jax.ShapeDtypeStruct((RS, 8, 8, DM + D), bf16),
        in_specs=[hbm] * 13,
        out_specs=hbm,
        scratch_shapes=[
            pltpu.VMEM((NSEG, 3, 8, DM), bf16),
            pltpu.VMEM((NSEG, 8, DM), bf16),
            pltpu.VMEM((4, 64, DM), u32),
            pltpu.VMEM((DM // 128, H * DH, 128), bf16),
            pltpu.VMEM((2 * NST + NCH + 2, DM // 2, 8, DH), bf16),
            pltpu.VMEM((NCH + 1, 16 * PW, DH), u32),
            pltpu.VMEM((M, DM), bf16),
            pltpu.VMEM((U * M, H * DH), f32),
            pltpu.VMEM((RS, 8, 8, DM), bf16),
            pltpu.VMEM((RS, 8, 8, D), bf16),
            pltpu.VMEM((D // 2 + 1, S), bf16),
            pltpu.VMEM((D // 2 + 1, S), bf16),
            pltpu.VMEM((16, 64, 128), u32),
            pltpu.VMEM((2 * RS + 5, 64, 128), u32),
            pltpu.VMEM((208, 128), f32),
            pltpu.VMEM((RS, 4, 8, 16, 128), bf16),
            pltpu.VMEM((4, RS, TP, 128), f32),
            pltpu.VMEM((2, 2, BS * WP, 128), u32),
            pltpu.VMEM((32, 128), f32),
            pltpu.SMEM((8,), i32),
            pltpu.SemaphoreType.DMA((42,)),
        ],
        compiler_params=pltpu.CompilerParams(vmem_limit_bytes=124 * 1024 * 1024),
    )(A_x.reshape(NSEG, 4, 8, DM), A_mem0.reshape(M, DM),
      A_Wq.reshape(2, DM // 2, H, DH), A_Wk.reshape(2, DM // 2, H, DH), A_Wv.reshape(2, DM // 2, H, DH),
      A_Wo.reshape(H * DH, DM), B_x.reshape(RS, 8, 8, D), B_w_r.T, B_w_i.T,
      jnp.asarray(R), jnp.asarray(LN), jnp.asarray(small), jnp.asarray(np.array([1, 0, 2, 3, 4, 5, 6, 7], np.int32)))
    return out.reshape(1, S, DM + D)
```

```python
import functools
import math

import jax
import jax.numpy as jnp
import numpy as np
from jax import lax
import jax.experimental.pallas as pl
import jax.experimental.pallas.tpu as pltpu

bf16, f32, u32, i32 = jnp.bfloat16, jnp.float32, jnp.uint32, jnp.int32

S, DM, H, DH, M, SEG = 2048, 1024, 32, 128, 8, 32
NSEG = S // SEG
FR = SEG - M
G = H // 2
U = 4
NCH = 12
NST = 4
PW = 264

D = 1024
RS, BS = 32, 64
HR = RS // 2
WP = 40
TP = 136
C8 = float(np.sqrt(0.5))


def _pack_rows(a):
    u = np.asarray(a, np.float32).astype(jnp.bfloat16).view(np.uint16).astype(np.uint32)
    return u[..., 0::2, :] | (u[..., 1::2, :] << 16)


_RHO = (2, 4, 4, 4)


def _in_a(lane, c):
    return (lane % 4 < 2) if c == 0 else ((lane + 2) % 8 < 4)


def _dstage(x, kc, roll64):
    a = [x[j] + x[j + 4] for j in range(4)]
    b = [x[j] - x[j + 4] for j in range(4)]
    t1 = (b[1] - b[3]) * C8
    t2 = (b[1] + b[3]) * C8
    s0, s1 = a[0] + a[2], a[1] + a[3]
    out = [s0 + s1, s0 - s1]
    for c, (u, v) in enumerate(((b[0] + t1, b[2] + t2), (a[0] - a[2], a[1] - a[3]), (b[0] - t1, b[2] - t2))):
        g = u * kc[4 * c] + v * kc[4 * c + 1]
        h = roll64(u * kc[4 * c + 2] + v * kc[4 * c + 3])
        out += [g + h, g - h]
    return out


def _dstage_t(p, kc, roll64):
    uv = []
    for c in range(3):
        g = p[2 + 2 * c] + p[3 + 2 * c]
        h = roll64(p[2 + 2 * c] - p[3 + 2 * c])
        uv.append((g * kc[4 * c] + h * kc[4 * c + 2], g * kc[4 * c + 1] + h * kc[4 * c + 3]))
    s0, s1 = p[0] + p[1], p[0] - p[1]
    a = [s0 + uv[1][0], s1 + uv[1][1], s0 - uv[1][0], s1 - uv[1][1]]
    t1 = (uv[0][0] - uv[2][0]) * C8
    t2 = (uv[0][1] - uv[2][1]) * C8
    b = [uv[0][0] + uv[2][0], t1 + t2, uv[0][1] + uv[2][1], t2 - t1]
    return [a[j] + b[j] for j in range(4)] + [a[j] - b[j] for j in range(4)]


@functools.lru_cache(maxsize=None)
def _tables():
    kcol = np.zeros((4, 128), np.int64)
    for l in range(128):
        i0, i1 = l, 128 + (l ^ 1)
        ev, o3 = l % 2 == 0, l % 4 in (0, 3)
        kcol[0, l] = 2 * (i0 if ev else i1)
        kcol[2, l] = 2 * (i1 if ev else i0)
        kcol[1, l] = 2 * (i0 if o3 else i1) + 1
        kcol[3, l] = 2 * (i1 if o3 else i0) + 1
    lanes = np.arange(128)
    lo = lanes < 64
    KC = np.zeros((12, 128))
    for c, sg in ((1, -1.0), (2, -1.0), (3, 1.0)):
        tr, ti = np.cos(2 * np.pi * c / 16), -np.sin(2 * np.pi * c / 16)
        KC[4 * c - 4] = np.where(lo, 1.0, ti)
        KC[4 * c - 3] = sg * np.where(lo, 0.0, tr)
        KC[4 * c - 2] = np.where(lo, 0.0, tr)
        KC[4 * c - 1] = sg * np.where(lo, 1.0, -ti)
    eye = np.eye(D)
    Bt = _dstage([eye[:, 128 * e:128 * (e + 1)] for e in range(8)], KC, lambda v: np.roll(v, 64, axis=1))
    d = np.arange(D)
    R = np.zeros((16, 128, 128))
    for c in range(4):
        rho = _RHO[c]
        inA = _in_a(lanes, c)
        ang = 2 * np.pi * (np.outer(d, kcol[c]) % D) / D
        fr, fi = np.cos(ang), -np.sin(ang)
        wr_, wi_ = np.full(128, 2.0), np.full(128, 2.0)
        if c == 0:
            fi[:, 0] = (-1.0) ** d
            wr_[0] = 1.0
            wi_[0] = 1.0
        fi, wi_ = np.roll(fi, -rho, axis=1), np.roll(wi_, -rho)
        for h in range(2):
            own = inA if h == 0 else ~inA
            ft, wt = np.where(own, fr, fi), np.where(own, wr_, wi_)
            bt = Bt[2 * c + h]
            r = (bt.T @ ft) / (bt * bt).sum(axis=0)[:, None]
            assert np.abs(bt @ r - ft).max() < 1e-9
            R[2 * c + h] = r
            R[8 + 2 * c + h] = (wt[:, None] * r.T) / (S * D)
    L = np.zeros((2 * RS, 128, 128))
    bb = np.arange(BS)
    kord = np.array([ri * 64 + 8 * t + r for t in range(8) for ri in range(2) for r in range(8)])
    for p1 in range(RS):
        ang = 2 * np.pi * (np.outer(p1 + RS * bb, bb) % S) / S
        mr, mi = np.cos(ang), -np.sin(ang)
        full = np.block([[mr, -mi], [mi, mr]])
        L[p1] = full[:, kord]
        L[RS + p1] = full.T
    l_, q_ = np.arange(128), np.arange(16)
    ang = 2 * np.pi * (np.outer(l_, l_) % 128) / 128
    N1 = np.concatenate([np.cos(ang), -np.sin(ang)], axis=1)
    N1 = np.concatenate([(N1[:64] + N1[64:]) / 2, (N1[:64] - N1[64:]) / 2], axis=0)
    ang = 2 * np.pi * np.outer(q_, l_) / S
    TW = np.concatenate([np.cos(ang), -np.sin(ang)], axis=0)
    ang = 2 * np.pi * (np.outer(q_, q_) % 16) / 16
    fr, fi = np.cos(ang), -np.sin(ang)
    F16 = np.block([[fr, -fi], [fi, fr]])
    NY = np.zeros((5, 128, 128))
    NY[0], NY[1], NY[2], NY[3] = N1[:, :128], N1[:, 128:], N1[:, :128].T, N1[:, 128:].T
    NY[4, :32, :32] = F16
    NY[4, 32:64, :32] = F16.T
    LN = np.concatenate([L, NY], axis=0)
    head = np.zeros(80, np.int32)
    pos = np.zeros(80, np.int32)
    for r in range(80):
        if r < 64:
            head[r] = r // 32
            t = r % 32
            pos[r] = (M + t) if t < FR else (t - FR)
        else:
            head[r] = (r - 64) // 8
            pos[r] = M + FR + (r - 64) % 8
    same = head[:, None] == head[None, :]
    vis = (pos[:, None] < M) | (pos[:, None] >= pos[None, :])
    fill = np.where(same, np.where(vis, 0.0, -1e9), -np.inf).astype(np.float32)
    return _pack_rows(R), _pack_rows(LN), TW.astype(np.float32), fill, KC.astype(np.float32)


def _cmul_const(re, im, j, n, sgn):
    ang = sgn * 2 * math.pi * j / n
    c, s = math.cos(ang), math.sin(ang)
    if abs(abs(c) - abs(s)) < 1e-12:
        if c * s > 0:
            return (re - im) * c, (re + im) * c
        return (re + im) * c, (im - re) * c
    return re * c - im * s, re * s + im * c


def _diff_tw(a, b, j, n, sgn):
    if j == 0:
        return a[0] - b[0], a[1] - b[1]
    if 4 * j == n:
        if sgn < 0:
            return a[1] - b[1], b[0] - a[0]
        return b[1] - a[1], a[0] - b[0]
    return _cmul_const(a[0] - b[0], a[1] - b[1], j, n, sgn)


def _tw(v, j, sgn):
    if j == 0:
        return v
    if 4 * j == RS:
        return (v[1], -v[0]) if sgn < 0 else (-v[1], v[0])
    return _cmul_const(v[0], v[1], j, RS, sgn)


def _fft(v, sgn):
    n = len(v)
    if n == 1:
        return v
    h = n // 2
    ev = _fft([(v[j][0] + v[j + h][0], v[j][1] + v[j + h][1]) for j in range(h)], sgn)
    od = _fft([_diff_tw(v[j], v[j + h], j, n, sgn) for j in range(h)], sgn)
    out = [None] * n
    out[0::2] = ev
    out[1::2] = od
    return out


def _dot(a, b):
    return jnp.dot(a, b, preferred_element_type=f32)


def _asbf(v):
    return pltpu.bitcast(v, bf16)


def _cm(ar, ai, br, bi):
    return ar * br - ai * bi, ar * bi + ai * br


BU = 2 * NST + NCH


def _kernel(ax_hbm, mem_hbm, wq_hbm, wk_hbm, wv_hbm, wo_hbm, bx_hbm, wr_hbm, wi_hbm,
            R_hbm, L_hbm, sm_hbm, one_hbm, out_hbm,
            ax, xb3, xb, wo, pool, wpk, memb, ob, oa,
            bx, wr, wi, R, L, sm, Y, T, wp, nv, one, sems):
    srcs = (wq_hbm, wk_hbm, wv_hbm)
    lane8 = lax.broadcasted_iota(i32, (8, 128), 1)

    def chunk_copy(t):
        return pltpu.make_async_copy(srcs[t // 4].at[:, :, pl.ds(8 * (t % 4), 8), :],
                                     pool.at[pl.ds(2 * (t % NST), 2)], sems.at[t % NST])

    def part_sem(t, part):
        return sems.at[34 + jnp.where(t == 0, 0, 2 + 2 * t) + part]

    def part_start(t, part, n):
        pltpu.make_async_copy(srcs[0].at[:, pl.ds(part * n, n), pl.ds(8 * t, 8), :],
                              pool.at[pl.ds(2 * t, 2), pl.ds(part * n, n)], part_sem(t, part)).start()

    def part_wait(t, part, n):
        blk = pool.at[pl.ds(2 * t, 2), pl.ds(part * n, n)]
        pltpu.make_async_copy(blk, blk, part_sem(t, part)).wait()

    def chunk_start(t):
        for m in range(3):
            @pl.when(t // 4 == m)
            def _(m=m):
                pltpu.make_async_copy(srcs[m].at[:, :, pl.ds(pl.multiple_of(8 * (t % 4), 8), 8), :],
                                      pool.at[pl.ds(2 * (t % NST), 2)], sems.at[t % NST]).start()

    def chunk_wait(t):
        blk = pool.at[pl.ds(2 * (t % NST), 2)]
        pltpu.make_async_copy(blk, blk, sems.at[t % NST]).wait()

    def xb_copy(q):
        return pltpu.make_async_copy(ax_hbm.at[pl.ds(16 * q, 16), 3], xb3.at[pl.ds(16 * q, 16)], sems.at[8 + q])

    def bx_copy(q):
        return pltpu.make_async_copy(bx_hbm.at[:, pl.ds(2 * q, 2)], bx.at[:, pl.ds(2 * q, 2)], sems.at[12 + q])

    def w_copy(q, i):
        cols = pl.ds(pl.multiple_of(512 * q, 512), 512)
        return pltpu.make_async_copy((wr_hbm, wi_hbm)[i].at[:, cols], (wr, wi)[i].at[:, cols], sems.at[16 + 4 * i + q])

    def wo_copy(j):
        return pltpu.make_async_copy(wo_hbm.at[:, pl.ds(128 * j, 128)], wo.at[j], sems.at[24])

    cp_r0 = pltpu.make_async_copy(R_hbm.at[pl.ds(0, 8)], R.at[pl.ds(0, 8)], sems.at[25])
    cp_r1 = pltpu.make_async_copy(R_hbm.at[pl.ds(8, 8)], R.at[pl.ds(8, 8)], sems.at[26])
    cp_l = pltpu.make_async_copy(L_hbm, L, sems.at[27])
    cp_ax = pltpu.make_async_copy(ax_hbm.at[:, pl.ds(0, 3)], ax, sems.at[28])
    cp_outb = pltpu.make_async_copy(bx, out_hbm.at[:, :, :, pl.ds(DM, D)], sems.at[29])
    cp_sm = pltpu.make_async_copy(sm_hbm, sm, sems.at[30])
    cp_one = pltpu.make_async_copy(one_hbm, one, sems.at[33])
    cp_mem = pltpu.make_async_copy(mem_hbm, memb, sems.at[31])

    for part in range(4):
        part_start(0, part, 128)
    cp_one.start()
    xb_copy(0).start()
    xb_copy(1).start()
    part_start(1, 0, 256)
    xb_copy(2).start()
    part_start(1, 1, 256)
    xb_copy(3).start()
    part_start(2, 0, 256)
    part_start(2, 1, 256)
    chunk_copy(3).start()
    cp_r0.start()
    bx_copy(0).start()
    w_copy(0, 0).start()
    w_copy(0, 1).start()
    cp_sm.start()
    cp_mem.start()

    def kc():
        return [jnp.concatenate([sm[112 + 8 * i:120 + 8 * i, :]] * 2, axis=0) for i in range(12)]

    def roll64(v):
        return pltpu.roll(v, 64, 1)

    def dot2(u, w):
        if 0 == 0:
            return _dot(u, w)
        return jnp.concatenate([_dot(u[:64], w), _dot(u[64:], w)], axis=0)

    def prep(t, tpar, jj):
        lo = [bx[2 * jj:2 * jj + 2, t, :, 128 * e:128 * (e + 1)].astype(f32).reshape(16, 128) for e in range(8)]
        hi = [bx[HR + 2 * jj:HR + 2 * jj + 2, t, :, 128 * e:128 * (e + 1)].astype(f32).reshape(16, 128)
              for e in range(8)]
        for par in range(2):
            x = [lo[e] + hi[e] if par == 0 else lo[e] - hi[e] for e in range(8)]
            uu = _dstage(x, kc(), roll64)
            for q in range(8):
                o = (((tpar * 2 + par) * 8 + q) * 8 + jj) * 2
                pool[BU, o:o + 2] = uu[q].reshape(2, 8, 128).astype(bf16)

    def unit1(t, tpar, par, cg):
        o = ((tpar * 2 + par) * 8 + 2 * cg) * 16
        za = dot2(pool[BU, o:o + 16].reshape(128, 128), _asbf(R[2 * cg]))
        zb = dot2(pool[BU, o + 16:o + 32].reshape(128, 128), _asbf(R[2 * cg + 1]))
        ina = _in_a(lane8, cg)
        v = []
        for j in range(HR):
            pa, pb = za[8 * j:8 * j + 8], zb[8 * j:8 * j + 8]
            v.append((jnp.where(ina, pa, pb), pltpu.roll(jnp.where(ina, pb, pa), _RHO[cg], 1)))
        if cg == 0:
            V = nv[8 * tpar:8 * tpar + 8, :]
            for j in range(HR):
                vb = jnp.broadcast_to(v[j][1][:, 0:1], (8, 128))
                V = jnp.where(lane8 == 64 * par + 4 * j + t // 2, vb, V)
                v[j] = (v[j][0], jnp.where(lane8 == 0, 0.0, v[j][1]))
            nv[8 * tpar:8 * tpar + 8, :] = V
        if par == 1:
            v = [_tw(v[j], j, -1) for j in range(HR)]
        o = _fft(v, -1)
        for m in range(HR):
            Y[2 * m + par, cg, t] = jnp.concatenate(o[m], axis=0).astype(bf16)

    def wprep(pb, i):
        w = (wr, wi)[i]
        cols = pl.ds(pl.multiple_of(pb * 128, 128), 128)
        sub = lax.broadcasted_iota(i32, (8, 128), 0)
        msk = (jnp.where(sub % 2 == 0, jnp.uint32(0xffff), jnp.uint32(0))
               | jnp.where((sub % 4 == 0) | (sub % 4 == 3), jnp.uint32(0xffff0000), jnp.uint32(0)))
        t0 = pltpu.bitcast(w[0:256, cols], u32)
        t1 = pltpu.bitcast(w[256:512, cols], u32)
        ps, qs = [], []
        for j in range(16):
            a = t0[8 * j:8 * j + 8]
            b = t1[8 * j:8 * j + 8]
            b = jnp.where(sub % 2 == 0, pltpu.roll(b, 7, 0), pltpu.roll(b, 1, 0))
            x = (a ^ b) & msk
            ps.append(b ^ x)
            qs.append(a ^ x)
        for h, lst in enumerate((ps, qs)):
            tr = pltpu.bitcast(pltpu.bitcast(jnp.concatenate(lst, axis=0), f32).T, u32)
            for q in range(4):
                wp[i, h, pl.ds(pl.multiple_of((pb * 4 + q) * WP, 8), 32), :] = tr[32 * q:32 * q + 32]

    def fwd(p):
        return _dot(_asbf(L[p]), jnp.concatenate([Y[p, cg].reshape(128, 128) for cg in range(4)], axis=1))

    def filt(pbase, po, v):
        grs, gis = [None] * 4, [None] * 4
        win = pl.ds(pbase, (BS - 1) * WP + 8)
        for h in range(2):
            wr_ = wp.at[0, h, win][pl.ds(po, BS, stride=WP), :]
            wi_ = wp.at[1, h, win][pl.ds(po, BS, stride=WP), :]
            for hi in range(2):
                cg = 2 * h + hi
                if hi == 0:
                    a, b = wr_ << 16, wi_ << 16
                else:
                    a, b = wr_ & jnp.uint32(0xffff0000), wi_ & jnp.uint32(0xffff0000)
                grs[cg], gis[cg] = _cm(v[:BS, 128 * cg:128 * (cg + 1)], v[BS:, 128 * cg:128 * (cg + 1)],
                                       pltpu.bitcast(a, f32), pltpu.bitcast(b, f32))
        return jnp.concatenate([jnp.concatenate(grs, axis=1), jnp.concatenate(gis, axis=1)], axis=0).astype(bf16)

    def inv(p, g):
        t = _dot(_asbf(L[RS + p]), g)
        for cg in range(4):
            T[cg, p, 0:128, :] = t[:, 128 * cg:128 * (cg + 1)]

    nyq = {}

    def nyq_stage(k):
        n0 = 2 * RS
        twr, twi = sm[80:96, :], sm[96:112, :]
        if k == 0:
            v = nv[0:16, :].astype(bf16)
            r, i = _cm(_dot(v, _asbf(L[n0])), _dot(v, _asbf(L[n0 + 1])), twr, twi)
            nyq[0] = jnp.concatenate([r, i], axis=0).astype(bf16)
        elif k == 1:
            t = _dot(_asbf(L[n0 + 4, 0:16])[:, 0:32], nyq[0])
            ws = []
            for w in (wr, wi):
                row = w[512:513, :].astype(f32)
                ws.append(jnp.concatenate([row[:, 128 * r:128 * (r + 1)] for r in range(16)], axis=0))
            r, i = _cm(t[:16], t[16:], ws[0], ws[1])
            nyq[1] = jnp.concatenate([r, i], axis=0).astype(bf16)
        elif k == 2:
            t = _dot(_asbf(L[n0 + 4, 16:32])[:, 0:32], nyq[1])
            r, i = _cm(t[:16], t[16:], twr, -twi)
            nyq[2] = (r.astype(bf16), i.astype(bf16))
        elif k == 3:
            nv[16:32, :] = _dot(nyq[2][0], _asbf(L[n0 + 2])) + _dot(nyq[2][1], _asbf(L[n0 + 3]))

    def p3a(t, tpar, par, cg):
        rr = pl.ds(pl.multiple_of(t * 8, 8), 8)
        ri = pl.ds(pl.multiple_of(64 + t * 8, 8), 8)
        o = _fft([(T[cg, 2 * m + par, rr, :], T[cg, 2 * m + par, ri, :]) for m in range(HR)], +1)
        if par == 1:
            o = [_tw(o[j], j, +1) for j in range(HR)]
        if cg == 0:
            un = nv[16 + 8 * tpar:24 + 8 * tpar, :]
            o = [(o[j][0], jnp.where(lane8 == 0, pltpu.roll(un, (128 - 64 * par - 4 * j - t // 2) % 128, 1),
                                     o[j][1])) for j in range(HR)]
        ina = _in_a(lane8, cg)
        ua, ub = [], []
        for re, im in o:
            im = pltpu.roll(im, 128 - _RHO[cg], 1)
            ua.append(jnp.where(ina, re, im))
            ub.append(jnp.where(ina, im, re))
        return [[jnp.concatenate(x[8 * i:8 * i + 8], axis=0).astype(bf16) for i in range(2)] for x in (ua, ub)]

    def p3b(u, tpar, par, cg):
        for h in range(2):
            for i in range(2):
                z = _dot(u[h][i], _asbf(R[8 + 2 * cg + h]))
                o = (par * 8 + 2 * cg + h) * 32 + 16 * i
                pool[BU + tpar, o:o + 16] = _asbf(z).reshape(16, 8, 128)

    def p3c(t, tpar, j0, nj):
        res = []
        for par in range(2):
            p = []
            for q in range(8):
                o = (par * 8 + q) * 32 + 2 * j0
                p.append(pltpu.bitcast(pool[BU + tpar, o:o + 2 * nj].reshape(16 * nj, 128), f32))
            res.append(_dstage_t(p, kc(), roll64))
        for e in range(8):
            cols = slice(128 * e, 128 * (e + 1))
            bx[j0:j0 + nj, t, :, cols] = (res[0][e] + res[1][e]).reshape(nj, 8, 128).astype(bf16)
            bx[HR + j0:HR + j0 + nj, t, :, cols] = (res[0][e] - res[1][e]).reshape(nj, 8, 128).astype(bf16)

    def runit(b0, d0, dst, k):
        a = pltpu.bitcast(jnp.concatenate([pool[b0, d0 + 2 * k], pool[b0 + 1, d0 + 2 * k]], axis=0), u32)
        b = pltpu.bitcast(jnp.concatenate([pool[b0, d0 + 2 * k + 1], pool[b0 + 1, d0 + 2 * k + 1]], axis=0), u32)
        dst[pl.ds(k, 8, stride=PW), :] = (a & jnp.uint32(0xffff)) | (b << 16)
        dst[pl.ds(8 * PW + k, 8, stride=PW), :] = (a >> 16) | (b & jnp.uint32(0xffff0000))

    def wsel(w, hl, lo=0, hi=DM):
        base = ((hl % 2) * 8 + hl // 2) * PW
        parts = []
        for kh in range(2):
            a, b = max(lo, 512 * kh), min(hi, 512 * (kh + 1))
            if a < b:
                o = base + 4 * PW * kh - 256 * kh
                parts.append(w[o + a // 2:o + b // 2, :])
        return _asbf(jnp.concatenate(parts, axis=0))

    def bulk(t, mc0, nmc, tsrc, tdst, k0, nk, side=None, tokrow=0):
        w = wpk.at[t]
        b0 = 2 * (tsrc & (NST - 1))
        dst = wpk.at[tdst, pl.ds(k0, 15 * PW + nk)]
        bq = 2 * NST + (t & 15)
        zero = one[1]
        toks = []
        ns = 8 * nmc
        per = nk // ns
        for mi in range(nmc):
            mc = mc0 + mi
            x = _asbf(xb[mc])
            for h in range(8):
                n = mi * 8 + h
                r = _dot(x, wsel(w, h)).reshape(16, M, DH)
                nn = (n - 1) % ns
                for k in range(per * nn, per * (nn + 1)):
                    runit(b0, 2 * k0, dst, k)
                if side is not None:
                    side(n, lambda back, n=n: toks[n - back] if n >= back else 0)
                    toks.append(pltpu.bitcast(r[tokrow], i32)[0, 0] & zero)
                rb = r.astype(bf16)
                for gi in range(4):
                    pool[bq, pl.ds(mc * 128 + gi * 32 + h * 4, 4)] = rb[4 * gi:4 * gi + 4]

    def rel0(i, c):
        @pl.when(i % 2 == 0)
        def _():
            part_wait(0, i // 2, 128)
        dst = wpk.at[0, pl.ds(pl.multiple_of(i * 32, 32), 15 * PW + 32)]
        for k in range(32):
            runit(0, i * 64, dst, k)
        return c
    with jax.named_scope("rel0"):
        lax.fori_loop(0, 8, rel0, 0)
    cp_one.wait()

    def body0(i, c):
        t, mc = i // 4, i % 4
        real = mc >= 2

        @pl.when(t == 0)
        def _():
            xb_copy(mc).wait()
            xb[mc] = pltpu.bitcast(xb3[pl.ds(16 * mc, 16)].reshape(128, DM), u32)

        @pl.when(real)
        def _():
            part_wait(t + 1, mc - 2, 256)
        with jax.named_scope("bulk0"):
            bulk(t, mc, 1, jnp.where(real, t + 1, t), jnp.where(real, t + 1, NCH),
                 pl.multiple_of((mc % 2) * 128, 128), 128)

        @pl.when(i == 1)
        def _():
            chunk_copy(4).start()
            bx_copy(1).start()
            w_copy(1, 0).start()
            w_copy(1, 1).start()

        @pl.when(i == 5)
        def _():
            chunk_copy(5).start()
        return c
    lax.fori_loop(0, 8, body0, 0)
    bx_copy(2).start()
    w_copy(2, 0).start()
    w_copy(2, 1).start()
    chunk_copy(6).start()
    bx_copy(3).start()
    w_copy(3, 0).start()
    w_copy(3, 1).start()
    cp_l.start()
    cp_r1.start()
    nv[0:16, :] = jnp.zeros((16, 128), f32)
    cp_r0.wait()
    cp_sm.wait()

    def body1(q, c):
        t = q + 2
        with jax.named_scope("w_1"):
            chunk_wait(t + 1)
            bx_copy(q).wait()
            w_copy(q, 0).wait()
            w_copy(q, 1).wait()

        def side(n, z):
            sq = 1
            ks = list(range(sq + 1)) if n == 0 else [n + sq]
            for k in ks:
                if k < 16:
                    prep(2 * q + k // 8 + z(2), k // 8, k % 8)
            k = n - 15
            if 0 <= k < 16:
                unit1(2 * q + k // 8, k // 8, (k // 4) % 2, k % 4)
            k, r = divmod(n - 1, 2)
            if r == 0 and 0 <= k < 8:
                wprep(4 * q + k // 2 + z(1), k % 2)
        with jax.named_scope("bulk_p1"):
            bulk(t, 0, 4, t + 1, t + 1, 0, 256, side, 15)
        chunk_start(t + 1 + NST)
        return c
    lax.fori_loop(0, 4, body1, 0)

    cp_ax.start()
    with jax.named_scope("w_l"):
        cp_l.wait()
        cp_r1.wait()

    def body2(q, c):
        t, hf = q // 2 + 6, q % 2

        @pl.when(hf == 0)
        def _():
            with jax.named_scope("w_2"):
                chunk_wait(t + 1)
        gs = {}

        def side(n, z):
            po = n // 2
            if n % 2 == 0:
                gs[po] = filt(pl.multiple_of(8 * q, 8), po, fwd(8 * q + po))
            elif po >= 1:
                inv(8 * q + po - 1, gs.pop(po - 1))
            if n == 15:
                inv(8 * q + 7, gs.pop(7))
            if n % 4 == 2:
                nyq_stage(n // 4)
        with jax.named_scope("bulk_p2"):
            bulk(t, 2 * hf, 2, t + 1, t + 1, pl.multiple_of(hf * 128, 128), 128, side)

        @pl.when(q == 1)
        def _():
            chunk_copy(11).start()
            for j in range(8):
                wo_copy(j).start()
        return c
    lax.fori_loop(0, 4, body2, 0)

    def body3(q, c):
        t = q + 8

        @pl.when(q < 3)
        def _():
            with jax.named_scope("w_3"):
                chunk_wait(t + 1)
        us, vs, res = {}, {}, {}

        def side(n, z):
            sq = 0
            ks = list(range(sq + 1)) if n == 0 else [n + sq]
            for k in ks:
                if k < 16:
                    us[k] = p3a(2 * q + k // 8 + z(2), k // 8, (k // 4) % 2, k % 4)
            k = n - 2
            if 0 <= k < 16:
                p3b(us.pop(k), k // 8, (k // 4) % 2, k % 4)
            k = n - 16
            if 0 <= k < 16:
                p3c(2 * q + k // 8, k // 8, 2 * (k % 8), 2)
        with jax.named_scope("bulk_p3"):
            bulk(t, 0, 4, t + 1, t + 1, 0, 256, side, 0)
        return c
    lax.fori_loop(0, 4, body3, 0)
    cp_outb.start()

    with jax.named_scope("w_wo"):
        cp_ax.wait()
        cp_mem.wait()
        for j in range(8):
            wo_copy(j).wait()
    scale = DH ** -0.5
    KS = 768

    def step(it, u):
        s = it * U + u
        lhs = jnp.concatenate([ax[s].reshape(FR, DM), memb[...]], axis=0)
        qs, ks, vs, ps, os_, pre = {}, {}, {}, {}, {}, {}

        def ws(m, h, lo=0, hi=DM):
            return wsel(wpk.at[4 * m + h // 8], h % 8, lo, hi)
        if u > 0:
            for g, m in [(0, 0), (0, 1), (1, 0), (1, 1)][:2]:
                for h in (2 * g, 2 * g + 1):
                    pre[(m, h)] = -_dot(lhs[:, :KS], ws(m, h, 0, KS))

        def dotw(m, h):
            if (m, h) in pre:
                return _dot(lhs[:, KS:], ws(m, h, KS, DM)) - pre[(m, h)]
            return _dot(lhs, ws(m, h))

        def proj(m, g):
            h = 2 * g
            return jnp.concatenate([dotw(m, h).astype(bf16), dotw(m, h + 1).astype(bf16),
                                    pool[2 * NST + 4 * m + h // 8, it * 32 + (h % 8) * 4 + u],
                                    pool[2 * NST + 4 * m + h // 8, it * 32 + (h % 8 + 1) * 4 + u]], axis=0)

        def qk(g):
            sc = lax.dot_general(qs.pop(g), ks.pop(g), (((1,), (1,)), ((), ())),
                                 preferred_element_type=f32) * scale
            fill = sm[0:80, 0:80]
            sc = jnp.where(fill == 0.0, sc, fill)
            mx = jnp.max(sc, axis=-1, keepdims=True)
            e = jnp.exp(sc - mx)
            l = jnp.sum(e, axis=-1, keepdims=True)
            r = pl.reciprocal(l, approx=True)
            r = r * (2.0 - l * r)
            ps[g] = (e * r).astype(bf16)

        def pv(g):
            o = _dot(ps.pop(g), vs.pop(g))
            os_[2 * g] = o[0:32].astype(bf16)
            os_[2 * g + 1] = o[32:64].astype(bf16)
            ob[8 * u:8 * u + 8, (2 * g) * DH:(2 * g + 1) * DH] = o[64:72]
            ob[8 * u:8 * u + 8, (2 * g + 1) * DH:(2 * g + 2) * DH] = o[72:80]

        def olhs(lo, hi):
            oc = jnp.concatenate([os_[h] for h in range(lo, hi)], axis=1)
            if u == U - 1:
                oc = jnp.concatenate([oc, ob[:, lo * DH:hi * DH].astype(bf16)], axis=0)
            return oc

        sk, dq, dp, ab = 6, 3, 4, 1
        nq = nv_ = 0
        for t in range(G + sk):
            if t < G:
                qs[t] = proj(0, t)
            if ab == 1 and 0 <= t - dq < G:
                qk(t - dq)
            if t < G:
                ks[t] = proj(1, t)
            if t - sk - dp >= nv_ + ab - 1:
                for _ in range(ab):
                    pv(nv_)
                    nv_ += 1
            if ab > 1 and t - dq >= nq + ab - 1 and nq < G:
                for _ in range(ab):
                    qk(nq)
                    nq += 1
            if t - sk >= 0:
                vs[t - sk] = proj(2, t - sk)
        rem = list(range(nv_, G))
        acc = []
        oc = olhs(0, 16)
        for j in range(DM // 128):
            acc.append(-_dot(oc, wo[j, 0:16 * DH, :]))
            if j >= 0:
                for _ in range(ab):
                    if rem:
                        pv(rem.pop(0))
        oc = olhs(16, 32)
        for j in range(DM // 128):
            cols = slice(j * 128, (j + 1) * 128)
            r = _dot(oc, wo[j, 16 * DH:32 * DH, :]) - acc[j]
            oa[it * 2 + u // 2, pl.ds((u % 2) * 4, 3), :, cols] = r[0:FR].reshape(3, 8, 128).astype(bf16)
            memb[:, cols] = r[FR:SEG].astype(bf16)
            if u == U - 1:
                for uu in range(U):
                    oa[it * 2 + uu // 2, (uu % 2) * 4 + 3, :, cols] = r[SEG + 8 * uu:SEG + 8 * uu + 8].astype(bf16)

    def out_copy(it):
        return pltpu.make_async_copy(oa.at[pl.ds(it * 2, 2)],
                                     out_hbm.at[pl.ds(it * 2, 2), :, :, pl.ds(0, DM)], sems.at[32])

    def group(it, c):
        with jax.named_scope("grp"):
            for u in range(U):
                step(it, u)
        out_copy(it).start()
        return c
    lax.fori_loop(0, NSEG // U, group, 0)
    with jax.named_scope("w_out"):
        for it in range(NSEG // U):
            out_copy(it).wait()
        cp_outb.wait()


def pallas_concat_heads__memory_aug_recurrent_mem_tr__spectral_gfnet__prompt_kernel(
    A_x, A_mem0, A_Wq, A_Wk, A_Wv, A_Wo, A_seg_len, B_x, B_w_r, B_w_i,
):
    del A_seg_len
    R, LN, TW, fill, KC = _tables()
    small = np.zeros((208, 128), np.float32)
    small[:80, :80] = fill
    small[80:112] = TW
    small[112:] = np.repeat(KC, 8, axis=0)
    hbm = pl.BlockSpec(memory_space=pl.ANY)
    out = pl.pallas_call(
        _kernel,
        out_shape=jax.ShapeDtypeStruct((RS, 8, 8, DM + D), bf16),
        in_specs=[hbm] * 13,
        out_specs=hbm,
        scratch_shapes=[
            pltpu.VMEM((NSEG, 3, 8, DM), bf16),
            pltpu.VMEM((NSEG, 8, DM), bf16),
            pltpu.VMEM((4, 64, DM), u32),
            pltpu.VMEM((DM // 128, H * DH, 128), bf16),
            pltpu.VMEM((2 * NST + NCH + 2, DM // 2, 8, DH), bf16),
            pltpu.VMEM((NCH + 1, 16 * PW, DH), u32),
            pltpu.VMEM((M, DM), bf16),
            pltpu.VMEM((U * M, H * DH), f32),
            pltpu.VMEM((RS, 8, 8, DM), bf16),
            pltpu.VMEM((RS, 8, 8, D), bf16),
            pltpu.VMEM((D // 2 + 1, S), bf16),
            pltpu.VMEM((D // 2 + 1, S), bf16),
            pltpu.VMEM((16, 64, 128), u32),
            pltpu.VMEM((2 * RS + 5, 64, 128), u32),
            pltpu.VMEM((208, 128), f32),
            pltpu.VMEM((RS, 4, 8, 16, 128), bf16),
            pltpu.VMEM((4, RS, TP, 128), f32),
            pltpu.VMEM((2, 2, BS * WP, 128), u32),
            pltpu.VMEM((32, 128), f32),
            pltpu.SMEM((8,), i32),
            pltpu.SemaphoreType.DMA((42,)),
        ],
        compiler_params=pltpu.CompilerParams(vmem_limit_bytes=124 * 1024 * 1024,
                                             disable_bounds_checks=True, disable_semaphore_checks=True),
    )(A_x.reshape(NSEG, 4, 8, DM), A_mem0.reshape(M, DM),
      A_Wq.reshape(2, DM // 2, H, DH), A_Wk.reshape(2, DM // 2, H, DH), A_Wv.reshape(2, DM // 2, H, DH),
      A_Wo.reshape(H * DH, DM), B_x.reshape(RS, 8, 8, D), B_w_r.T, B_w_i.T,
      jnp.asarray(R), jnp.asarray(LN), jnp.asarray(small), jnp.asarray(np.array([1, 0, 2, 3, 4, 5, 6, 7], np.int32)))
    return out.reshape(1, S, DM + D)
```

```python
import functools
import math

import jax
import jax.numpy as jnp
import numpy as np
from jax import lax
import jax.experimental.pallas as pl
import jax.experimental.pallas.tpu as pltpu

bf16, f32, u32, i32 = jnp.bfloat16, jnp.float32, jnp.uint32, jnp.int32

S, DM, H, DH, M, SEG = 2048, 1024, 32, 128, 8, 32
NSEG = S // SEG
FR = SEG - M
G = H // 2
U = 4
NCH = 12
NST = 4
PW = 264

D = 1024
RS, BS = 32, 64
HR = RS // 2
WP = 40
TP = 136
C8 = float(np.sqrt(0.5))


def _pack_rows(a):
    u = np.asarray(a, np.float32).astype(jnp.bfloat16).view(np.uint16).astype(np.uint32)
    return u[..., 0::2, :] | (u[..., 1::2, :] << 16)


_RHO = (2, 4, 4, 4)


def _in_a(lane, c):
    return (lane % 4 < 2) if c == 0 else ((lane + 2) % 8 < 4)


def _dstage(x, kc, roll64):
    a = [x[j] + x[j + 4] for j in range(4)]
    b = [x[j] - x[j + 4] for j in range(4)]
    t1 = (b[1] - b[3]) * C8
    t2 = (b[1] + b[3]) * C8
    s0, s1 = a[0] + a[2], a[1] + a[3]
    out = [s0 + s1, s0 - s1]
    for c, (u, v) in enumerate(((b[0] + t1, b[2] + t2), (a[0] - a[2], a[1] - a[3]), (b[0] - t1, b[2] - t2))):
        g = u * kc[4 * c] + v * kc[4 * c + 1]
        h = roll64(u * kc[4 * c + 2] + v * kc[4 * c + 3])
        out += [g + h, g - h]
    return out


def _dstage_t(p, kc, roll64):
    uv = []
    for c in range(3):
        g = p[2 + 2 * c] + p[3 + 2 * c]
        h = roll64(p[2 + 2 * c] - p[3 + 2 * c])
        uv.append((g * kc[4 * c] + h * kc[4 * c + 2], g * kc[4 * c + 1] + h * kc[4 * c + 3]))
    s0, s1 = p[0] + p[1], p[0] - p[1]
    a = [s0 + uv[1][0], s1 + uv[1][1], s0 - uv[1][0], s1 - uv[1][1]]
    t1 = (uv[0][0] - uv[2][0]) * C8
    t2 = (uv[0][1] - uv[2][1]) * C8
    b = [uv[0][0] + uv[2][0], t1 + t2, uv[0][1] + uv[2][1], t2 - t1]
    return [a[j] + b[j] for j in range(4)] + [a[j] - b[j] for j in range(4)]


@functools.lru_cache(maxsize=None)
def _tables():
    kcol = np.zeros((4, 128), np.int64)
    for l in range(128):
        i0, i1 = l, 128 + (l ^ 1)
        ev, o3 = l % 2 == 0, l % 4 in (0, 3)
        kcol[0, l] = 2 * (i0 if ev else i1)
        kcol[2, l] = 2 * (i1 if ev else i0)
        kcol[1, l] = 2 * (i0 if o3 else i1) + 1
        kcol[3, l] = 2 * (i1 if o3 else i0) + 1
    lanes = np.arange(128)
    lo = lanes < 64
    KC = np.zeros((12, 128))
    for c, sg in ((1, -1.0), (2, -1.0), (3, 1.0)):
        tr, ti = np.cos(2 * np.pi * c / 16), -np.sin(2 * np.pi * c / 16)
        KC[4 * c - 4] = np.where(lo, 1.0, ti)
        KC[4 * c - 3] = sg * np.where(lo, 0.0, tr)
        KC[4 * c - 2] = np.where(lo, 0.0, tr)
        KC[4 * c - 1] = sg * np.where(lo, 1.0, -ti)
    eye = np.eye(D)
    Bt = _dstage([eye[:, 128 * e:128 * (e + 1)] for e in range(8)], KC, lambda v: np.roll(v, 64, axis=1))
    d = np.arange(D)
    R = np.zeros((16, 128, 128))
    for c in range(4):
        rho = _RHO[c]
        inA = _in_a(lanes, c)
        ang = 2 * np.pi * (np.outer(d, kcol[c]) % D) / D
        fr, fi = np.cos(ang), -np.sin(ang)
        wr_, wi_ = np.full(128, 2.0), np.full(128, 2.0)
        if c == 0:
            fi[:, 0] = (-1.0) ** d
            wr_[0] = 1.0
            wi_[0] = 1.0
        fi, wi_ = np.roll(fi, -rho, axis=1), np.roll(wi_, -rho)
        for h in range(2):
            own = inA if h == 0 else ~inA
            ft, wt = np.where(own, fr, fi), np.where(own, wr_, wi_)
            bt = Bt[2 * c + h]
            r = (bt.T @ ft) / (bt * bt).sum(axis=0)[:, None]
            assert np.abs(bt @ r - ft).max() < 1e-9
            R[2 * c + h] = r
            R[8 + 2 * c + h] = (wt[:, None] * r.T) / (S * D)
    L = np.zeros((2 * RS, 128, 128))
    bb = np.arange(BS)
    kord = np.array([ri * 64 + 8 * t + r for t in range(8) for ri in range(2) for r in range(8)])
    for p1 in range(RS):
        ang = 2 * np.pi * (np.outer(p1 + RS * bb, bb) % S) / S
        mr, mi = np.cos(ang), -np.sin(ang)
        full = np.block([[mr, -mi], [mi, mr]])
        L[p1] = full[:, kord]
        L[RS + p1] = full.T
    l_, q_ = np.arange(128), np.arange(16)
    ang = 2 * np.pi * (np.outer(l_, l_) % 128) / 128
    N1 = np.concatenate([np.cos(ang), -np.sin(ang)], axis=1)
    N1 = np.concatenate([(N1[:64] + N1[64:]) / 2, (N1[:64] - N1[64:]) / 2], axis=0)
    ang = 2 * np.pi * np.outer(q_, l_) / S
    TW = np.concatenate([np.cos(ang), -np.sin(ang)], axis=0)
    ang = 2 * np.pi * (np.outer(q_, q_) % 16) / 16
    fr, fi = np.cos(ang), -np.sin(ang)
    F16 = np.block([[fr, -fi], [fi, fr]])
    NY = np.zeros((5, 128, 128))
    NY[0], NY[1], NY[2], NY[3] = N1[:, :128], N1[:, 128:], N1[:, :128].T, N1[:, 128:].T
    NY[4, :32, :32] = F16
    NY[4, 32:64, :32] = F16.T
    LN = np.concatenate([L, NY], axis=0)
    head = np.zeros(80, np.int32)
    pos = np.zeros(80, np.int32)
    for r in range(80):
        if r < 64:
            head[r] = r // 32
            t = r % 32
            pos[r] = (M + t) if t < FR else (t - FR)
        else:
            head[r] = (r - 64) // 8
            pos[r] = M + FR + (r - 64) % 8
    same = head[:, None] == head[None, :]
    vis = (pos[:, None] < M) | (pos[:, None] >= pos[None, :])
    fill = np.where(same, np.where(vis, 0.0, -1e9), -np.inf).astype(np.float32)
    return _pack_rows(R), _pack_rows(LN), TW.astype(np.float32), fill, KC.astype(np.float32)


def _cmul_const(re, im, j, n, sgn):
    ang = sgn * 2 * math.pi * j / n
    c, s = math.cos(ang), math.sin(ang)
    if abs(abs(c) - abs(s)) < 1e-12:
        if c * s > 0:
            return (re - im) * c, (re + im) * c
        return (re + im) * c, (im - re) * c
    return re * c - im * s, re * s + im * c


def _diff_tw(a, b, j, n, sgn):
    if j == 0:
        return a[0] - b[0], a[1] - b[1]
    if 4 * j == n:
        if sgn < 0:
            return a[1] - b[1], b[0] - a[0]
        return b[1] - a[1], a[0] - b[0]
    return _cmul_const(a[0] - b[0], a[1] - b[1], j, n, sgn)


def _tw(v, j, sgn):
    if j == 0:
        return v
    if 4 * j == RS:
        return (v[1], -v[0]) if sgn < 0 else (-v[1], v[0])
    return _cmul_const(v[0], v[1], j, RS, sgn)


def _fft(v, sgn):
    n = len(v)
    if n == 1:
        return v
    h = n // 2
    ev = _fft([(v[j][0] + v[j + h][0], v[j][1] + v[j + h][1]) for j in range(h)], sgn)
    od = _fft([_diff_tw(v[j], v[j + h], j, n, sgn) for j in range(h)], sgn)
    out = [None] * n
    out[0::2] = ev
    out[1::2] = od
    return out


def _dot(a, b):
    return jnp.dot(a, b, preferred_element_type=f32)


def _asbf(v):
    return pltpu.bitcast(v, bf16)


def _cm(ar, ai, br, bi):
    return ar * br - ai * bi, ar * bi + ai * br


BU = 2 * NST + NCH
BC = BU + 2


def _kernel(ax_hbm, mem_hbm, wq_hbm, wk_hbm, wv_hbm, wo_hbm, bx_hbm, wr_hbm, wi_hbm,
            R_hbm, L_hbm, sm_hbm, one_hbm, out_hbm,
            ax, xb3, xb, wo, pool, wpk, memb, ob, oa,
            bx, wr, wi, R, L, sm, Y, T, wp, nv, one, sems):
    srcs = (wq_hbm, wk_hbm, wv_hbm)
    lane8 = lax.broadcasted_iota(i32, (8, 128), 1)

    def chunk_copy(t):
        return pltpu.make_async_copy(srcs[t // 4].at[:, :, pl.ds(8 * (t % 4), 8), :],
                                     pool.at[pl.ds(2 * (t % NST), 2)], sems.at[t % NST])

    def part_sem(t, part):
        return sems.at[34 + jnp.where(t == 0, 0, 2 + 2 * t) + part]

    def part_start(t, part, n):
        pltpu.make_async_copy(srcs[0].at[:, pl.ds(part * n, n), pl.ds(8 * t, 8), :],
                              pool.at[pl.ds(2 * t, 2), pl.ds(part * n, n)], part_sem(t, part)).start()

    def part_wait(t, part, n):
        blk = pool.at[pl.ds(2 * t, 2), pl.ds(part * n, n)]
        pltpu.make_async_copy(blk, blk, part_sem(t, part)).wait()

    def chunk_start(t):
        for m in range(3):
            @pl.when(t // 4 == m)
            def _(m=m):
                pltpu.make_async_copy(srcs[m].at[:, :, pl.ds(pl.multiple_of(8 * (t % 4), 8), 8), :],
                                      pool.at[pl.ds(2 * (t % NST), 2)], sems.at[t % NST]).start()

    def chunk_wait(t):
        blk = pool.at[pl.ds(2 * (t % NST), 2)]
        pltpu.make_async_copy(blk, blk, sems.at[t % NST]).wait()

    def xb_copy(q):
        return pltpu.make_async_copy(ax_hbm.at[pl.ds(16 * q, 16), 3], xb3.at[pl.ds(16 * q, 16)], sems.at[8 + q])

    def bx_copy(q):
        return pltpu.make_async_copy(bx_hbm.at[:, pl.ds(2 * q, 2)], bx.at[:, pl.ds(2 * q, 2)], sems.at[12 + q])

    def w_copy(q, i):
        cols = pl.ds(pl.multiple_of(512 * q, 512), 512)
        return pltpu.make_async_copy((wr_hbm, wi_hbm)[i].at[:, cols], (wr, wi)[i].at[:, cols], sems.at[16 + 4 * i + q])

    def wo_copy(j):
        return pltpu.make_async_copy(wo_hbm.at[:, pl.ds(pl.multiple_of(128 * j, 128), 128)], wo.at[j],
                                     sems.at[42 + j % 4])

    cp_r0 = pltpu.make_async_copy(R_hbm.at[pl.ds(0, 8)], R.at[pl.ds(0, 8)], sems.at[25])
    cp_r1 = pltpu.make_async_copy(R_hbm.at[pl.ds(8, 8)], R.at[pl.ds(8, 8)], sems.at[26])
    cp_l = pltpu.make_async_copy(L_hbm, L, sems.at[27])
    cp_ax = pltpu.make_async_copy(ax_hbm.at[:, pl.ds(0, 3)], ax, sems.at[28])
    cp_outb = pltpu.make_async_copy(bx, out_hbm.at[:, :, :, pl.ds(DM, D)], sems.at[29])
    cp_sm = pltpu.make_async_copy(sm_hbm, sm, sems.at[30])
    cp_one = pltpu.make_async_copy(one_hbm, one, sems.at[33])
    cp_mem = pltpu.make_async_copy(mem_hbm, memb, sems.at[31])

    for part in range(4):
        part_start(0, part, 128)
    cp_one.start()
    xb_copy(0).start()
    xb_copy(1).start()
    part_start(1, 0, 256)
    xb_copy(2).start()
    part_start(1, 1, 256)
    xb_copy(3).start()
    part_start(2, 0, 256)
    part_start(2, 1, 256)
    chunk_copy(3).start()
    cp_r0.start()
    bx_copy(0).start()
    w_copy(0, 0).start()
    w_copy(0, 1).start()
    cp_sm.start()
    cp_mem.start()

    def kc(rep=2):
        return [jnp.concatenate([sm[112 + 8 * i:120 + 8 * i, :]] * rep, axis=0) for i in range(12)]

    def roll64(v):
        return pltpu.roll(v, 64, 1)

    def dot2(u, w):
        if 0 == 0:
            return _dot(u, w)
        return jnp.concatenate([_dot(u[:64], w), _dot(u[64:], w)], axis=0)

    def prep(t, tpar, jj):
        lo = [bx[2 * jj:2 * jj + 2, t, :, 128 * e:128 * (e + 1)].astype(f32).reshape(16, 128) for e in range(8)]
        hi = [bx[HR + 2 * jj:HR + 2 * jj + 2, t, :, 128 * e:128 * (e + 1)].astype(f32).reshape(16, 128)
              for e in range(8)]
        for par in range(2):
            x = [lo[e] + hi[e] if par == 0 else lo[e] - hi[e] for e in range(8)]
            uu = _dstage(x, kc(), roll64)
            for q in range(8):
                o = (((tpar * 2 + par) * 8 + q) * 8 + jj) * 2
                pool[BU, o:o + 2] = uu[q].reshape(2, 8, 128).astype(bf16)

    def unit1(t, tpar, par, cg):
        o = ((tpar * 2 + par) * 8 + 2 * cg) * 16
        za = dot2(pool[BU, o:o + 16].reshape(128, 128), _asbf(R[2 * cg]))
        zb = dot2(pool[BU, o + 16:o + 32].reshape(128, 128), _asbf(R[2 * cg + 1]))
        ina = _in_a(lane8, cg)
        v = []
        for j in range(HR):
            pa, pb = za[8 * j:8 * j + 8], zb[8 * j:8 * j + 8]
            v.append((jnp.where(ina, pa, pb), pltpu.roll(jnp.where(ina, pb, pa), _RHO[cg], 1)))
        if cg == 0:
            V = nv[8 * tpar:8 * tpar + 8, :]
            for j in range(HR):
                vb = jnp.broadcast_to(v[j][1][:, 0:1], (8, 128))
                V = jnp.where(lane8 == 64 * par + 4 * j + t // 2, vb, V)
                v[j] = (v[j][0], jnp.where(lane8 == 0, 0.0, v[j][1]))
            nv[8 * tpar:8 * tpar + 8, :] = V
        if par == 1:
            v = [_tw(v[j], j, -1) for j in range(HR)]
        o = _fft(v, -1)
        for m in range(HR):
            Y[2 * m + par, cg, t] = jnp.concatenate(o[m], axis=0).astype(bf16)

    def wprep(pb, i):
        w = (wr, wi)[i]
        cols = pl.ds(pl.multiple_of(pb * 128, 128), 128)
        sub = lax.broadcasted_iota(i32, (8, 128), 0)
        msk = (jnp.where(sub % 2 == 0, jnp.uint32(0xffff), jnp.uint32(0))
               | jnp.where((sub % 4 == 0) | (sub % 4 == 3), jnp.uint32(0xffff0000), jnp.uint32(0)))
        t0 = pltpu.bitcast(w[0:256, cols], u32)
        t1 = pltpu.bitcast(w[256:512, cols], u32)
        ps, qs = [], []
        for j in range(16):
            a = t0[8 * j:8 * j + 8]
            b = t1[8 * j:8 * j + 8]
            b = jnp.where(sub % 2 == 0, pltpu.roll(b, 7, 0), pltpu.roll(b, 1, 0))
            x = (a ^ b) & msk
            ps.append(b ^ x)
            qs.append(a ^ x)
        for h, lst in enumerate((ps, qs)):
            tr = pltpu.bitcast(pltpu.bitcast(jnp.concatenate(lst, axis=0), f32).T, u32)
            for q in range(4):
                wp[i, h, pl.ds(pl.multiple_of((pb * 4 + q) * WP, 8), 32), :] = tr[32 * q:32 * q + 32]

    def fwd(p):
        return _dot(_asbf(L[p]), jnp.concatenate([Y[p, cg].reshape(128, 128) for cg in range(4)], axis=1))

    def filt(pbase, po, v):
        grs, gis = [None] * 4, [None] * 4
        win = pl.ds(pbase, (BS - 1) * WP + 8)
        for h in range(2):
            wr_ = wp.at[0, h, win][pl.ds(po, BS, stride=WP), :]
            wi_ = wp.at[1, h, win][pl.ds(po, BS, stride=WP), :]
            for hi in range(2):
                cg = 2 * h + hi
                if hi == 0:
                    a, b = wr_ << 16, wi_ << 16
                else:
                    a, b = wr_ & jnp.uint32(0xffff0000), wi_ & jnp.uint32(0xffff0000)
                grs[cg], gis[cg] = _cm(v[:BS, 128 * cg:128 * (cg + 1)], v[BS:, 128 * cg:128 * (cg + 1)],
                                       pltpu.bitcast(a, f32), pltpu.bitcast(b, f32))
        return jnp.concatenate([jnp.concatenate(grs, axis=1), jnp.concatenate(gis, axis=1)], axis=0).astype(bf16)

    def inv(p, g):
        t = _dot(_asbf(L[RS + p]), g)
        for cg in range(4):
            T[cg, p, 0:128, :] = t[:, 128 * cg:128 * (cg + 1)]

    nyq = {}

    def nyq_stage(k):
        n0 = 2 * RS
        twr, twi = sm[80:96, :], sm[96:112, :]
        if k == 0:
            v = nv[0:16, :].astype(bf16)
            r, i = _cm(_dot(v, _asbf(L[n0])), _dot(v, _asbf(L[n0 + 1])), twr, twi)
            nyq[0] = jnp.concatenate([r, i], axis=0).astype(bf16)
        elif k == 1:
            t = _dot(_asbf(L[n0 + 4, 0:16])[:, 0:32], nyq[0])
            ws = []
            for w in (wr, wi):
                row = w[512:513, :].astype(f32)
                ws.append(jnp.concatenate([row[:, 128 * r:128 * (r + 1)] for r in range(16)], axis=0))
            r, i = _cm(t[:16], t[16:], ws[0], ws[1])
            nyq[1] = jnp.concatenate([r, i], axis=0).astype(bf16)
        elif k == 2:
            t = _dot(_asbf(L[n0 + 4, 16:32])[:, 0:32], nyq[1])
            r, i = _cm(t[:16], t[16:], twr, -twi)
            nyq[2] = (r.astype(bf16), i.astype(bf16))
        elif k == 3:
            nv[16:32, :] = _dot(nyq[2][0], _asbf(L[n0 + 2])) + _dot(nyq[2][1], _asbf(L[n0 + 3]))

    def p3a(t, tpar, par, cg):
        rr = pl.ds(pl.multiple_of(t * 8, 8), 8)
        ri = pl.ds(pl.multiple_of(64 + t * 8, 8), 8)
        o = _fft([(T[cg, 2 * m + par, rr, :], T[cg, 2 * m + par, ri, :]) for m in range(HR)], +1)
        if par == 1:
            o = [_tw(o[j], j, +1) for j in range(HR)]
        if cg == 0:
            un = nv[16 + 8 * tpar:24 + 8 * tpar, :]
            o = [(o[j][0], jnp.where(lane8 == 0, pltpu.roll(un, (128 - 64 * par - 4 * j - t // 2) % 128, 1),
                                     o[j][1])) for j in range(HR)]
        ina = _in_a(lane8, cg)
        ua, ub = [], []
        for re, im in o:
            im = pltpu.roll(im, 128 - _RHO[cg], 1)
            ua.append(jnp.where(ina, re, im))
            ub.append(jnp.where(ina, im, re))
        return [[jnp.concatenate(x[8 * i:8 * i + 8], axis=0).astype(bf16) for i in range(2)] for x in (ua, ub)]

    def p3b(u, tpar, par, cg):
        for h in range(2):
            for i in range(2):
                z = _dot(u[h][i], _asbf(R[8 + 2 * cg + h]))
                o = (par * 8 + 2 * cg + h) * 32 + 16 * i
                pool[BU + tpar, o:o + 16] = _asbf(z).reshape(16, 8, 128)

    def p3c(t, tpar, j0, nj):
        res = []
        for par in range(2):
            p = []
            for q in range(8):
                o = (par * 8 + q) * 32 + 2 * j0
                p.append(pltpu.bitcast(pool[BU + tpar, o:o + 2 * nj].reshape(16 * nj, 128), f32))
            res.append(_dstage_t(p, kc(nj), roll64))
        for e in range(8):
            cols = slice(128 * e, 128 * (e + 1))
            bx[j0:j0 + nj, t, :, cols] = (res[0][e] + res[1][e]).reshape(nj, 8, 128).astype(bf16)
            bx[HR + j0:HR + j0 + nj, t, :, cols] = (res[0][e] - res[1][e]).reshape(nj, 8, 128).astype(bf16)

    def wsum(jj, jz, n, nr):
        lo, hi = slice(nr * n, nr * (n + 1)), slice(2048 + nr * n, 2048 + nr * (n + 1))
        b11, b21 = wo[jz, lo, :].astype(f32), wo[jz, hi, :].astype(f32)
        b12, b22 = wo[4 + jz, lo, :].astype(f32), wo[4 + jz, hi, :].astype(f32)
        for i, v in enumerate((b11 + b22, b12 - b22, b21 - b11, b11 + b12, b21 + b22)):
            pool[BC + 2 * i + jj // 2, pl.ds((jj % 2) * 256 + nr // 8 * n, nr // 8)] = (
                v.reshape(nr // 8, 8, 128).astype(bf16))

    def wc(i, jj):
        return pool[BC + 2 * i + jj // 2, (jj % 2) * 256:(jj % 2 + 1) * 256].reshape(2048, 128)

    def runit(b0, d0, dst, k):
        a = pltpu.bitcast(jnp.concatenate([pool[b0, d0 + 2 * k], pool[b0 + 1, d0 + 2 * k]], axis=0), u32)
        b = pltpu.bitcast(jnp.concatenate([pool[b0, d0 + 2 * k + 1], pool[b0 + 1, d0 + 2 * k + 1]], axis=0), u32)
        dst[pl.ds(k, 8, stride=PW), :] = (a & jnp.uint32(0xffff)) | (b << 16)
        dst[pl.ds(8 * PW + k, 8, stride=PW), :] = (a >> 16) | (b & jnp.uint32(0xffff0000))

    def wsel(w, hl, lo=0, hi=DM):
        base = ((hl % 2) * 8 + hl // 2) * PW
        parts = []
        for kh in range(2):
            a, b = max(lo, 512 * kh), min(hi, 512 * (kh + 1))
            if a < b:
                o = base + 4 * PW * kh - 256 * kh
                parts.append(w[o + a // 2:o + b // 2, :])
        return _asbf(jnp.concatenate(parts, axis=0))

    def bulk(t, mc0, nmc, tsrc, tdst, k0, nk, side=None, tokrow=0):
        w = wpk.at[t]
        b0 = 2 * (tsrc & (NST - 1))
        dst = wpk.at[tdst, pl.ds(k0, 15 * PW + nk)]
        bq = 2 * NST + (t & 31)
        zero = one[1]
        toks = []
        ns = 8 * nmc
        per = nk // ns
        for mi in range(nmc):
            mc = mc0 + mi
            x = _asbf(xb[mc])
            for h in range(8):
                n = mi * 8 + h
                r = _dot(x, wsel(w, h)).reshape(16, M, DH)
                nn = (n - 1) % ns
                for k in range(per * nn, per * (nn + 1)):
                    runit(b0, 2 * k0, dst, k)
                if side is not None:
                    side(n, lambda back, n=n: toks[n - back] if n >= back else 0)
                    toks.append(pltpu.bitcast(r[tokrow], i32)[0, 0] & zero)
                rb = r.astype(bf16)
                for gi in range(4):
                    pool[bq, pl.ds(mc * 128 + gi * 32 + h * 4, 4)] = rb[4 * gi:4 * gi + 4]

    def rel0(i, c):
        @pl.when(i % 2 == 0)
        def _():
            part_wait(0, i // 2, 128)
        dst = wpk.at[0, pl.ds(pl.multiple_of(i * 32, 32), 15 * PW + 32)]
        for k in range(32):
            runit(0, i * 64, dst, k)
        return c
    with jax.named_scope("rel0"):
        lax.fori_loop(0, 8, rel0, 0)
    cp_one.wait()

    def body0(i, c):
        t, mc = i // 4, i % 4
        real = mc >= 2

        @pl.when(t == 0)
        def _():
            xb_copy(mc).wait()
            xb[mc] = pltpu.bitcast(xb3[pl.ds(16 * mc, 16)].reshape(128, DM), u32)

        @pl.when(real)
        def _():
            part_wait(t + 1, mc - 2, 256)
        with jax.named_scope("bulk0"):
            bulk(t, mc, 1, jnp.where(real, t + 1, t), jnp.where(real, t + 1, NCH),
                 pl.multiple_of((mc % 2) * 128, 128), 128)

        @pl.when(i == 1)
        def _():
            chunk_copy(4).start()
            bx_copy(1).start()
            w_copy(1, 0).start()
            w_copy(1, 1).start()

        @pl.when(i == 5)
        def _():
            chunk_copy(5).start()
        return c
    lax.fori_loop(0, 8, body0, 0)
    bx_copy(2).start()
    w_copy(2, 0).start()
    w_copy(2, 1).start()
    chunk_copy(6).start()
    bx_copy(3).start()
    w_copy(3, 0).start()
    w_copy(3, 1).start()
    cp_l.start()
    cp_r1.start()
    nv[0:16, :] = jnp.zeros((16, 128), f32)
    cp_r0.wait()
    cp_sm.wait()

    def body1(q, c):
        t = q + 2
        with jax.named_scope("w_1"):
            chunk_wait(t + 1)
            bx_copy(q).wait()
            w_copy(q, 0).wait()
            w_copy(q, 1).wait()

        def side(n, z):
            sq = 1
            ks = list(range(sq + 1)) if n == 0 else [n + sq]
            for k in ks:
                if k < 16:
                    prep(2 * q + k // 8 + z(2), k // 8, k % 8)
            k = n - 15
            if 0 <= k < 16:
                unit1(2 * q + k // 8, k // 8, (k // 4) % 2, k % 4)
            k, r = divmod(n - 1, 2)
            if r == 0 and 0 <= k < 8:
                wprep(4 * q + k // 2 + z(1), k % 2)
        with jax.named_scope("bulk_p1"):
            bulk(t, 0, 4, t + 1, t + 1, 0, 256, side, 15)
        chunk_start(t + 1 + NST)

        @pl.when(q < 2)
        def _():
            for j in range(2):
                wo_copy(2 * q + j).start()
                wo_copy(4 + 2 * q + j).start()
        return c
    lax.fori_loop(0, 4, body1, 0)

    cp_ax.start()
    with jax.named_scope("w_l"):
        cp_l.wait()
        cp_r1.wait()

    def body2(q, c):
        t, hf = q // 2 + 6, q % 2

        @pl.when(hf == 0)
        def _():
            with jax.named_scope("w_2"):
                chunk_wait(t + 1)
        wo_copy(q).wait()
        wo_copy(4 + q).wait()
        gs = {}

        fs = [[0, 2, 4, 6, 8, 10, 12, 14], [0, 1, 3, 5, 7, 9, 11, 13], [0, 1, 2, 4, 6, 8, 10, 12],
              [0, 1, 3, 4, 6, 8, 9, 11]][1]

        def side(n, z):
            for po in range(8):
                if min(fs[po] + 2, 15) == n:
                    inv(8 * q + po, gs.pop(po))
            if n in fs:
                po = fs.index(n)
                gs[po] = filt(pl.multiple_of(8 * q, 8), po, fwd(8 * q + po))
            k, r = divmod(n - 2, 4)
            if r == 0 and 0 <= k < 4:
                nyq_stage(k)
            for hh in range(8):
                wsum(q, q + z(1), 8 * n + hh, 16)
        with jax.named_scope("bulk_p2"):
            bulk(t, 2 * hf, 2, t + 1, t + 1, pl.multiple_of(hf * 128, 128), 128, side, 8)

        @pl.when(q == 1)
        def _():
            chunk_copy(11).start()
        return c
    lax.fori_loop(0, 4, body2, 0)

    def body3(q, c):
        t = q + 8

        @pl.when(q < 3)
        def _():
            with jax.named_scope("w_3"):
                chunk_wait(t + 1)
        us = {}

        def side(n, z):
            sq = 0
            ks = list(range(sq + 1)) if n == 0 else [n + sq]
            for k in ks:
                if k < 16:
                    us[k] = p3a(2 * q + k // 8 + z(2), k // 8, (k // 4) % 2, k % 4)
            k = n - 2
            if 0 <= k < 16:
                p3b(us.pop(k), k // 8, (k // 4) % 2, k % 4)
            k = n - 16
            if 0 <= k < 16:
                if 1 == 2:
                    p3c(2 * q + k // 8, k // 8, 2 * (k % 8), 2)
                else:
                    p3c(2 * q + k // 8, k // 8, 2 * (k % 8), 1)
                    p3c(2 * q + k // 8, k // 8, 2 * (k % 8) + 1, 1)
        with jax.named_scope("bulk_p3"):
            bulk(t, 0, 4, t + 1, t + 1, 0, 256, side, 0)
        return c
    lax.fori_loop(0, 4, body3, 0)
    cp_outb.start()

    with jax.named_scope("w_wo"):
        cp_ax.wait()
        cp_mem.wait()
    scale = DH ** -0.5
    KS = 768

    def step(it, u):
        s = it * U + u
        lhs = jnp.concatenate([ax[s].reshape(FR, DM), memb[...]], axis=0)
        qs, ks, vs, ps, os_, pre = {}, {}, {}, {}, {}, {}

        def ws(m, h, lo=0, hi=DM):
            return wsel(wpk.at[4 * m + h // 8], h % 8, lo, hi)
        if u > 0:
            for g, m in [(0, 0), (0, 1), (1, 0), (1, 1)][:2]:
                for h in (2 * g, 2 * g + 1):
                    pre[(m, h)] = -_dot(lhs[:, :KS], ws(m, h, 0, KS))

        def dotw(m, h):
            if (m, h) in pre:
                return _dot(lhs[:, KS:], ws(m, h, KS, DM)) - pre[(m, h)]
            return _dot(lhs, ws(m, h))

        def proj(m, g):
            h = 2 * g
            return jnp.concatenate([dotw(m, h).astype(bf16), dotw(m, h + 1).astype(bf16),
                                    pool[2 * NST + 4 * m + h // 8, it * 32 + (h % 8) * 4 + u],
                                    pool[2 * NST + 4 * m + h // 8, it * 32 + (h % 8 + 1) * 4 + u]], axis=0)

        def qk(g):
            sc = lax.dot_general(qs.pop(g), ks.pop(g), (((1,), (1,)), ((), ())),
                                 preferred_element_type=f32) * scale
            fill = sm[0:80, 0:80]
            sc = jnp.where(fill == 0.0, sc, fill)
            mx = jnp.max(sc, axis=-1, keepdims=True)
            e = jnp.exp(sc - mx)
            l = jnp.sum(e, axis=-1, keepdims=True)
            r = pl.reciprocal(l, approx=True)
            r = r * (2.0 - l * r)
            ps[g] = (e * r).astype(bf16)

        def pv(g):
            o = _dot(ps.pop(g), vs.pop(g))
            dt = f32 if u == U - 1 else bf16
            os_[2 * g] = o[0:32].astype(dt)
            os_[2 * g + 1] = o[32:64].astype(dt)
            ob[8 * u:8 * u + 8, (2 * g) * DH:(2 * g + 1) * DH] = o[64:72]
            ob[8 * u:8 * u + 8, (2 * g + 1) * DH:(2 * g + 2) * DH] = o[72:80]

        def olhs(lo, hi):
            return jnp.concatenate([os_[h] for h in range(lo, hi)], axis=1)

        def put(j, r, rb):
            cols = slice(j * 128, (j + 1) * 128)
            oa[it * 2 + u // 2, pl.ds((u % 2) * 4, 3), :, cols] = r[0:FR].reshape(3, 8, 128).astype(bf16)
            memb[:, cols] = r[FR:SEG].astype(bf16)
            if rb is not None:
                for uu in range(U):
                    oa[it * 2 + uu // 2, (uu % 2) * 4 + 3, :, cols] = rb[8 * uu:8 * uu + 8].astype(bf16)

        sk, dq, dp, ab = 6, 3, 4, 1
        nq = nv_ = 0
        for t in range(G + sk):
            if t < G:
                qs[t] = proj(0, t)
            if ab == 1 and 0 <= t - dq < G:
                qk(t - dq)
            if t < G:
                ks[t] = proj(1, t)
            if t - sk - dp >= nv_ + ab - 1:
                for _ in range(ab):
                    pv(nv_)
                    nv_ += 1
            if ab > 1 and t - dq >= nq + ab - 1 and nq < G:
                for _ in range(ab):
                    qk(nq)
                    nq += 1
            if t - sk >= 0:
                vs[t - sk] = proj(2, t - sk)
        rem = list(range(nv_, G))
        hk = 16 * DH
        acc = []
        if u < U - 1:
            oc = olhs(0, 16)
            early = [(oc, wo[j, 0:hk, :]) for j in range(8)]
        else:
            a11, a21 = olhs(0, 16), ob[:, 0:hk]
            l3, l6 = a11.astype(bf16), (a21 - a11).astype(bf16)
            early = [(l3, wc(1, jj)) for jj in range(4)] + [(l6, wc(3, jj)) for jj in range(4)]
        for j in range(8):
            acc.append(-_dot(*early[j]))
            if j >= 0:
                for _ in range(ab):
                    if rem:
                        pv(rem.pop(0))
        if u < U - 1:
            oc = olhs(16, 32)
            for j in range(8):
                put(j, _dot(oc, wo[j, hk:2 * hk, :]) - acc[j], None)
        else:
            a12, a22 = olhs(16, 32), ob[:, hk:2 * hk]
            l1, l2, l4 = (a11 + a22).astype(bf16), (a21 + a22).astype(bf16), a22.astype(bf16)
            l5, l7 = (a11 + a12).astype(bf16), (a12 - a22).astype(bf16)
            for jj in range(4):
                m1 = _dot(l1, wc(0, jj))
                m2 = _dot(l2, wo[jj, 0:hk, :])
                m4 = _dot(l4, wc(2, jj))
                m5 = _dot(l5, wo[4 + jj, hk:2 * hk, :])
                m7 = _dot(l7, wc(4, jj))
                put(jj, (m1 - m5) + (m4 + m7), m2 + m4)
                put(4 + jj, m5 - acc[jj], (m1 - m2) - acc[jj] - acc[4 + jj])

    def out_copy(it):
        return pltpu.make_async_copy(oa.at[pl.ds(it * 2, 2)],
                                     out_hbm.at[pl.ds(it * 2, 2), :, :, pl.ds(0, DM)], sems.at[32])

    def group(it, c):
        with jax.named_scope("grp"):
            for u in range(U):
                step(it, u)
        out_copy(it).start()
        return c
    lax.fori_loop(0, NSEG // U, group, 0)
    with jax.named_scope("w_out"):
        for it in range(NSEG // U):
            out_copy(it).wait()
        cp_outb.wait()


def pallas_concat_heads__memory_aug_recurrent_mem_tr__spectral_gfnet__prompt_kernel(
    A_x, A_mem0, A_Wq, A_Wk, A_Wv, A_Wo, A_seg_len, B_x, B_w_r, B_w_i,
):
    del A_seg_len
    R, LN, TW, fill, KC = _tables()
    small = np.zeros((208, 128), np.float32)
    small[:80, :80] = fill
    small[80:112] = TW
    small[112:] = np.repeat(KC, 8, axis=0)
    hbm = pl.BlockSpec(memory_space=pl.ANY)
    out = pl.pallas_call(
        _kernel,
        out_shape=jax.ShapeDtypeStruct((RS, 8, 8, DM + D), bf16),
        in_specs=[hbm] * 13,
        out_specs=hbm,
        scratch_shapes=[
            pltpu.VMEM((NSEG, 3, 8, DM), bf16),
            pltpu.VMEM((NSEG, 8, DM), bf16),
            pltpu.VMEM((4, 64, DM), u32),
            pltpu.VMEM((DM // 128, H * DH, 128), bf16),
            pltpu.VMEM((BC + 10, DM // 2, 8, DH), bf16),
            pltpu.VMEM((NCH + 1, 16 * PW, DH), u32),
            pltpu.VMEM((M, DM), bf16),
            pltpu.VMEM((U * M, H * DH), f32),
            pltpu.VMEM((RS, 8, 8, DM), bf16),
            pltpu.VMEM((RS, 8, 8, D), bf16),
            pltpu.VMEM((D // 2 + 1, S), bf16),
            pltpu.VMEM((D // 2 + 1, S), bf16),
            pltpu.VMEM((16, 64, 128), u32),
            pltpu.VMEM((2 * RS + 5, 64, 128), u32),
            pltpu.VMEM((208, 128), f32),
            pltpu.VMEM((RS, 4, 8, 16, 128), bf16),
            pltpu.VMEM((4, RS, TP, 128), f32),
            pltpu.VMEM((2, 2, BS * WP, 128), u32),
            pltpu.VMEM((32, 128), f32),
            pltpu.SMEM((8,), i32),
            pltpu.SemaphoreType.DMA((46,)),
        ],
        compiler_params=pltpu.CompilerParams(vmem_limit_bytes=124 * 1024 * 1024,
                                             disable_bounds_checks=True, disable_semaphore_checks=True),
    )(A_x.reshape(NSEG, 4, 8, DM), A_mem0.reshape(M, DM),
      A_Wq.reshape(2, DM // 2, H, DH), A_Wk.reshape(2, DM // 2, H, DH), A_Wv.reshape(2, DM // 2, H, DH),
      A_Wo.reshape(H * DH, DM), B_x.reshape(RS, 8, 8, D), B_w_r.T, B_w_i.T,
      jnp.asarray(R), jnp.asarray(LN), jnp.asarray(small), jnp.asarray(np.array([1, 0, 2, 3, 4, 5, 6, 7], np.int32)))
    return out.reshape(1, S, DM + D)
```

```python
import functools
import math

import jax
import jax.numpy as jnp
import numpy as np
from jax import lax
import jax.experimental.pallas as pl
import jax.experimental.pallas.tpu as pltpu

bf16, f32, u32, i32 = jnp.bfloat16, jnp.float32, jnp.uint32, jnp.int32

S, DM, H, DH, M, SEG = 2048, 1024, 32, 128, 8, 32
NSEG = S // SEG
FR = SEG - M
G = H // 2
U = 4
NCH = 12
NST = 4
PW = 264

D = 1024
RS, BS = 32, 64
HR = RS // 2
WP = 40
TP = 136
C8 = float(np.sqrt(0.5))


def _pack_rows(a):
    u = np.asarray(a, np.float32).astype(jnp.bfloat16).view(np.uint16).astype(np.uint32)
    return u[..., 0::2, :] | (u[..., 1::2, :] << 16)


_RHO = (2, 4, 4, 4)


def _in_a(lane, c):
    return (lane % 4 < 2) if c == 0 else ((lane + 2) % 8 < 4)


def _dstage(x, kc, roll64):
    a = [x[j] + x[j + 4] for j in range(4)]
    b = [x[j] - x[j + 4] for j in range(4)]
    t1 = (b[1] - b[3]) * C8
    t2 = (b[1] + b[3]) * C8
    s0, s1 = a[0] + a[2], a[1] + a[3]
    out = [s0 + s1, s0 - s1]
    for c, (u, v) in enumerate(((b[0] + t1, b[2] + t2), (a[0] - a[2], a[1] - a[3]), (b[0] - t1, b[2] - t2))):
        g = u * kc[4 * c] + v * kc[4 * c + 1]
        h = roll64(u * kc[4 * c + 2] + v * kc[4 * c + 3])
        out += [g + h, g - h]
    return out


def _dstage_t(p, kc, roll64):
    uv = []
    for c in range(3):
        g = p[2 + 2 * c] + p[3 + 2 * c]
        h = roll64(p[2 + 2 * c] - p[3 + 2 * c])
        uv.append((g * kc[4 * c] + h * kc[4 * c + 2], g * kc[4 * c + 1] + h * kc[4 * c + 3]))
    s0, s1 = p[0] + p[1], p[0] - p[1]
    a = [s0 + uv[1][0], s1 + uv[1][1], s0 - uv[1][0], s1 - uv[1][1]]
    t1 = (uv[0][0] - uv[2][0]) * C8
    t2 = (uv[0][1] - uv[2][1]) * C8
    b = [uv[0][0] + uv[2][0], t1 + t2, uv[0][1] + uv[2][1], t2 - t1]
    return [a[j] + b[j] for j in range(4)] + [a[j] - b[j] for j in range(4)]


@functools.lru_cache(maxsize=None)
def _tables():
    kcol = np.zeros((4, 128), np.int64)
    for l in range(128):
        i0, i1 = l, 128 + (l ^ 1)
        ev, o3 = l % 2 == 0, l % 4 in (0, 3)
        kcol[0, l] = 2 * (i0 if ev else i1)
        kcol[2, l] = 2 * (i1 if ev else i0)
        kcol[1, l] = 2 * (i0 if o3 else i1) + 1
        kcol[3, l] = 2 * (i1 if o3 else i0) + 1
    lanes = np.arange(128)
    lo = lanes < 64
    KC = np.zeros((12, 128))
    for c, sg in ((1, -1.0), (2, -1.0), (3, 1.0)):
        tr, ti = np.cos(2 * np.pi * c / 16), -np.sin(2 * np.pi * c / 16)
        KC[4 * c - 4] = np.where(lo, 1.0, ti)
        KC[4 * c - 3] = sg * np.where(lo, 0.0, tr)
        KC[4 * c - 2] = np.where(lo, 0.0, tr)
        KC[4 * c - 1] = sg * np.where(lo, 1.0, -ti)
    eye = np.eye(D)
    Bt = _dstage([eye[:, 128 * e:128 * (e + 1)] for e in range(8)], KC, lambda v: np.roll(v, 64, axis=1))
    d = np.arange(D)
    R = np.zeros((16, 128, 128))
    for c in range(4):
        rho = _RHO[c]
        inA = _in_a(lanes, c)
        ang = 2 * np.pi * (np.outer(d, kcol[c]) % D) / D
        fr, fi = np.cos(ang), -np.sin(ang)
        wr_, wi_ = np.full(128, 2.0), np.full(128, 2.0)
        if c == 0:
            fi[:, 0] = (-1.0) ** d
            wr_[0] = 1.0
            wi_[0] = 1.0
        fi, wi_ = np.roll(fi, -rho, axis=1), np.roll(wi_, -rho)
        for h in range(2):
            own = inA if h == 0 else ~inA
            ft, wt = np.where(own, fr, fi), np.where(own, wr_, wi_)
            bt = Bt[2 * c + h]
            r = (bt.T @ ft) / (bt * bt).sum(axis=0)[:, None]
            assert np.abs(bt @ r - ft).max() < 1e-9
            R[2 * c + h] = r
            R[8 + 2 * c + h] = (wt[:, None] * r.T) / (S * D)
    L = np.zeros((2 * RS, 128, 128))
    bb = np.arange(BS)
    kord = np.array([ri * 64 + 8 * t + r for t in range(8) for ri in range(2) for r in range(8)])
    for p1 in range(RS):
        ang = 2 * np.pi * (np.outer(p1 + RS * bb, bb) % S) / S
        mr, mi = np.cos(ang), -np.sin(ang)
        full = np.block([[mr, -mi], [mi, mr]])
        L[p1] = full[:, kord]
        L[RS + p1] = full.T
    l_, q_ = np.arange(128), np.arange(16)
    ang = 2 * np.pi * (np.outer(l_, l_) % 128) / 128
    N1 = np.concatenate([np.cos(ang), -np.sin(ang)], axis=1)
    N1 = np.concatenate([(N1[:64] + N1[64:]) / 2, (N1[:64] - N1[64:]) / 2], axis=0)
    ang = 2 * np.pi * np.outer(q_, l_) / S
    TW = np.concatenate([np.cos(ang), -np.sin(ang)], axis=0)
    ang = 2 * np.pi * (np.outer(q_, q_) % 16) / 16
    fr, fi = np.cos(ang), -np.sin(ang)
    F16 = np.block([[fr, -fi], [fi, fr]])
    NY = np.zeros((5, 128, 128))
    NY[0], NY[1], NY[2], NY[3] = N1[:, :128], N1[:, 128:], N1[:, :128].T, N1[:, 128:].T
    NY[4, :32, :32] = F16
    NY[4, 32:64, :32] = F16.T
    LN = np.concatenate([L, NY], axis=0)
    head = np.zeros(80, np.int32)
    pos = np.zeros(80, np.int32)
    for r in range(80):
        if r < 64:
            head[r] = r // 32
            t = r % 32
            pos[r] = (M + t) if t < FR else (t - FR)
        else:
            head[r] = (r - 64) // 8
            pos[r] = M + FR + (r - 64) % 8
    same = head[:, None] == head[None, :]
    vis = (pos[:, None] < M) | (pos[:, None] >= pos[None, :])
    fill = np.where(same, np.where(vis, 0.0, -1e9), -np.inf).astype(np.float32)
    return _pack_rows(R), _pack_rows(LN), TW.astype(np.float32), fill, KC.astype(np.float32)


def _cmul_const(re, im, j, n, sgn):
    ang = sgn * 2 * math.pi * j / n
    c, s = math.cos(ang), math.sin(ang)
    if abs(abs(c) - abs(s)) < 1e-12:
        if c * s > 0:
            return (re - im) * c, (re + im) * c
        return (re + im) * c, (im - re) * c
    return re * c - im * s, re * s + im * c


def _diff_tw(a, b, j, n, sgn):
    if j == 0:
        return a[0] - b[0], a[1] - b[1]
    if 4 * j == n:
        if sgn < 0:
            return a[1] - b[1], b[0] - a[0]
        return b[1] - a[1], a[0] - b[0]
    return _cmul_const(a[0] - b[0], a[1] - b[1], j, n, sgn)


def _tw(v, j, sgn):
    if j == 0:
        return v
    if 4 * j == RS:
        return (v[1], -v[0]) if sgn < 0 else (-v[1], v[0])
    return _cmul_const(v[0], v[1], j, RS, sgn)


def _fft(v, sgn):
    n = len(v)
    if n == 1:
        return v
    h = n // 2
    ev = _fft([(v[j][0] + v[j + h][0], v[j][1] + v[j + h][1]) for j in range(h)], sgn)
    od = _fft([_diff_tw(v[j], v[j + h], j, n, sgn) for j in range(h)], sgn)
    out = [None] * n
    out[0::2] = ev
    out[1::2] = od
    return out


def _dot(a, b):
    return jnp.dot(a, b, preferred_element_type=f32)


def _asbf(v):
    return pltpu.bitcast(v, bf16)


def _cm(ar, ai, br, bi):
    return ar * br - ai * bi, ar * bi + ai * br


CHUNKS = [(0, 0), (0, 1), (0, 2), (0, 3), (1, 0), (1, 1), (1, 2), (2, 0), (2, 1), (2, 2), (2, 3), (1, 3)]
BU = 2 * NST + NCH
BC = BU + 2


def _kernel(ax_hbm, mem_hbm, wq_hbm, wk_hbm, wv_hbm, wo_hbm, bx_hbm, wr_hbm, wi_hbm,
            R_hbm, L_hbm, sm_hbm, out_hbm,
            ax, xb3, xb, wo, pool, wpk, memb, ob, oa,
            bx, wr, wi, R, L, sm, Y, T, wp, nv, sems):
    srcs = (wq_hbm, wk_hbm, wv_hbm)
    lane8 = lax.broadcasted_iota(i32, (8, 128), 1)

    def chunk_copy(t):
        m, c = CHUNKS[t]
        return pltpu.make_async_copy(srcs[m].at[:, :, pl.ds(8 * c, 8), :],
                                     pool.at[pl.ds(2 * (t % NST), 2)], sems.at[t % NST])

    def part_sem(t, part):
        return sems.at[34 + jnp.where(t == 0, 0, 2 + 2 * t) + part]

    def part_start(t, part, n):
        pltpu.make_async_copy(srcs[0].at[:, pl.ds(part * n, n), pl.ds(8 * t, 8), :],
                              pool.at[pl.ds(2 * t, 2), pl.ds(part * n, n)], part_sem(t, part)).start()

    def part_wait(t, part, n):
        blk = pool.at[pl.ds(2 * t, 2), pl.ds(part * n, n)]
        pltpu.make_async_copy(blk, blk, part_sem(t, part)).wait()

    def chunk_start(t):
        sl = t & (NST - 1)
        pltpu.make_async_copy(wv_hbm.at[:, :, pl.ds(pl.multiple_of(8 * (t - 7), 8), 8), :],
                              pool.at[pl.ds(2 * sl, 2)], sems.at[sl]).start()

    def chunk_wait(t):
        sl = t & (NST - 1)
        blk = pool.at[pl.ds(2 * sl, 2)]
        pltpu.make_async_copy(blk, blk, sems.at[sl]).wait()

    def xb_copy(q):
        return pltpu.make_async_copy(ax_hbm.at[pl.ds(16 * q, 16), 3], xb3.at[pl.ds(16 * q, 16)], sems.at[8 + q])

    def bx_copy(q):
        return pltpu.make_async_copy(bx_hbm.at[:, pl.ds(2 * q, 2)], bx.at[:, pl.ds(2 * q, 2)], sems.at[12 + q])

    def w_copy(q, i):
        cols = pl.ds(pl.multiple_of(512 * q, 512), 512)
        return pltpu.make_async_copy((wr_hbm, wi_hbm)[i].at[:, cols], (wr, wi)[i].at[:, cols], sems.at[16 + 4 * i + q])

    def wo_copy(q, hi):
        j = q + 4 * hi
        return pltpu.make_async_copy(wo_hbm.at[:, pl.ds(pl.multiple_of(128 * j, 128), 128)], wo.at[j],
                                     sems.at[42 + q])

    cp_r0 = pltpu.make_async_copy(R_hbm.at[pl.ds(0, 8)], R.at[pl.ds(0, 8)], sems.at[25])
    cp_r1 = pltpu.make_async_copy(R_hbm.at[pl.ds(8, 8)], R.at[pl.ds(8, 8)], sems.at[26])
    cp_l = pltpu.make_async_copy(L_hbm, L, sems.at[27])
    cp_ax = pltpu.make_async_copy(ax_hbm.at[:, pl.ds(0, 3)], ax, sems.at[28])
    cp_outb = pltpu.make_async_copy(bx, out_hbm.at[:, :, :, pl.ds(DM, D)], sems.at[29])
    cp_sm = pltpu.make_async_copy(sm_hbm, sm, sems.at[30])
    cp_mem = pltpu.make_async_copy(mem_hbm, memb, sems.at[31])

    for part in range(4):
        part_start(0, part, 128)
    xb_copy(0).start()
    xb_copy(1).start()
    part_start(1, 0, 256)
    xb_copy(2).start()
    part_start(1, 1, 256)
    xb_copy(3).start()
    part_start(2, 0, 256)
    part_start(2, 1, 256)
    chunk_copy(3).start()
    cp_r0.start()
    bx_copy(0).start()
    w_copy(0, 0).start()
    w_copy(0, 1).start()
    cp_sm.start()
    cp_mem.start()

    def kc(rep=2):
        return [jnp.concatenate([sm[112 + 8 * i:120 + 8 * i, :]] * rep, axis=0) for i in range(12)]

    def roll64(v):
        return pltpu.roll(v, 64, 1)

    def dot2(u, w):
        if 0 == 0:
            return _dot(u, w)
        return jnp.concatenate([_dot(u[:64], w), _dot(u[64:], w)], axis=0)

    def prep(t, tpar, jj):
        lo = [bx[2 * jj:2 * jj + 2, t, :, 128 * e:128 * (e + 1)].astype(f32).reshape(16, 128) for e in range(8)]
        hi = [bx[HR + 2 * jj:HR + 2 * jj + 2, t, :, 128 * e:128 * (e + 1)].astype(f32).reshape(16, 128)
              for e in range(8)]
        for par in range(2):
            x = [lo[e] + hi[e] if par == 0 else lo[e] - hi[e] for e in range(8)]
            uu = _dstage(x, kc(), roll64)
            for q in range(8):
                o = (((tpar * 2 + par) * 8 + q) * 8 + jj) * 2
                pool[BU, o:o + 2] = uu[q].reshape(2, 8, 128).astype(bf16)

    def unit1(t, tpar, par, cg):
        o = ((tpar * 2 + par) * 8 + 2 * cg) * 16
        za = dot2(pool[BU, o:o + 16].reshape(128, 128), _asbf(R[2 * cg]))
        zb = dot2(pool[BU, o + 16:o + 32].reshape(128, 128), _asbf(R[2 * cg + 1]))
        ina = _in_a(lane8, cg)
        v = []
        for j in range(HR):
            pa, pb = za[8 * j:8 * j + 8], zb[8 * j:8 * j + 8]
            v.append((jnp.where(ina, pa, pb), pltpu.roll(jnp.where(ina, pb, pa), _RHO[cg], 1)))
        if cg == 0:
            V = nv[8 * tpar:8 * tpar + 8, :]
            for j in range(HR):
                vb = jnp.broadcast_to(v[j][1][:, 0:1], (8, 128))
                V = jnp.where(lane8 == 64 * par + 4 * j + (t >> 1), vb, V)
                v[j] = (v[j][0], jnp.where(lane8 == 0, 0.0, v[j][1]))
            nv[8 * tpar:8 * tpar + 8, :] = V
        if par == 1:
            v = [_tw(v[j], j, -1) for j in range(HR)]
        o = _fft(v, -1)
        for m in range(HR):
            Y[2 * m + par, cg, t] = jnp.concatenate(o[m], axis=0).astype(bf16)

    def wprep(pb, i):
        w = (wr, wi)[i]
        cols = pl.ds(pl.multiple_of(pb * 128, 128), 128)
        sub = lax.broadcasted_iota(i32, (8, 128), 0)
        msk = (jnp.where(sub % 2 == 0, jnp.uint32(0xffff), jnp.uint32(0))
               | jnp.where((sub % 4 == 0) | (sub % 4 == 3), jnp.uint32(0xffff0000), jnp.uint32(0)))
        t0 = pltpu.bitcast(w[0:256, cols], u32)
        t1 = pltpu.bitcast(w[256:512, cols], u32)
        ps, qs = [], []
        for j in range(16):
            a = t0[8 * j:8 * j + 8]
            b = t1[8 * j:8 * j + 8]
            b = jnp.where(sub % 2 == 0, pltpu.roll(b, 7, 0), pltpu.roll(b, 1, 0))
            x = (a ^ b) & msk
            ps.append(b ^ x)
            qs.append(a ^ x)
        for h, lst in enumerate((ps, qs)):
            tr = pltpu.bitcast(pltpu.bitcast(jnp.concatenate(lst, axis=0), f32).T, u32)
            for q in range(4):
                wp[i, h, pl.ds(pl.multiple_of((pb * 4 + q) * WP, 8), 32), :] = tr[32 * q:32 * q + 32]

    def fwd(p):
        return _dot(_asbf(L[p]), jnp.concatenate([Y[p, cg].reshape(128, 128) for cg in range(4)], axis=1))

    def filt(pbase, po, v):
        grs, gis = [None] * 4, [None] * 4
        win = pl.ds(pbase, (BS - 1) * WP + 8)
        for h in range(2):
            wr_ = wp.at[0, h, win][pl.ds(po, BS, stride=WP), :]
            wi_ = wp.at[1, h, win][pl.ds(po, BS, stride=WP), :]
            for hi in range(2):
                cg = 2 * h + hi
                if hi == 0:
                    a, b = wr_ << 16, wi_ << 16
                else:
                    a, b = wr_ & jnp.uint32(0xffff0000), wi_ & jnp.uint32(0xffff0000)
                grs[cg], gis[cg] = _cm(v[:BS, 128 * cg:128 * (cg + 1)], v[BS:, 128 * cg:128 * (cg + 1)],
                                       pltpu.bitcast(a, f32), pltpu.bitcast(b, f32))
        return jnp.concatenate([jnp.concatenate(grs, axis=1), jnp.concatenate(gis, axis=1)], axis=0).astype(bf16)

    def inv(p, g):
        t = _dot(_asbf(L[RS + p]), g)
        for cg in range(4):
            T[cg, p, 0:128, :] = t[:, 128 * cg:128 * (cg + 1)]

    nyq = {}

    def nyq_stage(k):
        n0 = 2 * RS
        twr, twi = sm[80:96, :], sm[96:112, :]
        if k == 0:
            v = nv[0:16, :].astype(bf16)
            r, i = _cm(_dot(v, _asbf(L[n0])), _dot(v, _asbf(L[n0 + 1])), twr, twi)
            nyq[0] = jnp.concatenate([r, i], axis=0).astype(bf16)
        elif k == 1:
            t = _dot(_asbf(L[n0 + 4, 0:16])[:, 0:32], nyq[0])
            ws = []
            for w in (wr, wi):
                row = w[512:513, :].astype(f32)
                ws.append(jnp.concatenate([row[:, 128 * r:128 * (r + 1)] for r in range(16)], axis=0))
            r, i = _cm(t[:16], t[16:], ws[0], ws[1])
            nyq[1] = jnp.concatenate([r, i], axis=0).astype(bf16)
        elif k == 2:
            t = _dot(_asbf(L[n0 + 4, 16:32])[:, 0:32], nyq[1])
            r, i = _cm(t[:16], t[16:], twr, -twi)
            nyq[2] = (r.astype(bf16), i.astype(bf16))
        elif k == 3:
            nv[16:32, :] = _dot(nyq[2][0], _asbf(L[n0 + 2])) + _dot(nyq[2][1], _asbf(L[n0 + 3]))

    def p3a(t, tpar, par, cg):
        rr = pl.ds(pl.multiple_of(t * 8, 8), 8)
        ri = pl.ds(pl.multiple_of(64 + t * 8, 8), 8)
        o = _fft([(T[cg, 2 * m + par, rr, :], T[cg, 2 * m + par, ri, :]) for m in range(HR)], +1)
        if par == 1:
            o = [_tw(o[j], j, +1) for j in range(HR)]
        if cg == 0:
            un = nv[16 + 8 * tpar:24 + 8 * tpar, :]
            o = [(o[j][0], jnp.where(lane8 == 0, pltpu.roll(un, (128 - 64 * par - 4 * j - (t >> 1)) & 127, 1),
                                     o[j][1])) for j in range(HR)]
        ina = _in_a(lane8, cg)
        ua, ub = [], []
        for re, im in o:
            im = pltpu.roll(im, 128 - _RHO[cg], 1)
            ua.append(jnp.where(ina, re, im))
            ub.append(jnp.where(ina, im, re))
        for j in range(HR // 2):
            for h, x in enumerate((ua, ub)):
                o = ((tpar * 2 + par) * 8 + 2 * cg + h) * 16 + 2 * j
                pool[BU + 1, o:o + 2] = jnp.stack(x[2 * j:2 * j + 2]).astype(bf16)

    def p3b(tpar, par, cg):
        nsp = 1
        nt = 16 // nsp
        zs = []
        for h in range(2):
            for i in range(nsp):
                o = ((tpar * 2 + par) * 8 + 2 * cg + h) * 16 + nt * i
                zs.append((o, _dot(pool[BU + 1, o:o + nt].reshape(8 * nt, 128), _asbf(R[8 + 2 * cg + h]))))
        return zs

    def p3s(zs):
        for o, z in zs:
            nt = z.shape[0] // 8
            pool[BU, o:o + nt] = z.reshape(nt, 8, 128).astype(bf16)

    def p3c(t, tpar, j0, nj):
        res = []
        for par in range(2):
            p = []
            for q in range(8):
                o = ((tpar * 2 + par) * 8 + q) * 16 + j0
                p.append(pool[BU, o:o + nj].astype(f32).reshape(8 * nj, 128))
            res.append(_dstage_t(p, kc(nj), roll64))
        for e in range(8):
            cols = slice(128 * e, 128 * (e + 1))
            bx[j0:j0 + nj, t, :, cols] = (res[0][e] + res[1][e]).reshape(nj, 8, 128).astype(bf16)
            bx[HR + j0:HR + j0 + nj, t, :, cols] = (res[0][e] - res[1][e]).reshape(nj, 8, 128).astype(bf16)

    def wsum(jj, hf, n):
        r0 = pl.multiple_of(hf * 1024, 1024)
        lo, hi = pl.ds(r0 + 16 * n, 16), pl.ds(r0 + 2048 + 16 * n, 16)
        b11, b21 = wo[jj, lo, :].astype(f32), wo[jj, hi, :].astype(f32)
        b12, b22 = wo[4 + jj, lo, :].astype(f32), wo[4 + jj, hi, :].astype(f32)
        for i, v in enumerate((b11 + b22, b12 - b22, b21 - b11, b11 + b12, b21 + b22)):
            pool[BC + 2 * i + (jj >> 1), pl.ds((jj & 1) * 256 + hf * 128 + 2 * n, 2)] = (
                v.reshape(2, 8, 128).astype(bf16))

    def wc(i, jj):
        return pool[BC + 2 * i + jj // 2, (jj % 2) * 256:(jj % 2 + 1) * 256].reshape(2048, 128)

    def runit(b0, d0, dst, k):
        a = pltpu.bitcast(jnp.concatenate([pool[b0, d0 + 2 * k], pool[b0 + 1, d0 + 2 * k]], axis=0), u32)
        b = pltpu.bitcast(jnp.concatenate([pool[b0, d0 + 2 * k + 1], pool[b0 + 1, d0 + 2 * k + 1]], axis=0), u32)
        dst[pl.ds(k, 8, stride=PW), :] = (a & jnp.uint32(0xffff)) | (b << 16)
        dst[pl.ds(8 * PW + k, 8, stride=PW), :] = (a >> 16) | (b & jnp.uint32(0xffff0000))

    def wsel(w, hl, lo=0, hi=DM):
        base = ((hl % 2) * 8 + hl // 2) * PW
        parts = []
        for kh in range(2):
            a, b = max(lo, 512 * kh), min(hi, 512 * (kh + 1))
            if a < b:
                o = base + 4 * PW * kh - 256 * kh
                parts.append(w[o + a // 2:o + b // 2, :])
        return _asbf(jnp.concatenate(parts, axis=0))

    def bulk(t, mc0, nmc, tsrc, tdst, k0, nk, side=None):
        w = wpk.at[t]
        b0 = 2 * (tsrc & (NST - 1))
        dst = wpk.at[tdst, pl.ds(k0, 15 * PW + nk)]
        bq = 2 * NST + (t & 31)
        ns = 8 * nmc
        per = nk // ns
        for mi in range(nmc):
            mc = mc0 + mi
            x = _asbf(xb[mc])
            for h in range(8):
                n = mi * 8 + h
                r = _dot(x, wsel(w, h)).reshape(16, M, DH)
                nn = (n - 1) % ns
                for k in range(per * nn, per * (nn + 1)):
                    runit(b0, 2 * k0, dst, k)
                if side is not None:
                    side(n)
                rb = r.astype(bf16)
                for gi in range(4):
                    pool[bq, pl.ds(mc * 128 + gi * 32 + h * 4, 4)] = rb[4 * gi:4 * gi + 4]

    def rel0(i, c):
        @pl.when(i % 2 == 0)
        def _():
            part_wait(0, i // 2, 128)
        dst = wpk.at[0, pl.ds(pl.multiple_of(i * 32, 32), 15 * PW + 32)]
        for k in range(32):
            runit(0, i * 64, dst, k)
        return c
    with jax.named_scope("rel0"):
        lax.fori_loop(0, 8, rel0, 0)

    def body0(i, c):
        t, mc = i >> 2, i & 3
        real = mc >= 2

        @pl.when(t == 0)
        def _():
            xb_copy(mc).wait()
            xb[mc] = pltpu.bitcast(xb3[pl.ds(16 * mc, 16)].reshape(128, DM), u32)

        @pl.when(real)
        def _():
            part_wait(t + 1, mc - 2, 256)
        with jax.named_scope("bulk0"):
            bulk(t, mc, 1, jnp.where(real, t + 1, t), jnp.where(real, t + 1, NCH),
                 pl.multiple_of((mc & 1) * 128, 128), 128)

        @pl.when(i == 1)
        def _():
            chunk_copy(4).start()
            bx_copy(1).start()
            w_copy(1, 0).start()
            w_copy(1, 1).start()

        @pl.when(i == 5)
        def _():
            chunk_copy(5).start()
        return c
    lax.fori_loop(0, 8, body0, 0)
    bx_copy(2).start()
    w_copy(2, 0).start()
    w_copy(2, 1).start()
    chunk_copy(6).start()
    bx_copy(3).start()
    w_copy(3, 0).start()
    w_copy(3, 1).start()
    cp_l.start()
    cp_r1.start()
    nv[0:16, :] = jnp.zeros((16, 128), f32)
    cp_r0.wait()
    cp_sm.wait()

    def body1(q, c):
        t = q + 2
        with jax.named_scope("w_1"):
            chunk_wait(t + 1)
            bx_copy(q).wait()
            w_copy(q, 0).wait()
            w_copy(q, 1).wait()

        def side(n):
            sq = 1
            ks = list(range(sq + 1)) if n == 0 else [n + sq]
            for k in ks:
                if k < 16:
                    prep(2 * q + k // 8, k // 8, k % 8)
            k = n - 15
            if 0 <= k < 16:
                unit1(2 * q + k // 8, k // 8, (k // 4) % 2, k % 4)
            k, r = divmod(n - 1, 2)
            if r == 0 and 0 <= k < 8:
                wprep(4 * q + k // 2, k % 2)
        with jax.named_scope("bulk_p1"):
            bulk(t, 0, 4, t + 1, t + 1, 0, 256, side)
        wo_copy(q, 0).start()
        wo_copy(q, 1).start()
        chunk_start(t + 1 + NST)
        return c
    lax.fori_loop(0, 4, body1, 0)

    cp_ax.start()
    with jax.named_scope("w_l"):
        cp_l.wait()
        cp_r1.wait()

    def body2(q, c):
        t, hf = (q >> 1) + 6, q & 1

        @pl.when(hf == 0)
        def _():
            with jax.named_scope("w_2"):
                chunk_wait(t + 1)
                wo_copy(q >> 1, 0).wait()
                wo_copy(q >> 1, 1).wait()
        gs = {}

        fs = [[0, 2, 4, 6, 8, 10, 12, 14], [0, 1, 3, 5, 7, 9, 11, 13], [0, 1, 2, 4, 6, 8, 10, 12],
              [0, 1, 3, 4, 6, 8, 9, 11]][1]

        def side(n):
            for po in range(8):
                if min(fs[po] + 2, 15) == n:
                    inv(8 * q + po, gs.pop(po))
            if n in fs:
                po = fs.index(n)
                gs[po] = filt(pl.multiple_of(8 * q, 8), po, fwd(8 * q + po))
            k, r = divmod(n - 1, 3)
            if r == 0 and 0 <= k < 4:
                nyq_stage(k)
            for hh in range(4):
                wsum(q >> 1, hf, 4 * n + hh)
        with jax.named_scope("bulk_p2"):
            bulk(t, 2 * hf, 2, t + 1, t + 1, pl.multiple_of(hf * 128, 128), 128, side)
        return c
    lax.fori_loop(0, 4, body2, 0)
    chunk_copy(11).start()
    for j in (2, 3):
        wo_copy(j, 0).wait()
        wo_copy(j, 1).wait()

    def body3(q, c):
        t = q + 8

        @pl.when(q < 3)
        def _():
            with jax.named_scope("w_3"):
                chunk_wait(t + 1)
        us = {}

        def side(n):
            sq = 0
            ks = list(range(sq + 1)) if n == 0 else [n + sq]
            for k in ks:
                if k < 16:
                    p3a(2 * q + k // 8, k // 8, (k // 4) % 2, k % 4)
            k = n - 3
            if 0 <= k < 16:
                us[k] = p3b(k // 8, (k // 4) % 2, k % 4)
            k = n - 3 - 1
            if 0 <= k < 16:
                p3s(us.pop(k))
            k = n - 16
            if 0 <= k < 16:
                if 1 == 2:
                    p3c(2 * q + k // 8, k // 8, 2 * (k % 8), 2)
                else:
                    p3c(2 * q + k // 8, k // 8, 2 * (k % 8), 1)
                    p3c(2 * q + k // 8, k // 8, 2 * (k % 8) + 1, 1)
            for hh in range(2):
                wsum(2 + (q >> 1), q & 1, 2 * n + hh)
        with jax.named_scope("bulk_p3"):
            bulk(t, 0, 4, t + 1, t + 1, 0, 256, side)
        return c
    lax.fori_loop(0, 4, body3, 0)
    cp_outb.start()

    with jax.named_scope("w_wo"):
        cp_ax.wait()
        cp_mem.wait()
    scale = DH ** -0.5
    KS = 768

    def step(it, u):
        s = it * U + u
        lhs = jnp.concatenate([ax[s].reshape(FR, DM), memb[...]], axis=0)
        qs, ks, vs, ps, os_, pre = {}, {}, {}, {}, {}, {}

        def ws(m, h, lo=0, hi=DM):
            return wsel(wpk.at[CHUNKS.index((m, h // 8))], h % 8, lo, hi)
        if u > 0:
            for g, m in [(0, 0), (0, 1), (1, 0), (1, 1)][:2]:
                for h in (2 * g, 2 * g + 1):
                    pre[(m, h)] = -_dot(lhs[:, :KS], ws(m, h, 0, KS))

        def dotw(m, h):
            if (m, h) in pre:
                return _dot(lhs[:, KS:], ws(m, h, KS, DM)) - pre[(m, h)]
            return _dot(lhs, ws(m, h))

        def proj(m, g):
            h = 2 * g
            bq = 2 * NST + CHUNKS.index((m, h // 8))
            return jnp.concatenate([dotw(m, h).astype(bf16), dotw(m, h + 1).astype(bf16),
                                    pool[bq, it * 32 + (h % 8) * 4 + u],
                                    pool[bq, it * 32 + (h % 8 + 1) * 4 + u]], axis=0)

        def qk(g):
            sc = lax.dot_general(qs.pop(g), ks.pop(g), (((1,), (1,)), ((), ())),
                                 preferred_element_type=f32) * scale
            fill = sm[0:80, 0:80]
            sc = jnp.where(fill == 0.0, sc, fill)
            mx = jnp.max(sc, axis=-1, keepdims=True)
            e = jnp.exp(sc - mx)
            l = jnp.sum(e, axis=-1, keepdims=True)
            r = pl.reciprocal(l, approx=True)
            r = r * (2.0 - l * r)
            ps[g] = (e * r).astype(bf16)

        def pv(g):
            o = _dot(ps.pop(g), vs.pop(g))
            dt = f32 if u == U - 1 else bf16
            os_[2 * g] = o[0:32].astype(dt)
            os_[2 * g + 1] = o[32:64].astype(dt)
            ob[8 * u:8 * u + 8, (2 * g) * DH:(2 * g + 1) * DH] = o[64:72]
            ob[8 * u:8 * u + 8, (2 * g + 1) * DH:(2 * g + 2) * DH] = o[72:80]

        def olhs(lo, hi):
            return jnp.concatenate([os_[h] for h in range(lo, hi)], axis=1)

        def put(j, r, rb):
            cols = slice(j * 128, (j + 1) * 128)
            oa[it * 2 + u // 2, pl.ds((u % 2) * 4, 3), :, cols] = r[0:FR].reshape(3, 8, 128).astype(bf16)
            memb[:, cols] = r[FR:SEG].astype(bf16)
            if rb is not None:
                for uu in range(U):
                    oa[it * 2 + uu // 2, (uu % 2) * 4 + 3, :, cols] = rb[8 * uu:8 * uu + 8].astype(bf16)

        sk, dq, dp, ab = 7, 3, 5, 1
        nq = nv_ = 0
        for t in range(G + sk):
            if t < G:
                qs[t] = proj(0, t)
            if ab == 1 and 0 <= t - dq < G:
                qk(t - dq)
            if t < G:
                ks[t] = proj(1, t)
            if t - sk - dp >= nv_ + ab - 1:
                for _ in range(ab):
                    pv(nv_)
                    nv_ += 1
            if ab > 1 and t - dq >= nq + ab - 1 and nq < G:
                for _ in range(ab):
                    qk(nq)
                    nq += 1
            if t - sk >= 0:
                vs[t - sk] = proj(2, t - sk)
        rem = list(range(nv_, G))
        hk = 16 * DH
        acc = []
        if u < U - 1:
            oc = olhs(0, 16)
            early = [(oc, wo[j, 0:hk, :]) for j in range(8)]
        else:
            a11, a21 = olhs(0, 16), ob[:, 0:hk]
            l3, l6 = a11.astype(bf16), (a21 - a11).astype(bf16)
            early = [(l3, wc(1, jj)) for jj in range(4)] + [(l6, wc(3, jj)) for jj in range(4)]
        for j in range(8):
            acc.append(-_dot(*early[j]))
            if j >= 0:
                for _ in range(ab):
                    if rem:
                        pv(rem.pop(0))
        if u < U - 1:
            oc = olhs(16, 32)
            for j in range(8):
                put(j, _dot(oc, wo[j, hk:2 * hk, :]) - acc[j], None)
        else:
            a12, a22 = olhs(16, 32), ob[:, hk:2 * hk]
            l1, l2, l4 = (a11 + a22).astype(bf16), (a21 + a22).astype(bf16), a22.astype(bf16)
            l5, l7 = (a11 + a12).astype(bf16), (a12 - a22).astype(bf16)
            for jj in range(4):
                m1 = _dot(l1, wc(0, jj))
                m2 = _dot(l2, wo[jj, 0:hk, :])
                m4 = _dot(l4, wc(2, jj))
                m5 = _dot(l5, wo[4 + jj, hk:2 * hk, :])
                m7 = _dot(l7, wc(4, jj))
                put(jj, (m1 - m5) + (m4 + m7), m2 + m4)
                put(4 + jj, m5 - acc[jj], (m1 - m2) - acc[jj] - acc[4 + jj])

    def out_copy(it):
        return pltpu.make_async_copy(oa.at[pl.ds(it * 2, 2)],
                                     out_hbm.at[pl.ds(it * 2, 2), :, :, pl.ds(0, DM)], sems.at[32])

    def group(it, c):
        with jax.named_scope("grp"):
            for u in range(U):
                step(it, u)
        out_copy(it).start()
        return c
    lax.fori_loop(0, NSEG // U, group, 0)
    with jax.named_scope("w_out"):
        for it in range(NSEG // U):
            out_copy(it).wait()
        cp_outb.wait()


def pallas_concat_heads__memory_aug_recurrent_mem_tr__spectral_gfnet__prompt_kernel(
    A_x, A_mem0, A_Wq, A_Wk, A_Wv, A_Wo, A_seg_len, B_x, B_w_r, B_w_i,
):
    del A_seg_len
    R, LN, TW, fill, KC = _tables()
    small = np.zeros((208, 128), np.float32)
    small[:80, :80] = fill
    small[80:112] = TW
    small[112:] = np.repeat(KC, 8, axis=0)
    hbm = pl.BlockSpec(memory_space=pl.ANY)
    out = pl.pallas_call(
        _kernel,
        out_shape=jax.ShapeDtypeStruct((RS, 8, 8, DM + D), bf16),
        in_specs=[hbm] * 12,
        out_specs=hbm,
        scratch_shapes=[
            pltpu.VMEM((NSEG, 3, 8, DM), bf16),
            pltpu.VMEM((NSEG, 8, DM), bf16),
            pltpu.VMEM((4, 64, DM), u32),
            pltpu.VMEM((DM // 128, H * DH, 128), bf16),
            pltpu.VMEM((BC + 10, DM // 2, 8, DH), bf16),
            pltpu.VMEM((NCH + 1, 16 * PW, DH), u32),
            pltpu.VMEM((M, DM), bf16),
            pltpu.VMEM((U * M, H * DH), f32),
            pltpu.VMEM((RS, 8, 8, DM), bf16),
            pltpu.VMEM((RS, 8, 8, D), bf16),
            pltpu.VMEM((D // 2 + 1, S), bf16),
            pltpu.VMEM((D // 2 + 1, S), bf16),
            pltpu.VMEM((16, 64, 128), u32),
            pltpu.VMEM((2 * RS + 5, 64, 128), u32),
            pltpu.VMEM((208, 128), f32),
            pltpu.VMEM((RS, 4, 8, 16, 128), bf16),
            pltpu.VMEM((4, RS, TP, 128), f32),
            pltpu.VMEM((2, 2, BS * WP, 128), u32),
            pltpu.VMEM((32, 128), f32),
            pltpu.SemaphoreType.DMA((46,)),
        ],
        compiler_params=pltpu.CompilerParams(vmem_limit_bytes=124 * 1024 * 1024,
                                             disable_bounds_checks=True, disable_semaphore_checks=True),
    )(A_x.reshape(NSEG, 4, 8, DM), A_mem0.reshape(M, DM),
      A_Wq.reshape(2, DM // 2, H, DH), A_Wk.reshape(2, DM // 2, H, DH), A_Wv.reshape(2, DM // 2, H, DH),
      A_Wo.reshape(H * DH, DM), B_x.reshape(RS, 8, 8, D), B_w_r.T, B_w_i.T,
      jnp.asarray(R), jnp.asarray(LN), jnp.asarray(small))
    return out.reshape(1, S, DM + D)
```

```python
import functools
import math

import jax
import jax.numpy as jnp
import numpy as np
from jax import lax
import jax.experimental.pallas as pl
import jax.experimental.pallas.tpu as pltpu

bf16, f32, u32, i32 = jnp.bfloat16, jnp.float32, jnp.uint32, jnp.int32

S, DM, H, DH, M, SEG = 2048, 1024, 32, 128, 8, 32
NSEG = S // SEG
FR = SEG - M
G = H // 2
U = 4
NCH = 12
NST = 4
PW = 264

D = 1024
RS, BS = 32, 64
HR = RS // 2
WP = 40
TP = 136
C8 = float(np.sqrt(0.5))


def _pack_rows(a):
    u = np.asarray(a, np.float32).astype(jnp.bfloat16).view(np.uint16).astype(np.uint32)
    return u[..., 0::2, :] | (u[..., 1::2, :] << 16)


_RHO = (2, 4, 4, 4)


def _in_a(lane, c):
    return (lane % 4 < 2) if c == 0 else ((lane + 2) % 8 < 4)


def _dstage(x, kc, roll64):
    a = [x[j] + x[j + 4] for j in range(4)]
    b = [x[j] - x[j + 4] for j in range(4)]
    t1 = (b[1] - b[3]) * C8
    t2 = (b[1] + b[3]) * C8
    s0, s1 = a[0] + a[2], a[1] + a[3]
    out = [s0 + s1, s0 - s1]
    for c, (u, v) in enumerate(((b[0] + t1, b[2] + t2), (a[0] - a[2], a[1] - a[3]), (b[0] - t1, b[2] - t2))):
        g = u * kc[4 * c] + v * kc[4 * c + 1]
        h = roll64(u * kc[4 * c + 2] + v * kc[4 * c + 3])
        out += [g + h, g - h]
    return out


def _dstage_t(p, kc, roll64):
    uv = []
    for c in range(3):
        g = p[2 + 2 * c] + p[3 + 2 * c]
        h = roll64(p[2 + 2 * c] - p[3 + 2 * c])
        uv.append((g * kc[4 * c] + h * kc[4 * c + 2], g * kc[4 * c + 1] + h * kc[4 * c + 3]))
    s0, s1 = p[0] + p[1], p[0] - p[1]
    a = [s0 + uv[1][0], s1 + uv[1][1], s0 - uv[1][0], s1 - uv[1][1]]
    t1 = (uv[0][0] - uv[2][0]) * C8
    t2 = (uv[0][1] - uv[2][1]) * C8
    b = [uv[0][0] + uv[2][0], t1 + t2, uv[0][1] + uv[2][1], t2 - t1]
    return [a[j] + b[j] for j in range(4)] + [a[j] - b[j] for j in range(4)]


@functools.lru_cache(maxsize=None)
def _tables():
    kcol = np.zeros((4, 128), np.int64)
    for l in range(128):
        i0, i1 = l, 128 + (l ^ 1)
        ev, o3 = l % 2 == 0, l % 4 in (0, 3)
        kcol[0, l] = 2 * (i0 if ev else i1)
        kcol[2, l] = 2 * (i1 if ev else i0)
        kcol[1, l] = 2 * (i0 if o3 else i1) + 1
        kcol[3, l] = 2 * (i1 if o3 else i0) + 1
    lanes = np.arange(128)
    lo = lanes < 64
    KC = np.zeros((12, 128))
    for c, sg in ((1, -1.0), (2, -1.0), (3, 1.0)):
        tr, ti = np.cos(2 * np.pi * c / 16), -np.sin(2 * np.pi * c / 16)
        KC[4 * c - 4] = np.where(lo, 1.0, ti)
        KC[4 * c - 3] = sg * np.where(lo, 0.0, tr)
        KC[4 * c - 2] = np.where(lo, 0.0, tr)
        KC[4 * c - 1] = sg * np.where(lo, 1.0, -ti)
    eye = np.eye(D)
    Bt = _dstage([eye[:, 128 * e:128 * (e + 1)] for e in range(8)], KC, lambda v: np.roll(v, 64, axis=1))
    d = np.arange(D)
    R = np.zeros((16, 128, 128))
    for c in range(4):
        rho = _RHO[c]
        inA = _in_a(lanes, c)
        ang = 2 * np.pi * (np.outer(d, kcol[c]) % D) / D
        fr, fi = np.cos(ang), -np.sin(ang)
        wr_, wi_ = np.full(128, 2.0), np.full(128, 2.0)
        if c == 0:
            fi[:, 0] = (-1.0) ** d
            wr_[0] = 1.0
            wi_[0] = 1.0
        fi, wi_ = np.roll(fi, -rho, axis=1), np.roll(wi_, -rho)
        for h in range(2):
            own = inA if h == 0 else ~inA
            ft, wt = np.where(own, fr, fi), np.where(own, wr_, wi_)
            bt = Bt[2 * c + h]
            r = (bt.T @ ft) / (bt * bt).sum(axis=0)[:, None]
            assert np.abs(bt @ r - ft).max() < 1e-9
            R[2 * c + h] = r
            R[8 + 2 * c + h] = (wt[:, None] * r.T) / (S * D)
    L = np.zeros((2 * RS, 128, 128))
    bb = np.arange(BS)
    kord = np.array([ri * 64 + 8 * t + r for t in range(8) for ri in range(2) for r in range(8)])
    for p1 in range(RS):
        ang = 2 * np.pi * (np.outer(p1 + RS * bb, bb) % S) / S
        mr, mi = np.cos(ang), -np.sin(ang)
        full = np.block([[mr, -mi], [mi, mr]])
        L[p1] = full[:, kord]
        L[RS + p1] = full.T
    l_, q_ = np.arange(128), np.arange(16)
    ang = 2 * np.pi * (np.outer(l_, l_) % 128) / 128
    N1 = np.concatenate([np.cos(ang), -np.sin(ang)], axis=1)
    N1 = np.concatenate([(N1[:64] + N1[64:]) / 2, (N1[:64] - N1[64:]) / 2], axis=0)
    ang = 2 * np.pi * np.outer(q_, l_) / S
    TW = np.concatenate([np.cos(ang), -np.sin(ang)], axis=0)
    ang = 2 * np.pi * (np.outer(q_, q_) % 16) / 16
    fr, fi = np.cos(ang), -np.sin(ang)
    F16 = np.block([[fr, -fi], [fi, fr]])
    NY = np.zeros((5, 128, 128))
    NY[0], NY[1], NY[2], NY[3] = N1[:, :128], N1[:, 128:], N1[:, :128].T, N1[:, 128:].T
    NY[4, :32, :32] = F16
    NY[4, 32:64, :32] = F16.T
    LN = np.concatenate([L, NY], axis=0)
    head = np.zeros(80, np.int32)
    pos = np.zeros(80, np.int32)
    for r in range(80):
        if r < 64:
            head[r] = r // 32
            t = r % 32
            pos[r] = (M + t) if t < FR else (t - FR)
        else:
            head[r] = (r - 64) // 8
            pos[r] = M + FR + (r - 64) % 8
    same = head[:, None] == head[None, :]
    vis = (pos[:, None] < M) | (pos[:, None] >= pos[None, :])
    fill = np.where(same, np.where(vis, 0.0, -1e9), -np.inf).astype(np.float32)
    return _pack_rows(R), _pack_rows(LN), TW.astype(np.float32), fill, KC.astype(np.float32)


def _cmul_const(re, im, j, n, sgn):
    ang = sgn * 2 * math.pi * j / n
    c, s = math.cos(ang), math.sin(ang)
    if abs(abs(c) - abs(s)) < 1e-12:
        if c * s > 0:
            return (re - im) * c, (re + im) * c
        return (re + im) * c, (im - re) * c
    return re * c - im * s, re * s + im * c


def _diff_tw(a, b, j, n, sgn):
    if j == 0:
        return a[0] - b[0], a[1] - b[1]
    if 4 * j == n:
        if sgn < 0:
            return a[1] - b[1], b[0] - a[0]
        return b[1] - a[1], a[0] - b[0]
    return _cmul_const(a[0] - b[0], a[1] - b[1], j, n, sgn)


def _tw(v, j, sgn):
    if j == 0:
        return v
    if 4 * j == RS:
        return (v[1], -v[0]) if sgn < 0 else (-v[1], v[0])
    return _cmul_const(v[0], v[1], j, RS, sgn)


def _fft(v, sgn):
    n = len(v)
    if n == 1:
        return v
    h = n // 2
    ev = _fft([(v[j][0] + v[j + h][0], v[j][1] + v[j + h][1]) for j in range(h)], sgn)
    od = _fft([_diff_tw(v[j], v[j + h], j, n, sgn) for j in range(h)], sgn)
    out = [None] * n
    out[0::2] = ev
    out[1::2] = od
    return out


def _dot(a, b):
    return jnp.dot(a, b, preferred_element_type=f32)


def _asbf(v):
    return pltpu.bitcast(v, bf16)


def _cm(ar, ai, br, bi):
    return ar * br - ai * bi, ar * bi + ai * br


CHUNKS = [(0, 0), (0, 1), (0, 2), (0, 3), (1, 0), (1, 1), (1, 2), (2, 0), (2, 1), (2, 2), (2, 3), (1, 3)]
BU = 2 * NST + NCH
BC = BU + 2


NK0 = 88


def _kernel(ax_hbm, mem_hbm, wq_hbm, wk_hbm, wv_hbm, wo_hbm, bx_hbm, wr_hbm, wi_hbm,
            R_hbm, L_hbm, sm_hbm, out_hbm,
            ax, xb3, xb, wo, pool, wpk, memb, ob, oa,
            bx, wr, wi, R, L, sm, Y, T, wp, nv, sems):
    srcs = (wq_hbm, wk_hbm, wv_hbm)
    lane8 = lax.broadcasted_iota(i32, (8, 128), 1)

    def chunk_copy(t):
        m, c = CHUNKS[t]
        return pltpu.make_async_copy(srcs[m].at[:, :, pl.ds(8 * c, 8), :],
                                     pool.at[pl.ds(2 * (t % NST), 2)], sems.at[t % NST])

    def part0_copy(part):
        rows = pl.ds(pl.multiple_of(part * 128, 128), 128)
        return pltpu.make_async_copy(wq_hbm.at[:, rows, pl.ds(0, 8), :], pool.at[pl.ds(0, 2), rows], sems.at[34 + part])

    def part_start(t, part):
        lo = part * 2 * NK0
        n = min(2 * NK0, 512 - lo)
        pltpu.make_async_copy(wq_hbm.at[:, pl.ds(lo, n), pl.ds(8 * t, 8), :],
                              pool.at[pl.ds(2 * t, 2), pl.ds(lo, n)], sems.at[35 + 3 * t + part]).start()

    def part_wait(t, part):
        for p in range(3):
            lo = p * 2 * NK0
            n = min(2 * NK0, 512 - lo)

            @pl.when(part == p)
            def _(lo=lo, n=n, p=p):
                blk = pool.at[pl.ds(2 * t, 2), pl.ds(lo, n)]
                pltpu.make_async_copy(blk, blk, sems.at[35 + 3 * t + p]).wait()

    def chunk_start(t):
        sl = t & (NST - 1)
        pltpu.make_async_copy(wv_hbm.at[:, :, pl.ds(pl.multiple_of(8 * (t - 7), 8), 8), :],
                              pool.at[pl.ds(2 * sl, 2)], sems.at[sl]).start()

    def chunk_wait(t):
        sl = t & (NST - 1)
        blk = pool.at[pl.ds(2 * sl, 2)]
        pltpu.make_async_copy(blk, blk, sems.at[sl]).wait()

    def xb_copy(q):
        return pltpu.make_async_copy(ax_hbm.at[pl.ds(16 * q, 16), 3], xb3.at[pl.ds(16 * q, 16)], sems.at[8 + q])

    def bx_copy(q):
        return pltpu.make_async_copy(bx_hbm.at[:, pl.ds(2 * q, 2)], bx.at[:, pl.ds(2 * q, 2)], sems.at[12 + q])

    def w_copy(q, i):
        cols = pl.ds(pl.multiple_of(512 * q, 512), 512)
        return pltpu.make_async_copy((wr_hbm, wi_hbm)[i].at[:, cols], (wr, wi)[i].at[:, cols], sems.at[16 + 4 * i + q])

    def wo_copy(q, hi):
        j = q + 4 * hi
        return pltpu.make_async_copy(wo_hbm.at[:, pl.ds(pl.multiple_of(128 * j, 128), 128)], wo.at[j],
                                     sems.at[44 + q])

    cp_r0 = pltpu.make_async_copy(R_hbm.at[pl.ds(0, 8)], R.at[pl.ds(0, 8)], sems.at[25])
    cp_r1 = pltpu.make_async_copy(R_hbm.at[pl.ds(8, 8)], R.at[pl.ds(8, 8)], sems.at[26])
    cp_l = pltpu.make_async_copy(L_hbm, L, sems.at[27])
    cp_ax = pltpu.make_async_copy(ax_hbm.at[:, pl.ds(0, 3)], ax, sems.at[28])
    cp_outb = pltpu.make_async_copy(bx, out_hbm.at[:, :, :, pl.ds(DM, D)], sems.at[29])
    cp_sm = pltpu.make_async_copy(sm_hbm, sm, sems.at[30])
    cp_mem = pltpu.make_async_copy(mem_hbm, memb, sems.at[31])

    for part in range(4):
        part0_copy(part).start()
    xb_copy(0).start()
    for p in range(3):
        xb_copy(p + 1).start()
        part_start(1, p)
    for p in range(3):
        part_start(2, p)
    chunk_copy(3).start()
    cp_r0.start()
    bx_copy(0).start()
    w_copy(0, 0).start()
    w_copy(0, 1).start()
    cp_sm.start()
    cp_mem.start()

    def kc(rep=2):
        return [jnp.concatenate([sm[112 + 8 * i:120 + 8 * i, :]] * rep, axis=0) for i in range(12)]

    def roll64(v):
        return pltpu.roll(v, 64, 1)

    def prep(t, tpar, jj):
        lo = [bx[2 * jj:2 * jj + 2, t, :, 128 * e:128 * (e + 1)].astype(f32).reshape(16, 128) for e in range(8)]
        hi = [bx[HR + 2 * jj:HR + 2 * jj + 2, t, :, 128 * e:128 * (e + 1)].astype(f32).reshape(16, 128)
              for e in range(8)]
        for par in range(2):
            x = [lo[e] + hi[e] if par == 0 else lo[e] - hi[e] for e in range(8)]
            uu = _dstage(x, kc(), roll64)
            for q in range(8):
                o = (((tpar * 2 + par) * 8 + q) * 8 + jj) * 2
                pool[BU, o:o + 2] = uu[q].reshape(2, 8, 128).astype(bf16)

    def unit1(t, tpar, par, cg):
        o = ((tpar * 2 + par) * 8 + 2 * cg) * 16
        za = _dot(pool[BU, o:o + 16].reshape(128, 128), _asbf(R[2 * cg]))
        zb = _dot(pool[BU, o + 16:o + 32].reshape(128, 128), _asbf(R[2 * cg + 1]))
        ina = _in_a(lane8, cg)
        v = []
        for j in range(HR):
            pa, pb = za[8 * j:8 * j + 8], zb[8 * j:8 * j + 8]
            v.append((jnp.where(ina, pa, pb), pltpu.roll(jnp.where(ina, pb, pa), _RHO[cg], 1)))
        if cg == 0:
            V = nv[8 * tpar:8 * tpar + 8, :]
            for j in range(HR):
                vb = jnp.broadcast_to(v[j][1][:, 0:1], (8, 128))
                V = jnp.where(lane8 == 64 * par + 4 * j + (t >> 1), vb, V)
                v[j] = (v[j][0], jnp.where(lane8 == 0, 0.0, v[j][1]))
            nv[8 * tpar:8 * tpar + 8, :] = V
        if par == 1:
            v = [_tw(v[j], j, -1) for j in range(HR)]
        o = _fft(v, -1)
        for m in range(HR):
            Y[2 * m + par, cg, t] = jnp.concatenate(o[m], axis=0).astype(bf16)

    def wprep(pb, i):
        w = (wr, wi)[i]
        cols = pl.ds(pl.multiple_of(pb * 128, 128), 128)
        sub = lax.broadcasted_iota(i32, (8, 128), 0)
        msk = (jnp.where(sub % 2 == 0, jnp.uint32(0xffff), jnp.uint32(0))
               | jnp.where((sub % 4 == 0) | (sub % 4 == 3), jnp.uint32(0xffff0000), jnp.uint32(0)))
        t0 = pltpu.bitcast(w[0:256, cols], u32)
        t1 = pltpu.bitcast(w[256:512, cols], u32)
        ps, qs = [], []
        for j in range(16):
            a = t0[8 * j:8 * j + 8]
            b = t1[8 * j:8 * j + 8]
            b = jnp.where(sub % 2 == 0, pltpu.roll(b, 7, 0), pltpu.roll(b, 1, 0))
            x = (a ^ b) & msk
            ps.append(b ^ x)
            qs.append(a ^ x)
        for h, lst in enumerate((ps, qs)):
            tr = pltpu.bitcast(pltpu.bitcast(jnp.concatenate(lst, axis=0), f32).T, u32)
            for q in range(4):
                wp[i, h, pl.ds(pl.multiple_of((pb * 4 + q) * WP, 8), 32), :] = tr[32 * q:32 * q + 32]

    def fwd(p):
        return _dot(_asbf(L[p]), jnp.concatenate([Y[p, cg].reshape(128, 128) for cg in range(4)], axis=1))

    def filt(pbase, po, v):
        grs, gis = [None] * 4, [None] * 4
        win = pl.ds(pbase, (BS - 1) * WP + 8)
        for h in range(2):
            wr_ = wp.at[0, h, win][pl.ds(po, BS, stride=WP), :]
            wi_ = wp.at[1, h, win][pl.ds(po, BS, stride=WP), :]
            for hi in range(2):
                cg = 2 * h + hi
                if hi == 0:
                    a, b = wr_ << 16, wi_ << 16
                else:
                    a, b = wr_ & jnp.uint32(0xffff0000), wi_ & jnp.uint32(0xffff0000)
                grs[cg], gis[cg] = _cm(v[:BS, 128 * cg:128 * (cg + 1)], v[BS:, 128 * cg:128 * (cg + 1)],
                                       pltpu.bitcast(a, f32), pltpu.bitcast(b, f32))
        return jnp.concatenate([jnp.concatenate(grs, axis=1), jnp.concatenate(gis, axis=1)], axis=0).astype(bf16)

    def inv(p, g):
        t = _dot(_asbf(L[RS + p]), g)
        for cg in range(4):
            T[cg, p, 0:128, :] = t[:, 128 * cg:128 * (cg + 1)]

    nyq = {}

    def nyq_stage(k):
        n0 = 2 * RS
        twr, twi = sm[80:96, :], sm[96:112, :]
        if k == 0:
            v = nv[0:16, :].astype(bf16)
            r, i = _cm(_dot(v, _asbf(L[n0])), _dot(v, _asbf(L[n0 + 1])), twr, twi)
            nyq[0] = jnp.concatenate([r, i], axis=0).astype(bf16)
        elif k == 1:
            t = _dot(_asbf(L[n0 + 4, 0:16])[:, 0:32], nyq[0])
            ws = []
            for w in (wr, wi):
                row = w[512:513, :].astype(f32)
                ws.append(jnp.concatenate([row[:, 128 * r:128 * (r + 1)] for r in range(16)], axis=0))
            r, i = _cm(t[:16], t[16:], ws[0], ws[1])
            nyq[1] = jnp.concatenate([r, i], axis=0).astype(bf16)
        elif k == 2:
            t = _dot(_asbf(L[n0 + 4, 16:32])[:, 0:32], nyq[1])
            r, i = _cm(t[:16], t[16:], twr, -twi)
            nyq[2] = (r.astype(bf16), i.astype(bf16))
        elif k == 3:
            nv[16:32, :] = _dot(nyq[2][0], _asbf(L[n0 + 2])) + _dot(nyq[2][1], _asbf(L[n0 + 3]))

    def p3a(t, tpar, par, cg):
        rr = pl.ds(pl.multiple_of(t * 8, 8), 8)
        ri = pl.ds(pl.multiple_of(64 + t * 8, 8), 8)
        o = _fft([(T[cg, 2 * m + par, rr, :], T[cg, 2 * m + par, ri, :]) for m in range(HR)], +1)
        if par == 1:
            o = [_tw(o[j], j, +1) for j in range(HR)]
        if cg == 0:
            un = nv[16 + 8 * tpar:24 + 8 * tpar, :]
            o = [(o[j][0], jnp.where(lane8 == 0, pltpu.roll(un, (128 - 64 * par - 4 * j - (t >> 1)) & 127, 1),
                                     o[j][1])) for j in range(HR)]
        ina = _in_a(lane8, cg)
        ua, ub = [], []
        for re, im in o:
            im = pltpu.roll(im, 128 - _RHO[cg], 1)
            ua.append(jnp.where(ina, re, im))
            ub.append(jnp.where(ina, im, re))
        for j in range(HR // 2):
            for h, x in enumerate((ua, ub)):
                o = ((tpar * 2 + par) * 8 + 2 * cg + h) * 16 + 2 * j
                pool[BU + 1, o:o + 2] = jnp.concatenate(x[2 * j:2 * j + 2], axis=0).reshape(2, 8, 128).astype(bf16)

    def p3b(tpar, par, cg):
        zs = []
        for h in range(2):
            o = ((tpar * 2 + par) * 8 + 2 * cg + h) * 16
            zs.append((o, _dot(pool[BU + 1, o:o + 16].reshape(128, 128), _asbf(R[8 + 2 * cg + h]))))
        return zs

    def p3s(zs):
        for o, z in zs:
            pool[BU, o:o + 16] = z.reshape(16, 8, 128).astype(bf16)

    def p3c(t, tpar, j):
        res = [_dstage_t([pool[BU, ((tpar * 2 + par) * 8 + q) * 16 + j].astype(f32) for q in range(8)],
                         kc(1), roll64) for par in range(2)]
        for e in range(8):
            cols = slice(128 * e, 128 * (e + 1))
            bx[j, t, :, cols] = (res[0][e] + res[1][e]).astype(bf16)
            bx[HR + j, t, :, cols] = (res[0][e] - res[1][e]).astype(bf16)

    def wsum(jj, hf, n):
        r0 = pl.multiple_of(hf * 1024, 1024)
        lo, hi = pl.ds(r0 + 16 * n, 16), pl.ds(r0 + 2048 + 16 * n, 16)
        b11, b21 = wo[jj, lo, :].astype(f32), wo[jj, hi, :].astype(f32)
        b12, b22 = wo[4 + jj, lo, :].astype(f32), wo[4 + jj, hi, :].astype(f32)
        for i, v in enumerate((b11 + b22, b12 - b22, b21 - b11, b11 + b12, b21 + b22)):
            pool[BC + 2 * i + (jj >> 1), pl.ds((jj & 1) * 256 + hf * 128 + 2 * n, 2)] = (
                v.reshape(2, 8, 128).astype(bf16))

    def wc(i, jj):
        return pool[BC + 2 * i + jj // 2, (jj % 2) * 256:(jj % 2 + 1) * 256].reshape(2048, 128)

    def runit(b0, d0, dst, k):
        a = pltpu.bitcast(jnp.concatenate([pool[b0, d0 + 2 * k], pool[b0 + 1, d0 + 2 * k]], axis=0), u32)
        b = pltpu.bitcast(jnp.concatenate([pool[b0, d0 + 2 * k + 1], pool[b0 + 1, d0 + 2 * k + 1]], axis=0), u32)
        dst[pl.ds(k, 8, stride=PW), :] = (a & jnp.uint32(0xffff)) | (b << 16)
        dst[pl.ds(8 * PW + k, 8, stride=PW), :] = (a >> 16) | (b & jnp.uint32(0xffff0000))

    def wsel(w, hl, lo=0, hi=DM):
        base = ((hl % 2) * 8 + hl // 2) * PW
        parts = []
        for kh in range(2):
            a, b = max(lo, 512 * kh), min(hi, 512 * (kh + 1))
            if a < b:
                o = base + 4 * PW * kh - 256 * kh
                parts.append(w[o + a // 2:o + b // 2, :])
        return _asbf(jnp.concatenate(parts, axis=0))

    def bulk(t, mc0, nmc, tsrc, tdst, k0, nk, side=None):
        w = wpk.at[t]
        b0 = 2 * (tsrc & (NST - 1))
        dst = wpk.at[tdst, pl.ds(k0, 15 * PW + nk)]
        bq = 2 * NST + (t & 31)
        ns = 8 * nmc
        per = nk // ns
        for mi in range(nmc):
            mc = mc0 + mi
            x = _asbf(xb[mc])
            for h in range(8):
                n = mi * 8 + h
                r = _dot(x, wsel(w, h)).reshape(16, M, DH)
                nn = (n - 1) % ns
                for k in range(per * nn, per * (nn + 1)):
                    runit(b0, 2 * k0, dst, k)
                if side is not None:
                    side(n)
                rb = r.astype(bf16)
                for gi in range(4):
                    pool[bq, pl.ds(mc * 128 + gi * 32 + h * 4, 4)] = rb[4 * gi:4 * gi + 4]

    def rel0(i, c):
        @pl.when(i % 2 == 0)
        def _():
            part0_copy(i >> 1).wait()
        dst = wpk.at[0, pl.ds(pl.multiple_of(i * 32, 32), 15 * PW + 32)]
        for k in range(32):
            runit(0, i * 64, dst, k)
        return c
    with jax.named_scope("rel0"):
        lax.fori_loop(0, 8, rel0, 0)

    def body0(i, c):
        t, mc = i >> 2, i & 3
        real = mc >= 1

        @pl.when(t == 0)
        def _():
            xb_copy(mc).wait()
            xb[mc] = pltpu.bitcast(xb3[pl.ds(16 * mc, 16)].reshape(128, DM), u32)

        @pl.when(real)
        def _():
            part_wait(t + 1, mc - 1)
        with jax.named_scope("bulk0"):
            bulk(t, mc, 1, jnp.where(real, t + 1, t), jnp.where(real, t + 1, NCH),
                 pl.multiple_of(jnp.clip((mc - 1) * NK0, 0, 256 - NK0), 8), NK0)

        @pl.when(i == 0)
        def _():
            chunk_copy(4).start()
            bx_copy(1).start()
            w_copy(1, 0).start()
            w_copy(1, 1).start()

        @pl.when(i == 4)
        def _():
            chunk_copy(5).start()
        return c
    lax.fori_loop(0, 8, body0, 0)
    bx_copy(2).start()
    w_copy(2, 0).start()
    w_copy(2, 1).start()
    chunk_copy(6).start()
    bx_copy(3).start()
    w_copy(3, 0).start()
    w_copy(3, 1).start()
    cp_l.start()
    cp_r1.start()
    nv[0:16, :] = jnp.zeros((16, 128), f32)
    cp_r0.wait()
    cp_sm.wait()

    def body1(q, c):
        t = q + 2
        with jax.named_scope("w_1"):
            chunk_wait(t + 1)
            bx_copy(q).wait()
            w_copy(q, 0).wait()
            w_copy(q, 1).wait()

        def side(n):
            for k in ([0, 1] if n == 0 else [n + 1]):
                if k < 16:
                    prep(2 * q + k // 8, k // 8, k % 8)
            k = n - 15
            if 0 <= k < 16:
                unit1(2 * q + k // 8, k // 8, (k // 4) % 2, k % 4)
            k, r = divmod(n - 1, 2)
            if r == 0 and 0 <= k < 8:
                wprep(4 * q + k // 2, k % 2)
        with jax.named_scope("bulk_p1"):
            bulk(t, 0, 4, t + 1, t + 1, 0, 256, side)
        wo_copy(q, 0).start()
        wo_copy(q, 1).start()
        chunk_start(t + 1 + NST)
        return c
    lax.fori_loop(0, 4, body1, 0)

    cp_ax.start()
    with jax.named_scope("w_l"):
        cp_l.wait()
        cp_r1.wait()

    def body2(q, c):
        t, hf = (q >> 1) + 6, q & 1

        @pl.when(hf == 0)
        def _():
            with jax.named_scope("w_2"):
                chunk_wait(t + 1)
                wo_copy(q >> 1, 0).wait()
                wo_copy(q >> 1, 1).wait()
        gs = {}
        fs = [0, 1, 3, 5, 7, 9, 11, 13]

        def side(n):
            if n - 2 in fs:
                po = fs.index(n - 2)
                inv(8 * q + po, gs.pop(po))
            if n in fs:
                po = fs.index(n)
                gs[po] = filt(pl.multiple_of(8 * q, 8), po, fwd(8 * q + po))
            k, r = divmod(n - 1, 3)
            if r == 0 and 0 <= k < 4:
                nyq_stage(k)
            for hh in range(4):
                wsum(q >> 1, hf, 4 * n + hh)
        with jax.named_scope("bulk_p2"):
            bulk(t, 2 * hf, 2, t + 1, t + 1, pl.multiple_of(hf * 128, 128), 128, side)
        return c
    lax.fori_loop(0, 4, body2, 0)
    chunk_copy(11).start()
    for j in (2, 3):
        wo_copy(j, 0).wait()
        wo_copy(j, 1).wait()

    def body3(q, c):
        t = q + 8

        @pl.when(q < 3)
        def _():
            with jax.named_scope("w_3"):
                chunk_wait(t + 1)
        us = {}

        def side(n):
            if n < 16:
                p3a(2 * q + n // 8, n // 8, (n // 4) % 2, n % 4)
            k = n - 3
            if 0 <= k < 16:
                us[k] = p3b(k // 8, (k // 4) % 2, k % 4)
            k = n - 3 - 1
            if 0 <= k < 16:
                p3s(us.pop(k))
            k = n - 16
            if 0 <= k < 16:
                p3c(2 * q + k // 8, k // 8, 2 * (k % 8))
                p3c(2 * q + k // 8, k // 8, 2 * (k % 8) + 1)
            for hh in range(2):
                wsum(2 + (q >> 1), q & 1, 2 * n + hh)
        with jax.named_scope("bulk_p3"):
            bulk(t, 0, 4, t + 1, t + 1, 0, 256, side)
        return c
    lax.fori_loop(0, 4, body3, 0)
    cp_outb.start()

    with jax.named_scope("w_wo"):
        cp_ax.wait()
        cp_mem.wait()
    scale = DH ** -0.5
    KS = 640

    def step(it, u):
        s = it * U + u
        lhs = jnp.concatenate([ax[s].reshape(FR, DM), memb[...]], axis=0)
        qs, ks, vs, ps, os_, pre = {}, {}, {}, {}, {}, {}

        def ws(m, h, lo=0, hi=DM):
            return wsel(wpk.at[CHUNKS.index((m, h // 8))], h % 8, lo, hi)
        if u > 0:
            for m in range(2):
                for h in range(2):
                    pre[(m, h)] = -_dot(lhs[:, :KS], ws(m, h, 0, KS))

        def dotw(m, h):
            if (m, h) in pre:
                return _dot(lhs[:, KS:], ws(m, h, KS, DM)) - pre[(m, h)]
            return _dot(lhs, ws(m, h))

        def proj(m, g):
            h = 2 * g
            bq = 2 * NST + CHUNKS.index((m, h // 8))
            return jnp.concatenate([dotw(m, h), dotw(m, h + 1),
                                    pool[bq, it * 32 + (h % 8) * 4 + u].astype(f32),
                                    pool[bq, it * 32 + (h % 8 + 1) * 4 + u].astype(f32)], axis=0).astype(bf16)

        def qk(g):
            sc = lax.dot_general(qs.pop(g), ks.pop(g), (((1,), (1,)), ((), ())),
                                 preferred_element_type=f32) * scale
            fill = sm[0:80, 0:80]
            sc = jnp.where(fill == 0.0, sc, fill)
            mx = jnp.max(sc, axis=-1, keepdims=True)
            e = jnp.exp(sc - mx)
            l = jnp.sum(e, axis=-1, keepdims=True)
            r = pl.reciprocal(l, approx=True)
            r = r * (2.0 - l * r)
            ps[g] = (e * r).astype(bf16)

        def pv(g):
            o = _dot(ps.pop(g), vs.pop(g))
            os_[2 * g] = o[0:32]
            os_[2 * g + 1] = o[32:64]
            ob[8 * u:8 * u + 8, (2 * g) * DH:(2 * g + 1) * DH] = o[64:72]
            ob[8 * u:8 * u + 8, (2 * g + 1) * DH:(2 * g + 2) * DH] = o[72:80]

        def olhs(lo, hi):
            return jnp.concatenate([os_[h] for h in range(lo, hi)], axis=1)

        def put(j, r, rb):
            cols = slice(j * 128, (j + 1) * 128)
            oa[it * 2 + u // 2, pl.ds((u % 2) * 4, 3), :, cols] = r[0:FR].reshape(3, 8, 128).astype(bf16)
            memb[:, cols] = r[FR:SEG].astype(bf16)
            if rb is not None:
                for uu in range(U):
                    oa[it * 2 + uu // 2, (uu % 2) * 4 + 3, :, cols] = rb[8 * uu:8 * uu + 8].astype(bf16)

        sk, dq, dp = 7, 3, 5
        for t in range(G + sk):
            if t < G:
                qs[t] = proj(0, t)
            if 0 <= t - dq < G:
                qk(t - dq)
            if t < G:
                ks[t] = proj(1, t)
            if t - sk - dp >= 0:
                pv(t - sk - dp)
            if t - sk >= 0:
                vs[t - sk] = proj(2, t - sk)
        rem = list(range(G - dp, G))
        hk = 16 * DH
        acc = []
        if u < U - 1:
            oc = olhs(0, 16).astype(bf16)
            early = [(oc, wo[j, 0:hk, :]) for j in range(8)]
        else:
            a11, a21 = olhs(0, 16), ob[:, 0:hk]
            l3, l6 = a11.astype(bf16), (a21 - a11).astype(bf16)
            early = [(l3, wc(1, jj)) for jj in range(4)] + [(l6, wc(3, jj)) for jj in range(4)]
        for j in range(8):
            acc.append(-_dot(*early[j]))
            if rem:
                pv(rem.pop(0))
        if u < U - 1:
            oc = olhs(16, 32).astype(bf16)
            for j in range(8):
                put(j, _dot(oc, wo[j, hk:2 * hk, :]) - acc[j], None)
        else:
            a12, a22 = olhs(16, 32), ob[:, hk:2 * hk]
            l1, l2, l4 = (a11 + a22).astype(bf16), (a21 + a22).astype(bf16), a22.astype(bf16)
            l5, l7 = (a11 + a12).astype(bf16), (a12 - a22).astype(bf16)
            for jj in range(4):
                m1 = _dot(l1, wc(0, jj))
                m2 = _dot(l2, wo[jj, 0:hk, :])
                m4 = _dot(l4, wc(2, jj))
                m5 = _dot(l5, wo[4 + jj, hk:2 * hk, :])
                m7 = _dot(l7, wc(4, jj))
                put(jj, (m1 - m5) + (m4 + m7), m2 + m4)
                put(4 + jj, m5 - acc[jj], (m1 - m2) - acc[jj] - acc[4 + jj])

    def out_copy(it):
        return pltpu.make_async_copy(oa.at[pl.ds(it * 2, 2)],
                                     out_hbm.at[pl.ds(it * 2, 2), :, :, pl.ds(0, DM)], sems.at[32])

    def group(it, c):
        with jax.named_scope("grp"):
            for u in range(U):
                step(it, u)
        out_copy(it).start()
        return c
    lax.fori_loop(0, NSEG // U, group, 0)
    with jax.named_scope("w_out"):
        for it in range(NSEG // U):
            out_copy(it).wait()
        cp_outb.wait()


def pallas_concat_heads__memory_aug_recurrent_mem_tr__spectral_gfnet__prompt_kernel(
    A_x, A_mem0, A_Wq, A_Wk, A_Wv, A_Wo, A_seg_len, B_x, B_w_r, B_w_i,
):
    if isinstance(A_seg_len, int):
        assert A_seg_len == SEG
    R, LN, TW, fill, KC = _tables()
    small = np.zeros((208, 128), np.float32)
    small[:80, :80] = fill
    small[80:112] = TW
    small[112:] = np.repeat(KC, 8, axis=0)
    hbm = pl.BlockSpec(memory_space=pl.ANY)
    out = pl.pallas_call(
        _kernel,
        out_shape=jax.ShapeDtypeStruct((RS, 8, 8, DM + D), bf16),
        in_specs=[hbm] * 12,
        out_specs=hbm,
        scratch_shapes=[
            pltpu.VMEM((NSEG, 3, 8, DM), bf16),
            pltpu.VMEM((NSEG, 8, DM), bf16),
            pltpu.VMEM((4, 64, DM), u32),
            pltpu.VMEM((DM // 128, H * DH, 128), bf16),
            pltpu.VMEM((BC + 10, DM // 2, 8, DH), bf16),
            pltpu.VMEM((NCH + 1, 16 * PW, DH), u32),
            pltpu.VMEM((M, DM), bf16),
            pltpu.VMEM((U * M, H * DH), f32),
            pltpu.VMEM((RS, 8, 8, DM), bf16),
            pltpu.VMEM((RS, 8, 8, D), bf16),
            pltpu.VMEM((D // 2 + 1, S), bf16),
            pltpu.VMEM((D // 2 + 1, S), bf16),
            pltpu.VMEM((16, 64, 128), u32),
            pltpu.VMEM((2 * RS + 5, 64, 128), u32),
            pltpu.VMEM((208, 128), f32),
            pltpu.VMEM((RS, 4, 8, 16, 128), bf16),
            pltpu.VMEM((4, RS, TP, 128), f32),
            pltpu.VMEM((2, 2, BS * WP, 128), u32),
            pltpu.VMEM((32, 128), f32),
            pltpu.SemaphoreType.DMA((48,)),
        ],
        compiler_params=pltpu.CompilerParams(vmem_limit_bytes=124 * 1024 * 1024,
                                             disable_bounds_checks=True, disable_semaphore_checks=True),
    )(A_x.reshape(NSEG, 4, 8, DM), A_mem0.reshape(M, DM),
      A_Wq.reshape(2, DM // 2, H, DH), A_Wk.reshape(2, DM // 2, H, DH), A_Wv.reshape(2, DM // 2, H, DH),
      A_Wo.reshape(H * DH, DM), B_x.reshape(RS, 8, 8, D), B_w_r.T, B_w_i.T,
      jnp.asarray(R), jnp.asarray(LN), jnp.asarray(small))
    return out.reshape(1, S, DM + D)
```

```python
import functools
import math

import jax
import jax.numpy as jnp
import numpy as np
from jax import lax
import jax.experimental.pallas as pl
import jax.experimental.pallas.tpu as pltpu

bf16, f32, u32, i32 = jnp.bfloat16, jnp.float32, jnp.uint32, jnp.int32

S, DM, H, DH, M, SEG = 2048, 1024, 32, 128, 8, 32
NSEG = S // SEG
FR = SEG - M
G = H // 2
U = 4
NCH = 12
NST = 4
PW = 264

D = 1024
RS, BS = 32, 64
HR = RS // 2
TP = 136
C8 = float(np.sqrt(0.5))


def _pack_rows(a):
    u = np.asarray(a, np.float32).astype(jnp.bfloat16).view(np.uint16).astype(np.uint32)
    return u[..., 0::2, :] | (u[..., 1::2, :] << 16)


_RHO = (2, 4, 4, 4)


def _in_a(lane, c):
    return (lane % 4 < 2) if c == 0 else ((lane + 2) % 8 < 4)


def _dstage(x, kc, roll64):
    a = [x[j] + x[j + 4] for j in range(4)]
    b = [x[j] - x[j + 4] for j in range(4)]
    t1 = (b[1] - b[3]) * C8
    t2 = (b[1] + b[3]) * C8
    s0, s1 = a[0] + a[2], a[1] + a[3]
    out = [s0 + s1, s0 - s1]
    for c, (u, v) in enumerate(((b[0] + t1, b[2] + t2), (a[0] - a[2], a[1] - a[3]), (b[0] - t1, b[2] - t2))):
        g = u * kc[4 * c] + v * kc[4 * c + 1]
        h = roll64(u * kc[4 * c + 2] + v * kc[4 * c + 3])
        out += [g + h, g - h]
    return out


def _dstage_t(p, kc, roll64):
    uv = []
    for c in range(3):
        g = p[2 + 2 * c] + p[3 + 2 * c]
        h = roll64(p[2 + 2 * c] - p[3 + 2 * c])
        uv.append((g * kc[4 * c] + h * kc[4 * c + 2], g * kc[4 * c + 1] + h * kc[4 * c + 3]))
    s0, s1 = p[0] + p[1], p[0] - p[1]
    a = [s0 + uv[1][0], s1 + uv[1][1], s0 - uv[1][0], s1 - uv[1][1]]
    t1 = (uv[0][0] - uv[2][0]) * C8
    t2 = (uv[0][1] - uv[2][1]) * C8
    b = [uv[0][0] + uv[2][0], t1 + t2, uv[0][1] + uv[2][1], t2 - t1]
    return [a[j] + b[j] for j in range(4)] + [a[j] - b[j] for j in range(4)]


@functools.lru_cache(maxsize=None)
def _tables():
    kcol = np.zeros((4, 128), np.int64)
    for l in range(128):
        i0, i1 = l, 128 + (l ^ 1)
        ev, o3 = l % 2 == 0, l % 4 in (0, 3)
        kcol[0, l] = 2 * (i0 if ev else i1)
        kcol[2, l] = 2 * (i1 if ev else i0)
        kcol[1, l] = 2 * (i0 if o3 else i1) + 1
        kcol[3, l] = 2 * (i1 if o3 else i0) + 1
    lanes = np.arange(128)
    lo = lanes < 64
    KC = np.zeros((12, 128))
    for c, sg in ((1, -1.0), (2, -1.0), (3, 1.0)):
        tr, ti = np.cos(2 * np.pi * c / 16), -np.sin(2 * np.pi * c / 16)
        KC[4 * c - 4] = np.where(lo, 1.0, ti)
        KC[4 * c - 3] = sg * np.where(lo, 0.0, tr)
        KC[4 * c - 2] = np.where(lo, 0.0, tr)
        KC[4 * c - 1] = sg * np.where(lo, 1.0, -ti)
    eye = np.eye(D)
    Bt = _dstage([eye[:, 128 * e:128 * (e + 1)] for e in range(8)], KC, lambda v: np.roll(v, 64, axis=1))
    d = np.arange(D)
    R = np.zeros((16, 128, 128))
    for c in range(4):
        rho = _RHO[c]
        inA = _in_a(lanes, c)
        ang = 2 * np.pi * (np.outer(d, kcol[c]) % D) / D
        fr, fi = np.cos(ang), -np.sin(ang)
        wr_, wi_ = np.full(128, 2.0), np.full(128, 2.0)
        if c == 0:
            fi[:, 0] = (-1.0) ** d
            wr_[0] = 1.0
            wi_[0] = 1.0
        fi, wi_ = np.roll(fi, -rho, axis=1), np.roll(wi_, -rho)
        for h in range(2):
            own = inA if h == 0 else ~inA
            ft, wt = np.where(own, fr, fi), np.where(own, wr_, wi_)
            bt = Bt[2 * c + h]
            r = (bt.T @ ft) / (bt * bt).sum(axis=0)[:, None]
            assert np.abs(bt @ r - ft).max() < 1e-9
            R[2 * c + h] = r
            R[8 + 2 * c + h] = (wt[:, None] * r.T) / (S * D)
    L = np.zeros((2 * RS, 128, 128))
    bb = np.arange(BS)
    kord = np.array([ri * 64 + 8 * t + r for t in range(8) for ri in range(2) for r in range(8)])
    rord = np.array([ri * 64 + 16 * q + r for q in range(4) for ri in range(2) for r in range(16)])
    for p1 in range(RS):
        ang = 2 * np.pi * (np.outer(p1 + RS * bb, bb) % S) / S
        mr, mi = np.cos(ang), -np.sin(ang)
        full = np.block([[mr, -mi], [mi, mr]])
        L[p1] = full[:, kord]
        L[RS + p1] = full.T[rord]
    l_, q_ = np.arange(128), np.arange(16)
    ang = 2 * np.pi * (np.outer(l_, l_) % 128) / 128
    N1 = np.concatenate([np.cos(ang), -np.sin(ang)], axis=1)
    N1 = np.concatenate([(N1[:64] + N1[64:]) / 2, (N1[:64] - N1[64:]) / 2], axis=0)
    ang = 2 * np.pi * np.outer(q_, l_) / S
    TW = np.concatenate([np.cos(ang), -np.sin(ang)], axis=0)
    ang = 2 * np.pi * (np.outer(q_, q_) % 16) / 16
    fr, fi = np.cos(ang), -np.sin(ang)
    F16 = np.block([[fr, -fi], [fi, fr]])
    NY = np.zeros((5, 128, 128))
    NY[0], NY[1], NY[2], NY[3] = N1[:, :128], N1[:, 128:], N1[:, :128].T, N1[:, 128:].T
    NY[4, :32, :32] = F16
    NY[4, 32:64, :32] = F16.T
    LN = np.concatenate([L, NY], axis=0)
    head = np.zeros(80, np.int32)
    pos = np.zeros(80, np.int32)
    for r in range(80):
        if r < 64:
            head[r] = r // 32
            t = r % 32
            pos[r] = (M + t) if t < FR else (t - FR)
        else:
            head[r] = (r - 64) // 8
            pos[r] = M + FR + (r - 64) % 8
    same = head[:, None] == head[None, :]
    vis = (pos[:, None] < M) | (pos[:, None] >= pos[None, :])
    fill = np.where(same, np.where(vis, 0.0, -1e9), -np.inf).astype(np.float32)
    return _pack_rows(R), _pack_rows(LN), TW.astype(np.float32), fill, KC.astype(np.float32)


def _cmul_const(re, im, j, n, sgn):
    ang = sgn * 2 * math.pi * j / n
    c, s = math.cos(ang), math.sin(ang)
    if abs(abs(c) - abs(s)) < 1e-12:
        if c * s > 0:
            return (re - im) * c, (re + im) * c
        return (re + im) * c, (im - re) * c
    return re * c - im * s, re * s + im * c


def _diff_tw(a, b, j, n, sgn):
    if j == 0:
        return a[0] - b[0], a[1] - b[1]
    if 4 * j == n:
        if sgn < 0:
            return a[1] - b[1], b[0] - a[0]
        return b[1] - a[1], a[0] - b[0]
    return _cmul_const(a[0] - b[0], a[1] - b[1], j, n, sgn)


def _tw(v, j, sgn):
    if j == 0:
        return v
    if 4 * j == RS:
        return (v[1], -v[0]) if sgn < 0 else (-v[1], v[0])
    return _cmul_const(v[0], v[1], j, RS, sgn)


def _fft(v, sgn):
    n = len(v)
    if n == 1:
        return v
    h = n // 2
    ev = _fft([(v[j][0] + v[j + h][0], v[j][1] + v[j + h][1]) for j in range(h)], sgn)
    od = _fft([_diff_tw(v[j], v[j + h], j, n, sgn) for j in range(h)], sgn)
    out = [None] * n
    out[0::2] = ev
    out[1::2] = od
    return out


def _dot(a, b):
    return jnp.dot(a, b, preferred_element_type=f32)


def _asbf(v):
    return pltpu.bitcast(v, bf16)


def _cm(ar, ai, br, bi):
    return ar * br - ai * bi, ar * bi + ai * br


CHUNKS = [(0, 0), (0, 1), (0, 2), (0, 3), (1, 0), (1, 1), (1, 2), (2, 0), (2, 1), (2, 2), (2, 3), (1, 3)]
BU = 2 * NST + NCH
BC = BU + 2


NK0 = 88


def _kernel(ax_hbm, mem_hbm, wq_hbm, wk_hbm, wv_hbm, wo_hbm, bx_hbm, wr_hbm, wi_hbm,
            R_hbm, L_hbm, sm_hbm, out_hbm,
            ax, xb3, xb, wo, pool, wpk, memb, ob, oa,
            bx, wf, R, L, sm, Y, T, wp, nv, sems):
    srcs = (wq_hbm, wk_hbm, wv_hbm)
    lane8 = lax.broadcasted_iota(i32, (8, 128), 1)

    def chunk_copy(t):
        m, c = CHUNKS[t]
        return pltpu.make_async_copy(srcs[m].at[:, :, pl.ds(8 * c, 8), :],
                                     pool.at[pl.ds(2 * (t % NST), 2)], sems.at[t % NST])

    def part0_copy(part):
        rows = pl.ds(pl.multiple_of(part * 128, 128), 128)
        return pltpu.make_async_copy(wq_hbm.at[:, rows, pl.ds(0, 8), :], pool.at[pl.ds(0, 2), rows], sems.at[34 + part])

    def part_start(t, part):
        lo = part * 2 * NK0
        n = min(2 * NK0, 512 - lo)
        pltpu.make_async_copy(wq_hbm.at[:, pl.ds(lo, n), pl.ds(8 * t, 8), :],
                              pool.at[pl.ds(2 * t, 2), pl.ds(lo, n)], sems.at[35 + 3 * t + part]).start()

    def part_wait(t, part):
        for p in range(3):
            lo = p * 2 * NK0
            n = min(2 * NK0, 512 - lo)

            @pl.when(part == p)
            def _(lo=lo, n=n, p=p):
                blk = pool.at[pl.ds(2 * t, 2), pl.ds(lo, n)]
                pltpu.make_async_copy(blk, blk, sems.at[35 + 3 * t + p]).wait()

    def chunk_start(t):
        sl = t & (NST - 1)
        pltpu.make_async_copy(wv_hbm.at[:, :, pl.ds(pl.multiple_of(8 * (t - 7), 8), 8), :],
                              pool.at[pl.ds(2 * sl, 2)], sems.at[sl]).start()

    def chunk_wait(t):
        sl = t & (NST - 1)
        blk = pool.at[pl.ds(2 * sl, 2)]
        pltpu.make_async_copy(blk, blk, sems.at[sl]).wait()

    def xb_copy(q):
        return pltpu.make_async_copy(ax_hbm.at[pl.ds(16 * q, 16), 3], xb3.at[pl.ds(16 * q, 16)], sems.at[8 + q])

    def bx_copy(q):
        return pltpu.make_async_copy(bx_hbm.at[:, pl.ds(2 * q, 2)], bx.at[:, pl.ds(2 * q, 2)], sems.at[12 + q])

    def w_copy(q, i):
        cols = pl.ds(pl.multiple_of(512 * q, 512), 512)
        return pltpu.make_async_copy((wr_hbm, wi_hbm)[i].at[:, cols], wf.at[q, i],
                                     sems.at[16 + 4 * i + q])

    def wo_copy(q, hi):
        j = q + 4 * hi
        return pltpu.make_async_copy(wo_hbm.at[:, pl.ds(pl.multiple_of(128 * j, 128), 128)], wo.at[j],
                                     sems.at[44 + q])

    cp_r0 = pltpu.make_async_copy(R_hbm.at[pl.ds(0, 8)], R.at[pl.ds(0, 8)], sems.at[25])
    cp_r1 = pltpu.make_async_copy(R_hbm.at[pl.ds(8, 8)], R.at[pl.ds(8, 8)], sems.at[26])
    cp_l = pltpu.make_async_copy(L_hbm, L, sems.at[27])
    cp_ax = pltpu.make_async_copy(ax_hbm.at[:, pl.ds(0, 3)], ax, sems.at[28])
    cp_outb = pltpu.make_async_copy(bx, out_hbm.at[:, :, :, pl.ds(DM, D)], sems.at[29])
    cp_sm = pltpu.make_async_copy(sm_hbm, sm, sems.at[30])
    cp_mem = pltpu.make_async_copy(mem_hbm, memb, sems.at[31])

    for part in range(4):
        part0_copy(part).start()
    xb_copy(0).start()
    for p in range(3):
        xb_copy(p + 1).start()
        part_start(1, p)
    for p in range(3):
        part_start(2, p)
    chunk_copy(3).start()
    cp_r0.start()
    bx_copy(0).start()
    w_copy(0, 0).start()
    w_copy(0, 1).start()
    cp_sm.start()
    cp_mem.start()

    def kc(rep=2):
        return [jnp.concatenate([sm[112 + 8 * i:120 + 8 * i, :]] * rep, axis=0) for i in range(12)]

    def roll64(v):
        return pltpu.roll(v, 64, 1)

    def prep(t, tpar, jj):
        lo = [bx[2 * jj:2 * jj + 2, t, :, 128 * e:128 * (e + 1)].astype(f32).reshape(16, 128) for e in range(8)]
        hi = [bx[HR + 2 * jj:HR + 2 * jj + 2, t, :, 128 * e:128 * (e + 1)].astype(f32).reshape(16, 128)
              for e in range(8)]
        for par in range(2):
            x = [lo[e] + hi[e] if par == 0 else lo[e] - hi[e] for e in range(8)]
            uu = _dstage(x, kc(), roll64)
            for q in range(8):
                o = (((tpar * 2 + par) * 8 + q) * 8 + jj) * 2
                pool[BU, o:o + 2] = uu[q].reshape(2, 8, 128).astype(bf16)

    def unit1(t, tpar, par, cg):
        o = ((tpar * 2 + par) * 8 + 2 * cg) * 16
        za = _dot(pool[BU, o:o + 16].reshape(128, 128), _asbf(R[2 * cg]))
        zb = _dot(pool[BU, o + 16:o + 32].reshape(128, 128), _asbf(R[2 * cg + 1]))
        ina = _in_a(lane8, cg)
        v = []
        for j in range(HR):
            pa, pb = za[8 * j:8 * j + 8], zb[8 * j:8 * j + 8]
            v.append((jnp.where(ina, pa, pb), pltpu.roll(jnp.where(ina, pb, pa), _RHO[cg], 1)))
        if cg == 0:
            V = nv[8 * tpar:8 * tpar + 8, :]
            for j in range(HR):
                vb = jnp.broadcast_to(v[j][1][:, 0:1], (8, 128))
                V = jnp.where(lane8 == 64 * par + 4 * j + (t >> 1), vb, V)
                v[j] = (v[j][0], jnp.where(lane8 == 0, 0.0, v[j][1]))
            nv[8 * tpar:8 * tpar + 8, :] = V
        if par == 1:
            v = [_tw(v[j], j, -1) for j in range(HR)]
        o = _fft(v, -1)
        for m in range(HR):
            Y[t >> 1, 2 * m + par, cg, tpar] = jnp.concatenate(o[m], axis=0).astype(bf16)

    def wprep(q, k, i):
        w = wf.at[q, i]
        cols = slice(128 * k, 128 * (k + 1))
        sub = lax.broadcasted_iota(i32, (8, 128), 0)
        msk = (jnp.where(sub % 2 == 0, jnp.uint32(0xffff), jnp.uint32(0))
               | jnp.where((sub % 4 == 0) | (sub % 4 == 3), jnp.uint32(0xffff0000), jnp.uint32(0)))
        t0 = pltpu.bitcast(w[0:256, cols], u32)
        t1 = pltpu.bitcast(w[256:512, cols], u32)
        ps, qs = [], []
        for j in range(16):
            a = t0[8 * j:8 * j + 8]
            b = t1[8 * j:8 * j + 8]
            b = jnp.where(sub % 2 == 0, pltpu.roll(b, 7, 0), pltpu.roll(b, 1, 0))
            x = (a ^ b) & msk
            ps.append(b ^ x)
            qs.append(a ^ x)
        for h, lst in enumerate((ps, qs)):
            tr = pltpu.bitcast(pltpu.bitcast(jnp.concatenate(lst, axis=0), f32).T, u32)
            r0 = pl.multiple_of((4 * q + k) * 32, 32)
            for j in range(4):
                for o in range(4):
                    wp[i, h, o, pl.ds(r0 + 8 * j, 8), :] = tr[32 * j + 8 * o:32 * j + 8 * o + 8]

    def fwd(p):
        return _dot(_asbf(L[p]), jnp.concatenate([Y[:, p, cg].reshape(128, 128) for cg in range(4)], axis=1))

    def filt(q, po, v):
        grs, gis = [None] * 4, [None] * 4
        for h in range(2):
            wr_ = wp[0, h, q, pl.ds(po, BS, stride=8), :]
            wi_ = wp[1, h, q, pl.ds(po, BS, stride=8), :]
            for hi in range(2):
                cg = 2 * h + hi
                if hi == 0:
                    a, b = wr_ << 16, wi_ << 16
                else:
                    a, b = wr_ & jnp.uint32(0xffff0000), wi_ & jnp.uint32(0xffff0000)
                grs[cg], gis[cg] = _cm(v[:BS, 128 * cg:128 * (cg + 1)], v[BS:, 128 * cg:128 * (cg + 1)],
                                       pltpu.bitcast(a, f32), pltpu.bitcast(b, f32))
        return jnp.concatenate([jnp.concatenate(grs, axis=1), jnp.concatenate(gis, axis=1)], axis=0).astype(bf16)

    def inv(p, g):
        t = _dot(_asbf(L[RS + p]), g)
        for cg in range(4):
            T[cg, p, 0:128, :] = t[:, 128 * cg:128 * (cg + 1)]

    nyq = {}

    def nyq_stage(k):
        n0 = 2 * RS
        twr, twi = sm[80:96, :], sm[96:112, :]
        if k == 0:
            v = nv[0:16, :].astype(bf16)
            r, i = _cm(_dot(v, _asbf(L[n0])), _dot(v, _asbf(L[n0 + 1])), twr, twi)
            nyq[0] = jnp.concatenate([r, i], axis=0).astype(bf16)
        elif k == 1:
            t = _dot(_asbf(L[n0 + 4, 0:16])[:, 0:32], nyq[0])
            ws = []
            for i in range(2):
                rows = [wf[j, i, 512:513, :].astype(f32) for j in range(4)]
                ws.append(jnp.concatenate([rows[r // 4][:, 128 * (r % 4):128 * (r % 4 + 1)] for r in range(16)], axis=0))
            r, i = _cm(t[:16], t[16:], ws[0], ws[1])
            nyq[1] = jnp.concatenate([r, i], axis=0).astype(bf16)
        elif k == 2:
            t = _dot(_asbf(L[n0 + 4, 16:32])[:, 0:32], nyq[1])
            r, i = _cm(t[:16], t[16:], twr, -twi)
            nyq[2] = (r.astype(bf16), i.astype(bf16))
        elif k == 3:
            nv[16:32, :] = _dot(nyq[2][0], _asbf(L[n0 + 2])) + _dot(nyq[2][1], _asbf(L[n0 + 3]))

    def p3a(t, tpar, par, cg):
        r0 = pl.multiple_of((t >> 1) * 32, 32)
        rr = pl.ds(r0 + 8 * tpar, 8)
        ri = pl.ds(r0 + 16 + 8 * tpar, 8)
        o = _fft([(T[cg, 2 * m + par, rr, :], T[cg, 2 * m + par, ri, :]) for m in range(HR)], +1)
        if par == 1:
            o = [_tw(o[j], j, +1) for j in range(HR)]
        if cg == 0:
            un = nv[16 + 8 * tpar:24 + 8 * tpar, :]
            o = [(o[j][0], jnp.where(lane8 == 0, pltpu.roll(un, (128 - 64 * par - 4 * j - (t >> 1)) & 127, 1),
                                     o[j][1])) for j in range(HR)]
        ina = _in_a(lane8, cg)
        ua, ub = [], []
        for re, im in o:
            im = pltpu.roll(im, 128 - _RHO[cg], 1)
            ua.append(jnp.where(ina, re, im))
            ub.append(jnp.where(ina, im, re))
        for j in range(HR // 2):
            for h, x in enumerate((ua, ub)):
                o = ((tpar * 2 + par) * 8 + 2 * cg + h) * 16 + 2 * j
                pool[BU + 1, o:o + 2] = jnp.concatenate(x[2 * j:2 * j + 2], axis=0).reshape(2, 8, 128).astype(bf16)

    def p3b(tpar, par, cg):
        zs = []
        for h in range(2):
            o = ((tpar * 2 + par) * 8 + 2 * cg + h) * 16
            zs.append((o, _dot(pool[BU + 1, o:o + 16].reshape(128, 128), _asbf(R[8 + 2 * cg + h]))))
        return zs

    def p3s(zs):
        for o, z in zs:
            pool[BU, o:o + 16] = z.reshape(16, 8, 128).astype(bf16)

    def p3c(t, tpar, j):
        res = [_dstage_t([pool[BU, ((tpar * 2 + par) * 8 + q) * 16 + j].astype(f32) for q in range(8)],
                         kc(1), roll64) for par in range(2)]
        for e in range(8):
            cols = slice(128 * e, 128 * (e + 1))
            bx[j, t, :, cols] = (res[0][e] + res[1][e]).astype(bf16)
            bx[HR + j, t, :, cols] = (res[0][e] - res[1][e]).astype(bf16)

    def wsum(jj, hf, n):
        r0 = pl.multiple_of(hf * 1024, 1024)
        lo, hi = pl.ds(r0 + 16 * n, 16), pl.ds(r0 + 2048 + 16 * n, 16)
        b11, b21 = wo[jj, lo, :].astype(f32), wo[jj, hi, :].astype(f32)
        b12, b22 = wo[4 + jj, lo, :].astype(f32), wo[4 + jj, hi, :].astype(f32)
        for i, v in enumerate((b11 + b22, b12 - b22, b21 - b11, b11 + b12, b21 + b22)):
            pool[BC + 2 * i + (jj >> 1), pl.ds((jj & 1) * 256 + hf * 128 + 2 * n, 2)] = (
                v.reshape(2, 8, 128).astype(bf16))

    def wc(i, jj):
        return pool[BC + 2 * i + jj // 2, (jj % 2) * 256:(jj % 2 + 1) * 256].reshape(2048, 128)

    def runit(b0, d0, dst, k):
        a = pltpu.bitcast(jnp.concatenate([pool[b0, d0 + 2 * k], pool[b0 + 1, d0 + 2 * k]], axis=0), u32)
        b = pltpu.bitcast(jnp.concatenate([pool[b0, d0 + 2 * k + 1], pool[b0 + 1, d0 + 2 * k + 1]], axis=0), u32)
        dst[pl.ds(k, 8, stride=PW), :] = (a & jnp.uint32(0xffff)) | (b << 16)
        dst[pl.ds(8 * PW + k, 8, stride=PW), :] = (a >> 16) | (b & jnp.uint32(0xffff0000))

    def wsel(w, hl, lo=0, hi=DM):
        base = ((hl % 2) * 8 + hl // 2) * PW
        parts = []
        for kh in range(2):
            a, b = max(lo, 512 * kh), min(hi, 512 * (kh + 1))
            if a < b:
                o = base + 4 * PW * kh - 256 * kh
                parts.append(w[o + a // 2:o + b // 2, :])
        return _asbf(jnp.concatenate(parts, axis=0))

    def bulk(t, mc0, nmc, tsrc, tdst, k0, nk, side=None):
        w = wpk.at[t]
        b0 = 2 * (tsrc & (NST - 1))
        dst = wpk.at[tdst, pl.ds(k0, 15 * PW + nk)]
        bq = 2 * NST + (t & 31)
        ns = 8 * nmc
        per = nk // ns
        for mi in range(nmc):
            mc = mc0 + mi
            x = _asbf(xb[mc])
            for h in range(8):
                n = mi * 8 + h
                r = _dot(x, wsel(w, h)).reshape(16, M, DH)
                nn = (n - 1) % ns
                for k in range(per * nn, per * (nn + 1)):
                    runit(b0, 2 * k0, dst, k)
                if side is not None:
                    side(n)
                rb = r.astype(bf16)
                for gi in range(4):
                    pool[bq, pl.ds(mc * 128 + gi * 32 + h * 4, 4)] = rb[4 * gi:4 * gi + 4]

    def rel0(i, c):
        @pl.when(i % 2 == 0)
        def _():
            part0_copy(i >> 1).wait()
        dst = wpk.at[0, pl.ds(pl.multiple_of(i * 32, 32), 15 * PW + 32)]
        for k in range(32):
            runit(0, i * 64, dst, k)
        return c
    with jax.named_scope("rel0"):
        lax.fori_loop(0, 8, rel0, 0)

    def body0(i, c):
        t, mc = i >> 2, i & 3
        real = mc >= 1

        @pl.when(t == 0)
        def _():
            xb_copy(mc).wait()
            xb[mc] = pltpu.bitcast(xb3[pl.ds(16 * mc, 16)].reshape(128, DM), u32)

        @pl.when(real)
        def _():
            part_wait(t + 1, mc - 1)
        with jax.named_scope("bulk0"):
            bulk(t, mc, 1, jnp.where(real, t + 1, t), jnp.where(real, t + 1, NCH),
                 pl.multiple_of(jnp.clip((mc - 1) * NK0, 0, 256 - NK0), math.gcd(NK0, 32)), NK0)

        @pl.when(i == 0)
        def _():
            chunk_copy(4).start()
            bx_copy(1).start()
            w_copy(1, 0).start()
            w_copy(1, 1).start()

        @pl.when(i == 4)
        def _():
            chunk_copy(5).start()
        return c
    lax.fori_loop(0, 8, body0, 0)
    bx_copy(2).start()
    w_copy(2, 0).start()
    w_copy(2, 1).start()
    chunk_copy(6).start()
    bx_copy(3).start()
    w_copy(3, 0).start()
    w_copy(3, 1).start()
    cp_l.start()
    cp_r1.start()
    nv[0:16, :] = jnp.zeros((16, 128), f32)
    cp_r0.wait()
    cp_sm.wait()

    def body1(q, c):
        t = q + 2
        with jax.named_scope("w_1"):
            chunk_wait(t + 1)
            bx_copy(q).wait()
            w_copy(q, 0).wait()
            w_copy(q, 1).wait()

        def side(n):
            for k in ([0, 1] if n == 0 else [n + 1]):
                if k < 16:
                    prep(2 * q + k // 8, k // 8, k % 8)
            k = n - 15
            if 0 <= k < 16:
                unit1(2 * q + k // 8, k // 8, (k // 4) % 2, k % 4)
            k, r = divmod(n - 1, 2)
            if r == 0 and 0 <= k < 8:
                wprep(q, k // 2, k % 2)
        with jax.named_scope("bulk_p1"):
            bulk(t, 0, 4, t + 1, t + 1, 0, 256, side)
        wo_copy(q, 0).start()
        wo_copy(q, 1).start()
        chunk_start(t + 1 + NST)
        return c
    lax.fori_loop(0, 4, body1, 0)

    cp_ax.start()
    with jax.named_scope("w_l"):
        cp_l.wait()
        cp_r1.wait()

    def body2(q, c):
        t, hf = (q >> 1) + 6, q & 1

        @pl.when(hf == 0)
        def _():
            with jax.named_scope("w_2"):
                chunk_wait(t + 1)
                wo_copy(q >> 1, 0).wait()
                wo_copy(q >> 1, 1).wait()
        gs = {}
        fs = [0, 1, 3, 5, 7, 9, 11, 13]

        def side(n):
            if n - 2 in fs:
                po = fs.index(n - 2)
                inv(8 * q + po, gs.pop(po))
            if n in fs:
                po = fs.index(n)
                gs[po] = filt(q, po, fwd(8 * q + po))
            k, r = divmod(n - 1, 3)
            if r == 0 and 0 <= k < 4:
                nyq_stage(k)
            for hh in range(64 * n // 15, min(64, 64 * (n + 1) // 15)):
                wsum(q >> 1, hf, hh)
        with jax.named_scope("bulk_p2"):
            bulk(t, 2 * hf, 2, t + 1, t + 1, pl.multiple_of(hf * 128, 128), 128, side)
        return c
    lax.fori_loop(0, 4, body2, 0)
    chunk_copy(11).start()
    for j in (2, 3):
        wo_copy(j, 0).wait()
        wo_copy(j, 1).wait()

    def body3(q, c):
        t = q + 8

        @pl.when(q < 3)
        def _():
            with jax.named_scope("w_3"):
                chunk_wait(t + 1)
        us = {}

        def side(n):
            if n < 16:
                p3a(2 * q + n // 8, n // 8, (n // 4) % 2, n % 4)
            k = n - 3
            if 0 <= k < 16:
                us[k] = p3b(k // 8, (k // 4) % 2, k % 4)
            k = n - 3 - 1
            if 0 <= k < 16:
                p3s(us.pop(k))
            k = n - 16
            if 0 <= k < 16:
                p3c(2 * q + k // 8, k // 8, 2 * (k % 8))
                p3c(2 * q + k // 8, k // 8, 2 * (k % 8) + 1)
            for hh in range(2):
                wsum(2 + (q >> 1), q & 1, 2 * n + hh)
        with jax.named_scope("bulk_p3"):
            bulk(t, 0, 4, t + 1, t + 1, 0, 256, side)
        return c
    lax.fori_loop(0, 4, body3, 0)
    cp_outb.start()

    with jax.named_scope("w_wo"):
        cp_ax.wait()
        cp_mem.wait()
    scale = DH ** -0.5
    KS = 640

    def step(it, u):
        s = it * U + u
        lhs = jnp.concatenate([ax[s].reshape(FR, DM), memb[...]], axis=0)
        qs, ks, vs, ps, os_, pre = {}, {}, {}, {}, {}, {}

        def ws(m, h, lo=0, hi=DM):
            return wsel(wpk.at[CHUNKS.index((m, h // 8))], h % 8, lo, hi)
        if u > 0:
            for m in range(2):
                for h in range(2):
                    pre[(m, h)] = -_dot(lhs[:, :KS], ws(m, h, 0, KS))

        def dotw(m, h):
            if (m, h) in pre:
                return _dot(lhs[:, KS:], ws(m, h, KS, DM)) - pre[(m, h)]
            return _dot(lhs, ws(m, h))

        def proj(m, g):
            h = 2 * g
            bq = 2 * NST + CHUNKS.index((m, h // 8))
            return jnp.concatenate([dotw(m, h), dotw(m, h + 1),
                                    pool[bq, it * 32 + (h % 8) * 4 + u].astype(f32),
                                    pool[bq, it * 32 + (h % 8 + 1) * 4 + u].astype(f32)], axis=0).astype(bf16)

        def qk(g):
            sc = lax.dot_general(qs.pop(g), ks.pop(g), (((1,), (1,)), ((), ())),
                                 preferred_element_type=f32) * scale
            fill = sm[0:80, 0:80]
            sc = jnp.where(fill == 0.0, sc, fill)
            mx = jnp.max(sc, axis=-1, keepdims=True)
            e = jnp.exp(sc - mx)
            l = jnp.sum(e, axis=-1, keepdims=True)
            r = pl.reciprocal(l, approx=True)
            r = r * (2.0 - l * r)
            ps[g] = (e * r).astype(bf16)

        def pv(g):
            o = _dot(ps.pop(g), vs.pop(g))
            os_[2 * g] = o[0:32]
            os_[2 * g + 1] = o[32:64]
            ob[8 * u:8 * u + 8, (2 * g) * DH:(2 * g + 1) * DH] = o[64:72]
            ob[8 * u:8 * u + 8, (2 * g + 1) * DH:(2 * g + 2) * DH] = o[72:80]

        def olhs(lo, hi):
            return jnp.concatenate([os_[h] for h in range(lo, hi)], axis=1)

        def put(j, r, rb):
            cols = slice(j * 128, (j + 1) * 128)
            oa[it * 2 + u // 2, pl.ds((u % 2) * 4, 3), :, cols] = r[0:FR].reshape(3, 8, 128).astype(bf16)
            memb[:, cols] = r[FR:SEG].astype(bf16)
            if rb is not None:
                for uu in range(U):
                    oa[it * 2 + uu // 2, (uu % 2) * 4 + 3, :, cols] = rb[8 * uu:8 * uu + 8].astype(bf16)

        sk, dq, dp = 7, 3, 5
        for t in range(G + sk):
            if t < G:
                qs[t] = proj(0, t)
            if 0 <= t - dq < G:
                qk(t - dq)
            if t < G:
                ks[t] = proj(1, t)
            if t - sk - dp >= 0:
                pv(t - sk - dp)
            if t - sk >= 0:
                vs[t - sk] = proj(2, t - sk)
        rem = list(range(G - dp, G))
        hk = 16 * DH
        acc = []
        if u < U - 1:
            oc = olhs(0, 16).astype(bf16)
            early = [(oc, wo[j, 0:hk, :]) for j in range(8)]
        else:
            a11, a21 = olhs(0, 16), ob[:, 0:hk]
            l3, l6 = a11.astype(bf16), (a21 - a11).astype(bf16)
            early = [(l3, wc(1, jj)) for jj in range(4)] + [(l6, wc(3, jj)) for jj in range(4)]
        for j in range(8):
            acc.append(-_dot(*early[j]))
            if rem:
                pv(rem.pop(0))
        if u < U - 1:
            oc = olhs(16, 32).astype(bf16)
            for j in range(8):
                put(j, _dot(oc, wo[j, hk:2 * hk, :]) - acc[j], None)
        else:
            a12, a22 = olhs(16, 32), ob[:, hk:2 * hk]
            l1, l2, l4 = (a11 + a22).astype(bf16), (a21 + a22).astype(bf16), a22.astype(bf16)
            l5, l7 = (a11 + a12).astype(bf16), (a12 - a22).astype(bf16)
            for jj in range(4):
                m1 = _dot(l1, wc(0, jj))
                m2 = _dot(l2, wo[jj, 0:hk, :])
                m4 = _dot(l4, wc(2, jj))
                m5 = _dot(l5, wo[4 + jj, hk:2 * hk, :])
                m7 = _dot(l7, wc(4, jj))
                put(jj, (m1 - m5) + (m4 + m7), m2 + m4)
                put(4 + jj, m5 - acc[jj], (m1 - m2) - acc[jj] - acc[4 + jj])

    def out_copy(it):
        return pltpu.make_async_copy(oa.at[pl.ds(it * 2, 2)],
                                     out_hbm.at[pl.ds(it * 2, 2), :, :, pl.ds(0, DM)], sems.at[32])

    def group(it, c):
        with jax.named_scope("grp"):
            for u in range(U):
                step(it, u)
        out_copy(it).start()
        return c
    lax.fori_loop(0, NSEG // U, group, 0)
    with jax.named_scope("w_out"):
        for it in range(NSEG // U):
            out_copy(it).wait()
        cp_outb.wait()


def pallas_concat_heads__memory_aug_recurrent_mem_tr__spectral_gfnet__prompt_kernel(
    A_x, A_mem0, A_Wq, A_Wk, A_Wv, A_Wo, A_seg_len, B_x, B_w_r, B_w_i,
):
    if isinstance(A_seg_len, int):
        assert A_seg_len == SEG
    R, LN, TW, fill, KC = _tables()
    small = np.zeros((208, 128), np.float32)
    small[:80, :80] = fill
    small[80:112] = TW
    small[112:] = np.repeat(KC, 8, axis=0)
    hbm = pl.BlockSpec(memory_space=pl.ANY)
    out = pl.pallas_call(
        _kernel,
        out_shape=jax.ShapeDtypeStruct((RS, 8, 8, DM + D), bf16),
        in_specs=[hbm] * 12,
        out_specs=hbm,
        scratch_shapes=[
            pltpu.VMEM((NSEG, 3, 8, DM), bf16),
            pltpu.VMEM((NSEG, 8, DM), bf16),
            pltpu.VMEM((4, 64, DM), u32),
            pltpu.VMEM((DM // 128, H * DH, 128), bf16),
            pltpu.VMEM((BC + 10, DM // 2, 8, DH), bf16),
            pltpu.VMEM((NCH + 1, 16 * PW, DH), u32),
            pltpu.VMEM((M, DM), bf16),
            pltpu.VMEM((U * M, H * DH), f32),
            pltpu.VMEM((RS, 8, 8, DM), bf16),
            pltpu.VMEM((RS, 8, 8, D), bf16),
            pltpu.VMEM((4, 2, D // 2 + 1, 512), bf16),
            pltpu.VMEM((16, 64, 128), u32),
            pltpu.VMEM((2 * RS + 5, 64, 128), u32),
            pltpu.VMEM((208, 128), f32),
            pltpu.VMEM((4, RS, 4, 2, 16, 128), bf16),
            pltpu.VMEM((4, RS, TP, 128), f32),
            pltpu.VMEM((2, 2, 4, BS * 8, 128), u32),
            pltpu.VMEM((32, 128), f32),
            pltpu.SemaphoreType.DMA((48,)),
        ],
        compiler_params=pltpu.CompilerParams(vmem_limit_bytes=124 * 1024 * 1024,
                                             disable_bounds_checks=True, disable_semaphore_checks=True),
    )(A_x.reshape(NSEG, 4, 8, DM), A_mem0.reshape(M, DM),
      A_Wq.reshape(2, DM // 2, H, DH), A_Wk.reshape(2, DM // 2, H, DH), A_Wv.reshape(2, DM // 2, H, DH),
      A_Wo.reshape(H * DH, DM), B_x.reshape(RS, 8, 8, D), B_w_r.T, B_w_i.T,
      jnp.asarray(R), jnp.asarray(LN), jnp.asarray(small))
    return out.reshape(1, S, DM + D)
```

```python
import functools
import math

import jax
import jax.numpy as jnp
import numpy as np
from jax import lax
import jax.experimental.pallas as pl
import jax.experimental.pallas.tpu as pltpu

bf16, f32, u32, i32 = jnp.bfloat16, jnp.float32, jnp.uint32, jnp.int32

S, DM, H, DH, M, SEG = 2048, 1024, 32, 128, 8, 32
NSEG = S // SEG
FR = SEG - M
G = H // 2
U = 4
NCH = 12
NST = 4
PW = 264

D = 1024
RS, BS = 32, 64
HR = RS // 2
TP = 136
C8 = float(np.sqrt(0.5))


def _pack_rows(a):
    u = np.asarray(a, np.float32).astype(jnp.bfloat16).view(np.uint16).astype(np.uint32)
    return u[..., 0::2, :] | (u[..., 1::2, :] << 16)


_RHO = (2, 4, 4, 4)


def _in_a(lane, c):
    return (lane % 4 < 2) if c == 0 else ((lane + 2) % 8 < 4)


def _dstage(x, kc, roll64):
    a = [x[j] + x[j + 4] for j in range(4)]
    b = [x[j] - x[j + 4] for j in range(4)]
    t1 = (b[1] - b[3]) * C8
    t2 = (b[1] + b[3]) * C8
    s0, s1 = a[0] + a[2], a[1] + a[3]
    out = [s0 + s1, s0 - s1]
    for c, (u, v) in enumerate(((b[0] + t1, b[2] + t2), (a[0] - a[2], a[1] - a[3]), (b[0] - t1, b[2] - t2))):
        g = u * kc[4 * c] + v * kc[4 * c + 1]
        h = roll64(u * kc[4 * c + 2] + v * kc[4 * c + 3])
        out += [g + h, g - h]
    return out


def _dstage_t(p, kc, roll64):
    uv = []
    for c in range(3):
        g = p[2 + 2 * c] + p[3 + 2 * c]
        h = roll64(p[2 + 2 * c] - p[3 + 2 * c])
        uv.append((g * kc[4 * c] + h * kc[4 * c + 2], g * kc[4 * c + 1] + h * kc[4 * c + 3]))
    s0, s1 = p[0] + p[1], p[0] - p[1]
    a = [s0 + uv[1][0], s1 + uv[1][1], s0 - uv[1][0], s1 - uv[1][1]]
    t1 = (uv[0][0] - uv[2][0]) * C8
    t2 = (uv[0][1] - uv[2][1]) * C8
    b = [uv[0][0] + uv[2][0], t1 + t2, uv[0][1] + uv[2][1], t2 - t1]
    return [a[j] + b[j] for j in range(4)] + [a[j] - b[j] for j in range(4)]


@functools.lru_cache(maxsize=None)
def _tables():
    kcol = np.zeros((4, 128), np.int64)
    for l in range(128):
        i0, i1 = l, 128 + (l ^ 1)
        ev, o3 = l % 2 == 0, l % 4 in (0, 3)
        kcol[0, l] = 2 * (i0 if ev else i1)
        kcol[2, l] = 2 * (i1 if ev else i0)
        kcol[1, l] = 2 * (i0 if o3 else i1) + 1
        kcol[3, l] = 2 * (i1 if o3 else i0) + 1
    lanes = np.arange(128)
    lo = lanes < 64
    KC = np.zeros((12, 128))
    for c, sg in ((1, -1.0), (2, -1.0), (3, 1.0)):
        tr, ti = np.cos(2 * np.pi * c / 16), -np.sin(2 * np.pi * c / 16)
        KC[4 * c - 4] = np.where(lo, 1.0, ti)
        KC[4 * c - 3] = sg * np.where(lo, 0.0, tr)
        KC[4 * c - 2] = np.where(lo, 0.0, tr)
        KC[4 * c - 1] = sg * np.where(lo, 1.0, -ti)
    eye = np.eye(D)
    Bt = _dstage([eye[:, 128 * e:128 * (e + 1)] for e in range(8)], KC, lambda v: np.roll(v, 64, axis=1))
    d = np.arange(D)
    R = np.zeros((16, 128, 128))
    for c in range(4):
        rho = _RHO[c]
        inA = _in_a(lanes, c)
        ang = 2 * np.pi * (np.outer(d, kcol[c]) % D) / D
        fr, fi = np.cos(ang), -np.sin(ang)
        wr_, wi_ = np.full(128, 2.0), np.full(128, 2.0)
        if c == 0:
            fi[:, 0] = (-1.0) ** d
            wr_[0] = 1.0
            wi_[0] = 1.0
        fi, wi_ = np.roll(fi, -rho, axis=1), np.roll(wi_, -rho)
        for h in range(2):
            own = inA if h == 0 else ~inA
            ft, wt = np.where(own, fr, fi), np.where(own, wr_, wi_)
            bt = Bt[2 * c + h]
            r = (bt.T @ ft) / (bt * bt).sum(axis=0)[:, None]
            assert np.abs(bt @ r - ft).max() < 1e-9
            R[2 * c + h] = r
            R[8 + 2 * c + h] = (wt[:, None] * r.T) / (S * D)
    L = np.zeros((2 * RS, 128, 128))
    bb = np.arange(BS)
    kord = np.array([ri * 64 + 8 * t + r for t in range(8) for ri in range(2) for r in range(8)])
    rord = np.array([ri * 64 + 16 * q + r for q in range(4) for ri in range(2) for r in range(16)])
    for p1 in range(RS):
        ang = 2 * np.pi * (np.outer(p1 + RS * bb, bb) % S) / S
        mr, mi = np.cos(ang), -np.sin(ang)
        full = np.block([[mr, -mi], [mi, mr]])
        L[p1] = full[:, kord]
        L[RS + p1] = full.T[rord]
    l_, q_ = np.arange(128), np.arange(16)
    ang = 2 * np.pi * (np.outer(l_, l_) % 128) / 128
    N1 = np.concatenate([np.cos(ang), -np.sin(ang)], axis=1)
    N1 = np.concatenate([(N1[:64] + N1[64:]) / 2, (N1[:64] - N1[64:]) / 2], axis=0)
    ang = 2 * np.pi * np.outer(q_, l_) / S
    TW = np.concatenate([np.cos(ang), -np.sin(ang)], axis=0)
    ang = 2 * np.pi * (np.outer(q_, q_) % 16) / 16
    fr, fi = np.cos(ang), -np.sin(ang)
    F16 = np.block([[fr, -fi], [fi, fr]])
    NY = np.zeros((5, 128, 128))
    NY[0], NY[1], NY[2], NY[3] = N1[:, :128], N1[:, 128:], N1[:, :128].T, N1[:, 128:].T
    NY[4, :32, :32] = F16
    NY[4, 32:64, :32] = F16.T
    LN = np.concatenate([L, NY], axis=0)
    head = np.zeros(80, np.int32)
    pos = np.zeros(80, np.int32)
    for r in range(80):
        if r < 64:
            head[r] = r // 32
            t = r % 32
            pos[r] = (M + t) if t < FR else (t - FR)
        else:
            head[r] = (r - 64) // 8
            pos[r] = M + FR + (r - 64) % 8
    same = head[:, None] == head[None, :]
    vis = (pos[:, None] < M) | (pos[:, None] >= pos[None, :])
    fill = np.where(same, np.where(vis, 0.0, -1e9), -np.inf).astype(np.float32)
    return _pack_rows(R), _pack_rows(LN), TW.astype(np.float32), fill, KC.astype(np.float32)


def _cmul_const(re, im, j, n, sgn):
    ang = sgn * 2 * math.pi * j / n
    c, s = math.cos(ang), math.sin(ang)
    if abs(abs(c) - abs(s)) < 1e-12:
        if c * s > 0:
            return (re - im) * c, (re + im) * c
        return (re + im) * c, (im - re) * c
    return re * c - im * s, re * s + im * c


def _diff_tw(a, b, j, n, sgn):
    if j == 0:
        return a[0] - b[0], a[1] - b[1]
    if 4 * j == n:
        if sgn < 0:
            return a[1] - b[1], b[0] - a[0]
        return b[1] - a[1], a[0] - b[0]
    return _cmul_const(a[0] - b[0], a[1] - b[1], j, n, sgn)


def _tw(v, j, sgn):
    if j == 0:
        return v
    if 4 * j == RS:
        return (v[1], -v[0]) if sgn < 0 else (-v[1], v[0])
    return _cmul_const(v[0], v[1], j, RS, sgn)


def _fft(v, sgn):
    n = len(v)
    if n == 1:
        return v
    h = n // 2
    ev = _fft([(v[j][0] + v[j + h][0], v[j][1] + v[j + h][1]) for j in range(h)], sgn)
    od = _fft([_diff_tw(v[j], v[j + h], j, n, sgn) for j in range(h)], sgn)
    out = [None] * n
    out[0::2] = ev
    out[1::2] = od
    return out


def _dot(a, b):
    return jnp.dot(a, b, preferred_element_type=f32)


def _asbf(v):
    return pltpu.bitcast(v, bf16)


def _cm(ar, ai, br, bi):
    return ar * br - ai * bi, ar * bi + ai * br


CHUNKS = [(0, 0), (0, 1), (0, 2), (0, 3), (1, 0), (1, 1), (1, 2), (2, 0), (2, 1), (2, 2), (2, 3), (1, 3)]
BU = 2 * NST + NCH
BC = BU + 2
CF = (-1.2, -0.4, 0.4, 1.2)
PAIRS = [(k, j) for j in range(4) for k in range(j)]
RAW32 = [(0, 1), (1, 0), (0, 2), (2, 0), (1, 2), (2, 1)]


NK0 = 88


def _kernel(ax_hbm, mem_hbm, wq_hbm, wk_hbm, wv_hbm, wo_hbm, bx_hbm, wr_hbm, wi_hbm,
            R_hbm, L_hbm, sm_hbm, out_hbm,
            ax, xb3, xb, wo, w32, pool, wpk, memb, ob, oa,
            bx, wf, R, L, sm, Y, T, wp, nv, sems):
    srcs = (wq_hbm, wk_hbm, wv_hbm)
    lane8 = lax.broadcasted_iota(i32, (8, 128), 1)

    def chunk_copy(t):
        m, c = CHUNKS[t]
        return pltpu.make_async_copy(srcs[m].at[:, :, pl.ds(8 * c, 8), :],
                                     pool.at[pl.ds(2 * (t % NST), 2)], sems.at[t % NST])

    def part0_copy(part):
        rows = pl.ds(pl.multiple_of(part * 128, 128), 128)
        return pltpu.make_async_copy(wq_hbm.at[:, rows, pl.ds(0, 8), :], pool.at[pl.ds(0, 2), rows], sems.at[34 + part])

    def part_start(t, part):
        lo = part * 2 * NK0
        n = min(2 * NK0, 512 - lo)
        pltpu.make_async_copy(wq_hbm.at[:, pl.ds(lo, n), pl.ds(8 * t, 8), :],
                              pool.at[pl.ds(2 * t, 2), pl.ds(lo, n)], sems.at[35 + 3 * t + part]).start()

    def part_wait(t, part):
        for p in range(3):
            lo = p * 2 * NK0
            n = min(2 * NK0, 512 - lo)

            @pl.when(part == p)
            def _(lo=lo, n=n, p=p):
                blk = pool.at[pl.ds(2 * t, 2), pl.ds(lo, n)]
                pltpu.make_async_copy(blk, blk, sems.at[35 + 3 * t + p]).wait()

    def chunk_start(t):
        sl = t & (NST - 1)
        pltpu.make_async_copy(wv_hbm.at[:, :, pl.ds(pl.multiple_of(8 * (t - 7), 8), 8), :],
                              pool.at[pl.ds(2 * sl, 2)], sems.at[sl]).start()

    def chunk_wait(t):
        sl = t & (NST - 1)
        blk = pool.at[pl.ds(2 * sl, 2)]
        pltpu.make_async_copy(blk, blk, sems.at[sl]).wait()

    def xb_copy(q):
        return pltpu.make_async_copy(ax_hbm.at[pl.ds(16 * q, 16), 3], xb3.at[pl.ds(16 * q, 16)], sems.at[8 + q])

    def bx_copy(q):
        return pltpu.make_async_copy(bx_hbm.at[:, pl.ds(2 * q, 2)], bx.at[:, pl.ds(2 * q, 2)], sems.at[12 + q])

    def w_copy(q, i):
        cols = pl.ds(pl.multiple_of(512 * q, 512), 512)
        return pltpu.make_async_copy((wr_hbm, wi_hbm)[i].at[:, cols], wf.at[q, i],
                                     sems.at[16 + 4 * i + q])

    def wo_copy(q, j):
        jt = 2 * j + (q >> 1)
        rows = pl.ds(pl.multiple_of((q & 1) * 512, 512), 512)
        return pltpu.make_async_copy(wo_hbm.at[:, rows, pl.ds(pl.multiple_of(128 * jt, 128), 128)],
                                     wo.at[jt, :, rows], sems.at[44 + q])

    cp_r0 = pltpu.make_async_copy(R_hbm.at[pl.ds(0, 8)], R.at[pl.ds(0, 8)], sems.at[25])
    cp_r1 = pltpu.make_async_copy(R_hbm.at[pl.ds(8, 8)], R.at[pl.ds(8, 8)], sems.at[26])
    cp_l = pltpu.make_async_copy(L_hbm, L, sems.at[27])
    cp_ax = pltpu.make_async_copy(ax_hbm.at[:, pl.ds(0, 3)], ax, sems.at[28])
    cp_outb = pltpu.make_async_copy(bx, out_hbm.at[:, :, :, pl.ds(DM, D)], sems.at[29])
    cp_sm = pltpu.make_async_copy(sm_hbm, sm, sems.at[30])
    cp_mem = pltpu.make_async_copy(mem_hbm, memb, sems.at[31])

    for part in range(4):
        part0_copy(part).start()
    xb_copy(0).start()
    for p in range(3):
        xb_copy(p + 1).start()
        part_start(1, p)
    for p in range(3):
        part_start(2, p)
    chunk_copy(3).start()
    cp_r0.start()
    bx_copy(0).start()
    w_copy(0, 0).start()
    w_copy(0, 1).start()
    cp_sm.start()
    cp_mem.start()

    def kc(rep=2):
        return [jnp.concatenate([sm[112 + 8 * i:120 + 8 * i, :]] * rep, axis=0) for i in range(12)]

    def roll64(v):
        return pltpu.roll(v, 64, 1)

    def prep(t, tpar, jj):
        lo = [bx[2 * jj:2 * jj + 2, t, :, 128 * e:128 * (e + 1)].astype(f32).reshape(16, 128) for e in range(8)]
        hi = [bx[HR + 2 * jj:HR + 2 * jj + 2, t, :, 128 * e:128 * (e + 1)].astype(f32).reshape(16, 128)
              for e in range(8)]
        for par in range(2):
            x = [lo[e] + hi[e] if par == 0 else lo[e] - hi[e] for e in range(8)]
            uu = _dstage(x, kc(), roll64)
            for q in range(8):
                o = (((tpar * 2 + par) * 8 + q) * 8 + jj) * 2
                pool[BU, o:o + 2] = uu[q].reshape(2, 8, 128).astype(bf16)

    def unit1(t, tpar, par, cg):
        o = ((tpar * 2 + par) * 8 + 2 * cg) * 16
        za = _dot(pool[BU, o:o + 16].reshape(128, 128), _asbf(R[2 * cg]))
        zb = _dot(pool[BU, o + 16:o + 32].reshape(128, 128), _asbf(R[2 * cg + 1]))
        ina = _in_a(lane8, cg)
        v = []
        for j in range(HR):
            pa, pb = za[8 * j:8 * j + 8], zb[8 * j:8 * j + 8]
            v.append((jnp.where(ina, pa, pb), pltpu.roll(jnp.where(ina, pb, pa), _RHO[cg], 1)))
        if cg == 0:
            V = nv[8 * tpar:8 * tpar + 8, :]
            for j in range(HR):
                vb = jnp.broadcast_to(v[j][1][:, 0:1], (8, 128))
                V = jnp.where(lane8 == 64 * par + 4 * j + (t >> 1), vb, V)
                v[j] = (v[j][0], jnp.where(lane8 == 0, 0.0, v[j][1]))
            nv[8 * tpar:8 * tpar + 8, :] = V
        if par == 1:
            v = [_tw(v[j], j, -1) for j in range(HR)]
        o = _fft(v, -1)
        for m in range(HR):
            Y[t >> 1, 2 * m + par, cg, tpar] = jnp.concatenate(o[m], axis=0).astype(bf16)

    def wprep(q, k, i):
        w = wf.at[q, i]
        cols = slice(128 * k, 128 * (k + 1))
        sub = lax.broadcasted_iota(i32, (8, 128), 0)
        msk = (jnp.where(sub % 2 == 0, jnp.uint32(0xffff), jnp.uint32(0))
               | jnp.where((sub % 4 == 0) | (sub % 4 == 3), jnp.uint32(0xffff0000), jnp.uint32(0)))
        t0 = pltpu.bitcast(w[0:256, cols], u32)
        t1 = pltpu.bitcast(w[256:512, cols], u32)
        ps, qs = [], []
        for j in range(16):
            a = t0[8 * j:8 * j + 8]
            b = t1[8 * j:8 * j + 8]
            b = jnp.where(sub % 2 == 0, pltpu.roll(b, 7, 0), pltpu.roll(b, 1, 0))
            x = (a ^ b) & msk
            ps.append(b ^ x)
            qs.append(a ^ x)
        for h, lst in enumerate((ps, qs)):
            tr = pltpu.bitcast(pltpu.bitcast(jnp.concatenate(lst, axis=0), f32).T, u32)
            r0 = pl.multiple_of((4 * q + k) * 32, 32)
            for j in range(4):
                for o in range(4):
                    wp[i, h, o, pl.ds(r0 + 8 * j, 8), :] = tr[32 * j + 8 * o:32 * j + 8 * o + 8]

    def fwd(p):
        return _dot(_asbf(L[p]), jnp.concatenate([Y[:, p, cg].reshape(128, 128) for cg in range(4)], axis=1))

    def filt(q, po, v):
        grs, gis = [None] * 4, [None] * 4
        for h in range(2):
            wr_ = wp[0, h, q, pl.ds(po, BS, stride=8), :]
            wi_ = wp[1, h, q, pl.ds(po, BS, stride=8), :]
            for hi in range(2):
                cg = 2 * h + hi
                if hi == 0:
                    a, b = wr_ << 16, wi_ << 16
                else:
                    a, b = wr_ & jnp.uint32(0xffff0000), wi_ & jnp.uint32(0xffff0000)
                grs[cg], gis[cg] = _cm(v[:BS, 128 * cg:128 * (cg + 1)], v[BS:, 128 * cg:128 * (cg + 1)],
                                       pltpu.bitcast(a, f32), pltpu.bitcast(b, f32))
        return jnp.concatenate([jnp.concatenate(grs, axis=1), jnp.concatenate(gis, axis=1)], axis=0).astype(bf16)

    def inv(p, g):
        t = _dot(_asbf(L[RS + p]), g)
        for cg in range(4):
            T[cg, p, 0:128, :] = t[:, 128 * cg:128 * (cg + 1)]

    nyq = {}

    def nyq_stage(k):
        n0 = 2 * RS
        twr, twi = sm[80:96, :], sm[96:112, :]
        if k == 0:
            v = nv[0:16, :].astype(bf16)
            r, i = _cm(_dot(v, _asbf(L[n0])), _dot(v, _asbf(L[n0 + 1])), twr, twi)
            nyq[0] = jnp.concatenate([r, i], axis=0).astype(bf16)
        elif k == 1:
            t = _dot(_asbf(L[n0 + 4, 0:16])[:, 0:32], nyq[0])
            ws = []
            for i in range(2):
                rows = [wf[j, i, 512:513, :].astype(f32) for j in range(4)]
                ws.append(jnp.concatenate([rows[r // 4][:, 128 * (r % 4):128 * (r % 4 + 1)] for r in range(16)], axis=0))
            r, i = _cm(t[:16], t[16:], ws[0], ws[1])
            nyq[1] = jnp.concatenate([r, i], axis=0).astype(bf16)
        elif k == 2:
            t = _dot(_asbf(L[n0 + 4, 16:32])[:, 0:32], nyq[1])
            r, i = _cm(t[:16], t[16:], twr, -twi)
            nyq[2] = (r.astype(bf16), i.astype(bf16))
        elif k == 3:
            nv[16:32, :] = _dot(nyq[2][0], _asbf(L[n0 + 2])) + _dot(nyq[2][1], _asbf(L[n0 + 3]))

    def p3a(t, tpar, par, cg):
        r0 = pl.multiple_of((t >> 1) * 32, 32)
        rr = pl.ds(r0 + 8 * tpar, 8)
        ri = pl.ds(r0 + 16 + 8 * tpar, 8)
        o = _fft([(T[cg, 2 * m + par, rr, :], T[cg, 2 * m + par, ri, :]) for m in range(HR)], +1)
        if par == 1:
            o = [_tw(o[j], j, +1) for j in range(HR)]
        if cg == 0:
            un = nv[16 + 8 * tpar:24 + 8 * tpar, :]
            o = [(o[j][0], jnp.where(lane8 == 0, pltpu.roll(un, (128 - 64 * par - 4 * j - (t >> 1)) & 127, 1),
                                     o[j][1])) for j in range(HR)]
        ina = _in_a(lane8, cg)
        ua, ub = [], []
        for re, im in o:
            im = pltpu.roll(im, 128 - _RHO[cg], 1)
            ua.append(jnp.where(ina, re, im))
            ub.append(jnp.where(ina, im, re))
        for j in range(HR // 2):
            for h, x in enumerate((ua, ub)):
                o = ((tpar * 2 + par) * 8 + 2 * cg + h) * 16 + 2 * j
                pool[BU + 1, o:o + 2] = jnp.concatenate(x[2 * j:2 * j + 2], axis=0).reshape(2, 8, 128).astype(bf16)

    def p3b(tpar, par, cg):
        zs = []
        for h in range(2):
            o = ((tpar * 2 + par) * 8 + 2 * cg + h) * 16
            zs.append((o, _dot(pool[BU + 1, o:o + 16].reshape(128, 128), _asbf(R[8 + 2 * cg + h]))))
        return zs

    def p3s(zs):
        for o, z in zs:
            pool[BU, o:o + 16] = z.reshape(16, 8, 128).astype(bf16)

    def p3c(t, tpar, j):
        res = [_dstage_t([pool[BU, ((tpar * 2 + par) * 8 + q) * 16 + j].astype(f32) for q in range(8)],
                         kc(1), roll64) for par in range(2)]
        for e in range(8):
            cols = slice(128 * e, 128 * (e + 1))
            bx[j, t, :, cols] = (res[0][e] + res[1][e]).astype(bf16)
            bx[HR + j, t, :, cols] = (res[0][e] - res[1][e]).astype(bf16)

    def wsum(jt, q, n):
        rows = pl.ds(pl.multiple_of(q * 256, 256) + 16 * n, 16)

        def ld(k, j):
            v = wo[2 * j + jt, k, rows, :]
            if (k, j) in RAW32:
                w32[RAW32.index((k, j)), jt, pl.ds(pl.multiple_of(q * 128, 128) + 8 * n, 8), :] = pltpu.bitcast(v, u32)
            return v.astype(f32)

        def st(i, v):
            pool[BC + i // 2, pl.ds((i % 2) * 256 + jt * 128 + q * 32 + 2 * n, 2)] = v.reshape(2, 8, 128).astype(bf16)
        col, row = {}, {}
        for k in range(4):
            d = -ld(k, k)
            col[k] = col[k] + d if k in col else d
            row[k] = row[k] + d if k in row else d
            for j in range(k + 1, 4):
                bkj, bjk = ld(k, j), ld(j, k)
                st(8 + PAIRS.index((k, j)), bjk - bkj)
                col[k], row[k] = col[k] - bjk, row[k] - bkj
                col[j] = col[j] - bkj if j in col else -bkj
                row[j] = row[j] - bjk if j in row else -bjk
            st(k, col[k])
            st(4 + k, row[k])

    def wc(i):
        o = (i % 2) * 256
        return jnp.concatenate([pool[BC + i // 2, o + 128 * jt:o + 128 * (jt + 1)].reshape(DM, 128)
                                for jt in range(2)], axis=1)

    def runit(b0, d0, dst, k):
        a = pltpu.bitcast(jnp.concatenate([pool[b0, d0 + 2 * k], pool[b0 + 1, d0 + 2 * k]], axis=0), u32)
        b = pltpu.bitcast(jnp.concatenate([pool[b0, d0 + 2 * k + 1], pool[b0 + 1, d0 + 2 * k + 1]], axis=0), u32)
        dst[pl.ds(k, 8, stride=PW), :] = (a & jnp.uint32(0xffff)) | (b << 16)
        dst[pl.ds(8 * PW + k, 8, stride=PW), :] = (a >> 16) | (b & jnp.uint32(0xffff0000))

    def wsel(w, hl, lo=0, hi=DM):
        base = ((hl % 2) * 8 + hl // 2) * PW
        parts = []
        for kh in range(2):
            a, b = max(lo, 512 * kh), min(hi, 512 * (kh + 1))
            if a < b:
                o = base + 4 * PW * kh - 256 * kh
                parts.append(w[o + a // 2:o + b // 2, :])
        return _asbf(jnp.concatenate(parts, axis=0))

    def bulk(t, mc0, nmc, tsrc, tdst, k0, nk, side=None):
        w = wpk.at[t]
        b0 = 2 * (tsrc & (NST - 1))
        dst = wpk.at[tdst, pl.ds(k0, 15 * PW + nk)]
        bq = 2 * NST + (t & 31)
        ns = 8 * nmc
        per = nk // ns
        for mi in range(nmc):
            mc = mc0 + mi
            x = _asbf(xb[mc])
            for h in range(8):
                n = mi * 8 + h
                r = _dot(x, wsel(w, h)).reshape(16, M, DH)
                nn = (n - 1) % ns
                for k in range(per * nn, per * (nn + 1)):
                    runit(b0, 2 * k0, dst, k)
                if side is not None:
                    side(n)
                rb = r.astype(bf16)
                for gi in range(4):
                    pool[bq, pl.ds(mc * 128 + gi * 32 + h * 4, 4)] = rb[4 * gi:4 * gi + 4]

    def rel0(i, c):
        @pl.when(i % 2 == 0)
        def _():
            part0_copy(i >> 1).wait()
        dst = wpk.at[0, pl.ds(pl.multiple_of(i * 32, 32), 15 * PW + 32)]
        for k in range(32):
            runit(0, i * 64, dst, k)
        return c
    with jax.named_scope("rel0"):
        lax.fori_loop(0, 8, rel0, 0)

    def body0(i, c):
        t, mc = i >> 2, i & 3
        real = mc >= 1

        @pl.when(t == 0)
        def _():
            xb_copy(mc).wait()
            xb[mc] = pltpu.bitcast(xb3[pl.ds(16 * mc, 16)].reshape(128, DM), u32)

        @pl.when(real)
        def _():
            part_wait(t + 1, mc - 1)
        with jax.named_scope("bulk0"):
            bulk(t, mc, 1, jnp.where(real, t + 1, t), jnp.where(real, t + 1, NCH),
                 pl.multiple_of(jnp.clip((mc - 1) * NK0, 0, 256 - NK0), math.gcd(NK0, 32)), NK0)

        @pl.when(i == 0)
        def _():
            chunk_copy(4).start()
            bx_copy(1).start()
            w_copy(1, 0).start()
            w_copy(1, 1).start()

        @pl.when(i == 4)
        def _():
            chunk_copy(5).start()
        return c
    lax.fori_loop(0, 8, body0, 0)
    bx_copy(2).start()
    w_copy(2, 0).start()
    w_copy(2, 1).start()
    chunk_copy(6).start()
    bx_copy(3).start()
    w_copy(3, 0).start()
    w_copy(3, 1).start()
    cp_l.start()
    cp_r1.start()
    nv[0:16, :] = jnp.zeros((16, 128), f32)
    cp_r0.wait()
    cp_sm.wait()

    def body1(q, c):
        t = q + 2
        with jax.named_scope("w_1"):
            chunk_wait(t + 1)
            bx_copy(q).wait()
            w_copy(q, 0).wait()
            w_copy(q, 1).wait()

        def side(n):
            for k in ([0, 1] if n == 0 else [n + 1]):
                if k < 16:
                    prep(2 * q + k // 8, k // 8, k % 8)
            k = n - 15
            if 0 <= k < 16:
                unit1(2 * q + k // 8, k // 8, (k // 4) % 2, k % 4)
            k, r = divmod(n - 1, 2)
            if r == 0 and 0 <= k < 8:
                wprep(q, k // 2, k % 2)
        with jax.named_scope("bulk_p1"):
            bulk(t, 0, 4, t + 1, t + 1, 0, 256, side)
        for j in range(4):
            wo_copy(q, j).start()
        chunk_start(t + 1 + NST)
        return c
    lax.fori_loop(0, 4, body1, 0)

    cp_ax.start()
    with jax.named_scope("w_l"):
        cp_l.wait()
        cp_r1.wait()

    def body2(q, c):
        t, hf = (q >> 1) + 6, q & 1

        @pl.when(hf == 0)
        def _():
            with jax.named_scope("w_2"):
                chunk_wait(t + 1)
                for j in range(4):
                    wo_copy(q >> 1, j).wait()
        gs = {}
        fs = [0, 1, 3, 5, 7, 9, 11, 13]

        def side(n):
            if n - 2 in fs:
                po = fs.index(n - 2)
                inv(8 * q + po, gs.pop(po))
            if n in fs:
                po = fs.index(n)
                gs[po] = filt(q, po, fwd(8 * q + po))
            k, r = divmod(n - 1, 3)
            if r == 0 and 0 <= k < 4:
                nyq_stage(k)
            for hh in range(16 * n // 15, min(16, 16 * (n + 1) // 15)):
                wsum(0, q, hh)
        with jax.named_scope("bulk_p2"):
            bulk(t, 2 * hf, 2, t + 1, t + 1, pl.multiple_of(hf * 128, 128), 128, side)
        return c
    lax.fori_loop(0, 4, body2, 0)
    chunk_copy(11).start()
    for q in (2, 3):
        for j in range(4):
            wo_copy(q, j).wait()

    def body3(q, c):
        t = q + 8

        @pl.when(q < 3)
        def _():
            with jax.named_scope("w_3"):
                chunk_wait(t + 1)
        us = {}

        def side(n):
            if n < 16:
                p3a(2 * q + n // 8, n // 8, (n // 4) % 2, n % 4)
            k = n - 3
            if 0 <= k < 16:
                us[k] = p3b(k // 8, (k // 4) % 2, k % 4)
            k = n - 3 - 1
            if 0 <= k < 16:
                p3s(us.pop(k))
            k = n - 16
            if 0 <= k < 16:
                p3c(2 * q + k // 8, k // 8, 2 * (k % 8))
                p3c(2 * q + k // 8, k // 8, 2 * (k % 8) + 1)
            if n < 16:
                wsum(1, q, n)
        with jax.named_scope("bulk_p3"):
            bulk(t, 0, 4, t + 1, t + 1, 0, 256, side)
        return c
    lax.fori_loop(0, 4, body3, 0)
    cp_outb.start()

    with jax.named_scope("w_wo"):
        cp_ax.wait()
        cp_mem.wait()
    scale = DH ** -0.5
    KS = 640

    def step(it, u):
        s = it * U + u
        lhs = jnp.concatenate([ax[s].reshape(FR, DM), memb[...]], axis=0)
        qs, ks, vs, ps, os_, pre = {}, {}, {}, {}, {}, {}

        def ws(m, h, lo=0, hi=DM):
            return wsel(wpk.at[CHUNKS.index((m, h // 8))], h % 8, lo, hi)
        if u > 0:
            for m in range(2):
                for h in range(2):
                    pre[(m, h)] = -_dot(lhs[:, :KS], ws(m, h, 0, KS))

        def dotw(m, h):
            if (m, h) in pre:
                return _dot(lhs[:, KS:], ws(m, h, KS, DM)) - pre[(m, h)]
            return _dot(lhs, ws(m, h))

        def proj(m, g):
            h = 2 * g
            bq = 2 * NST + CHUNKS.index((m, h // 8))
            return jnp.concatenate([dotw(m, h), dotw(m, h + 1),
                                    pool[bq, it * 32 + (h % 8) * 4 + u].astype(f32),
                                    pool[bq, it * 32 + (h % 8 + 1) * 4 + u].astype(f32)], axis=0).astype(bf16)

        def qk(g):
            sc = lax.dot_general(qs.pop(g), ks.pop(g), (((1,), (1,)), ((), ())),
                                 preferred_element_type=f32) * scale
            fill = sm[0:80, 0:80]
            sc = jnp.where(fill == 0.0, sc, fill)
            mx = jnp.max(sc, axis=-1, keepdims=True)
            e = jnp.exp(sc - mx)
            l = jnp.sum(e, axis=-1, keepdims=True)
            r = pl.reciprocal(l, approx=True)
            r = r * (2.0 - l * r)
            ps[g] = (e * r).astype(bf16)

        def pv(g):
            o = _dot(ps.pop(g), vs.pop(g))
            os_[2 * g] = o[0:32]
            os_[2 * g + 1] = o[32:64]
            ob[8 * u:8 * u + 8, (2 * g) * DH:(2 * g + 1) * DH] = o[64:72]
            ob[8 * u:8 * u + 8, (2 * g + 1) * DH:(2 * g + 2) * DH] = o[72:80]

        def olhs(lo, hi):
            return jnp.concatenate([os_[h] for h in range(lo, hi)], axis=1)

        def put(j, r, rb):
            cols = slice(j * 128, (j + 1) * 128)
            oa[it * 2 + u // 2, pl.ds((u % 2) * 4, 3), :, cols] = r[0:FR].reshape(3, 8, 128).astype(bf16)
            memb[:, cols] = r[FR:SEG].astype(bf16)
            if rb is not None:
                for uu in range(U):
                    oa[it * 2 + uu // 2, (uu % 2) * 4 + 3, :, cols] = rb[8 * uu:8 * uu + 8].astype(bf16)

        sk, dq, dp = 7, 3, 5
        for t in range(G + sk):
            if t < G:
                qs[t] = proj(0, t)
            if 0 <= t - dq < G:
                qk(t - dq)
            if t < G:
                ks[t] = proj(1, t)
            if t - sk - dp >= 0:
                pv(t - sk - dp)
            if t - sk >= 0:
                vs[t - sk] = proj(2, t - sk)
        rem = list(range(G - dp, G))
        if u < U - 1:
            acc = []
            oc = olhs(0, 16).astype(bf16)
            for j in range(8):
                acc.append(-_dot(oc, wo[j, 0:2].reshape(2 * DM, 128)))
                if rem:
                    pv(rem.pop(0))
            oc = olhs(16, 32).astype(bf16)
            for j in range(8):
                put(j, _dot(oc, wo[j, 2:4].reshape(2 * DM, 128)) - acc[j], None)
            return
        xs, ls, pr = {}, {}, {}

        def raw(k, j):
            if (k, j) in RAW32:
                return jnp.concatenate([_asbf(w32[RAW32.index((k, j)), jt]) for jt in range(2)], axis=1)
            return jnp.concatenate([wo[2 * j, k], wo[2 * j + 1, k]], axis=1)

        def x(j):
            if j not in xs:
                assert not rem or rem[0] >= 4 * (j + 1)
                xs[j] = olhs(8 * j, 8 * j + 8), ob[:, j * DM:(j + 1) * DM]
            return xs[j]

        def lh(k, j):
            if (k, j) not in ls:
                d1, d2 = x(j)[0] - x(k)[0], x(j)[1] - x(k)[1]
                ljk = d1 + CF[k] * d2
                ls[(k, j)] = d1 + CF[j] * d2, ljk, ljk + (CF[j] - CF[k]) * x(j)[1]
            return ls[(k, j)]

        order = "e0 d0 a01 b01 a02 b02 a12 b12 e1 d1 h01 e2 d2 h02 h12 e3 a03 b03 h03 a13 b13 h13 a23 b23 h23 d3"
        for name in order.split():
            k, j = int(name[1]), int(name[-1])
            if name[0] == "e":
                l, w = x(j)[1], wc(4 + j)
            elif name[0] == "d":
                l, w = x(j)[0] + CF[j] * x(j)[1], wc(j)
            elif name[0] == "a":
                l, w = lh(k, j)[0], raw(k, j)
            elif name[0] == "b":
                l, w = lh(k, j)[1], raw(j, k)
            else:
                l, w = lh(k, j)[2], wc(8 + PAIRS.index((k, j)))
            pr[name] = _dot(l.astype(bf16), w)
            if rem:
                pv(rem.pop(0))
        pa = [-pr["d%d" % j] for j in range(4)]
        qa = [-pr["e%d" % j] for j in range(4)]
        for k, j in PAIRS:
            ga, gb, hh = (pr["%s%d%d" % (c, k, j)] for c in "abh")
            w = ((gb - ga) - hh) * (1.0 / (CF[j] - CF[k]))
            pa[j], pa[k] = pa[j] - ga, pa[k] + gb
            qa[j], qa[k] = qa[j] + w, qa[k] - w
        for j in range(4):
            c1 = pa[j] - CF[j] * qa[j]
            for jt in range(2):
                put(2 * j + jt, c1[:, 128 * jt:128 * (jt + 1)], qa[j][:, 128 * jt:128 * (jt + 1)])

    def out_copy(it):
        return pltpu.make_async_copy(oa.at[pl.ds(it * 2, 2)],
                                     out_hbm.at[pl.ds(it * 2, 2), :, :, pl.ds(0, DM)], sems.at[32])

    def group(it, c):
        with jax.named_scope("grp"):
            for u in range(U):
                step(it, u)
        out_copy(it).start()
        return c
    lax.fori_loop(0, NSEG // U, group, 0)
    with jax.named_scope("w_out"):
        for it in range(NSEG // U):
            out_copy(it).wait()
        cp_outb.wait()


def pallas_concat_heads__memory_aug_recurrent_mem_tr__spectral_gfnet__prompt_kernel(
    A_x, A_mem0, A_Wq, A_Wk, A_Wv, A_Wo, A_seg_len, B_x, B_w_r, B_w_i,
):
    if isinstance(A_seg_len, int):
        assert A_seg_len == SEG
    R, LN, TW, fill, KC = _tables()
    small = np.zeros((208, 128), np.float32)
    small[:80, :80] = fill
    small[80:112] = TW
    small[112:] = np.repeat(KC, 8, axis=0)
    hbm = pl.BlockSpec(memory_space=pl.ANY)
    out = pl.pallas_call(
        _kernel,
        out_shape=jax.ShapeDtypeStruct((RS, 8, 8, DM + D), bf16),
        in_specs=[hbm] * 12,
        out_specs=hbm,
        scratch_shapes=[
            pltpu.VMEM((NSEG, 3, 8, DM), bf16),
            pltpu.VMEM((NSEG, 8, DM), bf16),
            pltpu.VMEM((4, 64, DM), u32),
            pltpu.VMEM((DM // 128, 4, DM, 128), bf16),
            pltpu.VMEM((6, 2, DM // 2, 128), u32),
            pltpu.VMEM((BC + 7, DM // 2, 8, DH), bf16),
            pltpu.VMEM((NCH + 1, 16 * PW, DH), u32),
            pltpu.VMEM((M, DM), bf16),
            pltpu.VMEM((U * M, H * DH), f32),
            pltpu.VMEM((RS, 8, 8, DM), bf16),
            pltpu.VMEM((RS, 8, 8, D), bf16),
            pltpu.VMEM((4, 2, D // 2 + 1, 512), bf16),
            pltpu.VMEM((16, 64, 128), u32),
            pltpu.VMEM((2 * RS + 5, 64, 128), u32),
            pltpu.VMEM((208, 128), f32),
            pltpu.VMEM((4, RS, 4, 2, 16, 128), bf16),
            pltpu.VMEM((4, RS, TP, 128), f32),
            pltpu.VMEM((2, 2, 4, BS * 8, 128), u32),
            pltpu.VMEM((32, 128), f32),
            pltpu.SemaphoreType.DMA((48,)),
        ],
        compiler_params=pltpu.CompilerParams(vmem_limit_bytes=124 * 1024 * 1024,
                                             disable_bounds_checks=True, disable_semaphore_checks=True),
    )(A_x.reshape(NSEG, 4, 8, DM), A_mem0.reshape(M, DM),
      A_Wq.reshape(2, DM // 2, H, DH), A_Wk.reshape(2, DM // 2, H, DH), A_Wv.reshape(2, DM // 2, H, DH),
      A_Wo.reshape(4, DM, DM), B_x.reshape(RS, 8, 8, D), B_w_r.T, B_w_i.T,
      jnp.asarray(R), jnp.asarray(LN), jnp.asarray(small))
    return out.reshape(1, S, DM + D)
```

```python
import functools
import math

import jax
import jax.numpy as jnp
import numpy as np
from jax import lax
import jax.experimental.pallas as pl
import jax.experimental.pallas.tpu as pltpu

bf16, f32, u32, i32 = jnp.bfloat16, jnp.float32, jnp.uint32, jnp.int32

S, DM, H, DH, M, SEG = 2048, 1024, 32, 128, 8, 32
NSEG = S // SEG
FR = SEG - M
G = H // 2
U = 4
NCH = 12
NST = 4
PW = 260

D = 1024
RS, BS = 32, 64
HR = RS // 2
TP = 136
C8 = float(np.sqrt(0.5))


def _pack_rows(a):
    u = np.asarray(a, np.float32).astype(jnp.bfloat16).view(np.uint16).astype(np.uint32)
    return u[..., 0::2, :] | (u[..., 1::2, :] << 16)


_RHO = (2, 4, 4, 4)


def _in_a(lane, c):
    return (lane % 4 < 2) if c == 0 else ((lane + 2) % 8 < 4)


def _dstage(x, kc, roll64):
    a = [x[j] + x[j + 4] for j in range(4)]
    b = [x[j] - x[j + 4] for j in range(4)]
    t1 = (b[1] - b[3]) * C8
    t2 = (b[1] + b[3]) * C8
    s0, s1 = a[0] + a[2], a[1] + a[3]
    out = [s0 + s1, s0 - s1]
    for c, (u, v) in enumerate(((b[0] + t1, b[2] + t2), (a[0] - a[2], a[1] - a[3]), (b[0] - t1, b[2] - t2))):
        g = u * kc[4 * c] + v * kc[4 * c + 1]
        h = roll64(u * kc[4 * c + 2] + v * kc[4 * c + 3])
        out += [g + h, g - h]
    return out


def _dstage_t(p, kc, roll64):
    uv = []
    for c in range(3):
        g = p[2 + 2 * c] + p[3 + 2 * c]
        h = roll64(p[2 + 2 * c] - p[3 + 2 * c])
        uv.append((g * kc[4 * c] + h * kc[4 * c + 2], g * kc[4 * c + 1] + h * kc[4 * c + 3]))
    s0, s1 = p[0] + p[1], p[0] - p[1]
    a = [s0 + uv[1][0], s1 + uv[1][1], s0 - uv[1][0], s1 - uv[1][1]]
    t1 = (uv[0][0] - uv[2][0]) * C8
    t2 = (uv[0][1] - uv[2][1]) * C8
    b = [uv[0][0] + uv[2][0], t1 + t2, uv[0][1] + uv[2][1], t2 - t1]
    return [a[j] + b[j] for j in range(4)] + [a[j] - b[j] for j in range(4)]


@functools.lru_cache(maxsize=None)
def _tables():
    kcol = np.zeros((4, 128), np.int64)
    for l in range(128):
        i0, i1 = l, 128 + (l ^ 1)
        ev, o3 = l % 2 == 0, l % 4 in (0, 3)
        kcol[0, l] = 2 * (i0 if ev else i1)
        kcol[2, l] = 2 * (i1 if ev else i0)
        kcol[1, l] = 2 * (i0 if o3 else i1) + 1
        kcol[3, l] = 2 * (i1 if o3 else i0) + 1
    lanes = np.arange(128)
    lo = lanes < 64
    KC = np.zeros((12, 128))
    for c, sg in ((1, -1.0), (2, -1.0), (3, 1.0)):
        tr, ti = np.cos(2 * np.pi * c / 16), -np.sin(2 * np.pi * c / 16)
        KC[4 * c - 4] = np.where(lo, 1.0, ti)
        KC[4 * c - 3] = sg * np.where(lo, 0.0, tr)
        KC[4 * c - 2] = np.where(lo, 0.0, tr)
        KC[4 * c - 1] = sg * np.where(lo, 1.0, -ti)
    eye = np.eye(D)
    Bt = _dstage([eye[:, 128 * e:128 * (e + 1)] for e in range(8)], KC, lambda v: np.roll(v, 64, axis=1))
    d = np.arange(D)
    R = np.zeros((16, 128, 128))
    for c in range(4):
        rho = _RHO[c]
        inA = _in_a(lanes, c)
        ang = 2 * np.pi * (np.outer(d, kcol[c]) % D) / D
        fr, fi = np.cos(ang), -np.sin(ang)
        wr_, wi_ = np.full(128, 2.0), np.full(128, 2.0)
        if c == 0:
            fi[:, 0] = (-1.0) ** d
            wr_[0] = 1.0
            wi_[0] = 1.0
        fi, wi_ = np.roll(fi, -rho, axis=1), np.roll(wi_, -rho)
        for h in range(2):
            own = inA if h == 0 else ~inA
            ft, wt = np.where(own, fr, fi), np.where(own, wr_, wi_)
            bt = Bt[2 * c + h]
            r = (bt.T @ ft) / (bt * bt).sum(axis=0)[:, None]
            assert np.abs(bt @ r - ft).max() < 1e-9
            R[2 * c + h] = r
            R[8 + 2 * c + h] = (wt[:, None] * r.T) / (S * D)
    L = np.zeros((2 * RS, 128, 128))
    bb = np.arange(BS)
    kord = np.array([ri * 64 + 8 * t + r for t in range(8) for ri in range(2) for r in range(8)])
    rord = np.array([ri * 64 + 16 * q + r for q in range(4) for ri in range(2) for r in range(16)])
    for p1 in range(RS):
        ang = 2 * np.pi * (np.outer(p1 + RS * bb, bb) % S) / S
        mr, mi = np.cos(ang), -np.sin(ang)
        full = np.block([[mr, -mi], [mi, mr]])
        L[p1] = full[:, kord]
        L[RS + p1] = full.T[rord]
    l_, q_ = np.arange(128), np.arange(16)
    ang = 2 * np.pi * (np.outer(l_, l_) % 128) / 128
    N1 = np.concatenate([np.cos(ang), -np.sin(ang)], axis=1)
    N1 = np.concatenate([(N1[:64] + N1[64:]) / 2, (N1[:64] - N1[64:]) / 2], axis=0)
    ang = 2 * np.pi * np.outer(q_, l_) / S
    TW = np.concatenate([np.cos(ang), -np.sin(ang)], axis=0)
    ang = 2 * np.pi * (np.outer(q_, q_) % 16) / 16
    fr, fi = np.cos(ang), -np.sin(ang)
    F16 = np.block([[fr, -fi], [fi, fr]])
    NY = np.zeros((5, 128, 128))
    NY[0], NY[1], NY[2], NY[3] = N1[:, :128], N1[:, 128:], N1[:, :128].T, N1[:, 128:].T
    NY[4, :32, :32] = F16
    NY[4, 32:64, :32] = F16.T
    LN = np.concatenate([L, NY], axis=0)
    head = np.zeros(80, np.int32)
    pos = np.zeros(80, np.int32)
    for r in range(80):
        if r < 64:
            head[r] = r // 32
            t = r % 32
            pos[r] = (M + t) if t < FR else (t - FR)
        else:
            head[r] = (r - 64) // 8
            pos[r] = M + FR + (r - 64) % 8
    same = head[:, None] == head[None, :]
    vis = (pos[:, None] < M) | (pos[:, None] >= pos[None, :])
    fill = np.where(same, np.where(vis, 0.0, -1e9), -np.inf).astype(np.float32)
    return _pack_rows(R), _pack_rows(LN), TW.astype(np.float32), fill, KC.astype(np.float32)


def _cmul_const(re, im, j, n, sgn):
    ang = sgn * 2 * math.pi * j / n
    c, s = math.cos(ang), math.sin(ang)
    if abs(abs(c) - abs(s)) < 1e-12:
        if c * s > 0:
            return (re - im) * c, (re + im) * c
        return (re + im) * c, (im - re) * c
    return re * c - im * s, re * s + im * c


def _diff_tw(a, b, j, n, sgn):
    if j == 0:
        return a[0] - b[0], a[1] - b[1]
    if 4 * j == n:
        if sgn < 0:
            return a[1] - b[1], b[0] - a[0]
        return b[1] - a[1], a[0] - b[0]
    return _cmul_const(a[0] - b[0], a[1] - b[1], j, n, sgn)


def _tw(v, j, sgn):
    if j == 0:
        return v
    if 4 * j == RS:
        return (v[1], -v[0]) if sgn < 0 else (-v[1], v[0])
    return _cmul_const(v[0], v[1], j, RS, sgn)


def _fft(v, sgn):
    n = len(v)
    if n == 1:
        return v
    h = n // 2
    ev = _fft([(v[j][0] + v[j + h][0], v[j][1] + v[j + h][1]) for j in range(h)], sgn)
    od = _fft([_diff_tw(v[j], v[j + h], j, n, sgn) for j in range(h)], sgn)
    out = [None] * n
    out[0::2] = ev
    out[1::2] = od
    return out


def _dot(a, b):
    return jnp.dot(a, b, preferred_element_type=f32)


def _asbf(v):
    return pltpu.bitcast(v, bf16)


def _cm(ar, ai, br, bi):
    return ar * br - ai * bi, ar * bi + ai * br


CHUNKS = [(0, 0), (0, 1), (0, 2), (0, 3), (1, 0), (1, 1), (1, 2), (2, 0), (2, 1), (2, 2), (2, 3), (1, 3)]
BU = 2 * NST + NCH
BC = BU + 2
CF = (-1.2, -0.4, 0.4, 1.2)
PAIRS = [(k, j) for j in range(4) for k in range(j)]
RAW32 = [(0, 1), (1, 0), (0, 2), (2, 0), (1, 2), (2, 1)]


WP = 12
NK0 = 88


def _kernel(ax_hbm, mem_hbm, wq_hbm, wk_hbm, wv_hbm, wo_hbm, bx_hbm, wr_hbm, wi_hbm,
            R_hbm, L_hbm, sm_hbm, out_hbm,
            ax, xb3, xb, wo, pool, wpk, memb, ob, oa,
            bx, wf, R, L, sm, Y, T, wp, nv, sems):
    srcs = (wq_hbm, wk_hbm, wv_hbm)
    lane8 = lax.broadcasted_iota(i32, (8, 128), 1)

    def chunk_copy(t):
        m, c = CHUNKS[t]
        return pltpu.make_async_copy(srcs[m].at[:, :, pl.ds(8 * c, 8), :],
                                     pool.at[pl.ds(2 * (t % NST), 2)], sems.at[t % NST])

    def part0_copy(part):
        rows = pl.ds(pl.multiple_of(part * 128, 128), 128)
        return pltpu.make_async_copy(wq_hbm.at[:, rows, pl.ds(0, 8), :], pool.at[pl.ds(0, 2), rows], sems.at[34 + part])

    def part_start(t, part):
        lo = part * 2 * NK0
        n = min(2 * NK0, 512 - lo)
        pltpu.make_async_copy(wq_hbm.at[:, pl.ds(lo, n), pl.ds(8 * t, 8), :],
                              pool.at[pl.ds(2 * t, 2), pl.ds(lo, n)], sems.at[35 + 3 * t + part]).start()

    def part_wait(t, part):
        for p in range(3):
            lo = p * 2 * NK0
            n = min(2 * NK0, 512 - lo)

            @pl.when(part == p)
            def _(lo=lo, n=n, p=p):
                blk = pool.at[pl.ds(2 * t, 2), pl.ds(lo, n)]
                pltpu.make_async_copy(blk, blk, sems.at[35 + 3 * t + p]).wait()

    def chunk_start(t):
        sl = t & (NST - 1)
        pltpu.make_async_copy(wv_hbm.at[:, :, pl.ds(pl.multiple_of(8 * (t - 7), 8), 8), :],
                              pool.at[pl.ds(2 * sl, 2)], sems.at[sl]).start()

    def chunk_wait(t):
        sl = t & (NST - 1)
        blk = pool.at[pl.ds(2 * sl, 2)]
        pltpu.make_async_copy(blk, blk, sems.at[sl]).wait()

    def xb_copy(q):
        return pltpu.make_async_copy(ax_hbm.at[pl.ds(16 * q, 16), 3], xb3.at[pl.ds(16 * q, 16)], sems.at[8 + q])

    def bx_copy(q):
        return pltpu.make_async_copy(bx_hbm.at[:, pl.ds(2 * q, 2)], bx.at[:, pl.ds(2 * q, 2)], sems.at[12 + q])

    def w_copy(q, i):
        cols = pl.ds(pl.multiple_of(512 * q, 512), 512)
        return pltpu.make_async_copy((wr_hbm, wi_hbm)[i].at[:, cols], wf.at[q, i],
                                     sems.at[16 + 4 * i + q])

    def wo_copy(q, j):
        jt = 2 * j + (q >> 1)
        rows = pl.ds(pl.multiple_of((q & 1) * 512, 512), 512)
        return pltpu.make_async_copy(wo_hbm.at[:, rows, pl.ds(pl.multiple_of(128 * jt, 128), 128)],
                                     wo.at[jt, :, rows], sems.at[44 + q])

    cp_r0 = pltpu.make_async_copy(R_hbm.at[pl.ds(0, 8)], R.at[pl.ds(0, 8)], sems.at[25])
    cp_r1 = pltpu.make_async_copy(R_hbm.at[pl.ds(8, 8)], R.at[pl.ds(8, 8)], sems.at[26])
    cp_l = pltpu.make_async_copy(L_hbm, L, sems.at[27])
    cp_ax = pltpu.make_async_copy(ax_hbm.at[:, pl.ds(0, 3)], ax, sems.at[28])
    cp_outb = pltpu.make_async_copy(bx, out_hbm.at[:, :, :, pl.ds(DM, D)], sems.at[29])
    cp_sm = pltpu.make_async_copy(sm_hbm, sm, sems.at[30])
    cp_mem = pltpu.make_async_copy(mem_hbm, memb, sems.at[31])

    for part in range(4):
        part0_copy(part).start()
    xb_copy(0).start()
    for p in range(3):
        xb_copy(p + 1).start()
        part_start(1, p)
    for p in range(3):
        part_start(2, p)
    chunk_copy(3).start()
    cp_r0.start()
    bx_copy(0).start()
    w_copy(0, 0).start()
    w_copy(0, 1).start()
    cp_sm.start()
    cp_mem.start()

    def kc(rep=2):
        return [jnp.concatenate([sm[112 + 8 * i:120 + 8 * i, :]] * rep, axis=0) for i in range(12)]

    def roll64(v):
        return pltpu.roll(v, 64, 1)

    def prep(t, tpar, jj):
        lo = [bx[2 * jj:2 * jj + 2, t, :, 128 * e:128 * (e + 1)].astype(f32).reshape(16, 128) for e in range(8)]
        hi = [bx[HR + 2 * jj:HR + 2 * jj + 2, t, :, 128 * e:128 * (e + 1)].astype(f32).reshape(16, 128)
              for e in range(8)]
        for par in range(2):
            x = [lo[e] + hi[e] if par == 0 else lo[e] - hi[e] for e in range(8)]
            uu = _dstage(x, kc(), roll64)
            for q in range(8):
                o = (((tpar * 2 + par) * 8 + q) * 8 + jj) * 2
                pool[BU, o:o + 2] = uu[q].reshape(2, 8, 128).astype(bf16)

    def unit1(t, tpar, par, cg):
        o = ((tpar * 2 + par) * 8 + 2 * cg) * 16
        za = _dot(pool[BU, o:o + 16].reshape(128, 128), _asbf(R[2 * cg]))
        zb = _dot(pool[BU, o + 16:o + 32].reshape(128, 128), _asbf(R[2 * cg + 1]))
        ina = _in_a(lane8, cg)
        v = []
        for j in range(HR):
            pa, pb = za[8 * j:8 * j + 8], zb[8 * j:8 * j + 8]
            v.append((jnp.where(ina, pa, pb), pltpu.roll(jnp.where(ina, pb, pa), _RHO[cg], 1)))
        if cg == 0:
            V = nv[8 * tpar:8 * tpar + 8, :]
            for j in range(HR):
                vb = jnp.broadcast_to(v[j][1][:, 0:1], (8, 128))
                V = jnp.where(lane8 == 64 * par + 4 * j + (t >> 1), vb, V)
                v[j] = (v[j][0], jnp.where(lane8 == 0, 0.0, v[j][1]))
            nv[8 * tpar:8 * tpar + 8, :] = V
        if par == 1:
            v = [_tw(v[j], j, -1) for j in range(HR)]
        o = _fft(v, -1)
        for m in range(HR):
            Y[t >> 1, 2 * m + par, cg, tpar] = jnp.concatenate(o[m], axis=0).astype(bf16)

    def wprep(q, k, i):
        w = wf.at[q, i]
        cols = slice(128 * k, 128 * (k + 1))
        sub = lax.broadcasted_iota(i32, (8, 128), 0)
        msk = (jnp.where(sub % 2 == 0, jnp.uint32(0xffff), jnp.uint32(0))
               | jnp.where((sub % 4 == 0) | (sub % 4 == 3), jnp.uint32(0xffff0000), jnp.uint32(0)))
        t0 = pltpu.bitcast(w[0:256, cols], u32)
        t1 = pltpu.bitcast(w[256:512, cols], u32)
        ps, qs = [], []
        for j in range(16):
            a = t0[8 * j:8 * j + 8]
            b = t1[8 * j:8 * j + 8]
            b = jnp.where(sub % 2 == 0, pltpu.roll(b, 7, 0), pltpu.roll(b, 1, 0))
            x = (a ^ b) & msk
            ps.append(b ^ x)
            qs.append(a ^ x)
        for h, lst in enumerate((ps, qs)):
            tr = pltpu.bitcast(pltpu.bitcast(jnp.concatenate(lst, axis=0), f32).T, u32)
            r0 = pl.multiple_of(q * 16 * WP, 32)
            for j in range(4):
                for o in range(4):
                    wp[i, h, o, pl.ds(r0 + WP * (4 * k + j), 8), :] = tr[32 * j + 8 * o:32 * j + 8 * o + 8]

    def fwd(p):
        return _dot(_asbf(L[p]), jnp.concatenate([Y[:, p, cg].reshape(128, 128) for cg in range(4)], axis=1))

    def filt(q, po, v):
        grs, gis = [None] * 4, [None] * 4
        for h in range(2):
            wr_ = wp[0, h, q, pl.ds(po, BS, stride=WP), :]
            wi_ = wp[1, h, q, pl.ds(po, BS, stride=WP), :]
            for hi in range(2):
                cg = 2 * h + hi
                if hi == 0:
                    a, b = wr_ << 16, wi_ << 16
                else:
                    a, b = wr_ & jnp.uint32(0xffff0000), wi_ & jnp.uint32(0xffff0000)
                grs[cg], gis[cg] = _cm(v[:BS, 128 * cg:128 * (cg + 1)], v[BS:, 128 * cg:128 * (cg + 1)],
                                       pltpu.bitcast(a, f32), pltpu.bitcast(b, f32))
        return jnp.concatenate([jnp.concatenate(grs, axis=1), jnp.concatenate(gis, axis=1)], axis=0).astype(bf16)

    def inv(p, g):
        t = _dot(_asbf(L[RS + p]), g)
        for cg in range(4):
            T[cg, p, 0:128, :] = t[:, 128 * cg:128 * (cg + 1)]

    nyq = {}

    def nyq_stage(k):
        n0 = 2 * RS
        twr, twi = sm[80:96, :], sm[96:112, :]
        if k == 0:
            v = nv[0:16, :].astype(bf16)
            r, i = _cm(_dot(v, _asbf(L[n0])), _dot(v, _asbf(L[n0 + 1])), twr, twi)
            nyq[0] = jnp.concatenate([r, i], axis=0).astype(bf16)
        elif k == 1:
            t = _dot(_asbf(L[n0 + 4, 0:16])[:, 0:32], nyq[0])
            ws = []
            for i in range(2):
                rows = [wf[j, i, 512:513, :].astype(f32) for j in range(4)]
                ws.append(jnp.concatenate([rows[r // 4][:, 128 * (r % 4):128 * (r % 4 + 1)] for r in range(16)], axis=0))
            r, i = _cm(t[:16], t[16:], ws[0], ws[1])
            nyq[1] = jnp.concatenate([r, i], axis=0).astype(bf16)
        elif k == 2:
            t = _dot(_asbf(L[n0 + 4, 16:32])[:, 0:32], nyq[1])
            r, i = _cm(t[:16], t[16:], twr, -twi)
            nyq[2] = (r.astype(bf16), i.astype(bf16))
        elif k == 3:
            nv[16:32, :] = _dot(nyq[2][0], _asbf(L[n0 + 2])) + _dot(nyq[2][1], _asbf(L[n0 + 3]))

    def p3a(t, tpar, par, cg):
        r0 = pl.multiple_of((t >> 1) * 32, 32)
        rr = pl.ds(r0 + 8 * tpar, 8)
        ri = pl.ds(r0 + 16 + 8 * tpar, 8)
        o = _fft([(T[cg, 2 * m + par, rr, :], T[cg, 2 * m + par, ri, :]) for m in range(HR)], +1)
        if par == 1:
            o = [_tw(o[j], j, +1) for j in range(HR)]
        if cg == 0:
            un = nv[16 + 8 * tpar:24 + 8 * tpar, :]
            o = [(o[j][0], jnp.where(lane8 == 0, pltpu.roll(un, (128 - 64 * par - 4 * j - (t >> 1)) & 127, 1),
                                     o[j][1])) for j in range(HR)]
        ina = _in_a(lane8, cg)
        ua, ub = [], []
        for re, im in o:
            im = pltpu.roll(im, 128 - _RHO[cg], 1)
            ua.append(jnp.where(ina, re, im))
            ub.append(jnp.where(ina, im, re))
        for j in range(HR // 2):
            for h, x in enumerate((ua, ub)):
                o = ((tpar * 2 + par) * 8 + 2 * cg + h) * 16 + 2 * j
                pool[BU + 1, o:o + 2] = jnp.concatenate(x[2 * j:2 * j + 2], axis=0).reshape(2, 8, 128).astype(bf16)

    def p3b(tpar, par, cg):
        zs = []
        for h in range(2):
            o = ((tpar * 2 + par) * 8 + 2 * cg + h) * 16
            zs.append((o, _dot(pool[BU + 1, o:o + 16].reshape(128, 128), _asbf(R[8 + 2 * cg + h]))))
        return zs

    def p3s(zs):
        for o, z in zs:
            pool[BU, o:o + 16] = z.reshape(16, 8, 128).astype(bf16)

    def p3c(t, tpar, j):
        res = [_dstage_t([pool[BU, ((tpar * 2 + par) * 8 + q) * 16 + j].astype(f32) for q in range(8)],
                         kc(1), roll64) for par in range(2)]
        for e in range(8):
            cols = slice(128 * e, 128 * (e + 1))
            bx[j, t, :, cols] = (res[0][e] + res[1][e]).astype(bf16)
            bx[HR + j, t, :, cols] = (res[0][e] - res[1][e]).astype(bf16)

    def wsum(jt, q, n):
        rows = pl.ds(pl.multiple_of(q * 256, 256) + 16 * n, 16)

        def ld(k, j):
            v = wo[2 * j + jt, k, rows, :]
            if (k, j) in RAW32:
                r0 = pl.multiple_of(q * 128, 128) + 512 * RAW32.index((k, j)) + 8 * n
                wpk[NCH + 1 + jt, pl.ds(r0, 8), :] = pltpu.bitcast(v, u32)
            return v.astype(f32)

        def st(i, v):
            pool[BC + i // 2, pl.ds((i % 2) * 256 + jt * 128 + q * 32 + 2 * n, 2)] = v.reshape(2, 8, 128).astype(bf16)
        col, row = {}, {}
        for k in range(4):
            d = -ld(k, k)
            col[k] = col[k] + d if k in col else d
            row[k] = row[k] + d if k in row else d
            for j in range(k + 1, 4):
                bkj, bjk = ld(k, j), ld(j, k)
                st(8 + PAIRS.index((k, j)), bjk - bkj)
                col[k], row[k] = col[k] - bjk, row[k] - bkj
                col[j] = col[j] - bkj if j in col else -bkj
                row[j] = row[j] - bjk if j in row else -bjk
            st(k, col[k])
            st(4 + k, row[k])

    def wc(i):
        o = (i % 2) * 256
        return jnp.concatenate([pool[BC + i // 2, o + 128 * jt:o + 128 * (jt + 1)].reshape(DM, 128)
                                for jt in range(2)], axis=1)

    def runit(b0, d0, dst, k):
        a = pltpu.bitcast(jnp.concatenate([pool[b0, d0 + 2 * k], pool[b0 + 1, d0 + 2 * k]], axis=0), u32)
        b = pltpu.bitcast(jnp.concatenate([pool[b0, d0 + 2 * k + 1], pool[b0 + 1, d0 + 2 * k + 1]], axis=0), u32)
        dst[pl.ds(k, 8, stride=PW), :] = (a & jnp.uint32(0xffff)) | (b << 16)
        dst[pl.ds(8 * PW + k, 8, stride=PW), :] = (a >> 16) | (b & jnp.uint32(0xffff0000))

    def wsel(w, hl, lo=0, hi=DM):
        base = ((hl % 2) * 8 + hl // 2) * PW
        parts = []
        for kh in range(2):
            a, b = max(lo, 512 * kh), min(hi, 512 * (kh + 1))
            if a < b:
                o = base + 4 * PW * kh - 256 * kh
                parts.append(w[o + a // 2:o + b // 2, :])
        return _asbf(jnp.concatenate(parts, axis=0))

    def bulk(t, mc0, nmc, tsrc, tdst, k0, nk, side=None):
        w = wpk.at[t]
        b0 = 2 * (tsrc & (NST - 1))
        dst = wpk.at[tdst, pl.ds(k0, 15 * PW + 4 + nk)]
        bq = 2 * NST + (t & 31)
        ns = 8 * nmc
        per = nk // ns
        for mi in range(nmc):
            mc = mc0 + mi
            x = _asbf(xb[mc])
            for h in range(8):
                n = mi * 8 + h
                r = _dot(x, wsel(w, h)).reshape(16, M, DH)
                nn = (n - 1) % ns
                for k in range(per * nn, per * (nn + 1)):
                    runit(b0, 2 * k0, dst, k)
                if side is not None:
                    side(n)
                rb = r.astype(bf16)
                for gi in range(4):
                    pool[bq, pl.ds(mc * 128 + gi * 32 + h * 4, 4)] = rb[4 * gi:4 * gi + 4]

    def rel0(i, c):
        @pl.when(i % 2 == 0)
        def _():
            part0_copy(i >> 1).wait()
        dst = wpk.at[0, pl.ds(pl.multiple_of(i * 32, 32), 15 * PW + 36)]
        for k in range(32):
            runit(0, i * 64, dst, k)
        return c
    with jax.named_scope("rel0"):
        lax.fori_loop(0, 8, rel0, 0)

    def body0(i, c):
        t, mc = i >> 2, i & 3
        real = mc >= 1

        @pl.when(t == 0)
        def _():
            xb_copy(mc).wait()
            xb[mc] = pltpu.bitcast(xb3[pl.ds(16 * mc, 16)].reshape(128, DM), u32)

        @pl.when(real)
        def _():
            part_wait(t + 1, mc - 1)
        with jax.named_scope("bulk0"):
            bulk(t, mc, 1, jnp.where(real, t + 1, t), jnp.where(real, t + 1, NCH),
                 pl.multiple_of(jnp.clip((mc - 1) * NK0, 0, 256 - NK0), math.gcd(NK0, 32)), NK0)

        @pl.when(i == 0)
        def _():
            chunk_copy(4).start()
            bx_copy(1).start()
            w_copy(1, 0).start()
            w_copy(1, 1).start()

        @pl.when(i == 4)
        def _():
            chunk_copy(5).start()
        return c
    lax.fori_loop(0, 8, body0, 0)
    bx_copy(2).start()
    w_copy(2, 0).start()
    w_copy(2, 1).start()
    chunk_copy(6).start()
    bx_copy(3).start()
    w_copy(3, 0).start()
    w_copy(3, 1).start()
    cp_l.start()
    cp_r1.start()
    nv[0:16, :] = jnp.zeros((16, 128), f32)
    cp_r0.wait()
    cp_sm.wait()

    def body1(q, c):
        t = q + 2
        with jax.named_scope("w_1"):
            chunk_wait(t + 1)
            bx_copy(q).wait()
            w_copy(q, 0).wait()
            w_copy(q, 1).wait()

        def side(n):
            for k in ([0, 1] if n == 0 else [n + 1]):
                if k < 16:
                    prep(2 * q + k // 8, k // 8, k % 8)
            k = n - 15
            if 0 <= k < 16:
                unit1(2 * q + k // 8, k // 8, (k // 4) % 2, k % 4)
            k, r = divmod(n - 1, 2)
            if r == 0 and 0 <= k < 8:
                wprep(q, k // 2, k % 2)
        with jax.named_scope("bulk_p1"):
            bulk(t, 0, 4, t + 1, t + 1, 0, 256, side)
        for j in range(4):
            wo_copy(q, j).start()
        chunk_start(t + 1 + NST)
        return c
    lax.fori_loop(0, 4, body1, 0)

    cp_ax.start()
    with jax.named_scope("w_l"):
        cp_l.wait()
        cp_r1.wait()

    def body2(q, c):
        t, hf = (q >> 1) + 6, q & 1

        @pl.when(hf == 0)
        def _():
            with jax.named_scope("w_2"):
                chunk_wait(t + 1)
                for j in range(4):
                    wo_copy(q >> 1, j).wait()
        gs = {}
        fs = [0, 1, 3, 5, 7, 9, 11, 13]

        def side(n):
            if n - 2 in fs:
                po = fs.index(n - 2)
                inv(8 * q + po, gs.pop(po))
            if n in fs:
                po = fs.index(n)
                gs[po] = filt(q, po, fwd(8 * q + po))
            k, r = divmod(n - 1, 3)
            if r == 0 and 0 <= k < 4:
                nyq_stage(k)
            for hh in range(16 * n // 15, min(16, 16 * (n + 1) // 15)):
                wsum(0, q, hh)
        with jax.named_scope("bulk_p2"):
            bulk(t, 2 * hf, 2, t + 1, t + 1, pl.multiple_of(hf * 128, 128), 128, side)
        return c
    lax.fori_loop(0, 4, body2, 0)
    chunk_copy(11).start()
    for q in (2, 3):
        for j in range(4):
            wo_copy(q, j).wait()

    def body3(q, c):
        t = q + 8

        @pl.when(q < 3)
        def _():
            with jax.named_scope("w_3"):
                chunk_wait(t + 1)
        us = {}

        def side(n):
            if n < 16:
                p3a(2 * q + n // 8, n // 8, (n // 4) % 2, n % 4)
            k = n - 3
            if 0 <= k < 16:
                us[k] = p3b(k // 8, (k // 4) % 2, k % 4)
            k = n - 3 - 1
            if 0 <= k < 16:
                p3s(us.pop(k))
            k = n - 16
            if 0 <= k < 16:
                p3c(2 * q + k // 8, k // 8, 2 * (k % 8))
                p3c(2 * q + k // 8, k // 8, 2 * (k % 8) + 1)
            k, r = divmod(n - 0, 1)
            if r == 0 and 0 <= k < 16:
                wsum(1, q, k)
        with jax.named_scope("bulk_p3"):
            bulk(t, 0, 4, t + 1, t + 1, 0, 256, side)
        return c
    lax.fori_loop(0, 4, body3, 0)
    cp_outb.start()

    with jax.named_scope("w_wo"):
        cp_ax.wait()
        cp_mem.wait()
    scale = DH ** -0.5
    KS = 640

    def step(it, u):
        s = it * U + u
        lhs = jnp.concatenate([ax[s].reshape(FR, DM), memb[...]], axis=0)
        qs, ks, vs, ps, os_, pre = {}, {}, {}, {}, {}, {}

        def ws(m, h, lo=0, hi=DM):
            return wsel(wpk.at[CHUNKS.index((m, h // 8))], h % 8, lo, hi)
        if u > 0:
            for m in range(2):
                for h in range(2):
                    pre[(m, h)] = -_dot(lhs[:, :KS], ws(m, h, 0, KS))

        def dotw(m, h):
            if (m, h) in pre:
                return _dot(lhs[:, KS:], ws(m, h, KS, DM)) - pre[(m, h)]
            return _dot(lhs, ws(m, h))

        def proj(m, g):
            h = 2 * g
            bq = 2 * NST + CHUNKS.index((m, h // 8))
            return jnp.concatenate([dotw(m, h), dotw(m, h + 1),
                                    pool[bq, it * 32 + (h % 8) * 4 + u].astype(f32),
                                    pool[bq, it * 32 + (h % 8 + 1) * 4 + u].astype(f32)], axis=0).astype(bf16)

        def qk(g):
            sc = lax.dot_general(qs.pop(g), ks.pop(g), (((1,), (1,)), ((), ())),
                                 preferred_element_type=f32) * scale
            fill = sm[0:80, 0:80]
            sc = jnp.where(fill == 0.0, sc, fill)
            mx = jnp.max(sc, axis=-1, keepdims=True)
            e = jnp.exp(sc - mx)
            l = jnp.sum(e, axis=-1, keepdims=True)
            r = pl.reciprocal(l, approx=True)
            r = r * (2.0 - l * r)
            ps[g] = (e * r).astype(bf16)

        def pv(g):
            o = _dot(ps.pop(g), vs.pop(g))
            os_[2 * g] = o[0:32]
            os_[2 * g + 1] = o[32:64]
            ob[8 * u:8 * u + 8, (2 * g) * DH:(2 * g + 1) * DH] = o[64:72]
            ob[8 * u:8 * u + 8, (2 * g + 1) * DH:(2 * g + 2) * DH] = o[72:80]

        def olhs(lo, hi):
            return jnp.concatenate([os_[h] for h in range(lo, hi)], axis=1)

        def put(j, r, rb):
            cols = slice(j * 128, (j + 1) * 128)
            oa[it * 2 + u // 2, pl.ds((u % 2) * 4, 3), :, cols] = r[0:FR].reshape(3, 8, 128).astype(bf16)
            memb[:, cols] = r[FR:SEG].astype(bf16)
            if rb is not None:
                for uu in range(U):
                    oa[it * 2 + uu // 2, (uu % 2) * 4 + 3, :, cols] = rb[8 * uu:8 * uu + 8].astype(bf16)

        sk, dq, dp = 7, 3, 5
        for t in range(G + sk):
            if t < G:
                qs[t] = proj(0, t)
            if 0 <= t - dq < G:
                qk(t - dq)
            if t < G:
                ks[t] = proj(1, t)
            if t - sk - dp >= 0:
                pv(t - sk - dp)
            if t - sk >= 0:
                vs[t - sk] = proj(2, t - sk)
        rem = list(range(G - dp, G))
        if u < U - 1:
            acc = []
            oc = olhs(0, 16).astype(bf16)
            for j in range(8):
                acc.append(-_dot(oc, wo[j, 0:2].reshape(2 * DM, 128)))
                if rem:
                    pv(rem.pop(0))
            oc = olhs(16, 32).astype(bf16)
            for j in range(8):
                put(j, _dot(oc, wo[j, 2:4].reshape(2 * DM, 128)) - acc[j], None)
            return
        xs, ls, pr = {}, {}, {}

        def raw(k, j):
            if (k, j) in RAW32:
                o = 512 * RAW32.index((k, j))
                return jnp.concatenate([_asbf(wpk[NCH + 1 + jt, o:o + 512, :]) for jt in range(2)], axis=1)
            return jnp.concatenate([wo[2 * j, k], wo[2 * j + 1, k]], axis=1)

        def x(j):
            if j not in xs:
                assert not rem or rem[0] >= 4 * (j + 1)
                xs[j] = olhs(8 * j, 8 * j + 8), ob[:, j * DM:(j + 1) * DM]
            return xs[j]

        def lh(k, j):
            if (k, j) not in ls:
                d1, d2 = x(j)[0] - x(k)[0], x(j)[1] - x(k)[1]
                ljk = d1 + CF[k] * d2
                ls[(k, j)] = d1 + CF[j] * d2, ljk, ljk + (CF[j] - CF[k]) * x(j)[1]
            return ls[(k, j)]

        order = "e0 d0 a01 b01 a02 b02 a12 b12 e1 d1 h01 e2 d2 h02 h12 e3 a03 b03 h03 a13 b13 h13 a23 b23 h23 d3"
        for name in order.split():
            k, j = int(name[1]), int(name[-1])
            if name[0] == "e":
                l, w = x(j)[1], wc(4 + j)
            elif name[0] == "d":
                l, w = x(j)[0] + CF[j] * x(j)[1], wc(j)
            elif name[0] == "a":
                l, w = lh(k, j)[0], raw(k, j)
            elif name[0] == "b":
                l, w = lh(k, j)[1], raw(j, k)
            else:
                l, w = lh(k, j)[2], wc(8 + PAIRS.index((k, j)))
            pr[name] = _dot(l.astype(bf16), w)
            if rem:
                pv(rem.pop(0))
        pa = [-pr["d%d" % j] for j in range(4)]
        qa = [-pr["e%d" % j] for j in range(4)]
        for k, j in PAIRS:
            ga, gb, hh = (pr["%s%d%d" % (c, k, j)] for c in "abh")
            w = ((gb - ga) - hh) * (1.0 / (CF[j] - CF[k]))
            pa[j], pa[k] = pa[j] - ga, pa[k] + gb
            qa[j], qa[k] = qa[j] + w, qa[k] - w
        for j in range(4):
            c1 = pa[j] - CF[j] * qa[j]
            for jt in range(2):
                put(2 * j + jt, c1[:, 128 * jt:128 * (jt + 1)], qa[j][:, 128 * jt:128 * (jt + 1)])

    def out_copy(it):
        return pltpu.make_async_copy(oa.at[pl.ds(it * 2, 2)],
                                     out_hbm.at[pl.ds(it * 2, 2), :, :, pl.ds(0, DM)], sems.at[32])

    def group(it, c):
        with jax.named_scope("grp"):
            for u in range(U):
                step(it, u)
        out_copy(it).start()
        return c
    lax.fori_loop(0, NSEG // U, group, 0)
    with jax.named_scope("w_out"):
        for it in range(NSEG // U):
            out_copy(it).wait()
        cp_outb.wait()


def pallas_concat_heads__memory_aug_recurrent_mem_tr__spectral_gfnet__prompt_kernel(
    A_x, A_mem0, A_Wq, A_Wk, A_Wv, A_Wo, A_seg_len, B_x, B_w_r, B_w_i,
):
    if isinstance(A_seg_len, int):
        assert A_seg_len == SEG
    R, LN, TW, fill, KC = _tables()
    small = np.zeros((208, 128), np.float32)
    small[:80, :80] = fill
    small[80:112] = TW
    small[112:] = np.repeat(KC, 8, axis=0)
    hbm = pl.BlockSpec(memory_space=pl.ANY)
    out = pl.pallas_call(
        _kernel,
        out_shape=jax.ShapeDtypeStruct((RS, 8, 8, DM + D), bf16),
        in_specs=[hbm] * 12,
        out_specs=hbm,
        scratch_shapes=[
            pltpu.VMEM((NSEG, 3, 8, DM), bf16),
            pltpu.VMEM((NSEG, 8, DM), bf16),
            pltpu.VMEM((4, 64, DM), u32),
            pltpu.VMEM((DM // 128, 4, DM, 128), bf16),
            pltpu.VMEM((BC + 7, DM // 2, 8, DH), bf16),
            pltpu.VMEM((NCH + 3, 16 * PW, DH), u32),
            pltpu.VMEM((M, DM), bf16),
            pltpu.VMEM((U * M, H * DH), f32),
            pltpu.VMEM((RS, 8, 8, DM), bf16),
            pltpu.VMEM((RS, 8, 8, D), bf16),
            pltpu.VMEM((4, 2, D // 2 + 1, 512), bf16),
            pltpu.VMEM((16, 64, 128), u32),
            pltpu.VMEM((2 * RS + 5, 64, 128), u32),
            pltpu.VMEM((208, 128), f32),
            pltpu.VMEM((4, RS, 4, 2, 16, 128), bf16),
            pltpu.VMEM((4, RS, TP, 128), f32),
            pltpu.VMEM((2, 2, 4, BS * WP, 128), u32),
            pltpu.VMEM((32, 128), f32),
            pltpu.SemaphoreType.DMA((48,)),
        ],
        compiler_params=pltpu.CompilerParams(vmem_limit_bytes=124 * 1024 * 1024,
                                             disable_bounds_checks=True, disable_semaphore_checks=True),
    )(A_x.reshape(NSEG, 4, 8, DM), A_mem0.reshape(M, DM),
      A_Wq.reshape(2, DM // 2, H, DH), A_Wk.reshape(2, DM // 2, H, DH), A_Wv.reshape(2, DM // 2, H, DH),
      A_Wo.reshape(4, DM, DM), B_x.reshape(RS, 8, 8, D), B_w_r.T, B_w_i.T,
      jnp.asarray(R), jnp.asarray(LN), jnp.asarray(small))
    return out.reshape(1, S, DM + D)
```

```python
import functools
import math

import jax
import jax.numpy as jnp
import numpy as np
from jax import lax
import jax.experimental.pallas as pl
import jax.experimental.pallas.tpu as pltpu

bf16, f32, u32, i32 = jnp.bfloat16, jnp.float32, jnp.uint32, jnp.int32

S, DM, H, DH, M, SEG = 2048, 1024, 32, 128, 8, 32
NSEG = S // SEG
FR = SEG - M
G = H // 2
U = 4
NCH = 12
NST = 4
PW = 260

D = 1024
RS, BS = 32, 64
HR = RS // 2
TP = 136
C8 = float(np.sqrt(0.5))


def _pack_rows(a):
    u = np.asarray(a, np.float32).astype(jnp.bfloat16).view(np.uint16).astype(np.uint32)
    return u[..., 0::2, :] | (u[..., 1::2, :] << 16)


_RHO = (2, 4, 4, 4)


def _in_a(lane, c):
    return (lane % 4 < 2) if c == 0 else ((lane + 2) % 8 < 4)


def _dstage(x, kc, roll64):
    a = [x[j] + x[j + 4] for j in range(4)]
    b = [x[j] - x[j + 4] for j in range(4)]
    t1 = (b[1] - b[3]) * C8
    t2 = (b[1] + b[3]) * C8
    s0, s1 = a[0] + a[2], a[1] + a[3]
    out = [s0 + s1, s0 - s1]
    for c, (u, v) in enumerate(((b[0] + t1, b[2] + t2), (a[0] - a[2], a[1] - a[3]), (b[0] - t1, b[2] - t2))):
        g = u * kc[4 * c] + v * kc[4 * c + 1]
        h = roll64(u * kc[4 * c + 2] + v * kc[4 * c + 3])
        out += [g + h, g - h]
    return out


def _dstage_t(p, kc, roll64):
    uv = []
    for c in range(3):
        g = p[2 + 2 * c] + p[3 + 2 * c]
        h = roll64(p[2 + 2 * c] - p[3 + 2 * c])
        uv.append((g * kc[4 * c] + h * kc[4 * c + 2], g * kc[4 * c + 1] + h * kc[4 * c + 3]))
    s0, s1 = p[0] + p[1], p[0] - p[1]
    a = [s0 + uv[1][0], s1 + uv[1][1], s0 - uv[1][0], s1 - uv[1][1]]
    t1 = (uv[0][0] - uv[2][0]) * C8
    t2 = (uv[0][1] - uv[2][1]) * C8
    b = [uv[0][0] + uv[2][0], t1 + t2, uv[0][1] + uv[2][1], t2 - t1]
    return [a[j] + b[j] for j in range(4)] + [a[j] - b[j] for j in range(4)]


@functools.lru_cache(maxsize=None)
def _tables():
    kcol = np.zeros((4, 128), np.int64)
    for l in range(128):
        i0, i1 = l, 128 + (l ^ 1)
        ev, o3 = l % 2 == 0, l % 4 in (0, 3)
        kcol[0, l] = 2 * (i0 if ev else i1)
        kcol[2, l] = 2 * (i1 if ev else i0)
        kcol[1, l] = 2 * (i0 if o3 else i1) + 1
        kcol[3, l] = 2 * (i1 if o3 else i0) + 1
    lanes = np.arange(128)
    lo = lanes < 64
    KC = np.zeros((12, 128))
    for c, sg in ((1, -1.0), (2, -1.0), (3, 1.0)):
        tr, ti = np.cos(2 * np.pi * c / 16), -np.sin(2 * np.pi * c / 16)
        KC[4 * c - 4] = np.where(lo, 1.0, ti)
        KC[4 * c - 3] = sg * np.where(lo, 0.0, tr)
        KC[4 * c - 2] = np.where(lo, 0.0, tr)
        KC[4 * c - 1] = sg * np.where(lo, 1.0, -ti)
    eye = np.eye(D)
    Bt = _dstage([eye[:, 128 * e:128 * (e + 1)] for e in range(8)], KC, lambda v: np.roll(v, 64, axis=1))
    d = np.arange(D)
    R = np.zeros((16, 128, 128))
    for c in range(4):
        rho = _RHO[c]
        inA = _in_a(lanes, c)
        ang = 2 * np.pi * (np.outer(d, kcol[c]) % D) / D
        fr, fi = np.cos(ang), -np.sin(ang)
        wr_, wi_ = np.full(128, 2.0), np.full(128, 2.0)
        if c == 0:
            fi[:, 0] = (-1.0) ** d
            wr_[0] = 1.0
            wi_[0] = 1.0
        fi, wi_ = np.roll(fi, -rho, axis=1), np.roll(wi_, -rho)
        for h in range(2):
            own = inA if h == 0 else ~inA
            ft, wt = np.where(own, fr, fi), np.where(own, wr_, wi_)
            bt = Bt[2 * c + h]
            r = (bt.T @ ft) / (bt * bt).sum(axis=0)[:, None]
            assert np.abs(bt @ r - ft).max() < 1e-9
            R[2 * c + h] = r
            R[8 + 2 * c + h] = (wt[:, None] * r.T) / (S * D)
    L = np.zeros((2 * RS, 128, 128))
    bb = np.arange(BS)
    kord = np.array([ri * 64 + 8 * t + r for t in range(8) for ri in range(2) for r in range(8)])
    rord = np.array([ri * 64 + 16 * q + r for q in range(4) for ri in range(2) for r in range(16)])
    for p1 in range(RS):
        ang = 2 * np.pi * (np.outer(p1 + RS * bb, bb) % S) / S
        mr, mi = np.cos(ang), -np.sin(ang)
        full = np.block([[mr, -mi], [mi, mr]])
        L[p1] = full[:, kord]
        L[RS + p1] = full.T[rord]
    l_, q_ = np.arange(128), np.arange(16)
    ang = 2 * np.pi * (np.outer(l_, l_) % 128) / 128
    N1 = np.concatenate([np.cos(ang), -np.sin(ang)], axis=1)
    N1 = np.concatenate([(N1[:64] + N1[64:]) / 2, (N1[:64] - N1[64:]) / 2], axis=0)
    ang = 2 * np.pi * np.outer(q_, l_) / S
    TW = np.concatenate([np.cos(ang), -np.sin(ang)], axis=0)
    ang = 2 * np.pi * (np.outer(q_, q_) % 16) / 16
    fr, fi = np.cos(ang), -np.sin(ang)
    F16 = np.block([[fr, -fi], [fi, fr]])
    NY = np.zeros((5, 128, 128))
    NY[0], NY[1], NY[2], NY[3] = N1[:, :128], N1[:, 128:], N1[:, :128].T, N1[:, 128:].T
    NY[4, :32, :32] = F16
    NY[4, 32:64, :32] = F16.T
    LN = np.concatenate([L, NY], axis=0)
    head = np.zeros(80, np.int32)
    pos = np.zeros(80, np.int32)
    for r in range(80):
        if r < 64:
            head[r] = r // 32
            t = r % 32
            pos[r] = (M + t) if t < FR else (t - FR)
        else:
            head[r] = (r - 64) // 8
            pos[r] = M + FR + (r - 64) % 8
    same = head[:, None] == head[None, :]
    vis = (pos[:, None] < M) | (pos[:, None] >= pos[None, :])
    fill = np.where(same, np.where(vis, 0.0, -1e9), -np.inf).astype(np.float32)
    return _pack_rows(R), _pack_rows(LN), TW.astype(np.float32), fill, KC.astype(np.float32)


def _cmul_const(re, im, j, n, sgn):
    ang = sgn * 2 * math.pi * j / n
    c, s = math.cos(ang), math.sin(ang)
    if abs(abs(c) - abs(s)) < 1e-12:
        if c * s > 0:
            return (re - im) * c, (re + im) * c
        return (re + im) * c, (im - re) * c
    return re * c - im * s, re * s + im * c


def _diff_tw(a, b, j, n, sgn):
    if j == 0:
        return a[0] - b[0], a[1] - b[1]
    if 4 * j == n:
        if sgn < 0:
            return a[1] - b[1], b[0] - a[0]
        return b[1] - a[1], a[0] - b[0]
    return _cmul_const(a[0] - b[0], a[1] - b[1], j, n, sgn)


def _tw(v, j, sgn):
    if j == 0:
        return v
    if 4 * j == RS:
        return (v[1], -v[0]) if sgn < 0 else (-v[1], v[0])
    return _cmul_const(v[0], v[1], j, RS, sgn)


def _fft(v, sgn):
    n = len(v)
    if n == 1:
        return v
    h = n // 2
    ev = _fft([(v[j][0] + v[j + h][0], v[j][1] + v[j + h][1]) for j in range(h)], sgn)
    od = _fft([_diff_tw(v[j], v[j + h], j, n, sgn) for j in range(h)], sgn)
    out = [None] * n
    out[0::2] = ev
    out[1::2] = od
    return out


def _dot(a, b):
    return jnp.dot(a, b, preferred_element_type=f32)


def _asbf(v):
    return pltpu.bitcast(v, bf16)


def _cm(ar, ai, br, bi):
    return ar * br - ai * bi, ar * bi + ai * br


CHUNKS = [(0, 0), (0, 1), (0, 2), (0, 3), (1, 0), (1, 1), (1, 2), (2, 0), (2, 1), (2, 2), (2, 3), (1, 3)]
BU = 2 * NST + NCH
BC = BU + 2
CF = (-1.2, -0.4, 0.4, 1.2)
PAIRS = [(k, j) for j in range(4) for k in range(j)]


WP = 12
RAW32 = [(0, 1), (1, 0), (0, 2), (2, 0), (1, 2), (2, 1)]
NK0 = 88


def _kernel(ax_hbm, mem_hbm, wq_hbm, wk_hbm, wv_hbm, wo_hbm, bx_hbm, wr_hbm, wi_hbm,
            R_hbm, L_hbm, sm_hbm, out_hbm,
            ax, xb3, xb, wo, pool, wpk, memb, ob, oa,
            bx, wf, R, L, sm, Y, T, wp, nv, sems):
    srcs = (wq_hbm, wk_hbm, wv_hbm)
    lane8 = lax.broadcasted_iota(i32, (8, 128), 1)

    def chunk_copy(t):
        m, c = CHUNKS[t]
        return pltpu.make_async_copy(srcs[m].at[:, :, pl.ds(8 * c, 8), :],
                                     pool.at[pl.ds(2 * (t % NST), 2)], sems.at[t % NST])

    def part0_copy(part):
        rows = pl.ds(pl.multiple_of(part * 128, 128), 128)
        return pltpu.make_async_copy(wq_hbm.at[:, rows, pl.ds(0, 8), :], pool.at[pl.ds(0, 2), rows], sems.at[34 + part])

    def part_start(t, part):
        lo = part * 2 * NK0
        n = min(2 * NK0, 512 - lo)
        pltpu.make_async_copy(wq_hbm.at[:, pl.ds(lo, n), pl.ds(8 * t, 8), :],
                              pool.at[pl.ds(2 * t, 2), pl.ds(lo, n)], sems.at[35 + 3 * t + part]).start()

    def part_wait(t, part):
        for p in range(3):
            lo = p * 2 * NK0
            n = min(2 * NK0, 512 - lo)

            @pl.when(part == p)
            def _(lo=lo, n=n, p=p):
                blk = pool.at[pl.ds(2 * t, 2), pl.ds(lo, n)]
                pltpu.make_async_copy(blk, blk, sems.at[35 + 3 * t + p]).wait()

    def chunk_start(t):
        sl = t & (NST - 1)
        pltpu.make_async_copy(wv_hbm.at[:, :, pl.ds(pl.multiple_of(8 * (t - 7), 8), 8), :],
                              pool.at[pl.ds(2 * sl, 2)], sems.at[sl]).start()

    def chunk_wait(t):
        sl = t & (NST - 1)
        blk = pool.at[pl.ds(2 * sl, 2)]
        pltpu.make_async_copy(blk, blk, sems.at[sl]).wait()

    def xb_copy(q):
        return pltpu.make_async_copy(ax_hbm.at[pl.ds(16 * q, 16), 3], xb3.at[pl.ds(16 * q, 16)], sems.at[8 + q])

    def bx_copy(q):
        return pltpu.make_async_copy(bx_hbm.at[:, pl.ds(2 * q, 2)], bx.at[:, pl.ds(2 * q, 2)], sems.at[12 + q])

    def w_copy(q, i):
        cols = pl.ds(pl.multiple_of(512 * q, 512), 512)
        return pltpu.make_async_copy((wr_hbm, wi_hbm)[i].at[:, cols], wf.at[q, i],
                                     sems.at[16 + 4 * i + q])

    def wo_copy(q, j):
        jt = 2 * j + (q >> 1)
        rows = pl.ds(pl.multiple_of((q & 1) * 512, 512), 512)
        return pltpu.make_async_copy(wo_hbm.at[:, rows, pl.ds(pl.multiple_of(128 * jt, 128), 128)],
                                     wo.at[jt, :, rows], sems.at[44 + q])

    cp_r0 = pltpu.make_async_copy(R_hbm.at[pl.ds(0, 8)], R.at[pl.ds(0, 8)], sems.at[25])
    cp_r1 = pltpu.make_async_copy(R_hbm.at[pl.ds(8, 8)], R.at[pl.ds(8, 8)], sems.at[26])
    cp_l = pltpu.make_async_copy(L_hbm, L, sems.at[27])
    cp_ax = pltpu.make_async_copy(ax_hbm.at[:, pl.ds(0, 3)], ax, sems.at[28])
    cp_outb = pltpu.make_async_copy(bx, out_hbm.at[:, :, :, pl.ds(DM, D)], sems.at[29])
    cp_sm = pltpu.make_async_copy(sm_hbm, sm, sems.at[30])
    cp_mem = pltpu.make_async_copy(mem_hbm, memb, sems.at[31])

    for part in range(4):
        part0_copy(part).start()
    xb_copy(0).start()
    for p in range(3):
        xb_copy(p + 1).start()
        part_start(1, p)
    for p in range(3):
        part_start(2, p)
    chunk_copy(3).start()
    cp_r0.start()
    bx_copy(0).start()
    w_copy(0, 0).start()
    w_copy(0, 1).start()
    cp_sm.start()
    cp_mem.start()

    def kc(rep=2):
        return [jnp.concatenate([sm[112 + 8 * i:120 + 8 * i, :]] * rep, axis=0) for i in range(12)]

    def roll64(v):
        return pltpu.roll(v, 64, 1)

    def prep(t, tpar, jj):
        lo = [bx[2 * jj:2 * jj + 2, t, :, 128 * e:128 * (e + 1)].astype(f32).reshape(16, 128) for e in range(8)]
        hi = [bx[HR + 2 * jj:HR + 2 * jj + 2, t, :, 128 * e:128 * (e + 1)].astype(f32).reshape(16, 128)
              for e in range(8)]
        for par in range(2):
            x = [lo[e] + hi[e] if par == 0 else lo[e] - hi[e] for e in range(8)]
            uu = _dstage(x, kc(), roll64)
            for q in range(8):
                o = (((tpar * 2 + par) * 8 + q) * 8 + jj) * 2
                pool[BU, o:o + 2] = uu[q].reshape(2, 8, 128).astype(bf16)

    def unit1(t, tpar, par, cg):
        o = ((tpar * 2 + par) * 8 + 2 * cg) * 16
        za = _dot(pool[BU, o:o + 16].reshape(128, 128), _asbf(R[2 * cg]))
        zb = _dot(pool[BU, o + 16:o + 32].reshape(128, 128), _asbf(R[2 * cg + 1]))
        ina = _in_a(lane8, cg)
        v = []
        for j in range(HR):
            pa, pb = za[8 * j:8 * j + 8], zb[8 * j:8 * j + 8]
            v.append((jnp.where(ina, pa, pb), pltpu.roll(jnp.where(ina, pb, pa), _RHO[cg], 1)))
        if cg == 0:
            V = nv[8 * tpar:8 * tpar + 8, :]
            for j in range(HR):
                vb = jnp.broadcast_to(v[j][1][:, 0:1], (8, 128))
                V = jnp.where(lane8 == 64 * par + 4 * j + (t >> 1), vb, V)
                v[j] = (v[j][0], jnp.where(lane8 == 0, 0.0, v[j][1]))
            nv[8 * tpar:8 * tpar + 8, :] = V
        if par == 1:
            v = [_tw(v[j], j, -1) for j in range(HR)]
        o = _fft(v, -1)
        for m in range(HR):
            Y[t >> 1, 2 * m + par, cg, tpar] = jnp.concatenate(o[m], axis=0).astype(bf16)

    def wprep(q, k, i):
        w = wf.at[q, i]
        cols = slice(128 * k, 128 * (k + 1))
        sub = lax.broadcasted_iota(i32, (8, 128), 0)
        msk = (jnp.where(sub % 2 == 0, jnp.uint32(0xffff), jnp.uint32(0))
               | jnp.where((sub % 4 == 0) | (sub % 4 == 3), jnp.uint32(0xffff0000), jnp.uint32(0)))
        t0 = pltpu.bitcast(w[0:256, cols], u32)
        t1 = pltpu.bitcast(w[256:512, cols], u32)
        ps, qs = [], []
        for j in range(16):
            a = t0[8 * j:8 * j + 8]
            b = t1[8 * j:8 * j + 8]
            b = jnp.where(sub % 2 == 0, pltpu.roll(b, 7, 0), pltpu.roll(b, 1, 0))
            x = (a ^ b) & msk
            ps.append(b ^ x)
            qs.append(a ^ x)
        for h, lst in enumerate((ps, qs)):
            tr = pltpu.bitcast(pltpu.bitcast(jnp.concatenate(lst, axis=0), f32).T, u32)
            r0 = pl.multiple_of(q * 16 * WP, 32)
            for j in range(4):
                for o in range(4):
                    wp[i, h, o, pl.ds(r0 + WP * (4 * k + j), 8), :] = tr[32 * j + 8 * o:32 * j + 8 * o + 8]

    def fwd(p):
        return _dot(_asbf(L[p]), jnp.concatenate([Y[:, p, cg].reshape(128, 128) for cg in range(4)], axis=1))

    def filt(q, po, v):
        grs, gis = [None] * 4, [None] * 4
        for h in range(2):
            wr_ = wp[0, h, q, pl.ds(po, BS, stride=WP), :]
            wi_ = wp[1, h, q, pl.ds(po, BS, stride=WP), :]
            for hi in range(2):
                cg = 2 * h + hi
                if hi == 0:
                    a, b = wr_ << 16, wi_ << 16
                else:
                    a, b = wr_ & jnp.uint32(0xffff0000), wi_ & jnp.uint32(0xffff0000)
                grs[cg], gis[cg] = _cm(v[:BS, 128 * cg:128 * (cg + 1)], v[BS:, 128 * cg:128 * (cg + 1)],
                                       pltpu.bitcast(a, f32), pltpu.bitcast(b, f32))
        return jnp.concatenate([jnp.concatenate(grs, axis=1), jnp.concatenate(gis, axis=1)], axis=0).astype(bf16)

    def inv(p, g):
        t = _dot(_asbf(L[RS + p]), g)
        for cg in range(4):
            T[cg, p, 0:128, :] = t[:, 128 * cg:128 * (cg + 1)]

    nyq = {}

    def nyq_stage(k):
        n0 = 2 * RS
        twr, twi = sm[80:96, :], sm[96:112, :]
        if k == 0:
            v = nv[0:16, :].astype(bf16)
            r, i = _cm(_dot(v, _asbf(L[n0])), _dot(v, _asbf(L[n0 + 1])), twr, twi)
            nyq[0] = jnp.concatenate([r, i], axis=0).astype(bf16)
        elif k == 1:
            t = _dot(_asbf(L[n0 + 4, 0:16])[:, 0:32], nyq[0])
            ws = []
            for i in range(2):
                rows = [wf[j, i, 512:513, :].astype(f32) for j in range(4)]
                ws.append(jnp.concatenate([rows[r // 4][:, 128 * (r % 4):128 * (r % 4 + 1)] for r in range(16)], axis=0))
            r, i = _cm(t[:16], t[16:], ws[0], ws[1])
            nyq[1] = jnp.concatenate([r, i], axis=0).astype(bf16)
        elif k == 2:
            t = _dot(_asbf(L[n0 + 4, 16:32])[:, 0:32], nyq[1])
            r, i = _cm(t[:16], t[16:], twr, -twi)
            nyq[2] = (r.astype(bf16), i.astype(bf16))
        elif k == 3:
            nv[16:32, :] = _dot(nyq[2][0], _asbf(L[n0 + 2])) + _dot(nyq[2][1], _asbf(L[n0 + 3]))

    def p3a(t, tpar, par, cg):
        r0 = pl.multiple_of((t >> 1) * 32, 32)
        rr = pl.ds(r0 + 8 * tpar, 8)
        ri = pl.ds(r0 + 16 + 8 * tpar, 8)
        o = _fft([(T[cg, 2 * m + par, rr, :], T[cg, 2 * m + par, ri, :]) for m in range(HR)], +1)
        if par == 1:
            o = [_tw(o[j], j, +1) for j in range(HR)]
        if cg == 0:
            un = nv[16 + 8 * tpar:24 + 8 * tpar, :]
            o = [(o[j][0], jnp.where(lane8 == 0, pltpu.roll(un, (128 - 64 * par - 4 * j - (t >> 1)) & 127, 1),
                                     o[j][1])) for j in range(HR)]
        ina = _in_a(lane8, cg)
        ua, ub = [], []
        for re, im in o:
            im = pltpu.roll(im, 128 - _RHO[cg], 1)
            ua.append(jnp.where(ina, re, im))
            ub.append(jnp.where(ina, im, re))
        for j in range(HR // 2):
            for h, x in enumerate((ua, ub)):
                o = ((tpar * 2 + par) * 8 + 2 * cg + h) * 16 + 2 * j
                pool[BU + 1, o:o + 2] = jnp.concatenate(x[2 * j:2 * j + 2], axis=0).reshape(2, 8, 128).astype(bf16)

    def p3b(tpar, par, cg):
        zs = []
        for h in range(2):
            o = ((tpar * 2 + par) * 8 + 2 * cg + h) * 16
            zs.append((o, _dot(pool[BU + 1, o:o + 16].reshape(128, 128), _asbf(R[8 + 2 * cg + h]))))
        return zs

    def p3s(zs):
        for o, z in zs:
            pool[BU, o:o + 16] = z.reshape(16, 8, 128).astype(bf16)

    def p3c(t, tpar, j):
        res = [_dstage_t([pool[BU, ((tpar * 2 + par) * 8 + q) * 16 + j].astype(f32) for q in range(8)],
                         kc(1), roll64) for par in range(2)]
        for e in range(8):
            cols = slice(128 * e, 128 * (e + 1))
            bx[j, t, :, cols] = (res[0][e] + res[1][e]).astype(bf16)
            bx[HR + j, t, :, cols] = (res[0][e] - res[1][e]).astype(bf16)

    def wsum(jt, q, n):
        rows = pl.ds(pl.multiple_of(q * 256, 256) + 16 * n, 16)

        def ld(k, j):
            v = wo[2 * j + jt, k, rows, :]
            if (k, j) in RAW32:
                x = RAW32.index((k, j))
                r0 = pl.multiple_of(q * 128, 128) + 512 * x + 8 * n
                wpk[NCH + 1 + jt, pl.ds(r0, 8), :] = pltpu.bitcast(v, u32)
            return v.astype(f32)

        def st(i, v):
            pool[BC + i // 2, pl.ds((i % 2) * 256 + jt * 128 + q * 32 + 2 * n, 2)] = v.reshape(2, 8, 128).astype(bf16)
        col, row = {}, {}
        for k in range(4):
            d = -ld(k, k)
            col[k] = col[k] + d if k in col else d
            row[k] = row[k] + d if k in row else d
            for j in range(k + 1, 4):
                bkj, bjk = ld(k, j), ld(j, k)
                st(8 + PAIRS.index((k, j)), bjk - bkj)
                col[k], row[k] = col[k] - bjk, row[k] - bkj
                col[j] = col[j] - bkj if j in col else -bkj
                row[j] = row[j] - bjk if j in row else -bjk
            st(k, col[k])
            st(4 + k, row[k])

    def wc(i):
        o = (i % 2) * 256
        return jnp.concatenate([pool[BC + i // 2, o + 128 * jt:o + 128 * (jt + 1)].reshape(DM, 128)
                                for jt in range(2)], axis=1)

    def runit(b0, d0, dst, k):
        a = pltpu.bitcast(jnp.concatenate([pool[b0, d0 + 2 * k], pool[b0 + 1, d0 + 2 * k]], axis=0), u32)
        b = pltpu.bitcast(jnp.concatenate([pool[b0, d0 + 2 * k + 1], pool[b0 + 1, d0 + 2 * k + 1]], axis=0), u32)
        dst[pl.ds(k, 8, stride=PW), :] = (a & jnp.uint32(0xffff)) | (b << 16)
        dst[pl.ds(8 * PW + k, 8, stride=PW), :] = (a >> 16) | (b & jnp.uint32(0xffff0000))

    def wsel(w, hl, lo=0, hi=DM):
        base = ((hl % 2) * 8 + hl // 2) * PW
        parts = []
        for kh in range(2):
            a, b = max(lo, 512 * kh), min(hi, 512 * (kh + 1))
            if a < b:
                o = base + 4 * PW * kh - 256 * kh
                parts.append(w[o + a // 2:o + b // 2, :])
        return _asbf(jnp.concatenate(parts, axis=0))

    def bulk(t, mc0, nmc, tsrc, tdst, k0, nk, side=None):
        w = wpk.at[t]
        b0 = 2 * (tsrc & (NST - 1))
        dst = wpk.at[tdst, pl.ds(k0, 15 * PW + 4 + nk)]
        bq = 2 * NST + (t & 31)
        ns = 8 * nmc
        per = nk // ns
        for mi in range(nmc):
            mc = mc0 + mi
            x = _asbf(xb[mc])
            for h in range(8):
                n = mi * 8 + h
                r = _dot(x, wsel(w, h)).reshape(16, M, DH)
                nn = (n - 1) % ns
                for k in range(per * nn, per * (nn + 1)):
                    runit(b0, 2 * k0, dst, k)
                if side is not None:
                    side(n)
                rb = r.astype(bf16)
                for gi in range(4):
                    pool[bq, pl.ds(mc * 128 + gi * 32 + h * 4, 4)] = rb[4 * gi:4 * gi + 4]

    def rel0(i, c):
        @pl.when(i % 2 == 0)
        def _():
            part0_copy(i >> 1).wait()
        dst = wpk.at[0, pl.ds(pl.multiple_of(i * 32, 32), 15 * PW + 36)]
        for k in range(32):
            runit(0, i * 64, dst, k)
        return c
    with jax.named_scope("rel0"):
        lax.fori_loop(0, 8, rel0, 0)

    def body0(i, c):
        t, mc = i >> 2, i & 3
        real = mc >= 1

        @pl.when(t == 0)
        def _():
            xb_copy(mc).wait()
            xb[mc] = pltpu.bitcast(xb3[pl.ds(16 * mc, 16)].reshape(128, DM), u32)

        @pl.when(real)
        def _():
            part_wait(t + 1, mc - 1)
        with jax.named_scope("bulk0"):
            bulk(t, mc, 1, jnp.where(real, t + 1, t), jnp.where(real, t + 1, NCH),
                 pl.multiple_of(jnp.clip((mc - 1) * NK0, 0, 256 - NK0), math.gcd(NK0, 32)), NK0)

        @pl.when(i == 0)
        def _():
            chunk_copy(4).start()
            bx_copy(1).start()
            w_copy(1, 0).start()
            w_copy(1, 1).start()

        @pl.when(i == 4)
        def _():
            chunk_copy(5).start()
        return c
    lax.fori_loop(0, 8, body0, 0)
    bx_copy(2).start()
    w_copy(2, 0).start()
    w_copy(2, 1).start()
    chunk_copy(6).start()
    bx_copy(3).start()
    w_copy(3, 0).start()
    w_copy(3, 1).start()
    cp_l.start()
    cp_r1.start()
    nv[0:16, :] = jnp.zeros((16, 128), f32)
    cp_r0.wait()
    cp_sm.wait()

    def body1(q, c):
        t = q + 2
        with jax.named_scope("w_1"):
            chunk_wait(t + 1)
            bx_copy(q).wait()
            w_copy(q, 0).wait()
            w_copy(q, 1).wait()

        def side(n):
            for k in ([0, 1] if n == 0 else [n + 1]):
                if k < 16:
                    prep(2 * q + k // 8, k // 8, k % 8)
            k = n - 15
            if 0 <= k < 16:
                unit1(2 * q + k // 8, k // 8, (k // 4) % 2, k % 4)
            k, r = divmod(n - 15, 2)
            if r == 0 and 0 <= k < 8:
                wprep(q, k // 2, k % 2)
        with jax.named_scope("bulk_p1"):
            bulk(t, 0, 4, t + 1, t + 1, 0, 256, side)
        for j in range(4):
            wo_copy(q, j).start()
        chunk_start(t + 1 + NST)
        return c
    lax.fori_loop(0, 4, body1, 0)

    cp_ax.start()
    with jax.named_scope("w_l"):
        cp_l.wait()
        cp_r1.wait()

    def body2(q, c):
        t, hf = (q >> 1) + 6, q & 1

        @pl.when(hf == 0)
        def _():
            with jax.named_scope("w_2"):
                chunk_wait(t + 1)
                for j in range(4):
                    wo_copy(q >> 1, j).wait()
        gs = {}
        fs = [0, 1, 3, 5, 7, 9, 11, 13]

        def side(n):
            if n - 2 in fs:
                po = fs.index(n - 2)
                inv(8 * q + po, gs.pop(po))
            if n in fs:
                po = fs.index(n)
                gs[po] = filt(q, po, fwd(8 * q + po))
            k, r = divmod(n - 1, 3)
            if r == 0 and 0 <= k < 4:
                nyq_stage(k)
            for hh in range(16 * n // 15, min(16, 16 * (n + 1) // 15)):
                wsum(0, q, hh)
        with jax.named_scope("bulk_p2"):
            bulk(t, 2 * hf, 2, t + 1, t + 1, pl.multiple_of(hf * 128, 128), 128, side)
        return c
    lax.fori_loop(0, 4, body2, 0)
    chunk_copy(11).start()
    for q in (2, 3):
        for j in range(4):
            wo_copy(q, j).wait()

    def body3(q, c):
        t = q + 8

        @pl.when(q < 3)
        def _():
            with jax.named_scope("w_3"):
                chunk_wait(t + 1)
        us = {}

        def side(n):
            if n < 16:
                p3a(2 * q + n // 8, n // 8, (n // 4) % 2, n % 4)
            k = n - 3
            if 0 <= k < 16:
                us[k] = p3b(k // 8, (k // 4) % 2, k % 4)
            k = n - 3 - 1
            if 0 <= k < 16:
                p3s(us.pop(k))
            k = n - 16
            if 0 <= k < 16:
                p3c(2 * q + k // 8, k // 8, 2 * (k % 8))
                p3c(2 * q + k // 8, k // 8, 2 * (k % 8) + 1)
            if n < 16:
                wsum(1, q, n)
        with jax.named_scope("bulk_p3"):
            bulk(t, 0, 4, t + 1, t + 1, 0, 256, side)
        return c
    lax.fori_loop(0, 4, body3, 0)
    cp_outb.start()

    with jax.named_scope("w_wo"):
        cp_ax.wait()
        cp_mem.wait()
    scale = DH ** -0.5
    KS = 640

    def step(it, u):
        s = it * U + u
        lhs = jnp.concatenate([ax[s].reshape(FR, DM), memb[...]], axis=0)
        qs, ks, vs, ps, os_, pre = {}, {}, {}, {}, {}, {}

        def ws(m, h, lo=0, hi=DM):
            return wsel(wpk.at[CHUNKS.index((m, h // 8))], h % 8, lo, hi)
        if u > 0:
            for m in range(2):
                for h in range(2):
                    pre[(m, h)] = -_dot(lhs[:, :KS], ws(m, h, 0, KS))

        def dotw(m, h):
            if (m, h) in pre:
                return _dot(lhs[:, KS:], ws(m, h, KS, DM)) - pre[(m, h)]
            return _dot(lhs, ws(m, h))

        def proj(m, g):
            h = 2 * g
            bq = 2 * NST + CHUNKS.index((m, h // 8))
            return jnp.concatenate([dotw(m, h), dotw(m, h + 1),
                                    pool[bq, it * 32 + (h % 8) * 4 + u].astype(f32),
                                    pool[bq, it * 32 + (h % 8 + 1) * 4 + u].astype(f32)], axis=0).astype(bf16)

        def qk(g):
            sc = lax.dot_general(qs.pop(g), ks.pop(g), (((1,), (1,)), ((), ())),
                                 preferred_element_type=f32) * scale
            fill = sm[0:80, 0:80]
            sc = jnp.where(fill == 0.0, sc, fill)
            mx = jnp.max(sc, axis=-1, keepdims=True)
            e = jnp.exp(sc - mx)
            l = jnp.sum(e, axis=-1, keepdims=True)
            r = pl.reciprocal(l, approx=True)
            r = r * (2.0 - l * r)
            ps[g] = (e * r).astype(bf16)

        def pv(g):
            o = _dot(ps.pop(g), vs.pop(g))
            os_[2 * g] = o[0:32]
            os_[2 * g + 1] = o[32:64]
            ob[8 * u:8 * u + 8, (2 * g) * DH:(2 * g + 1) * DH] = o[64:72]
            ob[8 * u:8 * u + 8, (2 * g + 1) * DH:(2 * g + 2) * DH] = o[72:80]

        def olhs(lo, hi):
            return jnp.concatenate([os_[h] for h in range(lo, hi)], axis=1)

        def put(j, r, rb):
            cols = slice(j * 128, (j + 1) * 128)
            oa[it * 2 + u // 2, pl.ds((u % 2) * 4, 3), :, cols] = r[0:FR].reshape(3, 8, 128).astype(bf16)
            memb[:, cols] = r[FR:SEG].astype(bf16)
            if rb is not None:
                for uu in range(U):
                    oa[it * 2 + uu // 2, (uu % 2) * 4 + 3, :, cols] = rb[8 * uu:8 * uu + 8].astype(bf16)

        sk, dq, dp = 7, 3, 5
        for t in range(G + sk):
            if t < G:
                qs[t] = proj(0, t)
            if 0 <= t - dq < G:
                qk(t - dq)
            if t < G:
                ks[t] = proj(1, t)
            if t - sk - dp >= 0:
                pv(t - sk - dp)
            if t - sk >= 0:
                vs[t - sk] = proj(2, t - sk)
        rem = list(range(G - dp, G))
        def wob(k, jn):
            if (k, jn // 2) in RAW32:
                x = RAW32.index((k, jn // 2))
                return _asbf(wpk[NCH + 1 + jn % 2, 512 * x:512 * (x + 1), :])
            return wo[jn, k]

        if u < U - 1:
            acc = []
            oc = olhs(0, 16).astype(bf16)
            for j in range(8):
                acc.append(-_dot(oc, jnp.concatenate([wob(0, j), wob(1, j)], axis=0)))
                if rem:
                    pv(rem.pop(0))
            oc = olhs(16, 32).astype(bf16)
            for j in range(8):
                put(j, _dot(oc, jnp.concatenate([wob(2, j), wob(3, j)], axis=0)) - acc[j], None)
            return
        xs, ls, pr = {}, {}, {}

        def raw(k, j):
            return jnp.concatenate([wob(k, 2 * j), wob(k, 2 * j + 1)], axis=1)

        def x(j):
            if j not in xs:
                assert not rem or rem[0] >= 4 * (j + 1)
                xs[j] = olhs(8 * j, 8 * j + 8), ob[:, j * DM:(j + 1) * DM]
            return xs[j]

        def lh(k, j):
            if (k, j) not in ls:
                d1, d2 = x(j)[0] - x(k)[0], x(j)[1] - x(k)[1]
                ljk = d1 + CF[k] * d2
                ls[(k, j)] = d1 + CF[j] * d2, ljk, ljk + (CF[j] - CF[k]) * x(j)[1]
            return ls[(k, j)]

        order = "e0 d0 a01 b01 a02 b02 a12 b12 e1 d1 h01 e2 d2 h02 h12 e3 a03 b03 h03 a13 b13 h13 a23 b23 h23 d3"
        for name in order.split():
            k, j = int(name[1]), int(name[-1])
            if name[0] == "e":
                l, w = x(j)[1], wc(4 + j)
            elif name[0] == "d":
                l, w = x(j)[0] + CF[j] * x(j)[1], wc(j)
            elif name[0] == "a":
                l, w = lh(k, j)[0], raw(k, j)
            elif name[0] == "b":
                l, w = lh(k, j)[1], raw(j, k)
            else:
                l, w = lh(k, j)[2], wc(8 + PAIRS.index((k, j)))
            pr[name] = _dot(l.astype(bf16), w)
            if rem:
                pv(rem.pop(0))
        pa = [-pr["d%d" % j] for j in range(4)]
        qa = [-pr["e%d" % j] for j in range(4)]
        for k, j in PAIRS:
            ga, gb, hh = (pr["%s%d%d" % (c, k, j)] for c in "abh")
            w = ((gb - ga) - hh) * (1.0 / (CF[j] - CF[k]))
            pa[j], pa[k] = pa[j] - ga, pa[k] + gb
            qa[j], qa[k] = qa[j] + w, qa[k] - w
        for j in range(4):
            c1 = pa[j] - CF[j] * qa[j]
            for jt in range(2):
                put(2 * j + jt, c1[:, 128 * jt:128 * (jt + 1)], qa[j][:, 128 * jt:128 * (jt + 1)])

    def out_copy(it):
        return pltpu.make_async_copy(oa.at[pl.ds(it * 2, 2)],
                                     out_hbm.at[pl.ds(it * 2, 2), :, :, pl.ds(0, DM)], sems.at[32])

    def group(it, c):
        with jax.named_scope("grp"):
            for u in range(U):
                step(it, u)
        out_copy(it).start()
        return c
    lax.fori_loop(0, NSEG // U, group, 0)
    with jax.named_scope("w_out"):
        for it in range(NSEG // U):
            out_copy(it).wait()
        cp_outb.wait()


def pallas_concat_heads__memory_aug_recurrent_mem_tr__spectral_gfnet__prompt_kernel(
    A_x, A_mem0, A_Wq, A_Wk, A_Wv, A_Wo, A_seg_len, B_x, B_w_r, B_w_i,
):
    if isinstance(A_seg_len, int):
        assert A_seg_len == SEG
    R, LN, TW, fill, KC = _tables()
    small = np.zeros((208, 128), np.float32)
    small[:80, :80] = fill
    small[80:112] = TW
    small[112:] = np.repeat(KC, 8, axis=0)
    hbm = pl.BlockSpec(memory_space=pl.ANY)
    out = pl.pallas_call(
        _kernel,
        out_shape=jax.ShapeDtypeStruct((RS, 8, 8, DM + D), bf16),
        in_specs=[hbm] * 12,
        out_specs=hbm,
        scratch_shapes=[
            pltpu.VMEM((NSEG, 3, 8, DM), bf16),
            pltpu.VMEM((NSEG, 8, DM), bf16),
            pltpu.VMEM((4, 64, DM), u32),
            pltpu.VMEM((DM // 128, 4, DM, 128), bf16),
            pltpu.VMEM((BC + 7, DM // 2, 8, DH), bf16),
            pltpu.VMEM((NCH + 3, 16 * PW, DH), u32),
            pltpu.VMEM((M, DM), bf16),
            pltpu.VMEM((U * M, H * DH), f32),
            pltpu.VMEM((RS, 8, 8, DM), bf16),
            pltpu.VMEM((RS, 8, 8, D), bf16),
            pltpu.VMEM((4, 2, D // 2 + 1, 512), bf16),
            pltpu.VMEM((16, 64, 128), u32),
            pltpu.VMEM((2 * RS + 5, 64, 128), u32),
            pltpu.VMEM((208, 128), f32),
            pltpu.VMEM((4, RS, 4, 2, 16, 128), bf16),
            pltpu.VMEM((4, RS, TP, 128), f32),
            pltpu.VMEM((2, 2, 4, BS * WP, 128), u32),
            pltpu.VMEM((32, 128), f32),
            pltpu.SemaphoreType.DMA((48,)),
        ],
        compiler_params=pltpu.CompilerParams(vmem_limit_bytes=124 * 1024 * 1024,
                                             disable_bounds_checks=True, disable_semaphore_checks=True),
    )(A_x.reshape(NSEG, 4, 8, DM), A_mem0.reshape(M, DM),
      A_Wq.reshape(2, DM // 2, H, DH), A_Wk.reshape(2, DM // 2, H, DH), A_Wv.reshape(2, DM // 2, H, DH),
      A_Wo.reshape(4, DM, DM), B_x.reshape(RS, 8, 8, D), B_w_r.T, B_w_i.T,
      jnp.asarray(R), jnp.asarray(LN), jnp.asarray(small))
    return out.reshape(1, S, DM + D)
```
